```python
import jax
import jax.numpy as jnp

def _softmax(x, axis=-1):
    return jax.nn.softmax(x, axis=axis)
def _gelu(x):
    return jax.nn.gelu(x, approximate=True)
def _silu(x):
    return jax.nn.silu(x)
def _sigmoid(x):
    return jax.nn.sigmoid(x)
def _layernorm(x, axis=-1, eps=1e-5):
    m = jnp.mean(x, axis=axis, keepdims=True)
    v = jnp.var(x, axis=axis, keepdims=True)
    return (x - m) / jnp.sqrt(v + eps)
def _scatter_add(tgt, idx, src, axis=0):
    return tgt.at[idx].add(src)
def _segment_sum(src, seg, n):
    return jax.ops.segment_sum(src, seg, n)
class _Rng:
    def __init__(self, key):
        self._k = key
    def _next(self):
        self._k, sub = jax.random.split(self._k)
        return sub
    def normal(self, shape):
        return jax.random.normal(self._next(), shape, dtype=jnp.bfloat16)
    def randint(self, lo, hi, shape):
        return jax.random.randint(self._next(), shape, lo, hi, dtype=jnp.int32)
    def uniform(self, shape, lo=0.0, hi=1.0):
        return jax.random.uniform(self._next(), shape, jnp.bfloat16, lo, hi)
    def permutation(self, n):
        return jax.random.permutation(self._next(), n)


kernel_name = 'recurrent_scan__ssm_conv_s4__moe_arch_mod__prompt'

def setup_inputs():
    _rng = _Rng(jax.random.key(int.from_bytes(__import__("os").urandom(4), "little")))
    _w = (lambda a: (lambda t: t.astype(jnp.bfloat16) if jnp.issubdtype(t.dtype, jnp.floating) else t)(jnp.asarray(a)))
    def _A_setup():
        B, L, D, N = 1, 2048, 576, 128
        A_re = -jnp.exp((lambda *s: _rng.normal(s) * 0.05)(D, N))
        A_im = jnp.pi * (lambda *s: _rng.normal(s) * 0.05)(D, N)
        B_re = (lambda *s: _rng.normal(s) * 0.05)(D, N)
        B_im = (lambda *s: _rng.normal(s) * 0.05)(D, N)
        C_re = (lambda *s: _rng.normal(s) * 0.05)(D, N)
        C_im = (lambda *s: _rng.normal(s) * 0.05)(D, N)
        log_dt = (lambda *s: _rng.normal(s) * 0.05)(D) * 0.5 - 4.0
        Dskip = (lambda *s: _rng.normal(s) * 0.05)(D)
        return {
            "u": _w((lambda *s: _rng.normal(s) * 0.05)(B, L, D)),
            "A_re": _w(A_re),
            "A_im": _w(A_im),
            "B_re": _w(B_re),
            "B_im": _w(B_im),
            "C_re": _w(C_re),
            "C_im": _w(C_im),
            "log_dt": _w(log_dt),
            "Dskip": _w(Dskip),
        }
    _A_in = _A_setup()

    def _B_setup():
        B, S, D, F, C = 1, 2048, 576, 4608, 8
        return {
            "x": _w((lambda *s: _rng.normal(s) * 0.05)(B, S, D)),
            "w_r": _w((lambda *s: _rng.normal(s) * 0.05)(D)),
            "w_gate": _w((lambda *s: _rng.normal(s) * 0.05)(D, F)),
            "w_up": _w((lambda *s: _rng.normal(s) * 0.05)(D, F)),
            "w_down": _w((lambda *s: _rng.normal(s) * 0.05)(F, D)),
        }
    _B_in = _B_setup()

    return {
        "A_u": _A_in["u"],
        "A_A_re": _A_in["A_re"],
        "A_A_im": _A_in["A_im"],
        "A_B_re": _A_in["B_re"],
        "A_B_im": _A_in["B_im"],
        "A_C_re": _A_in["C_re"],
        "A_C_im": _A_in["C_im"],
        "A_log_dt": _A_in["log_dt"],
        "A_Dskip": _A_in["Dskip"],
        "B_x": _B_in["x"],
        "B_w_r": _B_in["w_r"],
        "B_w_gate": _B_in["w_gate"],
        "B_w_up": _B_in["w_up"],
        "B_w_down": _B_in["w_down"],
    }

def reference(A_u, A_A_re, A_A_im, A_B_re, A_B_im, A_C_re, A_C_im, A_log_dt, A_Dskip, B_x, B_w_r, B_w_gate, B_w_up, B_w_down):
    def _A_ref(u, A_re, A_im, B_re, B_im, C_re, C_im, log_dt, Dskip):
        Bsz, L, D = u.shape
        dt = jnp.exp(log_dt)[:, None]
        A = A_re + 1j * A_im
        Bc = B_re + 1j * B_im
        Cc = C_re + 1j * C_im
        logdA = dt * A
        dB = dt * Bc
        l = (lambda x, dt: x.astype(dt))(jnp.arange(L), A_re.dtype)
        P = jnp.exp(logdA[:, :, None] * l[None, None, :])
        K = jnp.einsum("dn,dnl,dn->dl", Cc, P, dB).real
        L2 = 2 * L
        Kp = jnp.pad(K, ((0, 0), (0, L)))
        up = (lambda x, *d: x.transpose(*d))(u, 0, 2, 1)
        up = jnp.pad(up, ((0, 0), (0, 0), (0, L)))
        Kf = (lambda x, axes=(-2,-1): jnp.fft.rfft2(x.astype(jnp.float32), axes=axes))(Kp[:, None, :], axes=(-2, -1))
        Uf = (lambda x, axes=(-2,-1): jnp.fft.rfft2(x.astype(jnp.float32), axes=axes))(up[:, :, None, :], axes=(-2, -1))
        Yf = Uf * Kf[None, :, :, :]
        y = (lambda x, s, axes=(-2,-1): jnp.fft.irfft2(x, s=s, axes=axes).astype(jnp.bfloat16))(Yf, (1, L2), axes=(-2, -1))[:, :, 0, :L]
        y = (lambda x, *d: x.transpose(*d))(y, 0, 2, 1) + u * Dskip[None, None, :]
        return y

    def _B_ref(x, w_r, w_gate, w_up, w_down):
        B, S, D = x.shape
        C = 8
        r = x @ w_r
        idx = jnp.argsort(-r, axis=-1)[:, :C]
        idx_e = jnp.repeat(idx.reshape(B, C, 1), D, axis=2)
        x_sel = jnp.take_along_axis(x, idx_e, axis=1)
        g = _silu(x_sel @ w_gate)
        u = x_sel @ w_up
        y = (g * u) @ w_down
        r_sel = _sigmoid(jnp.take_along_axis(r, idx, axis=1))
        y = y * r_sel.reshape(B, C, 1)
        b_off = (jnp.arange(B) * S).reshape(B, 1)
        flat_idx = (idx + b_off).reshape(B * C)
        zero = (x * 0.0).reshape(B * S, D)
        upd = _scatter_add(zero, flat_idx, y.reshape(B * C, D), axis=0)
        return x + upd.reshape(B, S, D)

    x = A_u
    xn = _layernorm(x, axis=-1)
    s = _A_ref(xn, A_A_re, A_A_im, A_B_re, A_B_im, A_C_re, A_C_im, A_log_dt, A_Dskip)
    g = _silu(_B_ref(xn, B_w_r, B_w_gate, B_w_up, B_w_down))
    return x + s * g
```

```python
import numpy as np
import jax
import jax.numpy as jnp
from jax import lax
import jax.experimental.pallas as pl
import jax.experimental.pallas.tpu as pltpu

L, D, N, F, C = 2048, 576, 128, 4608, 8
NU = D // 16
CB = 32
NB = D // CB
F32, BF16, I32, U32 = jnp.float32, jnp.bfloat16, jnp.int32, jnp.uint32
EPS = 1e-5


def _bf16_round_np(x):
    u = np.asarray(x, np.float32).view(np.uint32).astype(np.uint64)
    r = ((u + 0x7FFF + ((u >> 16) & 1)) >> 16) << 16
    return r.astype(np.uint32)


_LROUND = _bf16_round_np(np.arange(L)).view(np.float32).astype(np.int64)
_HI = [(1, 3), (5, 7), (4, 260), (8, 264), (516, 1032), (520, 1288), (772, 1544), (776, 1800),
       (2, 258), (6, 262)]


def _lane_l1(l2):
    p = np.arange(128)
    return 32 * ((p // 32) ^ l2) + p % 32


def _make_tables():
    tab = {}
    for p, pair in enumerate(_HI):
        for r2, h in enumerate(pair):
            if p < 8:
                sid, q = 2 * (p // 4) + r2, p % 4
            else:
                sid, q = 4, (p - 8) + 2 * r2
            for jp in range(16):
                for j2 in range(2):
                    tab[h + 16 * jp + 8 * j2] = (sid, 8 * jp + 2 * q + j2)
    lane = np.arange(128)
    pats = []
    for j in range(4):
        pats.append(4 * (lane % 32) + ((lane // 32) ^ j))
    for j in range(4):
        pats.append(32 * ((lane % 4) ^ j) + lane // 4)
    plan = {}
    for dl in range(4):
        for l2 in range(4):
            v = _LROUND[512 * dl + 4 * _lane_l1(l2) + l2]
            sid = np.array([tab[x][0] if x else -1 for x in v])
            ln = np.array([tab[x][1] if x else 0 for x in v])
            steps = []
            for s in sorted(set(sid.tolist()), key=lambda s: -(sid == s).sum()):
                lanes = np.nonzero(sid == s)[0]
                if s < 0:
                    steps.append((-1, None, lanes))
                    continue
                if len(set(ln[lanes].tolist())) == 1:
                    pat = np.full(128, ln[lanes[0]])
                else:
                    pat = np.where(sid == s, ln, 0)
                key = None
                for k, old in enumerate(pats):
                    if np.array_equal(old, pat):
                        key = k
                if key is None:
                    pats.append(pat)
                    key = len(pats) - 1
                steps.append((s, key, lanes))
            plan[dl, l2] = steps
    pats = np.stack(pats).astype(np.int32)
    m = np.arange(128)
    fw = np.zeros((4, 128, 256), np.float64)
    for l2 in range(4):
        t = 4 * _lane_l1(l2) + l2
        th = 2 * np.pi * (2 * m[None, :] + 0.5) * t[:, None] / 1024
        fw[l2, :, :128] = np.cos(th)
        fw[l2, :, 128:] = -np.sin(th)
    fb = _bf16_round_np(fw) >> 16
    fpk = (fb[:, 0::2, :] | (fb[:, 1::2, :] << 16)).astype(np.uint32)
    return plan, pats, fpk


_PLAN, _PATS, _FPK = _make_tables()
_NPAT = _PATS.shape[0]
_PATS_PAD = np.zeros((-(-_NPAT // 8) * 8, 128), np.int32)
_PATS_PAD[:_NPAT] = _PATS


def _cmul(ar, ai, br, bi):
    return ar * br - ai * bi, ar * bi + ai * br


def _sincos(b):
    magic = jnp.float32(12582912.0)
    t = b * jnp.float32(2.0 / np.pi) + magic
    k = t - magic
    ki = pltpu.bitcast(t, I32)
    r = b - k * jnp.float32(1.5703125)
    r = r - k * jnp.float32(0.0004837512969970703)
    r = r - k * jnp.float32(7.549790126404332e-08)
    u = r * r
    ps = (jnp.float32(-0.0001958295761141926) * u + jnp.float32(0.008332725614309311)) * u \
        + jnp.float32(-0.166666641831398)
    sn = r + (r * u) * ps
    pc = ((jnp.float32(2.437065268168226e-05) * u + jnp.float32(-0.0013886778615415096)) * u
          + jnp.float32(0.04166663438081741)) * u + jnp.float32(-0.5)
    cs = pc * u + jnp.float32(1.0)
    odd = (ki & 1) == 1
    s1 = jnp.where(odd, cs, sn)
    c1 = jnp.where(odd, sn, cs)
    sign = jnp.int32(-2147483648)
    s1 = pltpu.bitcast(pltpu.bitcast(s1, I32) ^ ((ki << 30) & sign), F32)
    c1 = pltpu.bitcast(pltpu.bitcast(c1, I32) ^ (((ki + 1) << 30) & sign), F32)
    return s1, c1


def _gather(x, idx):
    return jnp.take_along_axis(x, idx, axis=1, mode="promise_in_bounds")


def _lanes_mask(lanes):
    lane = lax.broadcasted_iota(I32, (8, 128), 1)
    lanes = sorted(int(x) for x in lanes)
    runs, start, prev = [], lanes[0], lanes[0]
    for x in lanes[1:]:
        if x != prev + 1:
            runs.append((start, prev))
            start = x
        prev = x
    runs.append((start, prev))
    m = None
    for a, b in runs:
        t = (lane == a) if a == b else jnp.logical_and(lane >= a, lane <= b)
        m = t if m is None else jnp.logical_or(m, t)
    return m


def _butterfly(p):
    lane = lax.broadcasted_iota(I32, p[0].shape, 1)
    b0 = (lane & 32) != 0
    b1 = (lane & 64) != 0
    t = [jnp.where(b0, p[k ^ 1], p[k]) for k in range(4)]
    return [jnp.where(b1, t[k ^ 2], t[k]) for k in range(4)]


def _fft4(x, sgn):
    (ar, ai), (br, bi), (cr, ci), (dr, di) = x
    s0r, s0i, d0r, d0i = ar + cr, ai + ci, ar - cr, ai - ci
    s1r, s1i, d1r, d1i = br + dr, bi + di, br - dr, bi - di
    y0 = (s0r + s1r, s0i + s1i)
    y2 = (s0r - s1r, s0i - s1i)
    p = (d0r - d1i, d0i + d1r)
    m = (d0r + d1i, d0i - d1r)
    return [y0, p, y2, m] if sgn > 0 else [y0, m, y2, p]


def _silu(z):
    h = z * jnp.float32(0.5)
    return h + h * jnp.tanh(h)


def _rbf(x):
    return x.astype(BF16).astype(F32)


def _pack(x):
    return pltpu.bitcast(x.astype(BF16), I32)


def _unpack(x):
    return pltpu.bitcast(x, BF16).astype(F32)


_NT = (((1,), (1,)), ((), ()))


def _kernel(x_hbm, are_hbm, aim_hbm, bre_hbm, bim_hbm, cre_hbm, cim_hbm, ldt_hbm, dsk_hbm, wr_hbm,
            wg_hbm, wu_hbm, wd_hbm, f_hbm, pat_hbm,
            out_hbm,
            xbuf, par, ldt, dsk, wr, wg, wu, wd, fpk, patr, pats,
            dtcol, skip, hi_re, hi_im, lo_re, lo_im, comp, khat,
            xp, xnp, uhat, yhat, sbuf, oh_ref, yt_ref, obuf,
            sem_in, sem_out):
    small = [(ldt_hbm, ldt), (dsk_hbm, dsk), (pat_hbm, patr), (wr_hbm, wr)]
    small += [(h, par.at[i]) for i, h in enumerate((are_hbm, aim_hbm, bre_hbm, bim_hbm, cre_hbm, cim_hbm))]
    small += [(f_hbm, fpk)]
    cps = [pltpu.make_async_copy(s, d, sem_in.at[i]) for i, (s, d) in enumerate(small)]
    ns = len(cps)
    cp_x = pltpu.make_async_copy(x_hbm, xbuf, sem_in.at[ns])
    cp_g = pltpu.make_async_copy(wg_hbm, wg, sem_in.at[ns + 1])
    cp_u = pltpu.make_async_copy(wu_hbm, wu, sem_in.at[ns + 2])
    wd_rows = [(0, 128), (128, 128), (256, 128), (384, 128), (512, 64)]
    cp_d = [pltpu.make_async_copy(wd_hbm.at[pl.ds(a, n)], wd.at[pl.ds(a, n)], sem_in.at[ns + 3 + i])
            for i, (a, n) in enumerate(wd_rows)]
    for cp in cps + [cp_x, cp_g, cp_u] + cp_d:
        cp.start()

    for cp in cps[:3]:
        cp.wait()
    r128 = lax.broadcasted_iota(I32, (128, 128), 0)
    c128 = lax.broadcasted_iota(I32, (128, 128), 1)
    eye = jnp.where(r128 == c128, 1.0, 0.0).astype(BF16)
    dt_row = jnp.exp(ldt[...].astype(F32).reshape(1, D)).astype(BF16)
    dsk_row = dsk[...].reshape(1, D)
    for t in range(5):
        n = min(128, D - 128 * t)
        for row, dst in ((dt_row, dtcol), (dsk_row, skip)):
            b = jnp.broadcast_to(row[:, 128 * t:128 * t + n], (128, n))
            dst[pl.ds(128 * t, n), :] = lax.dot_general(eye[:n, :n], b, _NT, preferred_element_type=F32)
    for k in range(_NPAT):
        pats[k] = jnp.broadcast_to(patr[pl.ds(k, 1), :], (8, 128))
    for cp in cps[3:]:
        cp.wait()

    def a_prep(u):
        r0 = pl.multiple_of(u * 16, 16)
        rows = pl.ds(r0, 16)
        ev = pl.ds(2 * r0, 16, stride=2)
        od = pl.ds(2 * r0 + 1, 16, stride=2)
        dt = dtcol[rows, :]
        al = dt * par[0, rows, :].astype(F32)
        be = dt * par[1, rows, :].astype(F32)
        cr, ci = _cmul(par[4, rows, :].astype(F32), par[5, rows, :].astype(F32),
                       par[2, rows, :].astype(F32), par[3, rows, :].astype(F32))
        dts = dt * jnp.float32(1.0 / 512)
        cr, ci = cr * dts, ci * dts
        k0 = jnp.sum(cr, axis=1, keepdims=True) * jnp.float32(512.0)
        skip[rows, :] = skip[rows, :] + k0
        s, c = _sincos(be)
        pw = {1: (c, s)}
        e = 1
        while e < 256:
            c, s = (c - s) * (c + s), (c + c) * s
            e *= 2
            pw[e] = (c, s)
        z = {}
        for e in (1, 8, 16, 256):
            mag = jnp.exp(al * jnp.float32(e))
            c, s = pw[e]
            z[e] = (mag * c, mag * s)
        one = jnp.ones((16, 128), F32)
        lo_re[0, ev, :] = one
        lo_im[0, ev, :] = jnp.zeros((16, 128), F32)
        lo_re[0, od, :] = z[8][0]
        lo_im[0, od, :] = -z[8][1]
        n16 = -z[16][1]
        lo_re[1, ev, :] = z[16][0]
        lo_re[1, od, :] = z[16][0]
        lo_im[1, ev, :] = n16
        lo_im[1, od, :] = n16
        slot = {h: (p, r2) for p, pair in enumerate(_HI) for r2, h in enumerate(pair)}

        def put(e, v):
            p, r2 = slot[e]
            hi_re[p, od if r2 else ev, :] = v[0]
            hi_im[p, od if r2 else ev, :] = v[1]

        h = (cr, ci)
        for e in range(1, 9):
            h = _cmul(*h, *z[1])
            put(e, h)
            g, ee = h, e + 256
            while ee in slot:
                g = _cmul(*g, *z[256])
                put(ee, g)
                ee += 256

    sub8 = lax.broadcasted_iota(I32, (8, 128), 0)
    lane8 = lax.broadcasted_iota(I32, (8, 128), 1)

    def a_gen(u):
        cidx = (lane8 & (-8)) + (sub8 & 6) + (lane8 & 1)
        b0 = (lane8 & 2) != 0
        b1 = (lane8 & 4) != 0
        for k in range(4):
            rows = pl.ds(pl.multiple_of(u * 32 + 8 * k, 8), 8)
            vr, vi = lo_re[0, rows, :], lo_im[0, rows, :]
            wr_, wi_ = lo_re[1, rows, :], lo_im[1, rows, :]
            lr, li = [vr], [vi]
            for _ in range(15):
                vr, vi = _cmul(vr, vi, wr_, wi_)
                lr.append(vr)
                li.append(vi)
            lo = jnp.concatenate([jnp.concatenate(lr, axis=0).astype(BF16),
                                  jnp.concatenate(li, axis=0).astype(BF16)], axis=1)
            hi = jnp.concatenate([hi_re[:, rows, :].reshape(80, 128).astype(BF16),
                                  hi_im[:, rows, :].reshape(80, 128).astype(BF16)], axis=1)
            o = lax.dot_general(hi, lo, _NT, preferred_element_type=F32)
            g = [_gather(o[8 * p:8 * p + 8], cidx) for p in range(10)]
            for a in range(2):
                comp[a, rows, :] = jnp.where(b1, jnp.where(b0, g[4 * a + 3], g[4 * a + 2]),
                                             jnp.where(b0, g[4 * a + 1], g[4 * a]))
            comp[2, rows, :] = jnp.where(b0, g[9], g[8])

    def a_dft(u):
        r0 = pl.multiple_of(u * 16, 16)
        ev = pl.ds(2 * r0, 16, stride=2)
        od = pl.ds(2 * r0 + 1, 16, stride=2)
        src = [_pack(comp[0, ev, :]), _pack(comp[0, od, :]), _pack(comp[1, ev, :]), _pack(comp[1, od, :]),
               jnp.where((lane8 & 4) != 0, _pack(comp[2, od, :]), _pack(comp[2, ev, :]))]
        cache = {}

        def gat(s, key):
            if (s, key) not in cache:
                cache[s, key] = _gather(src[s], pats[key])
            return cache[s, key]

        for l2 in range(4):
            tiles = []
            for dl in range(4):
                t = None
                for s, key, lanes in _PLAN[dl, l2]:
                    v = jnp.zeros((8, 128), I32) if s < 0 else gat(s, key)
                    t = v if t is None else jnp.where(_lanes_mask(lanes), v, t)
                tiles.append(t)
            lhs = pltpu.bitcast(jnp.concatenate(tiles, axis=0), BF16)
            res = jnp.dot(lhs, pltpu.bitcast(fpk[l2], BF16), preferred_element_type=F32)
            khat[l2, :, pl.ds(r0, 16), :] = res.reshape(4, 16, 256)

    a_prep(0)
    a_gen(0)
    a_prep(1)

    def a_body(i, carry):
        a_dft(i - 1)
        a_gen(i)
        a_prep(i + 1)
        return carry

    lax.fori_loop(1, NU - 1, a_body, 0)
    a_dft(NU - 2)
    a_gen(NU - 1)
    a_dft(NU - 1)

    cp_x.wait()

    def b_body(b, carry):
        s1 = [jnp.zeros((8, 128), F32) for _ in range(4)]
        s2 = [jnp.zeros((8, 128), F32) for _ in range(4)]
        for u in range(NU):
            p = []
            for j in range(4):
                col = pl.ds(pl.multiple_of(b * 512 + 128 * j, 128), 128)
                p.append(_gather(pltpu.bitcast(xbuf[pl.ds(16 * u, 16), col], I32), pats[j]))
            o = _butterfly(p)
            for l2 in range(4):
                xp[l2, b, pl.ds(8 * u, 8), :] = o[l2]
                f = _unpack(o[l2])
                lo_, hi_ = f[:8], f[8:]
                s1[l2] = s1[l2] + (lo_ + hi_)
                s2[l2] = s2[l2] + (lo_ * lo_ + hi_ * hi_)
        for l2 in range(4):
            m = jnp.sum(s1[l2], axis=0, keepdims=True) * jnp.float32(1.0 / D)
            q = jnp.sum(s2[l2], axis=0, keepdims=True) * jnp.float32(1.0 / D)
            var = _rbf(jnp.maximum(q - m * m, 0.0))
            sd = _rbf(jnp.sqrt(_rbf(var + jnp.float32(EPS))))
            mb = jnp.broadcast_to(_rbf(m), (16, 128))
            rs = jnp.broadcast_to(1.0 / sd, (16, 128))
            for u in range(NU):
                f = _unpack(xp[l2, b, pl.ds(8 * u, 8), :])
                xnp[l2, b, pl.ds(8 * u, 8), :] = _pack((f - mb) * rs)
        return carry

    lax.fori_loop(0, 4, b_body, 0)

    wr16 = jnp.broadcast_to(wr[...].reshape(1, D), (16, D))
    keys, rvals = [], []
    for l2 in range(4):
        for b in range(4):
            r = jnp.dot(wr16, pltpu.bitcast(xnp[l2, b], BF16), preferred_element_type=F32)[:8]
            r = _rbf(r)
            r = jnp.where(r == 0.0, 0.0, r)
            bits = pltpu.bitcast(r, I32)
            mono = ((bits ^ ((bits >> 31) & jnp.int32(0x7FFFFFFF))) >> 16) + 32768
            tok = 512 * b + 4 * (32 * ((lane8 >> 5) ^ l2) + (lane8 & 31)) + l2
            keys.append(pltpu.bitcast((mono << 11) + (2047 - tok) + jnp.int32(0x00800000), F32))
            rvals.append(r)
    oh = [jnp.zeros((8, 128), F32) for _ in range(16)]
    for c in range(C):
        mx = keys[0]
        for t in range(1, 16):
            mx = jnp.maximum(mx, keys[t])
        mx = jnp.max(mx, axis=1, keepdims=True)
        for t in range(16):
            hit = keys[t] == mx
            oh[t] = jnp.where(jnp.logical_and(hit, sub8 == c), 1.0, oh[t])
            keys[t] = jnp.where(hit, 0.0, keys[t])
    rs_acc = oh[0] * rvals[0]
    for t in range(1, 16):
        rs_acc = rs_acc + oh[t] * rvals[t]
    r_sel = jnp.sum(rs_acc, axis=1, keepdims=True)
    gate_r = _rbf(jax.nn.sigmoid(r_sel))
    xsel = jnp.zeros((16, D), F32)
    for l2 in range(4):
        for b in range(4):
            t = 4 * l2 + b
            o16 = jnp.concatenate([oh[t], jnp.zeros((8, 128), F32)], axis=0).astype(BF16)
            oh_ref[t] = pltpu.bitcast(o16, I32)
            xsel = xsel + lax.dot_general(o16, pltpu.bitcast(xnp[l2, b], BF16), _NT,
                                          preferred_element_type=F32)
    xsel = xsel.astype(BF16)

    def c_fwd(i):
        h0 = pl.multiple_of(i * (CB // 2), CB // 2)
        r0 = pl.multiple_of(i * CB, CB)
        for l2 in range(4):
            lhs = pltpu.bitcast(xnp[l2, :, pl.ds(h0, CB // 2), :].reshape(2 * CB, 128), BF16)
            res = jnp.dot(lhs, pltpu.bitcast(fpk[l2], BF16), preferred_element_type=F32)
            uhat[l2, :, pl.ds(r0, CB), :] = res.reshape(4, CB, 256)

    def c_mid(i):
        for k in range(CB // 8):
            rows = pl.ds(pl.multiple_of(i * CB + 8 * k, 8), 8)
            uu = [_fft4([(uhat[l2, b, rows, 0:128], uhat[l2, b, rows, 128:256]) for l2 in range(4)], -1)
                  for b in range(4)]
            kk = [_fft4([(khat[l2, b, rows, 0:128], khat[l2, b, rows, 128:256]) for l2 in range(4)], -1)
                  for b in range(4)]
            yy = [[None] * 4 for _ in range(4)]
            for k2 in range(4):
                kp = [kk[0][k2]] + [(kk[b][k2][0] - kk[b - 1][k2][1], kk[b][k2][1] + kk[b - 1][k2][0])
                                    for b in range(1, 4)]
                for m in range(4):
                    acc = None
                    for b in range(m + 1):
                        t = _cmul(*uu[b][k2], *kp[m - b])
                        acc = t if acc is None else (acc[0] + t[0], acc[1] + t[1])
                    yy[m][k2] = acc
            ww = [_fft4(yy[m], 1) for m in range(4)]
            un = i * (CB // 8) + k
            for l2 in range(4):
                for bp in range(2):
                    for ri in range(2):
                        v = jnp.concatenate([ww[2 * bp][l2][ri], ww[2 * bp + 1][l2][ri]], axis=0)
                        yhat[l2, un, bp, :, 128 * ri:128 * ri + 128] = _pack(v)

    def c_inv(i):
        u0 = i * (CB // 8)
        for l2 in range(4):
            lhs = pltpu.bitcast(yhat[l2, pl.ds(u0, CB // 8)].reshape(2 * CB, 256), BF16)
            y = lax.dot_general(lhs, pltpu.bitcast(fpk[l2], BF16), _NT, preferred_element_type=F32)
            for k in range(CB // 16):
                r0 = pl.multiple_of(i * CB + 16 * k, 16)
                sk = skip[pl.ds(r0, 16), :]
                for b in range(4):
                    xn = _unpack(xnp[l2, b, pl.ds(pl.multiple_of(i * (CB // 2) + 8 * k, 8), 8), :])
                    yb = jnp.concatenate([y[64 * k + 8 * b:64 * k + 8 * b + 8],
                                          y[64 * k + 32 + 8 * b:64 * k + 32 + 8 * b + 8]], axis=0)
                    sbuf[l2, b, pl.ds(r0, 16), :] = yb + xn * sk

    c_fwd(0)
    c_mid(0)
    c_fwd(1)

    def c_body(i, carry):
        c_inv(i - 1)
        c_mid(i)
        c_fwd(i + 1)
        return carry

    lax.fori_loop(1, NB - 1, c_body, 0)
    c_inv(NB - 2)
    c_mid(NB - 1)
    c_inv(NB - 1)

    cp_g.wait()
    ga = _rbf(jnp.dot(xsel, wg[...], preferred_element_type=F32)[:8])
    ga = _rbf(ga * _rbf(jax.nn.sigmoid(ga)))
    cp_u.wait()
    up = _rbf(jnp.dot(xsel, wu[...], preferred_element_type=F32)[:8])
    hh = jnp.concatenate([ga * up, jnp.zeros((8, F), F32)], axis=0).astype(BF16)
    for (a, n), cp in zip(wd_rows, cp_d):
        cp.wait()
        y = lax.dot_general(hh, wd[pl.ds(a, n), :], _NT, preferred_element_type=F32)
        y = jnp.concatenate([_rbf(y[:8]) * gate_r, jnp.zeros((120, n), F32)], axis=0).astype(BF16)
        yt = lax.dot_general(eye[:n, :n], y, _NT, preferred_element_type=F32)
        yt_ref[pl.ds(a // 2, n // 2), :] = _pack(yt)

    def out_copy(i):
        rows = pl.ds(pl.multiple_of(i * CB, CB), CB)
        return pltpu.make_async_copy(obuf.at[rows], out_hbm.at[rows], sem_out.at[i])

    def o_body(i, carry):
        h0 = pl.multiple_of(i * (CB // 2), CB // 2)
        yt = pltpu.bitcast(yt_ref[pl.ds(h0, CB // 2), :], BF16)[:, :16]
        for b in range(4):
            upd = [jnp.dot(yt, pltpu.bitcast(oh_ref[4 * l2 + b], BF16), preferred_element_type=F32)
                   for l2 in range(4)]
            for k in range(CB // 16):
                hr = pl.ds(pl.multiple_of(h0 + 8 * k, 8), 8)
                r0 = pl.multiple_of(i * CB + 16 * k, 16)
                o = []
                for l2 in range(4):
                    z = _unpack(xnp[l2, b, hr, :]) + upd[l2][16 * k:16 * k + 16]
                    v = _unpack(xp[l2, b, hr, :]) + sbuf[l2, b, pl.ds(r0, 16), :] * _silu(z)
                    o.append(_pack(v))
                p = _butterfly(o)
                for j in range(4):
                    obuf[pl.ds(r0, 16), pl.ds(512 * b + 128 * j, 128)] = pltpu.bitcast(
                        _gather(p[j], pats[4 + j]), BF16)
        out_copy(i).start()
        return carry

    lax.fori_loop(0, NB, o_body, 0)
    for i in range(NB):
        out_copy(i).wait()


def _scratch():
    return [
        pltpu.VMEM((D, L), BF16),
        pltpu.VMEM((6, D, N), BF16),
        pltpu.VMEM((D,), BF16),
        pltpu.VMEM((D,), BF16),
        pltpu.VMEM((D,), BF16),
        pltpu.VMEM((D, F), BF16),
        pltpu.VMEM((D, F), BF16),
        pltpu.VMEM((D, F), BF16),
        pltpu.VMEM((4, 64, 256), U32),
        pltpu.VMEM(_PATS_PAD.shape, I32),
        pltpu.VMEM((_NPAT, 8, 128), I32),
        pltpu.VMEM((D, 128), F32),
        pltpu.VMEM((D, 128), F32),
        pltpu.VMEM((10, 2 * D, 128), F32),
        pltpu.VMEM((10, 2 * D, 128), F32),
        pltpu.VMEM((2, 2 * D, 128), F32),
        pltpu.VMEM((2, 2 * D, 128), F32),
        pltpu.VMEM((3, 2 * D, 128), F32),
        pltpu.VMEM((4, 4, D, 256), F32),
        pltpu.VMEM((4, 4, D // 2, 128), I32),
        pltpu.VMEM((4, 4, D // 2, 128), I32),
        pltpu.VMEM((4, 4, D, 256), F32),
        pltpu.VMEM((4, D // 8, 2, 8, 256), I32),
        pltpu.VMEM((4, 4, D, 128), F32),
        pltpu.VMEM((16, 8, 128), I32),
        pltpu.VMEM((D // 2, 128), I32),
        pltpu.VMEM((D, L), BF16),
        pltpu.SemaphoreType.DMA((19,)),
        pltpu.SemaphoreType.DMA((NB,)),
    ]


@jax.jit
def pallas_recurrent_scan__ssm_conv_s4__moe_arch_mod__prompt_kernel(
    A_u: jax.Array,
    A_A_re: jax.Array,
    A_A_im: jax.Array,
    A_B_re: jax.Array,
    A_B_im: jax.Array,
    A_C_re: jax.Array,
    A_C_im: jax.Array,
    A_log_dt: jax.Array,
    A_Dskip: jax.Array,
    B_x: jax.Array,
    B_w_r: jax.Array,
    B_w_gate: jax.Array,
    B_w_up: jax.Array,
    B_w_down: jax.Array,
):
    hbm = pl.BlockSpec(memory_space=pltpu.HBM)
    out = pl.pallas_call(
        _kernel,
        out_shape=jax.ShapeDtypeStruct((D, L), BF16),
        in_specs=[hbm] * 15,
        out_specs=hbm,
        scratch_shapes=_scratch(),
        compiler_params=pltpu.CompilerParams(vmem_limit_bytes=110 * 1024 * 1024),
        name="s4_mod",
    )(A_u[0].T, A_A_re, A_A_im, A_B_re, A_B_im, A_C_re, A_C_im, A_log_dt, A_Dskip, B_w_r,
      B_w_gate, B_w_up, B_w_down.T, jnp.asarray(_FPK), jnp.asarray(_PATS_PAD))
    return out.T[None]
```

```python
import numpy as np
import jax
import jax.numpy as jnp
from jax import lax
import jax.experimental.pallas as pl
import jax.experimental.pallas.tpu as pltpu

L, D, N, F, C = 2048, 576, 128, 4608, 8
NU = D // 16
CB = 32
NB = D // CB
UA = 2
GA = 4
GC = 4
F32, BF16, I32, U32 = jnp.float32, jnp.bfloat16, jnp.int32, jnp.uint32
EPS = 1e-5


def _bf16_round_np(x):
    u = np.asarray(x, np.float32).view(np.uint32).astype(np.uint64)
    r = ((u + 0x7FFF + ((u >> 16) & 1)) >> 16) << 16
    return r.astype(np.uint32)


_LROUND = _bf16_round_np(np.arange(L)).view(np.float32).astype(np.int64)
_HI = [(1, 3, 516, 1032), (5, 7, 520, 1288), (4, 260, 772, 1544), (8, 264, 776, 1800), (2, 6, 258, 262)]


def _lane_l1(l2):
    p = np.arange(128)
    return 32 * ((p // 32) ^ l2) + p % 32


def _comp_q():
    t = np.arange(8)[:, None]
    lane = np.arange(128)[None, :]
    return ((lane - 8 - 7 * (t % 4)) % 16) // 4


def _make_tables():
    lane = np.arange(128)
    lo = 16 * (2 * (7 - lane // 16) + lane % 2) + 8 * ((lane // 2) % 2)
    tab = [dict(), dict()]
    amask = np.zeros(128, bool)
    for q in range(5):
        for e in range(4):
            for par in range(2):
                t = 4 * par + e
                for h in range(2):
                    src = lane[(lane // 4) % 4 == 2 * h + par]
                    dst = (src + (4 * (q % 4) - 8 * h + 8) + 7 * t) % 128
                    assert np.all(_comp_q()[t, dst] == q % 4)
                    sid = e if q < 4 else 4 + e // 2
                    for sl, dl_ in zip(src, dst):
                        ent = (sid, int(dl_))
                        assert tab[par].setdefault(_HI[q][e] + int(lo[sl]), ent) == ent
                    if q == 4 and e % 2 == 1:
                        amask[dst % 16 + 16 * np.arange(8)[:, None]] = True
    pats = []
    for j in range(4):
        pats.append(np.tile(4 * (lane % 32) + ((lane // 32) ^ j), (8, 1)))
    for j in range(4):
        pats.append(np.tile(32 * ((lane % 4) ^ j) + lane // 4, (8, 1)))
    npat0 = len(pats)
    tiles, tile_of = [], {}
    for dl in range(4):
        for l2 in range(4):
            v = _LROUND[512 * dl + 4 * lane + l2]
            key = tuple(v.tolist())
            if key in tile_of:
                tile_of[dl, l2] = tile_of[key]
                continue
            sid = np.array([tab[0][x][0] if x else -1 for x in v])
            ln = np.array([[tab[s8 % 2][x][1] if x else 0 for x in v] for s8 in range(8)])
            steps = []
            for s in sorted(set(sid.tolist()), key=lambda s: -(sid == s).sum()):
                lanes = np.nonzero(sid == s)[0]
                if s < 0:
                    steps.append((-1, None, lanes))
                    continue
                care = sid == s
                kk = None
                for k in range(npat0, len(pats)):
                    oldp, oldc, olds = pats[k]
                    both = care & oldc
                    if olds == s and np.array_equal(oldp[:, both], ln[:, both]):
                        pats[k] = (np.where(care, ln, oldp), care | oldc, s)
                        kk = k
                        break
                if kk is None:
                    pats.append((np.where(care, ln, 0), care, s))
                    kk = len(pats) - 1
                steps.append((s, kk, lanes))
            tiles.append(steps)
            tile_of[key] = tile_of[dl, l2] = len(tiles) - 1
    pats = np.stack([p if k < npat0 else p[0] for k, p in enumerate(pats)]).astype(np.int32)
    tile_of = {k: v for k, v in tile_of.items() if len(k) == 2}
    m = np.arange(128)
    fw = np.zeros((4, 128, 256), np.float64)
    for l2 in range(4):
        t = 4 * _lane_l1(l2) + l2
        th = 2 * np.pi * (2 * m[None, :] + 0.5) * t[:, None] / 1024
        fw[l2, :, :128] = np.cos(th)
        fw[l2, :, 128:] = -np.sin(th)
    fb = _bf16_round_np(fw) >> 16
    fpk = (fb[:, 0::2, :] | (fb[:, 1::2, :] << 16)).astype(np.uint32)
    masks = np.stack([_comp_q() & 1, _comp_q() >> 1, np.tile(amask, (8, 1))]).astype(np.int32)
    return tiles, tile_of, np.concatenate([pats, masks]), fpk


_TILES, _TILE_OF, _PATS, _FPK = _make_tables()
_NPAT = _PATS.shape[0]
_NT_K = len(_TILES)


def _cmul(ar, ai, br, bi):
    return ar * br - ai * bi, ar * bi + ai * br


def _sincos(b):
    magic = jnp.float32(12582912.0)
    t = b * jnp.float32(2.0 / np.pi) + magic
    k = t - magic
    ki = pltpu.bitcast(t, I32)
    r = b - k * jnp.float32(1.5703125)
    r = r - k * jnp.float32(0.0004837512969970703)
    r = r - k * jnp.float32(7.549790126404332e-08)
    u = r * r
    ps = (jnp.float32(-0.0001958295761141926) * u + jnp.float32(0.008332725614309311)) * u \
        + jnp.float32(-0.166666641831398)
    sn = r + (r * u) * ps
    pc = ((jnp.float32(2.437065268168226e-05) * u + jnp.float32(-0.0013886778615415096)) * u
          + jnp.float32(0.04166663438081741)) * u + jnp.float32(-0.5)
    cs = pc * u + jnp.float32(1.0)
    odd = (ki & 1) == 1
    s1 = jnp.where(odd, cs, sn)
    c1 = jnp.where(odd, sn, cs)
    sign = jnp.int32(-2147483648)
    s1 = pltpu.bitcast(pltpu.bitcast(s1, I32) ^ ((ki << 30) & sign), F32)
    c1 = pltpu.bitcast(pltpu.bitcast(c1, I32) ^ (((ki + 1) << 30) & sign), F32)
    return s1, c1


def _gather(x, idx):
    return jnp.take_along_axis(x, idx, axis=1, mode="promise_in_bounds")


def _lanes_mask(lanes):
    lane = lax.broadcasted_iota(I32, (8, 128), 1)
    lanes = sorted(int(x) for x in lanes)
    runs, start, prev = [], lanes[0], lanes[0]
    for x in lanes[1:]:
        if x != prev + 1:
            runs.append((start, prev))
            start = x
        prev = x
    runs.append((start, prev))
    m = None
    for a, b in runs:
        t = (lane == a) if a == b else jnp.logical_and(lane >= a, lane <= b)
        m = t if m is None else jnp.logical_or(m, t)
    return m


def _butterfly(p):
    lane = lax.broadcasted_iota(I32, p[0].shape, 1)
    b0 = (lane & 32) != 0
    b1 = (lane & 64) != 0
    t = [jnp.where(b0, p[k ^ 1], p[k]) for k in range(4)]
    return [jnp.where(b1, t[k ^ 2], t[k]) for k in range(4)]


def _fft4(x, sgn):
    (ar, ai), (br, bi), (cr, ci), (dr, di) = x
    s0r, s0i, d0r, d0i = ar + cr, ai + ci, ar - cr, ai - ci
    s1r, s1i, d1r, d1i = br + dr, bi + di, br - dr, bi - di
    y0 = (s0r + s1r, s0i + s1i)
    y2 = (s0r - s1r, s0i - s1i)
    p = (d0r - d1i, d0i + d1r)
    m = (d0r + d1i, d0i - d1r)
    return [y0, p, y2, m] if sgn > 0 else [y0, m, y2, p]


def _silu(z):
    h = z * jnp.float32(0.5)
    return h + h * jnp.tanh(h)


def _rbf(x):
    return x.astype(BF16).astype(F32)


def _pack2(a, b):
    p = pltpu.pack_elementwise([a, b], packed_dtype=BF16)
    return p if p.dtype == I32 else pltpu.bitcast(p, I32)


def _unpack2(x):
    return [pltpu.unpack_elementwise(x, index=i, packed_dtype=BF16, unpacked_dtype=F32) for i in range(2)]


def _bf(x):
    return pltpu.bitcast(x, BF16)


_NT = (((1,), (1,)), ((), ()))


class _Idx:
    def __init__(self, i, lag):
        self.i, self.lag = i, lag

    def off(self, stride, const=0, align=None):
        c = const - self.lag * stride
        if isinstance(self.i, int):
            return self.i * stride + c
        v = self.i * stride + c
        return pl.multiple_of(v, align) if align else v


def _pipeline(stages, n):
    ns = len(stages)

    def step(i, lo, hi):
        for k in range(hi - 1, lo - 1, -1):
            stages[k](_Idx(i, k))

    for i in range(ns - 1):
        step(i, 0, i + 1)

    def body(i, carry):
        step(i, 0, ns)
        return carry

    lax.fori_loop(ns - 1, n, body, 0)
    return [lambda i=i: step(n + i, i + 1, ns) for i in range(ns - 1)]


def _kernel(x_hbm, are_hbm, aim_hbm, bre_hbm, bim_hbm, cre_hbm, cim_hbm, ldt_hbm, dsk_hbm, wr_hbm,
            wg_hbm, wu_hbm, wd_hbm, f_hbm, pat_hbm,
            out_hbm,
            xbuf, par, ldt, dsk, wr, wg, wu, wd, fpk, pats,
            dtcol, skip, hi_re, hi_im, lo_re, lo_im, comp, ktile, khat,
            xg, xp, xnp, uhat, yhat, ybuf, oh_ref, yt_ref, updb, opk, obuf,
            sem_in, sem_out):
    small = [(ldt_hbm, ldt), (dsk_hbm, dsk)]
    small += [(h, par.at[i]) for i, h in enumerate((are_hbm, aim_hbm, bre_hbm, bim_hbm, cre_hbm, cim_hbm))]
    small += [(pat_hbm, pats), (f_hbm, fpk), (wr_hbm, wr)]
    cps = [pltpu.make_async_copy(s, d, sem_in.at[i]) for i, (s, d) in enumerate(small)]
    ns = len(cps)
    cp_x = pltpu.make_async_copy(x_hbm, xbuf, sem_in.at[ns])
    cp_g = pltpu.make_async_copy(wg_hbm, wg, sem_in.at[ns + 1])
    cp_u = pltpu.make_async_copy(wu_hbm, wu, sem_in.at[ns + 2])
    wd_rows = [(0, 128), (128, 128), (256, 128), (384, 128), (512, 64)]
    cp_d = [pltpu.make_async_copy(wd_hbm.at[pl.ds(a, n)], wd.at[pl.ds(a, n)], sem_in.at[ns + 3 + i])
            for i, (a, n) in enumerate(wd_rows)]
    for cp in cps + [cp_x, cp_g, cp_u] + cp_d:
        cp.start()

    for cp in cps[:2]:
        cp.wait()
    r128 = lax.broadcasted_iota(I32, (128, 128), 0)
    c128 = lax.broadcasted_iota(I32, (128, 128), 1)
    eye = jnp.where(r128 == c128, 1.0, 0.0).astype(BF16)
    dt_row = jnp.exp(ldt[...].astype(F32).reshape(1, D)).astype(BF16)
    dsk_row = dsk[...].reshape(1, D)
    for t in range(5):
        n = min(128, D - 128 * t)
        for row, dst in ((dt_row, dtcol), (dsk_row, skip)):
            b = jnp.broadcast_to(row[:, 128 * t:128 * t + n], (128, n))
            dst[pl.ds(128 * t, n), :] = lax.dot_general(eye[:n, :n], b, _NT, preferred_element_type=F32)
    for cp in cps[2:]:
        cp.wait()

    sub8 = lax.broadcasted_iota(I32, (8, 128), 0)
    lane8 = lax.broadcasted_iota(I32, (8, 128), 1)

    def dft_fwd(lhs, fmat, store):
        re = [jnp.dot(lhs[l2], fmat(l2, 0), preferred_element_type=F32) for l2 in range(4)]
        s0, d0r, s1, d1r = re[0] + re[2], re[0] - re[2], re[1] + re[3], re[1] - re[3]
        store(0, 0, s0 + s1)
        store(2, 0, s0 - s1)
        im = [jnp.dot(lhs[l2], fmat(l2, 1), preferred_element_type=F32) for l2 in range(4)]
        s0, d0i, s1, d1i = im[0] + im[2], im[0] - im[2], im[1] + im[3], im[1] - im[3]
        store(0, 1, s0 + s1)
        store(2, 1, s0 - s1)
        store(1, 0, d0r + d1i)
        store(1, 1, d0i - d1r)
        store(3, 0, d0r - d1i)
        store(3, 1, d0i + d1r)

    slot = {h: (q, e) for q, ent in enumerate(_HI) for e, h in enumerate(ent)}

    def a_prep(i):
        for u in range(UA):
            rows = pl.ds(i.off(16 * UA, 16 * u, 16), 16)
            ev = pl.ds(i.off(32 * UA, 32 * u), 16, stride=2)
            od = pl.ds(i.off(32 * UA, 32 * u + 1), 16, stride=2)
            dt = dtcol[rows, :]
            al = dt * par[0, rows, :].astype(F32)
            be = dt * par[1, rows, :].astype(F32)
            cr, ci = _cmul(par[4, rows, :].astype(F32), par[5, rows, :].astype(F32),
                           par[2, rows, :].astype(F32), par[3, rows, :].astype(F32))
            dts = dt * jnp.float32(1.0 / 512)
            cr, ci = cr * dts, ci * dts
            k0 = jnp.sum(cr, axis=1, keepdims=True) * jnp.float32(512.0)
            skip[rows, :] = skip[rows, :] + k0
            s, c = _sincos(be)
            pw = {1: (c, s)}
            e = 1
            while e < 256:
                c, s = (c - s) * (c + s), (c + c) * s
                e *= 2
                pw[e] = (c, s)
            z = {}
            for e in (1, 8, 16, 256):
                mag = jnp.exp(al * jnp.float32(e))
                c, s = pw[e]
                z[e] = (mag * c, mag * s)
            lo_re[0, ev, :] = jnp.ones((16, 128), F32)
            lo_im[0, ev, :] = jnp.zeros((16, 128), F32)
            lo_re[0, od, :] = z[8][0]
            lo_im[0, od, :] = -z[8][1]
            n16 = -z[16][1]
            lo_re[1, ev, :] = z[16][0]
            lo_re[1, od, :] = z[16][0]
            lo_im[1, ev, :] = n16
            lo_im[1, od, :] = n16
            pend = {}

            def put(e, v):
                q, ee = slot[e]
                key = (q, ee // 2)
                if key not in pend:
                    pend[key] = (ee % 2, v)
                    return
                w, o = pend.pop(key)
                lo_, hi_ = (o, v) if w == 0 else (v, o)
                dst = od if ee // 2 else ev
                hi_re[q, dst, :] = _pack2(lo_[0], hi_[0])
                hi_im[q, dst, :] = _pack2(lo_[1], hi_[1])

            h = (cr, ci)
            for e in range(1, 9):
                h = _cmul(*h, *z[1])
                put(e, h)
                g, ee = h, e + 256
                while ee in slot:
                    g = _cmul(*g, *z[256])
                    put(ee, g)
                    ee += 256

    def a_gen(i):
        b0 = pats[_NPAT - 3] != 0
        b1 = pats[_NPAT - 2] != 0
        for k in range(4 * UA):
            rows = pl.ds(i.off(32 * UA, 8 * k, 8), 8)
            vr, vi = lo_re[0, rows, :], lo_im[0, rows, :]
            wr_, wi_ = lo_re[1, rows, :], lo_im[1, rows, :]
            lr, li = [], []
            for j in range(8):
                ur, ui = _cmul(vr, vi, wr_, wi_)
                lr.append(_pack2(vr, ur))
                li.append(_pack2(vi, ui))
                if j < 7:
                    vr, vi = _cmul(ur, ui, wr_, wi_)
            lo = jnp.concatenate([jnp.concatenate(lr[::-1], axis=0), jnp.concatenate(li[::-1], axis=0)], axis=1)
            hi = jnp.concatenate([hi_re[:, rows, :].reshape(40, 128), hi_im[:, rows, :].reshape(40, 128)], axis=1)
            o = lax.dot_general(_bf(hi), _bf(lo), _NT, preferred_element_type=F32)
            for h in range(2):
                g = [pltpu.roll(o[16 * q + 8 * h:16 * q + 8 * h + 8], 4 * (q % 4) - 8 * h + 8, 1,
                                stride=7, stride_axis=0) for q in range(5)]
                dst = pl.ds(i.off(64 * UA, 16 * k + 8 * h, 8), 8)
                comp[0, dst, :] = jnp.where(b1, jnp.where(b0, g[3], g[2]), jnp.where(b0, g[1], g[0]))
                comp[1, dst, :] = g[4]

    def a_exp(i):
        bm = pats[_NPAT - 1] != 0
        srcs = []
        for u in range(UA):
            def ld(a, e):
                return _pack2(comp[a, pl.ds(i.off(64 * UA, 64 * u + e), 8, stride=4), :],
                              comp[a, pl.ds(i.off(64 * UA, 64 * u + 32 + e), 8, stride=4), :])

            srcs.append([ld(0, e) for e in range(4)]
                        + [jnp.where(bm, ld(1, 2 * k + 1), ld(1, 2 * k)) for k in range(2)])
        cache = {}

        def gat(s, key):
            if key not in cache:
                cache[key] = [_gather(srcs[u][s], pats[key]) for u in range(UA)]
            return cache[key]

        for tid, steps in enumerate(_TILES):
            t = None
            for s, key, lanes in steps:
                v = [jnp.zeros((8, 128), I32)] * UA if s < 0 else gat(s, key)
                t = v if t is None else [jnp.where(_lanes_mask(lanes), v[u], t[u]) for u in range(UA)]
            ktile[tid, pl.ds(i.off(8 * UA, 0, 8), 8 * UA), :] = jnp.concatenate(t, axis=0)

    def f_nat(l2, ri):
        return _bf(jnp.concatenate([fpk[l2, pl.ds(16 * (j ^ l2), 16), pl.ds(128 * ri, 128)] for j in range(4)],
                                   axis=0))

    def f_swz(l2, ri):
        return _bf(fpk[l2, :, pl.ds(128 * ri, 128)])

    def a_dft(i):
        h0 = i.off(8 * UA, 0, 8)
        r0 = i.off(16 * UA, 0, 16)
        for d0 in range(0, 4, GA):
            lhs = [_bf(jnp.concatenate([ktile[_TILE_OF[dl, l2], pl.ds(h0, 8 * UA), :]
                                        for dl in range(d0, d0 + GA)], axis=0)) for l2 in range(4)]

            def store(k2, ri, v):
                khat[2 * k2 + ri, pl.ds(d0, GA), pl.ds(r0, 16 * UA), :] = v.reshape(GA, 16 * UA, 128)

            dft_fwd(lhs, f_nat, store)

    a_tail = _pipeline([a_prep, a_gen, a_exp, a_dft], NU // UA)

    cp_x.wait()

    def b_gather(b):
        for j in range(4):
            for u in range(NU):
                v = pltpu.bitcast(xbuf[pl.ds(16 * u, 16), pl.ds(512 * b + 128 * j, 128)], I32)
                xg[j, b, pl.ds(8 * u, 8), :] = _gather(v, pats[j])

    def b_norm(b):
        s1 = [jnp.zeros((8, 128), F32) for _ in range(4)]
        s2 = [jnp.zeros((8, 128), F32) for _ in range(4)]
        for u in range(NU):
            o = _butterfly([xg[j, b, pl.ds(8 * u, 8), :] for j in range(4)])
            for l2 in range(4):
                xp[l2, b, pl.ds(8 * u, 8), :] = o[l2]
                e_, o_ = _unpack2(o[l2])
                s1[l2] = s1[l2] + (e_ + o_)
                s2[l2] = s2[l2] + (e_ * e_ + o_ * o_)
        rr = []
        for l2 in range(4):
            m = jnp.sum(s1[l2], axis=0, keepdims=True) * jnp.float32(1.0 / D)
            q = jnp.sum(s2[l2], axis=0, keepdims=True) * jnp.float32(1.0 / D)
            var = _rbf(jnp.maximum(q - m * m, 0.0))
            sd = _rbf(jnp.sqrt(_rbf(var + jnp.float32(EPS))))
            mb = jnp.broadcast_to(_rbf(m), (8, 128))
            rs = jnp.broadcast_to(1.0 / sd, (8, 128))
            for u in range(NU):
                e_, o_ = _unpack2(xp[l2, b, pl.ds(8 * u, 8), :])
                xnp[l2, b, pl.ds(8 * u, 8), :] = _pack2((e_ - mb) * rs, (o_ - mb) * rs)
            rr.append(jnp.dot(wr16, _bf(xnp[l2, b]), preferred_element_type=F32)[:8])
        return rr

    wr16 = jnp.broadcast_to(wr[...].reshape(1, D), (16, D))
    a_tail[0]()
    b_gather(0)
    a_tail[1]()
    b_gather(1)
    a_tail[2]()
    b_gather(2)
    b_gather(3)
    rraw = [b_norm(b) for b in range(4)]

    def c_fwd(i):
        h0 = i.off(CB // 2, 0, 8)
        r0 = i.off(CB, 0, 8)
        for b0 in range(0, 4, GC):
            lhs = [_bf(xnp[l2, pl.ds(b0, GC), pl.ds(h0, CB // 2), :].reshape(GC * CB // 2, 128))
                   for l2 in range(4)]

            def store(k2, ri, v):
                uhat[2 * k2 + ri, pl.ds(b0, GC), pl.ds(r0, CB), :] = v.reshape(GC, CB, 128)

            dft_fwd(lhs, f_swz, store)

    def c_mid(i):
        for k in range(CB // 8):
            rows = pl.ds(i.off(CB, 8 * k, 8), 8)
            krows = pl.ds(i.off(CB, 16 * (k // 2) + k % 2), 8, stride=2)
            yy = [[None] * 4 for _ in range(4)]
            for k2 in range(4):
                uu = [(uhat[2 * k2, b, rows, :], uhat[2 * k2 + 1, b, rows, :]) for b in range(4)]
                kk = [(khat[2 * k2, b, krows, :], khat[2 * k2 + 1, b, krows, :]) for b in range(4)]
                pp = []
                for m in range(4):
                    acc = None
                    for b in range(m + 1):
                        t = _cmul(*uu[b], *kk[m - b])
                        acc = t if acc is None else (acc[0] + t[0], acc[1] + t[1])
                    pp.append(acc)
                    yy[m][k2] = acc if m == 0 else (acc[0] - pp[m - 1][1], acc[1] + pp[m - 1][0])
            ww = [_fft4(yy[m], 1) for m in range(4)]
            un = i.off(CB // 8, k)
            for l2 in range(4):
                for bp in range(2):
                    for ri in range(2):
                        yhat[l2, bp, un, :, pl.ds(128 * ri, 128)] = _pack2(ww[2 * bp][l2][ri],
                                                                           ww[2 * bp + 1][l2][ri])

    def c_inv(i):
        u0 = i.off(CB // 8)
        r0 = i.off(2 * CB, 0, 8)
        for l2 in range(4):
            lhs = _bf(yhat[l2, :, pl.ds(u0, CB // 8)].reshape(2 * CB, 256))
            y = lax.dot_general(lhs, _bf(fpk[l2]), _NT, preferred_element_type=F32)
            ybuf[l2, :, pl.ds(r0, 2 * CB), :] = y.reshape(2, 2 * CB, 128)

    keys, rvals = [], []
    for l2 in range(4):
        for b in range(4):
            r = _rbf(rraw[b][l2])
            r = jnp.where(r == 0.0, 0.0, r)
            bits = pltpu.bitcast(r, I32)
            mono = ((bits ^ ((bits >> 31) & jnp.int32(0x7FFFFFFF))) >> 16) + 32768
            tok = 512 * b + 4 * (32 * ((lane8 >> 5) ^ l2) + (lane8 & 31)) + l2
            keys.append(pltpu.bitcast((mono << 11) + (2047 - tok) + jnp.int32(0x00800000), F32))
            rvals.append(r)
    oh = [jnp.zeros((8, 128), F32) for _ in range(16)]
    for c in range(C):
        mx = keys[0]
        for t in range(1, 16):
            mx = jnp.maximum(mx, keys[t])
        mx = jnp.max(mx, axis=1, keepdims=True)
        for t in range(16):
            hit = keys[t] == mx
            oh[t] = jnp.where(jnp.logical_and(hit, sub8 == c), 1.0, oh[t])
            keys[t] = jnp.where(hit, 0.0, keys[t])
    rs_acc = oh[0] * rvals[0]
    for t in range(1, 16):
        rs_acc = rs_acc + oh[t] * rvals[t]
    r_sel = jnp.sum(rs_acc, axis=1, keepdims=True)
    gate_r = _rbf(jax.nn.sigmoid(r_sel))
    for t in range(16):
        o16 = jnp.concatenate([oh[t], jnp.zeros((8, 128), F32)], axis=0).astype(BF16)
        oh_ref[t] = pltpu.bitcast(o16, I32)

    c_tail = _pipeline([c_fwd, c_mid, c_inv], NB)
    c_tail[0]()
    xsel = jnp.zeros((16, D), F32)
    for l2 in range(4):
        for b in range(4):
            xsel = xsel + lax.dot_general(_bf(oh_ref[4 * l2 + b]), _bf(xnp[l2, b]), _NT,
                                          preferred_element_type=F32)
    xsel = xsel.astype(BF16)
    c_tail[1]()

    cp_g.wait()
    ga = _rbf(jnp.dot(xsel, wg[...], preferred_element_type=F32)[:8])
    ga = _rbf(ga * _rbf(jax.nn.sigmoid(ga)))
    cp_u.wait()
    up = _rbf(jnp.dot(xsel, wu[...], preferred_element_type=F32)[:8])
    hh = jnp.concatenate([ga * up, jnp.zeros((8, F), F32)], axis=0).astype(BF16)
    pr = (r128 & (-16)) + 4 * (r128 & 3) + ((r128 >> 2) & 1) + 2 * ((r128 >> 3) & 1)
    perm = jnp.where(pr == c128, 1.0, 0.0).astype(BF16)

    def transpose_y(a, n, y):
        y = jnp.concatenate([_rbf(y[:8]) * gate_r, jnp.zeros((8, n), F32)], axis=0).astype(BF16)
        yt = lax.dot_general(perm[:n, :n], y, _NT, preferred_element_type=F32)
        for u in range(n // 16):
            yt_ref[pl.ds(a // 2 + 8 * u, 8), :] = _pack2(yt[16 * u:16 * u + 8], yt[16 * u + 8:16 * u + 16])

    prev = None
    for (a, n), cp in zip(wd_rows, cp_d):
        cp.wait()
        y = lax.dot_general(hh, wd[pl.ds(a, n), :], _NT, preferred_element_type=F32)
        if prev is not None:
            transpose_y(*prev)
        prev = (a, n, y)
    transpose_y(*prev)

    def out_copy(i):
        rows = pl.ds(i.off(CB, 0, 16), CB)
        return pltpu.make_async_copy(obuf.at[rows], out_hbm.at[rows], sem_out.at[i.off(1)])

    def o_upd(i):
        yt = _bf(yt_ref[pl.ds(i.off(CB // 2, 0, 8), CB // 2), :])
        for t in range(16):
            updb[t, pl.ds(i.off(CB, 0, 8), CB), :] = jnp.dot(yt, _bf(oh_ref[t]),
                                                                         preferred_element_type=F32)

    def o_elt(i):
        for k in range(CB // 16):
            hr = pl.ds(i.off(CB // 2, 8 * k, 8), 8)
            sk = [skip[pl.ds(i.off(CB, 16 * k + e), 8, stride=2), :] for e in range(2)]
            for b in range(4):
                o = []
                for l2 in range(4):
                    xn = _unpack2(xnp[l2, b, hr, :])
                    xx = _unpack2(xp[l2, b, hr, :])
                    v = []
                    for e in range(2):
                        y = ybuf[l2, b // 2, pl.ds(i.off(2 * CB, 32 * k + 2 * e + b % 2), 8, stride=4), :]
                        z = xn[e] + updb[4 * l2 + b, pl.ds(i.off(CB, 16 * k + 8 * e, 8), 8), :]
                        v.append(xx[e] + (y + xn[e] * sk[e]) * _silu(z))
                    o.append(_pack2(*v))
                p = _butterfly(o)
                for j in range(4):
                    opk[j, b, hr, :] = p[j]

    def o_out(i):
        for j in range(4):
            for b in range(4):
                for k in range(CB // 16):
                    hr = pl.ds(i.off(CB // 2, 8 * k, 8), 8)
                    r0 = i.off(CB, 16 * k, 16)
                    obuf[pl.ds(r0, 16), pl.ds(512 * b + 128 * j, 128)] = _bf(_gather(opk[j, b, hr, :], pats[4 + j]))
        out_copy(i).start()

    for fn in _pipeline([o_upd, o_elt, o_out], NB):
        fn()
    for i in range(NB):
        out_copy(_Idx(i, 0)).wait()


def _scratch():
    return [
        pltpu.VMEM((D, L), BF16),
        pltpu.VMEM((6, D, N), BF16),
        pltpu.VMEM((D,), BF16),
        pltpu.VMEM((D,), BF16),
        pltpu.VMEM((D,), BF16),
        pltpu.VMEM((D, F), BF16),
        pltpu.VMEM((D, F), BF16),
        pltpu.VMEM((D, F), BF16),
        pltpu.VMEM((4, 64, 256), U32),
        pltpu.VMEM((_NPAT, 8, 128), I32),
        pltpu.VMEM((D, 128), F32),
        pltpu.VMEM((D, 128), F32),
        pltpu.VMEM((5, 2 * D, 128), I32),
        pltpu.VMEM((5, 2 * D, 128), I32),
        pltpu.VMEM((2, 2 * D, 128), F32),
        pltpu.VMEM((2, 2 * D, 128), F32),
        pltpu.VMEM((2, 4 * D, 128), F32),
        pltpu.VMEM((_NT_K, D // 2, 128), I32),
        pltpu.VMEM((8, 4, D, 128), F32),
        pltpu.VMEM((4, 4, D // 2, 128), I32),
        pltpu.VMEM((4, 4, D // 2, 128), I32),
        pltpu.VMEM((4, 4, D // 2, 128), I32),
        pltpu.VMEM((8, 4, D, 128), F32),
        pltpu.VMEM((4, 2, D // 8, 8, 256), I32),
        pltpu.VMEM((4, 2, 2 * D, 128), F32),
        pltpu.VMEM((16, 8, 128), I32),
        pltpu.VMEM((D // 2, 16), I32),
        pltpu.VMEM((16, D, 128), F32),
        pltpu.VMEM((4, 4, D // 2, 128), I32),
        pltpu.VMEM((D, L), BF16),
        pltpu.SemaphoreType.DMA((19,)),
        pltpu.SemaphoreType.DMA((NB,)),
    ]


@jax.jit
def pallas_recurrent_scan__ssm_conv_s4__moe_arch_mod__prompt_kernel(
    A_u: jax.Array,
    A_A_re: jax.Array,
    A_A_im: jax.Array,
    A_B_re: jax.Array,
    A_B_im: jax.Array,
    A_C_re: jax.Array,
    A_C_im: jax.Array,
    A_log_dt: jax.Array,
    A_Dskip: jax.Array,
    B_x: jax.Array,
    B_w_r: jax.Array,
    B_w_gate: jax.Array,
    B_w_up: jax.Array,
    B_w_down: jax.Array,
):
    hbm = pl.BlockSpec(memory_space=pltpu.HBM)
    out = pl.pallas_call(
        _kernel,
        out_shape=jax.ShapeDtypeStruct((D, L), BF16),
        in_specs=[hbm] * 15,
        out_specs=hbm,
        scratch_shapes=_scratch(),
        compiler_params=pltpu.CompilerParams(vmem_limit_bytes=110 * 1024 * 1024),
        name="s4_mod",
    )(A_u[0].T, A_A_re, A_A_im, A_B_re, A_B_im, A_C_re, A_C_im, A_log_dt, A_Dskip, B_w_r,
      B_w_gate, B_w_up, B_w_down.T, jnp.asarray(_FPK), jnp.asarray(_PATS))
    return out.T[None]
```

```python
import numpy as np
import jax
import jax.numpy as jnp
from jax import lax
import jax.experimental.pallas as pl
import jax.experimental.pallas.tpu as pltpu

L, D, N, F, C = 2048, 576, 128, 4608, 8
NU = D // 16
CB = 64
NB = D // CB
CO = 32
NO = D // CO
UA = 4
F32, BF16, I32, U32 = jnp.float32, jnp.bfloat16, jnp.int32, jnp.uint32
EPS = 1e-5
_DEV = {}


def _bf16_round_np(x):
    u = np.asarray(x, np.float32).view(np.uint32).astype(np.uint64)
    r = ((u + 0x7FFF + ((u >> 16) & 1)) >> 16) << 16
    return r.astype(np.uint32)


_LROUND = _bf16_round_np(np.arange(L)).view(np.float32).astype(np.int64)
_HI = [(1, 3, 516, 1032), (5, 7, 520, 1288), (4, 260, 772, 1544), (8, 264, 776, 1800), (2, 6, 258, 262)]


def _lane_l1(l2):
    p = np.arange(128)
    return 32 * ((p // 32) ^ l2) + p % 32


def _comp_q():
    t = np.arange(8)[:, None]
    lane = np.arange(128)[None, :]
    return ((lane - 8 - 7 * (t % 4)) % 16) // 4


def _make_tables():
    lane = np.arange(128)
    lo = 8 * (4 * (lane // 16) + lane % 4)
    tab = [dict(), dict()]
    amask = np.zeros(128, bool)
    for q in range(5):
        for e in range(4):
            for par in range(2):
                t = 4 * par + e
                for h in range(2):
                    src = lane[(lane // 4) % 4 == 2 * h + par]
                    dst = (src + (4 * (q % 4) - 8 * h + 8) + 7 * t) % 128
                    assert np.all(_comp_q()[t, dst] == q % 4)
                    sid = e if q < 4 else 4 + e // 2
                    for sl, dl_ in zip(src, dst):
                        ent = (sid, int(dl_))
                        assert tab[par].setdefault(_HI[q][e] + int(lo[sl]), ent) == ent
                    if q == 4 and e % 2 == 1:
                        amask[dst % 16 + 16 * np.arange(8)[:, None]] = True
    pats = []
    for j in range(4):
        pats.append(np.tile(4 * (lane % 32) + ((lane // 32) ^ j), (8, 1)))
    for j in range(4):
        pats.append(np.tile(32 * ((lane % 4) ^ j) + lane // 4, (8, 1)))
    npat0 = len(pats)
    tiles, tile_of = [], {}
    for dl in range(4):
        for l2 in range(4):
            v = _LROUND[512 * dl + 4 * lane + l2]
            key = tuple(v.tolist())
            if key in tile_of:
                tile_of[dl, l2] = tile_of[key]
                continue
            sid = np.array([tab[0][x][0] if x else -1 for x in v])
            ln = np.array([[tab[s8 % 2][x][1] if x else 0 for x in v] for s8 in range(8)])
            steps = []
            for s in sorted(set(sid.tolist()), key=lambda s: -(sid == s).sum()):
                lanes = np.nonzero(sid == s)[0]
                if s < 0:
                    steps.append((-1, None, lanes))
                    continue
                care = sid == s
                kk = None
                for k in range(npat0, len(pats)):
                    oldp, oldc, olds = pats[k]
                    both = care & oldc
                    if olds == s and np.array_equal(oldp[:, both], ln[:, both]):
                        pats[k] = (np.where(care, ln, oldp), care | oldc, s)
                        kk = k
                        break
                if kk is None:
                    pats.append((np.where(care, ln, 0), care, s))
                    kk = len(pats) - 1
                steps.append((s, kk, lanes))
            tiles.append(steps)
            tile_of[key] = tile_of[dl, l2] = len(tiles) - 1
    pats = np.stack([p if k < npat0 else p[0] for k, p in enumerate(pats)]).astype(np.int32)
    tile_of = {k: v for k, v in tile_of.items() if len(k) == 2}
    m = np.arange(128)
    fw = np.zeros((4, 128, 256), np.float64)
    for l2 in range(4):
        t = 4 * _lane_l1(l2) + l2
        th = 2 * np.pi * (2 * m[None, :] + 0.5) * t[:, None] / 1024
        fw[l2, :, :128] = np.cos(th)
        fw[l2, :, 128:] = -np.sin(th)
    fb = _bf16_round_np(fw) >> 16
    fpk = (fb[:, 0::2, :] | (fb[:, 1::2, :] << 16)).astype(np.uint32)
    masks = np.stack([_comp_q() & 1, _comp_q() >> 1, np.tile(amask, (8, 1))]).astype(np.int32)
    return tiles, tile_of, np.concatenate([pats, masks]), fpk


_TILES, _TILE_OF, _PATS, _FPK = _make_tables()
_NPAT = _PATS.shape[0]
_NT_K = len(_TILES)


def _cmul(ar, ai, br, bi):
    return ar * br - ai * bi, ar * bi + ai * br


def _sincos(b):
    magic = jnp.float32(12582912.0)
    t = b * jnp.float32(2.0 / np.pi) + magic
    k = t - magic
    ki = pltpu.bitcast(t, I32)
    r = b - k * jnp.float32(1.5703125)
    r = r - k * jnp.float32(0.0004837512969970703)
    r = r - k * jnp.float32(7.549790126404332e-08)
    u = r * r
    ps = (jnp.float32(-0.0001958295761141926) * u + jnp.float32(0.008332725614309311)) * u \
        + jnp.float32(-0.166666641831398)
    sn = r + (r * u) * ps
    pc = ((jnp.float32(2.437065268168226e-05) * u + jnp.float32(-0.0013886778615415096)) * u
          + jnp.float32(0.04166663438081741)) * u + jnp.float32(-0.5)
    cs = pc * u + jnp.float32(1.0)
    odd = (ki & 1) == 1
    s1 = jnp.where(odd, cs, sn)
    c1 = jnp.where(odd, sn, cs)
    sign = jnp.int32(-2147483648)
    s1 = pltpu.bitcast(pltpu.bitcast(s1, I32) ^ ((ki << 30) & sign), F32)
    c1 = pltpu.bitcast(pltpu.bitcast(c1, I32) ^ (((ki + 1) << 30) & sign), F32)
    return s1, c1


def _gather(x, idx):
    return jnp.take_along_axis(x, idx, axis=1, mode="promise_in_bounds")


def _lanes_mask(lanes):
    lane = lax.broadcasted_iota(I32, (8, 128), 1)
    lanes = sorted(int(x) for x in lanes)
    runs, start, prev = [], lanes[0], lanes[0]
    for x in lanes[1:]:
        if x != prev + 1:
            runs.append((start, prev))
            start = x
        prev = x
    runs.append((start, prev))
    m = None
    for a, b in runs:
        t = (lane == a) if a == b else jnp.logical_and(lane >= a, lane <= b)
        m = t if m is None else jnp.logical_or(m, t)
    return m


def _butterfly(p):
    lane = lax.broadcasted_iota(I32, p[0].shape, 1)
    b0 = (lane & 32) != 0
    b1 = (lane & 64) != 0
    t = [jnp.where(b0, p[k ^ 1], p[k]) for k in range(4)]
    return [jnp.where(b1, t[k ^ 2], t[k]) for k in range(4)]


def _fft4(x, sgn):
    (ar, ai), (br, bi), (cr, ci), (dr, di) = x
    s0r, s0i, d0r, d0i = ar + cr, ai + ci, ar - cr, ai - ci
    s1r, s1i, d1r, d1i = br + dr, bi + di, br - dr, bi - di
    y0 = (s0r + s1r, s0i + s1i)
    y2 = (s0r - s1r, s0i - s1i)
    p = (d0r - d1i, d0i + d1r)
    m = (d0r + d1i, d0i - d1r)
    return [y0, p, y2, m] if sgn > 0 else [y0, m, y2, p]


def _silu(z):
    h = z * jnp.float32(0.5)
    return h + h * jnp.tanh(h)


def _rbf(x):
    return x.astype(BF16).astype(F32)


def _pack2(a, b):
    p = pltpu.pack_elementwise([a, b], packed_dtype=BF16)
    return p if p.dtype == I32 else pltpu.bitcast(p, I32)


def _unpack2(x):
    return [pltpu.unpack_elementwise(x, index=i, packed_dtype=BF16, unpacked_dtype=F32) for i in range(2)]


def _bf(x):
    return pltpu.bitcast(x, BF16)


_NT = (((1,), (1,)), ((), ()))


class _Idx:
    def __init__(self, i, lag, z=None):
        self.i, self.lag, self.z = i, lag, z

    def off(self, stride, const=0, align=None):
        c = const - self.lag * stride
        if isinstance(self.i, int):
            if self.z is None:
                return self.i * stride + c
            v = self.z + (self.i * stride + c)
        else:
            v = self.i * stride + c
        return pl.multiple_of(v, align) if align else v

    def idx(self):
        return self.i - self.lag


def _pipeline(stages, n, newz, weave=None, reset=None):
    ns = len(stages)

    def step(i, lo, hi):
        z = newz() if isinstance(i, int) else None
        gens = {k: stages[k](_Idx(i, k, z)) for k in range(lo, hi)}
        if reset is not None:
            reset()
        if callable(weave):
            weave(gens)
        else:
            for k in weave or ():
                if k in gens:
                    next(gens[k], None)
        for k in range(hi - 1, lo - 1, -1):
            for _ in gens[k]:
                pass

    def body(i, carry):
        step(i, 0, ns)
        return carry

    return ([lambda i=i: step(i, 0, i + 1) for i in range(ns - 1)],
            lambda: lax.fori_loop(ns - 1, n, body, 0),
            [lambda i=i: step(n + i, i + 1, ns) for i in range(ns - 1)])


def _run(fns):
    for fn in fns:
        fn()


def _kernel(x_hbm, are_hbm, aim_hbm, bre_hbm, bim_hbm, cre_hbm, cim_hbm, ldt_hbm, dsk_hbm, wr_hbm,
            wg_hbm, wu_hbm, wd_hbm, f_hbm, pat_hbm,
            out_hbm,
            xbuf, par, ldt, dsk, wr, wg, wu, wd, fpk, pats,
            dtcol, skip, hi_re, hi_im, lo_re, lo_im, comp, khat,
            xp, xnp, uhat, yhat, ybuf, spk, topk, posv, cols, opk, og, obuf,
            sem_in, sem_out, *perb):
    xg = perb
    small = [(ldt_hbm, ldt), (dsk_hbm, dsk)]
    small += [(h, par.at[i]) for i, h in enumerate((are_hbm, aim_hbm, bre_hbm, bim_hbm, cre_hbm, cim_hbm))]
    small += [(pat_hbm, pats), (f_hbm, fpk), (wr_hbm, wr)]
    cps = [pltpu.make_async_copy(s, d, sem_in.at[i]) for i, (s, d) in enumerate(small)]
    ns = len(cps)
    cp_x = pltpu.make_async_copy(x_hbm, xbuf, sem_in.at[ns])
    cp_g = pltpu.make_async_copy(wg_hbm, wg, sem_in.at[ns + 1])
    cp_u = pltpu.make_async_copy(wu_hbm, wu, sem_in.at[ns + 2])
    wd_rows = [(0, 128), (128, 128), (256, 128), (384, 128), (512, 64)]
    cp_d = [pltpu.make_async_copy(wd_hbm.at[pl.ds(a, n)], wd.at[pl.ds(a, n)], sem_in.at[ns + 3 + i])
            for i, (a, n) in enumerate(wd_rows)]
    for cp in cps + [cp_x, cp_g, cp_u] + cp_d:
        cp.start()

    for cp in cps[:2]:
        cp.wait()
    r128 = lax.broadcasted_iota(I32, (128, 128), 0)
    c128 = lax.broadcasted_iota(I32, (128, 128), 1)
    eye = jnp.where(r128 == c128, 1.0, 0.0).astype(BF16)
    dt_row = jnp.exp(ldt[...].astype(F32).reshape(1, D)).astype(BF16)
    dsk_row = dsk[...].reshape(1, D)
    for t in range(5):
        n = min(128, D - 128 * t)
        for row, dst in ((dt_row, dtcol), (dsk_row, skip)):
            b = jnp.broadcast_to(row[:, 128 * t:128 * t + n], (128, n))
            dst[pl.ds(128 * t, n), :] = lax.dot_general(eye[:n, :n], b, _NT, preferred_element_type=F32)
    for cp in cps[2:]:
        cp.wait()

    sub8 = lax.broadcasted_iota(I32, (8, 128), 0)
    lane8 = lax.broadcasted_iota(I32, (8, 128), 1)
    zero = pats[0, 0, 0]
    zcount = [0]

    def newz():
        zcount[0] += 1
        return zero * (64 * zcount[0]) if _DEV.get("zpeel", 1) else None

    def after(x, deps):
        never = pats[0] < 0
        for v in deps:
            x = jnp.where(never, v if v.dtype == x.dtype else pltpu.bitcast(v, x.dtype), x)
        return x

    class Sched:
        tok, g, pre = {}, 0, []

        @classmethod
        def reset(cls):
            cls.tok, cls.g, cls.pre = {}, 0, []

        @classmethod
        def gate(cls, x):
            deps = cls.tok.pop(cls.g, [])
            cls.g += 1
            if not deps or not _DEV.get("gate", 1):
                return x
            return jnp.concatenate([after(x[:8], deps), after(x[8:], deps[-1:])], axis=0)

    slot = {h: (q, e) for q, ent in enumerate(_HI) for e, h in enumerate(ent)}

    def a_prep(i):
        gate = Sched.gate
        for u in range(UA):
            rows = pl.ds(i.off(16 * UA, 16 * u, 16), 16)
            ev = pl.ds(i.off(32 * UA, 32 * u), 16, stride=2)
            od = pl.ds(i.off(32 * UA, 32 * u + 1), 16, stride=2)
            dt = gate(dtcol[rows, :])
            al = dt * par[0, rows, :].astype(F32)
            be = dt * par[1, rows, :].astype(F32)
            cr, ci = _cmul(par[4, rows, :].astype(F32), par[5, rows, :].astype(F32),
                           par[2, rows, :].astype(F32), par[3, rows, :].astype(F32))
            dts = dt * jnp.float32(1.0 / 512)
            cr, ci = cr * dts, ci * dts
            k0 = jnp.sum(cr, axis=1, keepdims=True) * jnp.float32(512.0)
            skip[rows, :] = skip[rows, :] + k0
            yield cr
            s, c = _sincos(gate(be))
            yield c
            pw = {1: (c, s)}
            e = 1
            while e < 256:
                if e in (1, 16):
                    c = gate(c)
                c, s = (c - s) * (c + s), (c + c) * s
                e *= 2
                pw[e] = (c, s)
                if e in (16, 256):
                    yield c
            z = {}
            for e in (1, 8, 256):
                mag = jnp.exp(al * jnp.float32(e))
                c, s = pw[e]
                z[e] = (mag * c, mag * s)
            pend = {}

            def put(tab, q, ee, v):
                key = (tab[0] is hi_re, q, ee // 2)
                if key not in pend:
                    pend[key] = (ee % 2, v)
                    return
                w, o = pend.pop(key)
                lo_, hi_ = (o, v) if w == 0 else (v, o)
                dst = od if ee // 2 else ev
                tab[0][q, dst, :] = _pack2(lo_[0], hi_[0])
                tab[1][q, dst, :] = _pack2(lo_[1], hi_[1])

            h = (cr, ci)
            cnt = 0
            for e in range(1, 9):
                g, ee, m = h, e, z[1]
                while ee in slot:
                    if cnt % 4 == 0:
                        g = (gate(g[0]), g[1])
                    g = _cmul(*g, *m)
                    put((hi_re, hi_im), *slot[ee], g)
                    if ee == e:
                        h = g
                    ee, m = ee + 256, z[256]
                    cnt += 1
                    if cnt % 4 == 0:
                        yield g[0]
            w1 = (gate(z[8][0]), -z[8][1])
            v = [(jnp.ones((16, 128), F32), jnp.zeros((16, 128), F32)), w1]
            v.append(_cmul(*w1, *w1))
            v.append(_cmul(*v[2], *w1))
            w4 = _cmul(*v[2], *v[2])
            for j in range(8):
                for f in range(4):
                    put((lo_re, lo_im), j, f, v[f])
                yield v[3][0]
                if j < 7:
                    w4 = (gate(w4[0]), w4[1])
                    v = [w4 if (j == 0 and f == 0) else _cmul(*v[f], *w4) for f in range(4)]

    def a_gen(i):
        b0 = pats[_NPAT - 3] != 0
        b1 = pats[_NPAT - 2] != 0
        g0, gs = _DEV.get("g0", 13), _DEV.get("gs", 9)
        rate = _DEV.get("rate", 1.0)
        for k in range(4 * UA):
            rows = pl.ds(i.off(32 * UA, 8 * k, 8), 8)
            lo = jnp.concatenate([lo_re[:, rows, :].reshape(64, 128), lo_im[:, rows, :].reshape(64, 128)], axis=1)
            h0 = hi_re[0, rows, :]
            if k % 2 == 0 and Sched.pre and _DEV.get("gate", 1):
                h0 = after(h0, Sched.pre)
                Sched.pre = []
            hi = jnp.concatenate([jnp.concatenate([h0, hi_re[1:5, rows, :].reshape(32, 128)], axis=0),
                                  hi_im[:, rows, :].reshape(40, 128)], axis=1)
            o = lax.dot_general(_bf(hi), _bf(lo), _NT, preferred_element_type=F32)
            for q in range(5):
                Sched.tok.setdefault(g0 + int(rate * (5 * (k // 2) + q)), []).append(o[16 * q + 8:16 * q + 16])
            for h in range(2):
                g = [pltpu.roll(o[16 * q + 8 * h:16 * q + 8 * h + 8], 4 * (q % 4) - 8 * h + 8, 1,
                                stride=7, stride_axis=0) for q in range(5)]
                dst = pl.ds(i.off(64 * UA, 16 * k + 8 * h, 8), 8)
                v = jnp.where(b1, jnp.where(b0, g[3], g[2]), jnp.where(b0, g[1], g[0]))
                comp[0, dst, :] = v
                comp[1, dst, :] = g[4]
                if gs is not None:
                    Sched.tok.setdefault(g0 + gs + int(rate * (5 * (k // 2) + 4)), []).append(v)
            if k % 2 == 1:
                yield

    def a_exp(i):
        bm = pats[_NPAT - 1] != 0
        srcs = []
        for u in range(UA):
            def ld(a, e):
                return _pack2(comp[a, pl.ds(i.off(64 * UA, 64 * u + e), 8, stride=4), :],
                              comp[a, pl.ds(i.off(64 * UA, 64 * u + 32 + e), 8, stride=4), :])

            srcs.append([ld(0, e) for e in range(4)]
                        + [jnp.where(bm, ld(1, 2 * k + 1), ld(1, 2 * k)) for k in range(2)])
        cache = {}

        def gat(s, key):
            if key not in cache:
                pat = pats[key]
                cache[key] = [_gather(srcs[u][s], pat) for u in range(UA)]
            return cache[key]

        tiles = []
        for steps in _TILES:
            t = None
            for s, key, lanes in steps:
                v = [jnp.zeros((8, 128), I32)] * UA if s < 0 else gat(s, key)
                t = v if t is None else [jnp.where(_lanes_mask(lanes), v[u], t[u]) for u in range(UA)]
            tiles.append(t)
        yield
        for u0 in range(0, UA, 2):
            lhs = [_bf(jnp.concatenate([tiles[_TILE_OF[dl, l2]][u] for dl in range(4) for u in (u0, u0 + 1)], axis=0))
                   for l2 in range(4)]
            z0 = 0 if u0 == 0 else zero * 8

            def dots(ri):
                return [jnp.dot(lhs[l2], _bf(jnp.concatenate(
                    [fpk[l2, pl.ds(z0 + 16 * (j ^ l2), 16) if u0 == 0 else
                         pl.ds(pl.multiple_of(z0 + 16 * (j ^ l2), 8), 16), pl.ds(128 * ri, 128)]
                     for j in range(4)], axis=0)), preferred_element_type=F32) for l2 in range(4)]

            def store(k2, ri, v):
                khat[2 * k2 + ri, :, pl.ds(i.off(16 * UA, 16 * u0, 16), 32), :] = v.reshape(4, 32, 128)

            re = dots(0)
            s0, d0r, s1, d1r = re[0] + re[2], re[0] - re[2], re[1] + re[3], re[1] - re[3]
            store(0, 0, s0 + s1)
            store(2, 0, s0 - s1)
            im = dots(1)
            s0, d0i, s1, d1i = im[0] + im[2], im[0] - im[2], im[1] + im[3], im[1] - im[3]
            store(0, 1, s0 + s1)
            store(2, 1, s0 - s1)
            store(1, 0, d0r + d1i)
            store(1, 1, d0i - d1r)
            store(3, 0, d0r - d1i)
            store(3, 1, d0i + d1r)
            yield

    def bail(cl):
        for cp in cl:
            cp.wait()
        zr = pl.ds(pl.multiple_of(zero * 8, 8), 16)
        v = khat[zero, zero, zr, :] + skip[zr, :] + (spk[zero, zr, :] + opk[zero, zr, :]).astype(F32) + topk[zero][:1] + comp[zero, zr, :]
        v = v + (hi_re[zero, zr, :] + hi_im[zero, zr, :] + lo_re[zero, zr, :] + lo_im[zero, zr, :]).astype(F32)
        v = v + uhat[zero, zero, zr, :] + ybuf[zero, zero, zr, :] + yhat[zero, zero, zero][:1].astype(F32)
        obuf[pl.ds(0, 16), pl.ds(0, 128)] = v.astype(BF16)
        cp = pltpu.make_async_copy(obuf.at[pl.ds(0, 16)], out_hbm.at[pl.ds(0, 16)], sem_out.at[0])
        cp.start()
        cp.wait()

    if _DEV.get("only") == "C":
        a_tail = [lambda: None] * 2
    else:
        def a_weave(gens):
            if 2 in gens and _DEV.get("expfirst", 1):
                next(gens[2])
            if 0 in gens and 1 in gens:
                for n in _DEV.get("pre", (3, 5, 4)):
                    for _ in range(n):
                        v = next(gens[0])
                    Sched.pre = [v[:8], v[8:]]
                    next(gens[1])
            if 1 in gens:
                for _ in gens[1]:
                    pass
            if 0 in gens:
                for _ in gens[0]:
                    pass

        a_pro, a_loop, a_tail = _pipeline([a_prep, a_gen, a_exp], NU // UA, newz, reset=Sched.reset,
                                          weave=a_weave)
        _run(a_pro)
        a_loop()
    if _DEV.get("only") == "A":
        return bail([cp_x, cp_g, cp_u] + cp_d)

    cp_x.wait()

    def zrow(u):
        return pl.ds(pl.multiple_of(zero * 8 + 8 * u, 8), 8)

    def b_gather(b):
        for j in range(4):
            pat = pats[j]
            for u in range(NU):
                v = pltpu.bitcast(xbuf[pl.ds(16 * u, 16), pl.ds(512 * b + 128 * j, 128)], I32)
                xg[b][j, pl.ds(8 * u, 8), :] = _gather(v, pat)

    def b_stat(b):
        s1 = [jnp.zeros((8, 128), F32) for _ in range(4)]
        s2 = [jnp.zeros((8, 128), F32) for _ in range(4)]
        for u in range(NU):
            o = _butterfly([xg[b][j, zrow(u), :] for j in range(4)])
            for l2 in range(4):
                xp[4 * l2 + b, pl.ds(8 * u, 8), :] = o[l2]
                e_, o_ = _unpack2(o[l2])
                s1[l2] = s1[l2] + (e_ + o_)
                s2[l2] = s2[l2] + (e_ * e_ + o_ * o_)
        st = []
        for l2 in range(4):
            m = jnp.sum(s1[l2], axis=0, keepdims=True) * jnp.float32(1.0 / D)
            q = jnp.sum(s2[l2], axis=0, keepdims=True) * jnp.float32(1.0 / D)
            var = _rbf(jnp.maximum(q - m * m, 0.0))
            sd = _rbf(jnp.sqrt(_rbf(var + jnp.float32(EPS))))
            st.append((jnp.broadcast_to(_rbf(m), (8, 128)), jnp.broadcast_to(1.0 / sd, (8, 128))))
        return st

    def b_norm(b, st):
        rr = []
        for l2 in range(4):
            mb, rs = st[l2]
            vs = []
            for u in range(NU - 1, -1, -1):
                e_, o_ = _unpack2(xp[4 * l2 + b, zrow(u), :])
                vs.append(_pack2((e_ - mb) * rs, (o_ - mb) * rs))
                xnp[4 * l2 + b, pl.ds(8 * u, 8), :] = vs[-1]
            rr.append(jnp.dot(wr16, _bf(jnp.concatenate(vs[::-1], axis=0)), preferred_element_type=F32)[:8])
        return rr

    wr16 = jnp.broadcast_to(wr[...].reshape(1, D), (16, D))
    if _DEV.get("only") == "C":
        b_gather = lambda b: None
        b_stat = lambda b: None
        b_norm = lambda b, st: [jnp.zeros((8, 128), F32)] * 4
    b_gather(0)
    a_tail[0]()
    b_gather(1)
    a_tail[1]()
    b_gather(2)
    b_gather(3)
    rraw = [b_norm(b, b_stat(b)) for b in range(4)]

    def c_fwd(i):
        h0 = i.off(CB // 2, 0, 8)
        r0 = i.off(CB, 0, 8)
        for l2 in range(4):
            lhs = _bf(xnp[pl.ds(4 * l2, 4), pl.ds(h0, CB // 2), :].reshape(2 * CB, 128))
            res = jnp.dot(lhs, _bf(fpk[l2]), preferred_element_type=F32)
            for ri in range(2):
                uhat[2 * l2 + ri, :, pl.ds(r0, CB), :] = res[:, 128 * ri:128 * ri + 128].reshape(4, CB, 128)
            yield

    def c_mid(i):
        for k in range(CB // 8):
            rows = pl.ds(i.off(CB, 8 * k, 8), 8)
            krows = pl.ds(i.off(CB, 16 * (k // 2) + k % 2), 8, stride=2)
            uu = [_fft4([(uhat[2 * l2, b, rows, :], uhat[2 * l2 + 1, b, rows, :]) for l2 in range(4)], -1)
                  for b in range(4)]
            yy = [[None] * 4 for _ in range(4)]
            kmode = _DEV.get("kfft", 0)

            def khalf(dl, odd):
                kr = pl.ds(i.off(CB, 16 * (k // 2) + k % 2) + (zero if odd else 0), 8, stride=2)
                x = [(khat[2 * l2, dl, kr, :], khat[2 * l2 + 1, dl, kr, :]) for l2 in range(4)]
                if not odd:
                    s0 = (x[0][0] + x[2][0], x[0][1] + x[2][1])
                    s1 = (x[1][0] + x[3][0], x[1][1] + x[3][1])
                    return {0: (s0[0] + s1[0], s0[1] + s1[1]), 2: (s0[0] - s1[0], s0[1] - s1[1])}
                d0 = (x[0][0] - x[2][0], x[0][1] - x[2][1])
                d1 = (x[1][0] - x[3][0], x[1][1] - x[3][1])
                return {1: (d0[0] + d1[1], d0[1] - d1[0]), 3: (d0[0] - d1[1], d0[1] + d1[0])}

            def acc(pp, m, t):
                pp[m] = t if pp[m] is None else (pp[m][0] + t[0], pp[m][1] + t[1])

            for odd in range(2):
                pps = {k2: [None] * 4 for k2 in (odd, odd + 2)}
                if kmode == 0:
                    for k2 in pps:
                        for dl in range(3, -1, -1):
                            kk = (khat[2 * k2, dl, krows, :], khat[2 * k2 + 1, dl, krows, :])
                            for m in range(3, dl - 1, -1):
                                acc(pps[k2], m, _cmul(*uu[m - dl][k2], *kk))
                elif kmode == 1:
                    for dl in range(3, -1, -1):
                        kk = khalf(dl, odd)
                        for k2 in pps:
                            for m in range(3, dl - 1, -1):
                                acc(pps[k2], m, _cmul(*uu[m - dl][k2], *kk[k2]))
                else:
                    kk = [khalf(dl, odd) for dl in range(4)]
                    for k2 in pps:
                        for m in range(3, -1, -1):
                            for b in range(m, -1, -1):
                                acc(pps[k2], m, _cmul(*uu[b][k2], *kk[m - b][k2]))
                for k2, pp in pps.items():
                    for m in range(3, -1, -1):
                        yy[m][k2] = pp[0] if m == 0 else (pp[m][0] - pp[m - 1][1], pp[m][1] + pp[m - 1][0])
            un = i.off(CB // 8, k)
            for bp in range(2):
                ww = [_fft4(yy[m], 1) for m in (2 * bp, 2 * bp + 1)]
                for l2 in range(4):
                    for ri in range(2):
                        yhat[2 * l2 + ri, bp, un] = _pack2(ww[0][l2][ri], ww[1][l2][ri])
            yield

    def c_inv(i):
        u0 = i.off(CB // 8)
        r0 = i.off(2 * CB, 0, 8)
        for l2 in range(4):
            for ri in range(2):
                lhs = _bf(yhat[2 * l2 + ri, :, pl.ds(u0, CB // 8)].reshape(2 * CB, 128))
                y = lax.dot_general(lhs, _bf(fpk[l2, :, pl.ds(128 * ri, 128)]), _NT, preferred_element_type=F32)
                ybuf[2 * l2 + ri, :, pl.ds(r0, 2 * CB), :] = y.reshape(2, 2 * CB, 128)
            yield

    def c_elt(i):
        for k in range(CB // 16):
            hr = pl.ds(i.off(CB // 2, 8 * k, 8), 8)
            sk = [skip[pl.ds(i.off(CB, 16 * k + e), 8, stride=2), :] for e in range(2)]
            for b in range(4):
                o = []
                for l2 in range(4):
                    xn = _unpack2(xnp[4 * l2 + b, hr, :])
                    xx = _unpack2(xp[4 * l2 + b, hr, :])
                    ss, v = [], []
                    for e in range(2):
                        yr = pl.ds(i.off(2 * CB, 32 * k + 2 * e + b % 2), 8, stride=4)
                        ss.append(ybuf[2 * l2, b // 2, yr, :] + ybuf[2 * l2 + 1, b // 2, yr, :] + xn[e] * sk[e])
                        v.append(xx[e] + ss[e] * _silu(xn[e]))
                    spk[4 * l2 + b, hr, :] = _pack2(*ss)
                    o.append(_pack2(*v))
                p = _butterfly(o)
                for j in range(4):
                    opk[4 * b + j, hr, :] = p[j]
            yield

    kc = [None, None]
    for l2 in range(4):
        for b in range(4):
            t = 4 * l2 + b
            r = _rbf(rraw[b][l2])
            r = jnp.where(r == 0.0, 0.0, r)
            bits = pltpu.bitcast(r, I32)
            mono = ((bits ^ ((bits >> 31) & jnp.int32(0x7FFFFFFF))) >> 16) + 32768
            tok = 512 * b + 4 * (32 * ((lane8 >> 5) ^ l2) + (lane8 & 31)) + l2
            key = pltpu.bitcast((mono << 11) + (2047 - tok) + jnp.int32(0x00800000), F32)
            kc[t // 8] = key if t % 8 == 0 else jnp.where(sub8 == t % 8, key, kc[t // 8])
    topk[32] = kc[0]
    topk[33] = kc[1]
    topk[34] = jnp.zeros((8, 128), F32)

    def c_top(i):
        k0, k1 = topk[i.off(0, 32)], topk[i.off(0, 33)]
        mx = jnp.max(jnp.max(jnp.maximum(k0, k1), axis=0, keepdims=True), axis=1, keepdims=True)
        topk[i.off(0, 32)] = jnp.where(k0 == mx, 0.0, k0)
        topk[i.off(0, 33)] = jnp.where(k1 == mx, 0.0, k1)
        topk[i.off(0, 34)] = jnp.where(sub8 == i.idx(), mx, topk[i.off(0, 34)])
        yield

    def c_first(i):
        yield from c_top(i)
        yield from c_fwd(i)

    c_pro, c_loop, c_tail = _pipeline([c_first, c_mid, c_inv, c_elt], NB, newz,
                                      weave=_DEV.get("cweave", [0, 0, 0, 2, 2, 0, 0, 2, 2]))
    _run(c_pro)
    c_loop()
    if _DEV.get("only") == "C":
        return bail([cp_g, cp_u] + cp_d)

    sel = pltpu.bitcast(topk[34], I32) - jnp.int32(0x00800000)
    mono = (sel >> 11) - 32768
    r_sel = pltpu.bitcast((mono ^ ((mono >> 31) & jnp.int32(0x7FFF))) << 16, F32)
    gate_r = _rbf(jax.nn.sigmoid(r_sel))
    posv[...] = 2047 - (sel & 2047)
    tok = [posv[c, 0] for c in range(C)]
    nat = [(t >> 7, t & 127) for t in tok]
    prm = []
    for t in tok:
        l2, l1 = t & 3, (t >> 2) & 127
        prm.append((4 * l2 + (t >> 9), 32 * ((l1 >> 5) ^ l2) + (l1 & 31)))

    def extract(src, k):
        cols[k] = jnp.zeros((D // 2, 128), I32)
        for c, (tp, pp) in enumerate(prm):
            sh = (c - pp) & 127
            for u in range(NU):
                pltpu.store(cols.at[k, pl.ds(8 * u, 8), :], pltpu.roll(src[tp, pl.ds(8 * u, 8), :], sh, 1),
                            mask=lane8 == c)

    extract(xnp, 0)
    extract(xp, 1)
    _run(c_tail)
    z1 = newz()
    xsel = lax.dot_general(eye[:16], _bf(cols[0, pl.ds(pl.multiple_of(z1, 8), D // 2), :]), _NT,
                           preferred_element_type=F32)
    xsel_b = xsel.astype(BF16)

    def o_gather(js):
        for j in js:
            pat = pats[4 + j]
            for b in range(4):
                for u in range(NU):
                    og[4 * b + j, pl.ds(8 * u, 8), :] = _gather(opk[4 * b + j, zrow(u), :], pat)

    def o_store(t, u, v, col):
        obuf[pl.ds(16 * u, 8), col] = _bf(v[0:4])
        obuf[pl.ds(16 * u + 8, 8), col] = _bf(pltpu.roll(v, 4, 0)[0:4])

    def o_final(js):
        for j in js:
            for b in range(4):
                for u in range(NU):
                    o_store(4 * b + j, u, og[4 * b + j, zrow(u), :], pl.ds(512 * b + 128 * j, 128))

    def out_copy(t):
        col = pl.ds(128 * t, 128)
        return pltpu.make_async_copy(obuf.at[:, col], out_hbm.at[:, col], sem_out.at[t])

    def start_out(late):
        for t in range(16):
            hit = nat[0][0] == t
            for c in range(1, C):
                hit = jnp.logical_or(hit, nat[c][0] == t)

            @pl.when(hit if late else jnp.logical_not(hit))
            def _():
                out_copy(t).start()

    cp_g.wait()
    extract(spk, 2)
    o_gather((0, 1))
    ga = _rbf(jnp.dot(xsel_b, wg[...], preferred_element_type=F32)[:8])
    ga = _rbf(ga * _rbf(jax.nn.sigmoid(ga)))
    cp_u.wait()
    o_final((0, 1))
    o_gather((2, 3))
    up = _rbf(jnp.dot(xsel_b, wu[...], preferred_element_type=F32)[:8])
    hh = jnp.concatenate([ga * up, jnp.zeros((8, F), F32)], axis=0).astype(BF16)
    pr = (r128 & (-16)) + 2 * (r128 & 7) + ((r128 >> 3) & 1)
    perm = jnp.where(pr == c128, 1.0, 0.0).astype(BF16)

    def patch(a, n, y):
        z = _rbf(xsel[:8, a:a + n] + _rbf(_rbf(y[:8]) * gate_r[:, :1]))
        g = z * _rbf(jax.nn.sigmoid(z))
        g = jnp.concatenate([g, jnp.zeros((120, n), F32)], axis=0).astype(BF16)
        gt = lax.dot_general(perm[:n, :n], g, _NT, preferred_element_type=F32)
        us = range(a // 16, (a + n) // 16)
        zz = newz()
        for u in us:
            hr = pl.ds(pl.multiple_of(zz + 8 * u, 8), 8)
            xx, ss = _unpack2(cols[1, hr, :]), _unpack2(cols[2, hr, :])
            r0 = 16 * u - a
            w = _pack2(*[xx[e] + _rbf(ss[e] * gt[r0 + 8 * e:r0 + 8 * e + 8]) for e in range(2)])
            for c, (tn, pn) in enumerate(nat):
                tt = 4 * (tn >> 2) + (tn & 3)
                pltpu.store(og.at[tt, pl.ds(8 * u, 8), :], pltpu.roll(w, (pn - c) & 127, 1), mask=lane8 == pn)
        for c, (tn, pn) in enumerate(nat):
            for u in us:
                o_store(tn, u, og[tn, pl.ds(8 * u, 8), :], pl.ds(pl.multiple_of(tn * 128, 128), 128))

    prev = None
    for q, ((a, n), cp) in enumerate(zip(wd_rows, cp_d)):
        cp.wait()
        if q == 0:
            o_final((2, 3))
        y = lax.dot_general(hh, wd[pl.ds(a, n), :], _NT, preferred_element_type=F32)
        if prev is not None:
            patch(*prev)
        prev = (a, n, y)
        if q == _DEV.get("early", 0):
            start_out(False)
    patch(*prev)
    start_out(True)
    for t in range(16):
        out_copy(t).wait()


def _scratch():
    return [
        pltpu.VMEM((D, L), BF16),
        pltpu.VMEM((6, D, N), BF16),
        pltpu.VMEM((D,), BF16),
        pltpu.VMEM((D,), BF16),
        pltpu.VMEM((D,), BF16),
        pltpu.VMEM((D, F), BF16),
        pltpu.VMEM((D, F), BF16),
        pltpu.VMEM((D, F), BF16),
        pltpu.VMEM((4, 64, 256), U32),
        pltpu.VMEM((_NPAT, 8, 128), I32),
        pltpu.VMEM((D, 128), F32),
        pltpu.VMEM((D, 128), F32),
        pltpu.VMEM((5, 2 * D, 128), I32),
        pltpu.VMEM((5, 2 * D, 128), I32),
        pltpu.VMEM((8, 2 * D, 128), I32),
        pltpu.VMEM((8, 2 * D, 128), I32),
        pltpu.VMEM((2, 4 * D, 128), F32),
        pltpu.VMEM((8, 4, D, 128), F32),
        pltpu.VMEM((16, D // 2, 128), I32),
        pltpu.VMEM((16, D // 2, 128), I32),
        pltpu.VMEM((8, 4, D, 128), F32),
        pltpu.VMEM((8, 2, D // 8, 8, 128), I32),
        pltpu.VMEM((8, 2, 2 * D, 128), F32),
        pltpu.VMEM((16, D // 2, 128), I32),
        pltpu.VMEM((35, 8, 128), F32),
        pltpu.VMEM((8, 128), I32),
        pltpu.VMEM((3, D // 2, 128), I32),
        pltpu.VMEM((16, D // 2, 128), I32),
        pltpu.VMEM((16, D // 2, 128), I32),
        pltpu.VMEM((D, L), BF16),
        pltpu.SemaphoreType.DMA((19,)),
        pltpu.SemaphoreType.DMA((16,)),
    ] + [pltpu.VMEM((4, D // 2, 128), I32)] * 4


@jax.jit
def pallas_recurrent_scan__ssm_conv_s4__moe_arch_mod__prompt_kernel(
    A_u: jax.Array,
    A_A_re: jax.Array,
    A_A_im: jax.Array,
    A_B_re: jax.Array,
    A_B_im: jax.Array,
    A_C_re: jax.Array,
    A_C_im: jax.Array,
    A_log_dt: jax.Array,
    A_Dskip: jax.Array,
    B_x: jax.Array,
    B_w_r: jax.Array,
    B_w_gate: jax.Array,
    B_w_up: jax.Array,
    B_w_down: jax.Array,
):
    hbm = pl.BlockSpec(memory_space=pltpu.HBM)
    out = pl.pallas_call(
        _kernel,
        out_shape=jax.ShapeDtypeStruct((D, L), BF16),
        in_specs=[hbm] * 15,
        out_specs=hbm,
        scratch_shapes=_scratch(),
        compiler_params=pltpu.CompilerParams(vmem_limit_bytes=110 * 1024 * 1024),
        name="s4_mod",
    )(A_u[0].T, A_A_re, A_A_im, A_B_re, A_B_im, A_C_re, A_C_im, A_log_dt, A_Dskip, B_w_r,
      B_w_gate, B_w_up, B_w_down.T, jnp.asarray(_FPK), jnp.asarray(_PATS))
    return out.T[None]
```

```python
import numpy as np
import jax
import jax.numpy as jnp
from jax import lax
import jax.experimental.pallas as pl
import jax.experimental.pallas.tpu as pltpu

L, D, N, F, C = 2048, 576, 128, 4608, 8
NU = D // 16
CB = 64
NB = D // CB
CO = 32
NO = D // CO
UA = 4
F32, BF16, I32, U32 = jnp.float32, jnp.bfloat16, jnp.int32, jnp.uint32
EPS = 1e-5
_DEV = {}


def _bf16_round_np(x):
    u = np.asarray(x, np.float32).view(np.uint32).astype(np.uint64)
    r = ((u + 0x7FFF + ((u >> 16) & 1)) >> 16) << 16
    return r.astype(np.uint32)


_LROUND = _bf16_round_np(np.arange(L)).view(np.float32).astype(np.int64)
_HI = [(1, 3, 516, 1032), (5, 7, 520, 1288), (4, 260, 772, 1544), (8, 264, 776, 1800), (2, 6, 258, 262)]


def _lane_l1(l2):
    p = np.arange(128)
    return 32 * ((p // 32) ^ l2) + p % 32


def _comp_q():
    t = np.arange(8)[:, None]
    lane = np.arange(128)[None, :]
    return ((lane - 8 - 7 * (t % 4)) % 16) // 4


def _make_tables():
    lane = np.arange(128)
    lo = 8 * (4 * (lane // 16) + lane % 4)
    tab = [dict(), dict()]
    amask = np.zeros(128, bool)
    for q in range(5):
        for e in range(4):
            for par in range(2):
                t = 4 * par + e
                for h in range(2):
                    src = lane[(lane // 4) % 4 == 2 * h + par]
                    dst = (src + (4 * (q % 4) - 8 * h + 8) + 7 * t) % 128
                    assert np.all(_comp_q()[t, dst] == q % 4)
                    sid = e if q < 4 else 4 + e // 2
                    for sl, dl_ in zip(src, dst):
                        ent = (sid, int(dl_))
                        assert tab[par].setdefault(_HI[q][e] + int(lo[sl]), ent) == ent
                    if q == 4 and e % 2 == 1:
                        amask[dst % 16 + 16 * np.arange(8)[:, None]] = True
    pats = []
    for j in range(4):
        pats.append(np.tile(4 * (lane % 32) + ((lane // 32) ^ j), (8, 1)))
    for j in range(4):
        pats.append(np.tile(32 * ((lane % 4) ^ j) + lane // 4, (8, 1)))
    npat0 = len(pats)
    tiles, tile_of = [], {}
    for dl in range(4):
        for l2 in range(4):
            v = _LROUND[512 * dl + 4 * lane + l2]
            key = tuple(v.tolist())
            if key in tile_of:
                tile_of[dl, l2] = tile_of[key]
                continue
            sid = np.array([tab[0][x][0] if x else -1 for x in v])
            ln = np.array([[tab[s8 % 2][x][1] if x else 0 for x in v] for s8 in range(8)])
            steps = []
            for s in sorted(set(sid.tolist()), key=lambda s: -(sid == s).sum()):
                lanes = np.nonzero(sid == s)[0]
                if s < 0:
                    steps.append((-1, None, lanes))
                    continue
                care = sid == s
                kk = None
                for k in range(npat0, len(pats)):
                    oldp, oldc, olds = pats[k]
                    both = care & oldc
                    if olds == s and np.array_equal(oldp[:, both], ln[:, both]):
                        pats[k] = (np.where(care, ln, oldp), care | oldc, s)
                        kk = k
                        break
                if kk is None:
                    pats.append((np.where(care, ln, 0), care, s))
                    kk = len(pats) - 1
                steps.append((s, kk, lanes))
            tiles.append(steps)
            tile_of[key] = tile_of[dl, l2] = len(tiles) - 1
    pats = np.stack([p if k < npat0 else p[0] for k, p in enumerate(pats)]).astype(np.int32)
    tile_of = {k: v for k, v in tile_of.items() if len(k) == 2}
    m = np.arange(128)
    fw = np.zeros((4, 128, 256), np.float64)
    for l2 in range(4):
        t = 4 * _lane_l1(l2) + l2
        th = 2 * np.pi * (2 * m[None, :] + 0.5) * t[:, None] / 1024
        fw[l2, :, :128] = np.cos(th)
        fw[l2, :, 128:] = -np.sin(th)
    fb = _bf16_round_np(fw) >> 16
    fpk = (fb[:, 0::2, :] | (fb[:, 1::2, :] << 16)).astype(np.uint32)
    masks = np.stack([_comp_q() & 1, _comp_q() >> 1, np.tile(amask, (8, 1))]).astype(np.int32)
    return tiles, tile_of, np.concatenate([pats, masks]), fpk


_TILES, _TILE_OF, _PATS, _FPK = _make_tables()
_NPAT = _PATS.shape[0]
_NT_K = len(_TILES)


def _cmul(ar, ai, br, bi):
    return ar * br - ai * bi, ar * bi + ai * br


def _sincos(b):
    magic = jnp.float32(12582912.0)
    t = b * jnp.float32(2.0 / np.pi) + magic
    k = t - magic
    ki = pltpu.bitcast(t, I32)
    r = b - k * jnp.float32(1.5703125)
    r = r - k * jnp.float32(0.0004837512969970703)
    r = r - k * jnp.float32(7.549790126404332e-08)
    u = r * r
    ps = (jnp.float32(-0.0001958295761141926) * u + jnp.float32(0.008332725614309311)) * u \
        + jnp.float32(-0.166666641831398)
    sn = r + (r * u) * ps
    pc = ((jnp.float32(2.437065268168226e-05) * u + jnp.float32(-0.0013886778615415096)) * u
          + jnp.float32(0.04166663438081741)) * u + jnp.float32(-0.5)
    cs = pc * u + jnp.float32(1.0)
    odd = (ki & 1) == 1
    s1 = jnp.where(odd, cs, sn)
    c1 = jnp.where(odd, sn, cs)
    sign = jnp.int32(-2147483648)
    s1 = pltpu.bitcast(pltpu.bitcast(s1, I32) ^ ((ki << 30) & sign), F32)
    c1 = pltpu.bitcast(pltpu.bitcast(c1, I32) ^ (((ki + 1) << 30) & sign), F32)
    return s1, c1


def _gather(x, idx):
    return jnp.take_along_axis(x, idx, axis=1, mode="promise_in_bounds")


def _lanes_mask(lanes):
    lane = lax.broadcasted_iota(I32, (8, 128), 1)
    lanes = sorted(int(x) for x in lanes)
    runs, start, prev = [], lanes[0], lanes[0]
    for x in lanes[1:]:
        if x != prev + 1:
            runs.append((start, prev))
            start = x
        prev = x
    runs.append((start, prev))
    m = None
    for a, b in runs:
        t = (lane == a) if a == b else jnp.logical_and(lane >= a, lane <= b)
        m = t if m is None else jnp.logical_or(m, t)
    return m


def _butterfly(p):
    lane = lax.broadcasted_iota(I32, p[0].shape, 1)
    b0 = (lane & 32) != 0
    b1 = (lane & 64) != 0
    t = [jnp.where(b0, p[k ^ 1], p[k]) for k in range(4)]
    return [jnp.where(b1, t[k ^ 2], t[k]) for k in range(4)]


def _fft4(x, sgn):
    (ar, ai), (br, bi), (cr, ci), (dr, di) = x
    s0r, s0i, d0r, d0i = ar + cr, ai + ci, ar - cr, ai - ci
    s1r, s1i, d1r, d1i = br + dr, bi + di, br - dr, bi - di
    y0 = (s0r + s1r, s0i + s1i)
    y2 = (s0r - s1r, s0i - s1i)
    p = (d0r - d1i, d0i + d1r)
    m = (d0r + d1i, d0i - d1r)
    return [y0, p, y2, m] if sgn > 0 else [y0, m, y2, p]


def _silu(z):
    h = z * jnp.float32(0.5)
    return h + h * jnp.tanh(h)


def _rbf(x):
    return x.astype(BF16).astype(F32)


def _pack2(a, b):
    p = pltpu.pack_elementwise([a, b], packed_dtype=BF16)
    return p if p.dtype == I32 else pltpu.bitcast(p, I32)


def _unpack2(x):
    return [pltpu.unpack_elementwise(x, index=i, packed_dtype=BF16, unpacked_dtype=F32) for i in range(2)]


def _bf(x):
    return pltpu.bitcast(x, BF16)


_NT = (((1,), (1,)), ((), ()))


class _Idx:
    def __init__(self, i, lag, z=None):
        self.i, self.lag, self.z = i, lag, z

    def off(self, stride, const=0, align=None):
        c = const - self.lag * stride
        if isinstance(self.i, int):
            if self.z is None:
                return self.i * stride + c
            v = self.z + (self.i * stride + c)
        else:
            v = self.i * stride + c
        return pl.multiple_of(v, align) if align else v

    def idx(self):
        return self.i - self.lag


def _pipeline(stages, n, newz, weave=None, reset=None):
    ns = len(stages)

    def step(i, lo, hi):
        z = newz() if isinstance(i, int) else None
        gens = {k: stages[k](_Idx(i, k, z)) for k in range(lo, hi)}
        if reset is not None:
            reset()
        if callable(weave):
            weave(gens)
        else:
            for k in weave or ():
                if k in gens:
                    next(gens[k], None)
        for k in range(hi - 1, lo - 1, -1):
            for _ in gens[k]:
                pass

    def body(i, carry):
        step(i, 0, ns)
        return carry

    return ([lambda i=i: step(i, 0, i + 1) for i in range(ns - 1)],
            lambda: lax.fori_loop(ns - 1, n, body, 0),
            [lambda i=i: step(n + i, i + 1, ns) for i in range(ns - 1)])


def _run(fns):
    for fn in fns:
        fn()


def _kernel(x_hbm, are_hbm, aim_hbm, bre_hbm, bim_hbm, cre_hbm, cim_hbm, ldt_hbm, dsk_hbm, wr_hbm,
            wg_hbm, wu_hbm, wd_hbm, f_hbm, pat_hbm,
            out_hbm,
            xbuf, par, ldt, dsk, wr, wg, wu, wd, fpk, pats,
            dtcol, skip, hi_re, hi_im, lo_re, lo_im, comp, khat,
            xp, xnp, uhat, yhat, ybuf, spk, topk, posv, wr16b, wsum, xsel_ref, cols, opk, og, obuf,
            sem_in, sem_out, *perb):
    xi, xg, stat = perb[0:4], perb[4:8], perb[8:12]
    p_hbm = (are_hbm, aim_hbm, bre_hbm, bim_hbm, cre_hbm, cim_hbm)
    r1 = 16 * UA
    small = [(ldt_hbm, ldt), (pat_hbm.at[pl.ds(0, 1)], pats.at[pl.ds(0, 1)]), (dsk_hbm, dsk)]
    small += [(h.at[pl.ds(0, r1)], par.at[i, pl.ds(0, r1)]) for i, h in enumerate(p_hbm)]
    small += [(h.at[pl.ds(r1, D - r1)], par.at[i, pl.ds(r1, D - r1)]) for i, h in enumerate(p_hbm)]
    small += [(pat_hbm.at[pl.ds(1, _NPAT - 1)], pats.at[pl.ds(1, _NPAT - 1)]), (f_hbm, fpk), (wr_hbm, wr)]
    cps = [pltpu.make_async_copy(s, d, sem_in.at[i]) for i, (s, d) in enumerate(small)]
    ns = len(cps)
    cp_x = pltpu.make_async_copy(x_hbm, xbuf, sem_in.at[ns])
    cp_g = pltpu.make_async_copy(wg_hbm, wg, sem_in.at[ns + 1])
    cp_u = pltpu.make_async_copy(wu_hbm, wu, sem_in.at[ns + 2])
    wd_rows = [(0, 128), (128, 128), (256, 128), (384, 128), (512, 64)]
    cp_d = [pltpu.make_async_copy(wd_hbm.at[pl.ds(a, n)], wd.at[pl.ds(a, n)], sem_in.at[ns + 3 + i])
            for i, (a, n) in enumerate(wd_rows)]
    for cp in cps + [cp_x, cp_g, cp_u] + cp_d:
        cp.start()

    for cp in cps[:3]:
        cp.wait()
    r128 = lax.broadcasted_iota(I32, (128, 128), 0)
    c128 = lax.broadcasted_iota(I32, (128, 128), 1)
    eye = jnp.where(r128 == c128, 1.0, 0.0).astype(BF16)
    dt_row = jnp.exp(ldt[...].astype(F32).reshape(1, D)).astype(BF16)
    dsk_row = dsk[...].reshape(1, D)
    for t in range(5):
        n = min(128, D - 128 * t)
        for row, dst in ((dt_row, dtcol), (dsk_row, skip)):
            b = jnp.broadcast_to(row[:, 128 * t:128 * t + n], (128, n))
            dst[pl.ds(128 * t, n), :] = lax.dot_general(eye[:n, :n], b, _NT, preferred_element_type=F32)

    sub8 = lax.broadcasted_iota(I32, (8, 128), 0)
    lane8 = lax.broadcasted_iota(I32, (8, 128), 1)
    zero = pats[0, 0, 0]
    zcount = [0]

    def newz():
        zcount[0] += 1
        return zero * (64 * zcount[0]) if _DEV.get("zpeel", 1) else None

    def block(*fns):
        if not _DEV.get("blocks", 1):
            return _run(fns)

        def body(k, carry):
            _run(fns)
            return carry

        lax.fori_loop(0, zero + 1, body, 0)

    def slow_zero(i):
        t = i.off(1) * zero if not isinstance(i.i, int) or i.z is None else i.z
        for _ in range(_DEV.get("slow", 0)):
            t = t * t
        return pl.multiple_of(t * 8, 8)

    def after(x, deps):
        never = pats[0] < 0
        d = None
        for v in deps:
            v = v if v.dtype == I32 else pltpu.bitcast(v, I32)
            d = v if d is None else d ^ v
        return jnp.where(never, d if x.dtype == I32 else pltpu.bitcast(d, x.dtype), x)

    def pad_tail(y, i):
        n = _DEV.get("pad", 0)
        if not n:
            return y
        m = y.shape[0]
        base = i.off(1)
        k = m - 8 * _DEV.get("padpos", 4)
        mid = after(y[k:k + 8], [pats[j % _NPAT] * (base + j) for j in range(n)])
        return jnp.concatenate([y[:k], mid, y[k + 8:]], axis=0)

    class Sched:
        tok, g, pre = {}, 0, []

        @classmethod
        def reset(cls):
            cls.tok, cls.g, cls.pre = {}, 0, []

        @classmethod
        def gate(cls, x):
            deps = cls.tok.pop(cls.g, [])
            cls.g += 1
            if not deps or not _DEV.get("gate", 1):
                return x
            return jnp.concatenate([after(x[:8], deps), after(x[8:], deps[-1:])], axis=0)

    slot = {h: (q, e) for q, ent in enumerate(_HI) for e, h in enumerate(ent)}

    def a_prep(i):
        gate = Sched.gate
        for u in range(UA):
            rows = pl.ds(i.off(16 * UA, 16 * u, 16), 16)
            ev = pl.ds(i.off(32 * UA, 32 * u), 16, stride=2)
            od = pl.ds(i.off(32 * UA, 32 * u + 1), 16, stride=2)
            dt = gate(dtcol[rows, :])
            al = dt * par[0, rows, :].astype(F32)
            be = dt * par[1, rows, :].astype(F32)
            cr, ci = _cmul(par[4, rows, :].astype(F32), par[5, rows, :].astype(F32),
                           par[2, rows, :].astype(F32), par[3, rows, :].astype(F32))
            dts = dt * jnp.float32(1.0 / 512)
            cr, ci = cr * dts, ci * dts
            k0 = jnp.sum(cr, axis=1, keepdims=True) * jnp.float32(512.0)
            skip[rows, :] = skip[rows, :] + k0
            yield cr
            s, c = _sincos(gate(be))
            yield c
            pw = {1: (c, s)}
            e = 1
            while e < 256:
                if e in (1, 16):
                    c = gate(c)
                c, s = (c - s) * (c + s), (c + c) * s
                e *= 2
                pw[e] = (c, s)
                if e in (16, 256):
                    yield c
            z = {}
            for e in (1, 8, 256):
                mag = jnp.exp(al * jnp.float32(e))
                c, s = pw[e]
                z[e] = (mag * c, mag * s)
            pend = {}

            def put(tab, q, ee, v):
                key = (tab[0] is hi_re, q, ee // 2)
                if key not in pend:
                    pend[key] = (ee % 2, v)
                    return
                w, o = pend.pop(key)
                lo_, hi_ = (o, v) if w == 0 else (v, o)
                dst = od if ee // 2 else ev
                tab[0][q, dst, :] = _pack2(lo_[0], hi_[0])
                tab[1][q, dst, :] = _pack2(lo_[1], hi_[1])

            h = (cr, ci)
            cnt = 0
            for e in range(1, 9):
                g, ee, m = h, e, z[1]
                while ee in slot:
                    if cnt % 4 == 0:
                        g = (gate(g[0]), g[1])
                    g = _cmul(*g, *m)
                    put((hi_re, hi_im), *slot[ee], g)
                    if ee == e:
                        h = g
                    ee, m = ee + 256, z[256]
                    cnt += 1
                    if cnt % 4 == 0:
                        yield g[0]
            w1 = (gate(z[8][0]), -z[8][1])
            v = [(jnp.ones((16, 128), F32), jnp.zeros((16, 128), F32)), w1]
            v.append(_cmul(*w1, *w1))
            v.append(_cmul(*v[2], *w1))
            w4 = _cmul(*v[2], *v[2])
            for j in range(8):
                for f in range(4):
                    put((lo_re, lo_im), j, f, v[f])
                yield v[3][0]
                if j < 7:
                    w4 = (gate(w4[0]), w4[1])
                    v = [w4 if (j == 0 and f == 0) else _cmul(*v[f], *w4) for f in range(4)]

    def a_gen(i):
        b0 = pats[_NPAT - 3] != 0
        b1 = pats[_NPAT - 2] != 0
        g0, gs = _DEV.get("g0", 13), _DEV.get("gs", None)
        rate = _DEV.get("rate", 0.9)
        for k in range(4 * UA):
            rows = pl.ds(i.off(32 * UA, 8 * k, 8), 8)
            lo = jnp.concatenate([lo_re[:, rows, :].reshape(64, 128), lo_im[:, rows, :].reshape(64, 128)], axis=1)
            h0 = hi_re[0, rows, :]
            if k % 2 == 0 and Sched.pre and _DEV.get("gate", 1):
                h0 = after(h0, Sched.pre)
                Sched.pre = []
            hi = jnp.concatenate([jnp.concatenate([h0, hi_re[1:5, rows, :].reshape(32, 128)], axis=0),
                                  hi_im[:, rows, :].reshape(40, 128)], axis=1)
            o = lax.dot_general(_bf(hi), _bf(lo), _NT, preferred_element_type=F32)
            for q in range(5):
                Sched.tok.setdefault(g0 + int(rate * (5 * (k // 2) + q)), []).append(o[16 * q + 8:16 * q + 16])
            for h in range(2):
                g = [pltpu.roll(o[16 * q + 8 * h:16 * q + 8 * h + 8], 4 * (q % 4) - 8 * h + 8, 1,
                                stride=7, stride_axis=0) for q in range(5)]
                dst = pl.ds(i.off(64 * UA, 16 * k + 8 * h, 8), 8)
                v = jnp.where(b1, jnp.where(b0, g[3], g[2]), jnp.where(b0, g[1], g[0]))
                comp[0, dst, :] = v
                comp[1, dst, :] = g[4]
                if gs is not None:
                    Sched.tok.setdefault(g0 + gs + int(rate * (5 * (k // 2) + 4)), []).append(v)
            if k % 2 == 1:
                yield

    def a_exp(i):
        bm = pats[_NPAT - 1] != 0
        srcs = []
        for u in range(UA):
            def ld(a, e):
                return _pack2(comp[a, pl.ds(i.off(64 * UA, 64 * u + e), 8, stride=4), :],
                              comp[a, pl.ds(i.off(64 * UA, 64 * u + 32 + e), 8, stride=4), :])

            srcs.append([ld(0, e) for e in range(4)]
                        + [jnp.where(bm, ld(1, 2 * k + 1), ld(1, 2 * k)) for k in range(2)])
        cache = {}

        def gat(s, key):
            if key not in cache:
                pat = pats[key]
                cache[key] = [_gather(srcs[u][s], pat) for u in range(UA)]
            return cache[key]

        tiles = []
        for steps in _TILES:
            t = None
            for s, key, lanes in steps:
                v = [jnp.zeros((8, 128), I32)] * UA if s < 0 else gat(s, key)
                t = v if t is None else [jnp.where(_lanes_mask(lanes), v[u], t[u]) for u in range(UA)]
            tiles.append(t)
        yield
        for u0 in range(0, UA, 2):
            lhs = [_bf(jnp.concatenate([tiles[_TILE_OF[dl, l2]][u] for dl in range(4) for u in (u0, u0 + 1)], axis=0))
                   for l2 in range(4)]
            z0 = 0 if u0 == 0 else zero * 8

            def dots(ri):
                return [jnp.dot(lhs[l2], _bf(jnp.concatenate(
                    [fpk[l2, pl.ds(z0 + 16 * (j ^ l2), 16) if u0 == 0 else
                         pl.ds(pl.multiple_of(z0 + 16 * (j ^ l2), 8), 16), pl.ds(128 * ri, 128)]
                     for j in range(4)], axis=0)), preferred_element_type=F32) for l2 in range(4)]

            def store(k2, ri, v):
                khat[2 * k2 + ri, :, pl.ds(i.off(16 * UA, 16 * u0, 16), 32), :] = v.reshape(4, 32, 128)

            def toks(v, step0):
                g1 = _DEV.get("g0", 13) + int(_DEV.get("rate", 0.9) * 10 * UA) + _DEV.get("g1", 0)
                for j in range(8):
                    g = g1 + int(_DEV.get("rate2", 0.7) * (step0 + j))
                    Sched.tok.setdefault(g, []).append(v[16 * j + 8:16 * j + 16])

            re = dots(0)
            s0, d0r, s1, d1r = re[0] + re[2], re[0] - re[2], re[1] + re[3], re[1] - re[3]
            store(0, 0, s0 + s1)
            v = s0 - s1
            store(2, 0, v)
            toks(v, 8 * u0)
            im = dots(1)
            s0, d0i, s1, d1i = im[0] + im[2], im[0] - im[2], im[1] + im[3], im[1] - im[3]
            store(0, 1, s0 + s1)
            store(2, 1, s0 - s1)
            store(1, 0, d0r + d1i)
            store(1, 1, d0i - d1r)
            store(3, 0, d0r - d1i)
            v = d0i + d1r
            store(3, 1, v)
            toks(v, 8 * u0 + 8)
            yield

    def bail(cl):
        for cp in cl:
            cp.wait()
        zr = pl.ds(pl.multiple_of(zero * 8, 8), 16)
        v = khat[zero, zero, zr, :] + skip[zr, :] + (spk[zero, zr, :] + opk[zero, zr, :] + xnp[zero, zr, :] + xp[zero, zr, :]).astype(F32) + topk[zero][:1] + comp[zero, zr, :]
        v = v + (hi_re[zero, zr, :] + hi_im[zero, zr, :] + lo_re[zero, zr, :] + lo_im[zero, zr, :]).astype(F32)
        v = v + uhat[zero, zero, zr, :] + ybuf[zero, zero, zr, :] + yhat[zero, zero, zero][:1].astype(F32)
        obuf[pl.ds(0, 16), pl.ds(0, 128)] = v.astype(BF16)
        cp = pltpu.make_async_copy(obuf.at[pl.ds(0, 16)], out_hbm.at[pl.ds(0, 16)], sem_out.at[0])
        cp.start()
        cp.wait()

    if _DEV.get("only") == "C":
        a_tail = [lambda: None] * 2
    else:
        def a_weave(gens):
            if 2 in gens and _DEV.get("expfirst", 1):
                next(gens[2])
            if 0 in gens and 1 in gens:
                for n in _DEV.get("pre", (3, 5, 4)):
                    for _ in range(n):
                        v = next(gens[0])
                    Sched.pre = [v[:8], v[8:]]
                    next(gens[1])
            for k in (1, 2):
                if k in gens:
                    for _ in gens[k]:
                        pass
            if 0 in gens:
                for _ in gens[0]:
                    pass

        a_pro, a_loop, a_tail = _pipeline([a_prep, a_gen, a_exp], NU // UA, newz, reset=Sched.reset,
                                          weave=a_weave)
        for cp in cps[3:9]:
            cp.wait()
        a_pro[0]()
        for cp in cps[9:]:
            cp.wait()
        a_pro[1]()
        a_loop()
    if _DEV.get("only") == "A":
        return bail([cp_x, cp_g, cp_u] + cp_d)

    cp_x.wait()

    def zrow(u):
        return pl.ds(pl.multiple_of(zero * 8 + 8 * u, 8), 8)

    def b_join(b):
        for j in range(4):
            for u in range(NU):
                xi[b][j, pl.ds(8 * u, 8), :] = pltpu.bitcast(
                    xbuf[pl.ds(16 * u, 16), pl.ds(512 * b + 128 * j, 128)], I32)

    def b_gather(b):
        for j in range(4):
            pat = pats[j]
            for u in range(NU):
                xg[b][j, pl.ds(8 * u, 8), :] = _gather(xi[b][j, zrow(u), :], pat)

    def b_gather_direct(b):
        for j in range(4):
            pat = pats[j]
            for u in range(NU):
                v = pltpu.bitcast(xbuf[pl.ds(16 * u, 16), pl.ds(512 * b + 128 * j, 128)], I32)
                xg[b][j, pl.ds(8 * u, 8), :] = _gather(v, pat)

    def b_woven(k):
        st = [g for b in (0, 1) for g in [b_stat_gen(b)]]
        pend = []
        lag = _DEV.get("glag", 44)
        n = 0
        for b in (2, 3):
            for j in range(4):
                pat = pats[j]
                for u in range(NU):
                    v = pltpu.bitcast(xbuf[pl.ds(16 * u, 16), pl.ds(512 * b + 128 * j, 128)], I32)
                    pend.append((b, j, u, _gather(v, pat)))
                    if len(pend) > lag:
                        b_, j_, u_, v_ = pend.pop(0)
                        xg[b_][j_, pl.ds(8 * u_, 8), :] = v_
                    n += 1
                    if n % 4 == 0:
                        next(st[(n - 1) // 144], None)
        for b_, j_, u_, v_ in pend:
            xg[b_][j_, pl.ds(8 * u_, 8), :] = v_
        for g in st:
            for _ in g:
                pass

    def b_stat(b):
        for _ in b_stat_gen(b):
            pass

    def b_stat_gen(b):
        s2 = [jnp.zeros((8, 128), F32) for _ in range(4)]
        for u in range(NU):
            o = _butterfly([xg[b][j, zrow(u), :] for j in range(4)])
            for l2 in range(4):
                xp[4 * l2 + b, pl.ds(8 * u, 8), :] = o[l2]
                e_, o_ = _unpack2(o[l2])
                s2[l2] = s2[l2] + (e_ * e_ + o_ * o_)
            yield
        for l2 in range(4):
            stat[b][l2, pl.ds(16, 8), :] = s2[l2]

    def b_dot(b):
        lhs = _bf(wr16b[...])
        for j in range(4):
            stat[b][j, pl.ds(0, 16), :] = jnp.dot(lhs, _bf(xg[b][j, pl.ds(pl.multiple_of(zero * zero * 8, 8), D // 2), :]),
                                                  preferred_element_type=F32)

    def b_fin(b):
        st = []
        wxs = _butterfly([stat[b][j, zrow(0), :] for j in range(4)])
        sxs = _butterfly([stat[b][j, zrow(1), :] for j in range(4)])
        for l2 in range(4):
            wx, sx = wxs[l2], sxs[l2]
            m = sx * jnp.float32(1.0 / D)
            q = jnp.sum(stat[b][l2, zrow(2), :], axis=0, keepdims=True) * jnp.float32(1.0 / D)
            var = _rbf(jnp.maximum(q - m * m, 0.0))
            rs = 1.0 / _rbf(jnp.sqrt(_rbf(var + jnp.float32(EPS))))
            mb = _rbf(m)
            st.append((mb, rs))
            r = _rbf((wx - mb * wsum[...]) * rs)
            r = jnp.where(r == 0.0, 0.0, r)
            bits = pltpu.bitcast(r, I32)
            mono = ((bits ^ ((bits >> 31) & jnp.int32(0x7FFFFFFF))) >> 16) + 32768
            tok = 512 * b + 4 * (32 * ((lane8 >> 5) ^ l2) + (lane8 & 31)) + l2
            key = pltpu.bitcast((mono << 11) + (2047 - tok) + jnp.int32(0x00800000), F32)
            t = 4 * b + l2
            topk[t // 8] = key if t % 8 == 0 else jnp.where(sub8 == t % 8, key, topk[t // 8])
        return st

    def b_norm(b):
        st = b_fin(b)
        for us in (range(CB // 16), range(CB // 16, NU)):
            for l2 in range(4):
                mb, rs = st[l2]
                for u in us:
                    e_, o_ = _unpack2(xp[4 * l2 + b, zrow(u), :])
                    xnp[4 * l2 + b, pl.ds(8 * u, 8), :] = _pack2((e_ - mb) * rs, (o_ - mb) * rs)

    wrow = wr[...].reshape(1, D)
    wr16b[...] = pltpu.bitcast(jnp.concatenate([jnp.broadcast_to(wrow, (8, D)), jnp.ones((8, D), BF16)], axis=0), I32)
    wsum[...] = jnp.broadcast_to(jnp.sum(wrow.astype(F32), axis=1, keepdims=True), (8, 128))
    topk[2] = jnp.zeros((8, 128), F32)
    cols[...] = jnp.zeros(cols.shape, I32)

    ctok = {"mid": [], "n": 0}

    def c_reset():
        ctok["mid"], ctok["n"] = [], 0

    def pin_lhs(lhs):
        n = ctok["n"]
        ctok["n"] += 1
        nv = lhs.shape[0] // 8
        if n % 2 == 1 or not _DEV.get("cpin", 0):
            return lhs
        parts = [lhs[8 * j:8 * j + 8] for j in range(nv)]
        for k, tok in enumerate(ctok["mid"]):
            t = _DEV.get("cp0", 130) + _DEV.get("cp1", 128) * k - (n // 2) * nv * 16
            if 0 <= t < nv * 16:
                parts[t // 16] = after(parts[t // 16], [tok])
        return jnp.concatenate(parts, axis=0)

    def c_fwd(i):
        h0 = i.off(CB // 2, 0, 8)
        r0 = i.off(CB, 0, 8)
        for l2 in range(4):
            lhs = _bf(pin_lhs(xnp[pl.ds(4 * l2, 4), pl.ds(h0, CB // 2), :].reshape(2 * CB, 128)))
            res = jnp.dot(lhs, _bf(fpk[l2, pl.ds(slow_zero(i), 64), :]), preferred_element_type=F32)
            for ri in range(2):
                y = res[:, 128 * ri:128 * ri + 128]
                if l2 == 3 and ri == 1 and isinstance(i.i, int) and i.i < 2:
                    y = pad_tail(y, i)
                uhat[2 * l2 + ri, :, pl.ds(r0, CB), :] = y.reshape(4, CB, 128)
            yield

    def c_mid(i):
        for k in range(CB // 8):
            rows = pl.ds(i.off(CB, 8 * k, 8), 8)
            krows = pl.ds(i.off(CB, 16 * (k // 2) + k % 2), 8, stride=2)
            uu = [_fft4([(uhat[2 * l2, b, rows, :], uhat[2 * l2 + 1, b, rows, :]) for l2 in range(4)], -1)
                  for b in range(4)]
            yy = [[None] * 4 for _ in range(4)]
            kmode = _DEV.get("kfft", 0)

            def khalf(dl, odd):
                kr = pl.ds(i.off(CB, 16 * (k // 2) + k % 2) + (zero if odd else 0), 8, stride=2)
                x = [(khat[2 * l2, dl, kr, :], khat[2 * l2 + 1, dl, kr, :]) for l2 in range(4)]
                if not odd:
                    s0 = (x[0][0] + x[2][0], x[0][1] + x[2][1])
                    s1 = (x[1][0] + x[3][0], x[1][1] + x[3][1])
                    return {0: (s0[0] + s1[0], s0[1] + s1[1]), 2: (s0[0] - s1[0], s0[1] - s1[1])}
                d0 = (x[0][0] - x[2][0], x[0][1] - x[2][1])
                d1 = (x[1][0] - x[3][0], x[1][1] - x[3][1])
                return {1: (d0[0] + d1[1], d0[1] - d1[0]), 3: (d0[0] - d1[1], d0[1] + d1[0])}

            def acc(pp, m, t):
                pp[m] = t if pp[m] is None else (pp[m][0] + t[0], pp[m][1] + t[1])

            for odd in range(2):
                pps = {k2: [None] * 4 for k2 in (odd, odd + 2)}
                if kmode == 0:
                    for k2 in pps:
                        for dl in range(3, -1, -1):
                            kk = (khat[2 * k2, dl, krows, :], khat[2 * k2 + 1, dl, krows, :])
                            for m in range(3, dl - 1, -1):
                                acc(pps[k2], m, _cmul(*uu[m - dl][k2], *kk))
                elif kmode == 1:
                    for dl in range(3, -1, -1):
                        kk = khalf(dl, odd)
                        for k2 in pps:
                            for m in range(3, dl - 1, -1):
                                acc(pps[k2], m, _cmul(*uu[m - dl][k2], *kk[k2]))
                else:
                    kk = [khalf(dl, odd) for dl in range(4)]
                    for k2 in pps:
                        for m in range(3, -1, -1):
                            for b in range(m, -1, -1):
                                acc(pps[k2], m, _cmul(*uu[b][k2], *kk[m - b][k2]))
                for k2, pp in pps.items():
                    for m in range(3, -1, -1):
                        yy[m][k2] = pp[0] if m == 0 else (pp[m][0] - pp[m - 1][1], pp[m][1] + pp[m - 1][0])
            un = i.off(CB // 8, k)
            for bp in range(2):
                ww = [_fft4(yy[m], 1) for m in (2 * bp, 2 * bp + 1)]
                for l2 in range(4):
                    for ri in range(2):
                        v = _pack2(ww[0][l2][ri], ww[1][l2][ri])
                        yhat[2 * l2 + ri, bp, un] = v
            ctok["mid"].append(v)
            yield

    def c_inv(i):
        u0 = i.off(CB // 8)
        r0 = i.off(2 * CB, 0, 8)
        for l2 in range(4):
            for ri in range(2):
                lhs = yhat[2 * l2 + ri, :, pl.ds(u0, CB // 8)].reshape(2 * CB, 128)
                lhs = _bf(pin_lhs(lhs) if ri == 0 else lhs)
                y = lax.dot_general(lhs, _bf(fpk[l2, pl.ds(slow_zero(i), 64), pl.ds(128 * ri, 128)]), _NT, preferred_element_type=F32)
                if l2 == 3 and ri == 1:
                    y = pad_tail(y, i)
                ybuf[2 * l2 + ri, :, pl.ds(r0, 2 * CB), :] = y.reshape(2, 2 * CB, 128)
            yield

    def c_elt(i):
        for k in range(CB // 16):
            hr = pl.ds(i.off(CB // 2, 8 * k, 8), 8)
            sk = [skip[pl.ds(i.off(CB, 16 * k + e), 8, stride=2), :] for e in range(2)]
            for b in range(4):
                o = []
                for l2 in range(4):
                    xn = _unpack2(xnp[4 * l2 + b, hr, :])
                    xx = _unpack2(xp[4 * l2 + b, hr, :])
                    ss, v = [], []
                    for e in range(2):
                        yr = pl.ds(i.off(2 * CB, 32 * k + 2 * e + b % 2), 8, stride=4)
                        ss.append(ybuf[2 * l2, b // 2, yr, :] + ybuf[2 * l2 + 1, b // 2, yr, :] + xn[e] * sk[e])
                        v.append(xx[e] + ss[e] * _silu(xn[e]))
                    spk[4 * l2 + b, hr, :] = _pack2(*ss)
                    o.append(_pack2(*v))
                p = _butterfly(o)
                for j in range(4):
                    opk[4 * b + j, hr, :] = p[j]
            yield

    def c_top(i):
        k0, k1 = topk[i.off(0, 0)], topk[i.off(0, 1)]
        mx = jnp.max(jnp.max(jnp.maximum(k0, k1), axis=0, keepdims=True), axis=1, keepdims=True)
        topk[i.off(0, 0)] = jnp.where(k0 == mx, 0.0, k0)
        topk[i.off(0, 1)] = jnp.where(k1 == mx, 0.0, k1)
        topk[i.off(0, 2)] = jnp.where(sub8 == i.idx(), mx, topk[i.off(0, 2)])
        yield

    def c_first(i):
        if _DEV.get("toplast", 1):
            yield
            yield from c_fwd(i)
            yield from c_top(i)
        else:
            yield from c_top(i)
            yield from c_fwd(i)

    c_pro, c_loop, c_tail = _pipeline([c_first, c_mid, c_inv, c_elt], NB, newz, reset=c_reset,
                                      weave=_DEV.get("cweave", [1] * (CB // 8) + [3] * (CB // 16) + [0, 0, 0, 2, 2, 0, 0, 2, 2]))
    def first_fwd():
        i = _Idx(0, 0)
        for _ in c_fwd(i):
            pass
        for _ in c_top(i):
            pass

    if _DEV.get("only") != "C":
        ops = {"j": b_join, "g": b_gather, "G": b_gather_direct, "w": b_woven, "s": b_stat, "d": b_dot, "n": b_norm,
               "a": lambda k: a_tail[k](), "f": lambda k: first_fwd()}
        for blk in _DEV.get("bplan", "a0G0G1 a1G2G3d0d1s0s1 s2s3n0n1d2d3 n2n3f0").split():
            block(*[lambda k=k: ops[blk[k]](int(blk[k + 1])) for k in range(0, len(blk), 2)])
    if _DEV.get("only") == "B":
        return bail([cp_g, cp_u] + cp_d)
    for fn in c_pro[1:]:
        block(fn)
    c_loop()
    if _DEV.get("only") == "C":
        return bail([cp_g, cp_u] + cp_d)

    sel = pltpu.bitcast(topk[2], I32) - jnp.int32(0x00800000)
    mono = (sel >> 11) - 32768
    r_sel = pltpu.bitcast((mono ^ ((mono >> 31) & jnp.int32(0x7FFF))) << 16, F32)
    gate_r = _rbf(jax.nn.sigmoid(r_sel))
    posv[...] = 2047 - (sel & 2047)
    tok = [posv[c, 0] for c in range(C)]
    nat = [(t >> 7, t & 127) for t in tok]
    prm = []
    for t in tok:
        l2, l1 = t & 3, (t >> 2) & 127
        prm.append((4 * l2 + (t >> 9), 32 * ((l1 >> 5) ^ l2) + (l1 & 31)))

    def extract(src, k):
        for c, (tp, pp) in enumerate(prm):
            sh = (c - pp) & 127
            for u in range(NU):
                pltpu.store(cols.at[k, pl.ds(8 * u, 8), :], pltpu.roll(src[tp, pl.ds(8 * u, 8), :], sh, 1),
                            mask=lane8 == c)

    def take_rows():
        xs = lax.dot_general(eye[:16], _bf(cols[0, pl.ds(pl.multiple_of(newz(), 8), D // 2), :]), _NT,
                             preferred_element_type=F32)
        xsel_ref[...] = xs

    if _DEV.get("t1", 2) == 0:
        block(c_tail[0], lambda: extract(xnp, 0), lambda: extract(xp, 1))
    elif _DEV.get("t1", 2) == 1:
        block(lambda: extract(xnp, 0), lambda: extract(xp, 1), c_tail[0])
    else:
        block(c_tail[0], lambda: extract(xnp, 0))
    if _DEV.get("t1", 2) == 2:
        block(c_tail[1], take_rows, lambda: extract(xp, 1))
    else:
        block(c_tail[1], take_rows)

    def o_gather(us):
        for j in range(4):
            pat = pats[4 + j]
            for b in range(4):
                for u in us:
                    og[4 * b + j, pl.ds(8 * u, 8), :] = _gather(opk[4 * b + j, zrow(u), :], pat)

    def o_store(u, v, col):
        obuf[pl.ds(16 * u, 8), col] = _bf(v[0:4])
        obuf[pl.ds(16 * u + 8, 8), col] = _bf(pltpu.roll(v, 4, 0)[0:4])

    def o_final(us):
        for t in range(16):
            for u in us:
                o_store(u, og[t, zrow(u), :], pl.ds(128 * t, 128))

    def out_copy(t):
        col = pl.ds(128 * t, 128)
        return pltpu.make_async_copy(obuf.at[:, col], out_hbm.at[:, col], sem_out.at[t])

    def start_out(late):
        for t in range(16):
            hit = nat[0][0] == t
            for c in range(1, C):
                hit = jnp.logical_or(hit, nat[c][0] == t)

            @pl.when(hit if late else jnp.logical_not(hit))
            def _():
                out_copy(t).start()

    ul = NU - CB // 16
    cp_g.wait()
    c_tail[2]()
    xsel = xsel_ref[...]
    xsel_b = xsel.astype(BF16)
    ga = _rbf(jnp.dot(xsel_b, wg[...], preferred_element_type=F32)[:8])
    ga = _rbf(ga * _rbf(jax.nn.sigmoid(ga)))
    o_gather(range(ul))
    cp_u.wait()
    o_final(range(ul))
    up = _rbf(jnp.dot(xsel_b, wu[...], preferred_element_type=F32)[:8])
    o_gather(range(ul, NU))
    extract(spk, 2)
    hh = jnp.concatenate([ga * up, jnp.zeros((8, F), F32)], axis=0).astype(BF16)
    pr = (r128 & (-16)) + 2 * (r128 & 7) + ((r128 >> 3) & 1)
    perm = jnp.where(pr == c128, 1.0, 0.0).astype(BF16)

    def patch(a, n, y):
        z = _rbf(xsel[:8, a:a + n] + _rbf(_rbf(y[:8]) * gate_r[:, :1]))
        g = z * _rbf(jax.nn.sigmoid(z))
        g = jnp.concatenate([g, jnp.zeros((120, n), F32)], axis=0).astype(BF16)
        gt = lax.dot_general(perm[:n, :n], g, _NT, preferred_element_type=F32)
        us = range(a // 16, (a + n) // 16)
        zz = newz()
        for u in us:
            hr = pl.ds(pl.multiple_of(zz + 8 * u, 8), 8)
            xx, ss = _unpack2(cols[1, hr, :]), _unpack2(cols[2, hr, :])
            r0 = 16 * u - a
            w = _pack2(*[xx[e] + _rbf(ss[e] * gt[r0 + 8 * e:r0 + 8 * e + 8]) for e in range(2)])
            for c, (tn, pn) in enumerate(nat):
                tt = 4 * (tn >> 2) + (tn & 3)
                pltpu.store(og.at[tt, pl.ds(8 * u, 8), :], pltpu.roll(w, (pn - c) & 127, 1), mask=lane8 == pn)
        for c, (tn, pn) in enumerate(nat):
            for u in us:
                o_store(u, og[tn, pl.ds(8 * u, 8), :], pl.ds(pl.multiple_of(tn * 128, 128), 128))

    prev = None
    for q, ((a, n), cp) in enumerate(zip(wd_rows, cp_d)):
        cp.wait()
        if q == 0:
            o_final(range(ul, NU))
        if prev is not None:
            patch(*prev)
        y = lax.dot_general(hh, wd[pl.ds(a, n), :], _NT, preferred_element_type=F32)
        prev = (a, n, y)
        if q == _DEV.get("early", 0):
            start_out(False)
    patch(*prev)
    start_out(True)
    for t in range(16):
        out_copy(t).wait()


def _scratch():
    return [
        pltpu.VMEM((D, L), BF16),
        pltpu.VMEM((6, D, N), BF16),
        pltpu.VMEM((D,), BF16),
        pltpu.VMEM((D,), BF16),
        pltpu.VMEM((D,), BF16),
        pltpu.VMEM((D, F), BF16),
        pltpu.VMEM((D, F), BF16),
        pltpu.VMEM((D, F), BF16),
        pltpu.VMEM((4, 64, 256), U32),
        pltpu.VMEM((_NPAT, 8, 128), I32),
        pltpu.VMEM((D, 128), F32),
        pltpu.VMEM((D, 128), F32),
        pltpu.VMEM((5, 2 * D, 128), I32),
        pltpu.VMEM((5, 2 * D, 128), I32),
        pltpu.VMEM((8, 2 * D, 128), I32),
        pltpu.VMEM((8, 2 * D, 128), I32),
        pltpu.VMEM((2, 4 * D, 128), F32),
        pltpu.VMEM((8, 4, D, 128), F32),
        pltpu.VMEM((16, D // 2, 128), I32),
        pltpu.VMEM((16, D // 2, 128), I32),
        pltpu.VMEM((8, 4, D, 128), F32),
        pltpu.VMEM((8, 2, D // 8, 8, 128), I32),
        pltpu.VMEM((8, 2, 2 * D, 128), F32),
        pltpu.VMEM((16, D // 2, 128), I32),
        pltpu.VMEM((3, 8, 128), F32),
        pltpu.VMEM((8, 128), I32),
        pltpu.VMEM((8, D), I32),
        pltpu.VMEM((8, 128), F32),
        pltpu.VMEM((16, D), F32),
        pltpu.VMEM((3, D // 2, 128), I32),
        pltpu.VMEM((16, D // 2, 128), I32),
        pltpu.VMEM((16, D // 2, 128), I32),
        pltpu.VMEM((D, L), BF16),
        pltpu.SemaphoreType.DMA((26,)),
        pltpu.SemaphoreType.DMA((16,)),
    ] + [pltpu.VMEM((4, D // 2, 128), I32)] * 8 + [pltpu.VMEM((4, 24, 128), F32)] * 4


@jax.jit
def pallas_recurrent_scan__ssm_conv_s4__moe_arch_mod__prompt_kernel(
    A_u: jax.Array,
    A_A_re: jax.Array,
    A_A_im: jax.Array,
    A_B_re: jax.Array,
    A_B_im: jax.Array,
    A_C_re: jax.Array,
    A_C_im: jax.Array,
    A_log_dt: jax.Array,
    A_Dskip: jax.Array,
    B_x: jax.Array,
    B_w_r: jax.Array,
    B_w_gate: jax.Array,
    B_w_up: jax.Array,
    B_w_down: jax.Array,
):
    hbm = pl.BlockSpec(memory_space=pltpu.HBM)
    out = pl.pallas_call(
        _kernel,
        out_shape=jax.ShapeDtypeStruct((D, L), BF16),
        in_specs=[hbm] * 15,
        out_specs=hbm,
        scratch_shapes=_scratch(),
        compiler_params=pltpu.CompilerParams(vmem_limit_bytes=110 * 1024 * 1024),
        name="s4_mod",
    )(A_u[0].T, A_A_re, A_A_im, A_B_re, A_B_im, A_C_re, A_C_im, A_log_dt, A_Dskip, B_w_r,
      B_w_gate, B_w_up, B_w_down.T, jnp.asarray(_FPK), jnp.asarray(_PATS))
    return out.T[None]
```

```python
import numpy as np
import jax
import jax.numpy as jnp
from jax import lax
import jax.experimental.pallas as pl
import jax.experimental.pallas.tpu as pltpu

L, D, N, F, C = 2048, 576, 128, 4608, 8
NU = D // 16
CB = 64
NB = D // CB
CO = 32
NO = D // CO
UA = 4
F32, BF16, I32, U32 = jnp.float32, jnp.bfloat16, jnp.int32, jnp.uint32
EPS = 1e-5
_DEV = {}


def _bf16_round_np(x):
    u = np.asarray(x, np.float32).view(np.uint32).astype(np.uint64)
    r = ((u + 0x7FFF + ((u >> 16) & 1)) >> 16) << 16
    return r.astype(np.uint32)


_LROUND = _bf16_round_np(np.arange(L)).view(np.float32).astype(np.int64)
_HI = [(1, 3, 516, 1032), (5, 7, 520, 1288), (4, 260, 772, 1544), (8, 264, 776, 1800), (2, 6, 258, 262)]


def _lane_l1(l2):
    p = np.arange(128)
    return 32 * ((p // 32) ^ l2) + p % 32


def _comp_q():
    t = np.arange(8)[:, None]
    lane = np.arange(128)[None, :]
    return ((lane - 8 - 7 * (t % 4)) % 16) // 4


def _make_tables():
    lane = np.arange(128)
    lo = 8 * (4 * (lane // 16) + lane % 4)
    tab = [dict(), dict()]
    amask = np.zeros(128, bool)
    for q in range(5):
        for e in range(4):
            for par in range(2):
                t = 4 * par + e
                for h in range(2):
                    src = lane[(lane // 4) % 4 == 2 * h + par]
                    dst = (src + (4 * (q % 4) - 8 * h + 8) + 7 * t) % 128
                    assert np.all(_comp_q()[t, dst] == q % 4)
                    sid = e if q < 4 else 4 + e // 2
                    for sl, dl_ in zip(src, dst):
                        ent = (sid, int(dl_))
                        assert tab[par].setdefault(_HI[q][e] + int(lo[sl]), ent) == ent
                    if q == 4 and e % 2 == 1:
                        amask[dst % 16 + 16 * np.arange(8)[:, None]] = True
    pats = []
    for j in range(4):
        pats.append(np.tile(4 * (lane % 32) + ((lane // 32) ^ j), (8, 1)))
    for j in range(4):
        pats.append(np.tile(32 * ((lane % 4) ^ j) + lane // 4, (8, 1)))
    npat0 = len(pats)
    tiles, tile_of = [], {}
    for dl in range(4):
        for l2 in range(4):
            v = _LROUND[512 * dl + 4 * lane + l2]
            key = tuple(v.tolist())
            if key in tile_of:
                tile_of[dl, l2] = tile_of[key]
                continue
            sid = np.array([tab[0][x][0] if x else -1 for x in v])
            ln = np.array([[tab[s8 % 2][x][1] if x else 0 for x in v] for s8 in range(8)])
            steps = []
            for s in sorted(set(sid.tolist()), key=lambda s: -(sid == s).sum()):
                lanes = np.nonzero(sid == s)[0]
                if s < 0:
                    steps.append((-1, None, lanes))
                    continue
                care = sid == s
                kk = None
                for k in range(npat0, len(pats)):
                    oldp, oldc, olds = pats[k]
                    both = care & oldc
                    if olds == s and np.array_equal(oldp[:, both], ln[:, both]):
                        pats[k] = (np.where(care, ln, oldp), care | oldc, s)
                        kk = k
                        break
                if kk is None:
                    pats.append((np.where(care, ln, 0), care, s))
                    kk = len(pats) - 1
                steps.append((s, kk, lanes))
            tiles.append(steps)
            tile_of[key] = tile_of[dl, l2] = len(tiles) - 1
    pats = np.stack([p if k < npat0 else p[0] for k, p in enumerate(pats)]).astype(np.int32)
    tile_of = {k: v for k, v in tile_of.items() if len(k) == 2}
    m = np.arange(128)
    fw = np.zeros((4, 128, 256), np.float64)
    for l2 in range(4):
        t = 4 * _lane_l1(l2) + l2
        th = 2 * np.pi * (2 * m[None, :] + 0.5) * t[:, None] / 1024
        fw[l2, :, :128] = np.cos(th)
        fw[l2, :, 128:] = -np.sin(th)
    fb = _bf16_round_np(fw) >> 16
    fpk = (fb[:, 0::2, :] | (fb[:, 1::2, :] << 16)).astype(np.uint32)
    masks = np.stack([_comp_q() & 1, _comp_q() >> 1, np.tile(amask, (8, 1))]).astype(np.int32)
    return tiles, tile_of, np.concatenate([pats, masks]), fpk


_TILES, _TILE_OF, _PATS, _FPK = _make_tables()
_NPAT = _PATS.shape[0]
_NT_K = len(_TILES)


def _cmul(ar, ai, br, bi):
    return ar * br - ai * bi, ar * bi + ai * br


def _sincos(b):
    magic = jnp.float32(12582912.0)
    t = b * jnp.float32(2.0 / np.pi) + magic
    k = t - magic
    ki = pltpu.bitcast(t, I32)
    r = b - k * jnp.float32(1.5703125)
    r = r - k * jnp.float32(0.0004837512969970703)
    r = r - k * jnp.float32(7.549790126404332e-08)
    u = r * r
    ps = (jnp.float32(-0.0001958295761141926) * u + jnp.float32(0.008332725614309311)) * u \
        + jnp.float32(-0.166666641831398)
    sn = r + (r * u) * ps
    pc = ((jnp.float32(2.437065268168226e-05) * u + jnp.float32(-0.0013886778615415096)) * u
          + jnp.float32(0.04166663438081741)) * u + jnp.float32(-0.5)
    cs = pc * u + jnp.float32(1.0)
    odd = (ki & 1) == 1
    s1 = jnp.where(odd, cs, sn)
    c1 = jnp.where(odd, sn, cs)
    sign = jnp.int32(-2147483648)
    s1 = pltpu.bitcast(pltpu.bitcast(s1, I32) ^ ((ki << 30) & sign), F32)
    c1 = pltpu.bitcast(pltpu.bitcast(c1, I32) ^ (((ki + 1) << 30) & sign), F32)
    return s1, c1


def _gather(x, idx):
    return jnp.take_along_axis(x, idx, axis=1, mode="promise_in_bounds")


def _lanes_mask(lanes):
    lane = lax.broadcasted_iota(I32, (8, 128), 1)
    lanes = sorted(int(x) for x in lanes)
    runs, start, prev = [], lanes[0], lanes[0]
    for x in lanes[1:]:
        if x != prev + 1:
            runs.append((start, prev))
            start = x
        prev = x
    runs.append((start, prev))
    m = None
    for a, b in runs:
        t = (lane == a) if a == b else jnp.logical_and(lane >= a, lane <= b)
        m = t if m is None else jnp.logical_or(m, t)
    return m


def _butterfly(p):
    lane = lax.broadcasted_iota(I32, p[0].shape, 1)
    b0 = (lane & 32) != 0
    b1 = (lane & 64) != 0
    t = [jnp.where(b0, p[k ^ 1], p[k]) for k in range(4)]
    return [jnp.where(b1, t[k ^ 2], t[k]) for k in range(4)]


def _fft4(x, sgn):
    (ar, ai), (br, bi), (cr, ci), (dr, di) = x
    s0r, s0i, d0r, d0i = ar + cr, ai + ci, ar - cr, ai - ci
    s1r, s1i, d1r, d1i = br + dr, bi + di, br - dr, bi - di
    y0 = (s0r + s1r, s0i + s1i)
    y2 = (s0r - s1r, s0i - s1i)
    p = (d0r - d1i, d0i + d1r)
    m = (d0r + d1i, d0i - d1r)
    return [y0, p, y2, m] if sgn > 0 else [y0, m, y2, p]


def _silu(z):
    h = z * jnp.float32(0.5)
    return h + h * jnp.tanh(h)


def _rbf(x):
    return x.astype(BF16).astype(F32)


def _pack2(a, b):
    p = pltpu.pack_elementwise([a, b], packed_dtype=BF16)
    return p if p.dtype == I32 else pltpu.bitcast(p, I32)


def _unpack2(x):
    return [pltpu.unpack_elementwise(x, index=i, packed_dtype=BF16, unpacked_dtype=F32) for i in range(2)]


def _bf(x):
    return pltpu.bitcast(x, BF16)


_NT = (((1,), (1,)), ((), ()))


class _Idx:
    def __init__(self, i, lag, z=None):
        self.i, self.lag, self.z = i, lag, z

    def off(self, stride, const=0, align=None):
        c = const - self.lag * stride
        if isinstance(self.i, int):
            if self.z is None:
                return self.i * stride + c
            v = self.z + (self.i * stride + c)
        else:
            v = self.i * stride + c
        return pl.multiple_of(v, align) if align else v

    def idx(self):
        return self.i - self.lag


def _pipeline(stages, n, newz, weave=None, reset=None):
    ns = len(stages)

    def step(i, lo, hi):
        z = newz() if isinstance(i, int) else None
        gens = {k: stages[k](_Idx(i, k, z)) for k in range(lo, hi)}
        if reset is not None:
            reset()
        if callable(weave):
            weave(gens)
        else:
            for k in weave or ():
                if k in gens:
                    next(gens[k], None)
        for k in range(hi - 1, lo - 1, -1):
            for _ in gens[k]:
                pass

    def body(i, carry):
        step(i, 0, ns)
        return carry

    return ([lambda i=i: step(i, 0, i + 1) for i in range(ns - 1)],
            lambda: lax.fori_loop(ns - 1, n, body, 0),
            [lambda i=i: step(n + i, i + 1, ns) for i in range(ns - 1)])


def _run(fns):
    for fn in fns:
        fn()


def _kernel(x_hbm, are_hbm, aim_hbm, bre_hbm, bim_hbm, cre_hbm, cim_hbm, ldt_hbm, dsk_hbm, wr_hbm,
            wg_hbm, wu_hbm, wd_hbm, f_hbm, pat_hbm,
            out_hbm,
            xbuf, par, ldt, dsk, wr, wg, wu, wd, fpk, pats,
            dtcol, skip, hi_re, hi_im, lo_re, lo_im, comp, khat,
            xp, xnp, uhat, yhat, ybuf, spk, topk, posv, wr16b, wsum, ohb, xsel_ref, cols, opk, og, obuf,
            sem_in, sem_out, *perb):
    xi, xg, stat = perb[0:4], perb[4:8], perb[8:12]
    p_hbm = (are_hbm, aim_hbm, bre_hbm, bim_hbm, cre_hbm, cim_hbm)
    r1 = 16 * UA
    small = [(ldt_hbm, ldt), (pat_hbm.at[pl.ds(0, 1)], pats.at[pl.ds(0, 1)]), (dsk_hbm, dsk)]
    small += [(h.at[pl.ds(0, r1)], par.at[i, pl.ds(0, r1)]) for i, h in enumerate(p_hbm)]
    small += [(h.at[pl.ds(r1, D - r1)], par.at[i, pl.ds(r1, D - r1)]) for i, h in enumerate(p_hbm)]
    small += [(pat_hbm.at[pl.ds(1, _NPAT - 1)], pats.at[pl.ds(1, _NPAT - 1)]), (f_hbm, fpk), (wr_hbm, wr)]
    cps = [pltpu.make_async_copy(s, d, sem_in.at[0 if i < 3 else 1 if i < 9 else 2])
           for i, (s, d) in enumerate(small)]
    ns = 3
    cp_x = pltpu.make_async_copy(x_hbm, xbuf, sem_in.at[ns])
    cp_g = pltpu.make_async_copy(wg_hbm, wg, sem_in.at[ns + 1])
    cp_u = pltpu.make_async_copy(wu_hbm, wu, sem_in.at[ns + 2])
    wd_rows = [(0, 128), (128, 128), (256, 128), (384, 128), (512, 64)]
    waits = _DEV.get("waits", {0: (0, 1, 2, 3, 4)})
    wd_grp = {k: g for g, ks in enumerate(waits.values()) for k in ks}
    cp_d = [pltpu.make_async_copy(wd_hbm.at[pl.ds(a, n)], wd.at[pl.ds(a, n)], sem_in.at[ns + 3 + wd_grp[i]])
            for i, (a, n) in enumerate(wd_rows)]
    if _DEV.get("only"):
        cp_g, cp_u, cp_d = None, None, []
    for cp in cps + [cp_x, cp_g, cp_u] + cp_d:
        if cp is not None:
            cp.start()

    for cp in cps[:3]:
        cp.wait()
    r128 = lax.broadcasted_iota(I32, (128, 128), 0)
    c128 = lax.broadcasted_iota(I32, (128, 128), 1)
    eye = jnp.where(r128 == c128, 1.0, 0.0).astype(BF16)
    dt_row = jnp.exp(ldt[...].astype(F32).reshape(1, D)).astype(BF16)
    dsk_row = dsk[...].reshape(1, D)
    for t in range(5):
        n = min(128, D - 128 * t)
        for row, dst in ((dt_row, dtcol), (dsk_row, skip)):
            b = jnp.broadcast_to(row[:, 128 * t:128 * t + n], (128, n))
            dst[pl.ds(128 * t, n), :] = lax.dot_general(eye[:n, :n], b, _NT, preferred_element_type=F32)

    sub8 = lax.broadcasted_iota(I32, (8, 128), 0)
    lane8 = lax.broadcasted_iota(I32, (8, 128), 1)
    zero = pats[0, 0, 0]
    zcount = [0]

    def newz():
        zcount[0] += 1
        return zero * (64 * zcount[0]) if _DEV.get("zpeel", 1) else None

    def block(*fns):
        if not _DEV.get("blocks", 1):
            return _run(fns)

        def body(k, carry):
            _run(fns)
            return carry

        lax.fori_loop(0, zero + 1, body, 0)

    def slow_zero(i):
        t = i.off(1) * zero if not isinstance(i.i, int) or i.z is None else i.z
        for _ in range(_DEV.get("slow", 0)):
            t = t * t
        return pl.multiple_of(t * 8, 8)

    def after(x, deps):
        never = pats[0] < 0
        d = None
        for v in deps:
            v = v if v.dtype == I32 else pltpu.bitcast(v, I32)
            d = v if d is None else d ^ v
        return jnp.where(never, d if x.dtype == I32 else pltpu.bitcast(d, x.dtype), x)

    def pad_tail(y, i):
        n = _DEV.get("pad", 16)
        if not n:
            return y
        m = y.shape[0]
        base = i.off(1)
        k = m - 8 * _DEV.get("padpos", 8)
        mid = after(y[k:k + 8], [pats[j % _NPAT] * (base + j) for j in range(n)])
        return jnp.concatenate([y[:k], mid, y[k + 8:]], axis=0)

    class Sched:
        tok, g, pre = {}, 0, []

        @classmethod
        def reset(cls):
            cls.tok, cls.g, cls.pre = {}, 0, []

        @classmethod
        def gate(cls, x):
            deps = cls.tok.pop(cls.g, [])
            cls.g += 1
            if not deps or not _DEV.get("gate", 1):
                return x
            return jnp.concatenate([after(x[:8], deps), after(x[8:], deps[-1:])], axis=0)

    slot = {h: (q, e) for q, ent in enumerate(_HI) for e, h in enumerate(ent)}

    def a_prep(i):
        gate = Sched.gate
        for u in range(UA):
            rows = pl.ds(i.off(16 * UA, 16 * u, 16), 16)
            ev = pl.ds(i.off(32 * UA, 32 * u), 16, stride=2)
            od = pl.ds(i.off(32 * UA, 32 * u + 1), 16, stride=2)
            dt = gate(dtcol[rows, :])
            al = dt * par[0, rows, :].astype(F32)
            be = dt * par[1, rows, :].astype(F32)
            cr, ci = _cmul(par[4, rows, :].astype(F32), par[5, rows, :].astype(F32),
                           par[2, rows, :].astype(F32), par[3, rows, :].astype(F32))
            dts = dt * jnp.float32(1.0 / 512)
            cr, ci = cr * dts, ci * dts
            k0 = jnp.sum(cr, axis=1, keepdims=True) * jnp.float32(512.0)
            skip[rows, :] = skip[rows, :] + k0
            yield cr
            s, c = _sincos(gate(be))
            yield c
            pw = {1: (c, s)}
            e = 1
            while e < 256:
                if e in (1, 16):
                    c = gate(c)
                c, s = (c - s) * (c + s), (c + c) * s
                e *= 2
                pw[e] = (c, s)
                if e in (16, 256):
                    yield c
            z = {}
            for e in (1, 8, 256):
                mag = jnp.exp(al * jnp.float32(e))
                c, s = pw[e]
                z[e] = (mag * c, mag * s)
            pend = {}

            def put(tab, q, ee, v):
                key = (tab[0] is hi_re, q, ee // 2)
                if key not in pend:
                    pend[key] = (ee % 2, v)
                    return
                w, o = pend.pop(key)
                lo_, hi_ = (o, v) if w == 0 else (v, o)
                dst = od if ee // 2 else ev
                tab[0][q, dst, :] = _pack2(lo_[0], hi_[0])
                tab[1][q, dst, :] = _pack2(lo_[1], hi_[1])

            h = (cr, ci)
            cnt = 0
            for e in range(1, 9):
                g, ee, m = h, e, z[1]
                while ee in slot:
                    if cnt % 4 == 0:
                        g = (gate(g[0]), g[1])
                    g = _cmul(*g, *m)
                    put((hi_re, hi_im), *slot[ee], g)
                    if ee == e:
                        h = g
                    ee, m = ee + 256, z[256]
                    cnt += 1
                    if cnt % 4 == 0:
                        yield g[0]
            w1 = (gate(z[8][0]), -z[8][1])
            v = [(jnp.ones((16, 128), F32), jnp.zeros((16, 128), F32)), w1]
            v.append(_cmul(*w1, *w1))
            v.append(_cmul(*v[2], *w1))
            w4 = _cmul(*v[2], *v[2])
            for j in range(8):
                for f in range(4):
                    put((lo_re, lo_im), j, f, v[f])
                yield v[3][0]
                if j < 7:
                    w4 = (gate(w4[0]), w4[1])
                    v = [w4 if (j == 0 and f == 0) else _cmul(*v[f], *w4) for f in range(4)]

    def a_gen(i):
        b0 = pats[_NPAT - 3] != 0
        b1 = pats[_NPAT - 2] != 0
        g0, gs = _DEV.get("g0", 13), _DEV.get("gs", None)
        rate = _DEV.get("rate", 0.9)
        for k in range(4 * UA):
            rows = pl.ds(i.off(32 * UA, 8 * k, 8), 8)
            lo = jnp.concatenate([lo_re[:, rows, :].reshape(64, 128), lo_im[:, rows, :].reshape(64, 128)], axis=1)
            h0 = hi_re[0, rows, :]
            if k % 2 == 0 and Sched.pre and _DEV.get("gate", 1):
                h0 = after(h0, Sched.pre)
                Sched.pre = []
            hi = jnp.concatenate([jnp.concatenate([h0, hi_re[1:5, rows, :].reshape(32, 128)], axis=0),
                                  hi_im[:, rows, :].reshape(40, 128)], axis=1)
            o = lax.dot_general(_bf(hi), _bf(lo), _NT, preferred_element_type=F32)
            for q in range(5):
                Sched.tok.setdefault(g0 + int(rate * (5 * (k // 2) + q)), []).append(o[16 * q + 8:16 * q + 16])
            for h in range(2):
                g = [pltpu.roll(o[16 * q + 8 * h:16 * q + 8 * h + 8], 4 * (q % 4) - 8 * h + 8, 1,
                                stride=7, stride_axis=0) for q in range(5)]
                dst = pl.ds(i.off(64 * UA, 16 * k + 8 * h, 8), 8)
                v = jnp.where(b1, jnp.where(b0, g[3], g[2]), jnp.where(b0, g[1], g[0]))
                comp[0, dst, :] = v
                comp[1, dst, :] = g[4]
                if gs is not None:
                    Sched.tok.setdefault(g0 + gs + int(rate * (5 * (k // 2) + 4)), []).append(v)
            if k % 2 == 1:
                yield

    def a_exp(i):
        bm = pats[_NPAT - 1] != 0
        srcs = []
        for u in range(UA):
            def ld(a, e):
                return _pack2(comp[a, pl.ds(i.off(64 * UA, 64 * u + e), 8, stride=4), :],
                              comp[a, pl.ds(i.off(64 * UA, 64 * u + 32 + e), 8, stride=4), :])

            srcs.append([ld(0, e) for e in range(4)]
                        + [jnp.where(bm, ld(1, 2 * k + 1), ld(1, 2 * k)) for k in range(2)])
        cache = {}

        def gat(s, key):
            if key not in cache:
                pat = pats[key]
                cache[key] = [_gather(srcs[u][s], pat) for u in range(UA)]
            return cache[key]

        tiles = []
        for steps in _TILES:
            t = None
            for s, key, lanes in steps:
                v = [jnp.zeros((8, 128), I32)] * UA if s < 0 else gat(s, key)
                t = v if t is None else [jnp.where(_lanes_mask(lanes), v[u], t[u]) for u in range(UA)]
            tiles.append(t)
        yield
        for u0 in range(0, UA, 2):
            lhs = [_bf(jnp.concatenate([tiles[_TILE_OF[dl, l2]][u] for dl in range(4) for u in (u0, u0 + 1)], axis=0))
                   for l2 in range(4)]
            z0 = 0 if u0 == 0 else zero * 8

            def dots(ri):
                return [jnp.dot(lhs[l2], _bf(jnp.concatenate(
                    [fpk[l2, pl.ds(z0 + 16 * (j ^ l2), 16) if u0 == 0 else
                         pl.ds(pl.multiple_of(z0 + 16 * (j ^ l2), 8), 16), pl.ds(128 * ri, 128)]
                     for j in range(4)], axis=0)), preferred_element_type=F32) for l2 in range(4)]

            def store(k2, ri, v):
                khat[2 * k2 + ri, :, pl.ds(i.off(16 * UA, 16 * u0, 16), 32), :] = v.reshape(4, 32, 128)

            def toks(v, step0):
                g1 = _DEV.get("g0", 13) + int(_DEV.get("rate", 0.9) * 10 * UA) + _DEV.get("g1", 0)
                for j in range(8):
                    g = g1 + int(_DEV.get("rate2", 0.7) * (step0 + j))
                    Sched.tok.setdefault(g, []).append(v[16 * j + 8:16 * j + 16])

            re = dots(0)
            s0, d0r, s1, d1r = re[0] + re[2], re[0] - re[2], re[1] + re[3], re[1] - re[3]
            store(0, 0, s0 + s1)
            v = s0 - s1
            store(2, 0, v)
            toks(v, 8 * u0)
            im = dots(1)
            s0, d0i, s1, d1i = im[0] + im[2], im[0] - im[2], im[1] + im[3], im[1] - im[3]
            store(0, 1, s0 + s1)
            store(2, 1, s0 - s1)
            store(1, 0, d0r + d1i)
            store(1, 1, d0i - d1r)
            store(3, 0, d0r - d1i)
            v = d0i + d1r
            store(3, 1, v)
            toks(v, 8 * u0 + 8)
            yield

    def bail(cl):
        for cp in cl:
            if cp is not None:
                cp.wait()
        zr = pl.ds(pl.multiple_of(zero * 8, 8), 16)
        v = khat[zero, zero, zr, :] + skip[zr, :] + (spk[zero, zr, :] + opk[zero, zr, :] + xnp[zero, zr, :] + xp[zero, zr, :]).astype(F32) + topk[zero][:1] + comp[zero, zr, :]
        v = v + (hi_re[zero, zr, :] + hi_im[zero, zr, :] + lo_re[zero, zr, :] + lo_im[zero, zr, :]).astype(F32)
        v = v + uhat[zero, zero, zr, :] + ybuf[zero, zero, zr, :] + yhat[zero, zero, zero][:1].astype(F32)
        obuf[pl.ds(0, 16), pl.ds(0, 128)] = v.astype(BF16)
        cp = pltpu.make_async_copy(obuf.at[pl.ds(0, 16)], out_hbm.at[pl.ds(0, 16)], sem_out)
        cp.start()
        cp.wait()

    if _DEV.get("only") == "C":
        a_tail = [lambda: None] * 2
    else:
        def a_weave(gens):
            if 2 in gens and _DEV.get("expfirst", 1):
                next(gens[2])
            if 0 in gens and 1 in gens:
                for n in _DEV.get("pre", (3, 5, 4)):
                    for _ in range(n):
                        v = next(gens[0])
                    Sched.pre = [v[:8], v[8:]]
                    next(gens[1])
            for k in (1, 2):
                if k in gens:
                    for _ in gens[k]:
                        pass
            if 0 in gens:
                for _ in gens[0]:
                    pass

        a_pro, a_loop, a_tail = _pipeline([a_prep, a_gen, a_exp], NU // UA, newz, reset=Sched.reset,
                                          weave=a_weave)
        for cp in cps[3:9]:
            cp.wait()
        if _DEV.get("only") == "0":
            return bail(cps[9:] + [cp_x])
        a_pro[0]()
        for cp in cps[9:]:
            cp.wait()
        a_pro[1]()
        a_loop()
    if _DEV.get("only") == "A":
        return bail([cp_x, cp_g, cp_u] + cp_d)

    cp_x.wait()

    def zrow(u):
        return pl.ds(pl.multiple_of(zero * 8 + 8 * u, 8), 8)

    def b_gather_direct(b):
        for j in range(4):
            pat = pats[j]
            for u in range(NU):
                v = pltpu.bitcast(xbuf[pl.ds(16 * u, 16), pl.ds(512 * b + 128 * j, 128)], I32)
                xg[b][j, pl.ds(8 * u, 8), :] = _gather(v, pat)

    def b_stat(b):
        for _ in b_stat_gen(b):
            pass

    def b_stat_gen(b):
        s2 = [jnp.zeros((8, 128), F32) for _ in range(4)]
        for u in range(NU):
            o = _butterfly([xg[b][j, zrow(u), :] for j in range(4)])
            for l2 in range(4):
                xp[4 * l2 + b, pl.ds(8 * u, 8), :] = o[l2]
                e_, o_ = _unpack2(o[l2])
                s2[l2] = s2[l2] + (e_ * e_ + o_ * o_)
            yield
        for l2 in range(4):
            stat[b][l2, pl.ds(16, 8), :] = s2[l2]

    def b_dot(b):
        lhs = _bf(wr16b[...])
        for j in range(4):
            stat[b][j, pl.ds(0, 16), :] = jnp.dot(lhs, _bf(xg[b][j, pl.ds(pl.multiple_of(zero * zero * 8, 8), D // 2), :]),
                                                  preferred_element_type=F32)

    def b_fin(b):
        st = []
        wxs = _butterfly([stat[b][j, zrow(0), :] for j in range(4)])
        sxs = _butterfly([stat[b][j, zrow(1), :] for j in range(4)])
        for l2 in range(4):
            wx, sx = wxs[l2], sxs[l2]
            m = sx * jnp.float32(1.0 / D)
            q = jnp.sum(stat[b][l2, zrow(2), :], axis=0, keepdims=True) * jnp.float32(1.0 / D)
            var = _rbf(jnp.maximum(q - m * m, 0.0))
            rs = 1.0 / _rbf(jnp.sqrt(_rbf(var + jnp.float32(EPS))))
            mb = _rbf(m)
            st.append((mb, rs))
            r = _rbf((wx - mb * wsum[...]) * rs)
            r = jnp.where(r == 0.0, 0.0, r)
            bits = pltpu.bitcast(r, I32)
            mono = ((bits ^ ((bits >> 31) & jnp.int32(0x7FFFFFFF))) >> 16) + 32768
            tok = 512 * b + 4 * (32 * ((lane8 >> 5) ^ l2) + (lane8 & 31)) + l2
            key = pltpu.bitcast((mono << 11) + (2047 - tok) + jnp.int32(0x00800000), F32)
            t = 4 * b + l2
            topk[t // 8] = key if t % 8 == 0 else jnp.where(sub8 == t % 8, key, topk[t // 8])
        return st

    def b_norm(b):
        st = b_fin(b)
        for us in (range(CB // 16), range(CB // 16, NU)):
            for l2 in range(4):
                mb, rs = st[l2]
                for u in us:
                    e_, o_ = _unpack2(xp[4 * l2 + b, zrow(u), :])
                    xnp[4 * l2 + b, pl.ds(8 * u, 8), :] = _pack2((e_ - mb) * rs, (o_ - mb) * rs)

    wrow = wr[...].reshape(1, D)
    wr16b[...] = pltpu.bitcast(jnp.concatenate([jnp.broadcast_to(wrow, (8, D)), jnp.ones((8, D), BF16)], axis=0), I32)
    wsum[...] = jnp.broadcast_to(jnp.sum(wrow.astype(F32), axis=1, keepdims=True), (8, 128))
    topk[2] = jnp.zeros((8, 128), F32)
    cols[...] = jnp.zeros(cols.shape, I32)

    ctok = {"mid": [], "n": 0}

    def c_reset():
        ctok["mid"], ctok["n"] = [], 0

    def pin_lhs(lhs):
        n = ctok["n"]
        ctok["n"] += 1
        nv = lhs.shape[0] // 8
        if n % 2 == 1 or not _DEV.get("cpin", 0):
            return lhs
        parts = [lhs[8 * j:8 * j + 8] for j in range(nv)]
        for k, tok in enumerate(ctok["mid"]):
            t = _DEV.get("cp0", 130) + _DEV.get("cp1", 128) * k - (n // 2) * nv * 16
            if 0 <= t < nv * 16:
                parts[t // 16] = after(parts[t // 16], [tok])
        return jnp.concatenate(parts, axis=0)

    def c_fwd(i):
        h0 = i.off(CB // 2, 0, 8)
        r0 = i.off(CB, 0, 8)
        for l2 in range(4):
            lhs = _bf(pin_lhs(xnp[pl.ds(4 * l2, 4), pl.ds(h0, CB // 2), :].reshape(2 * CB, 128)))
            res = jnp.dot(lhs, _bf(fpk[l2, pl.ds(slow_zero(i), 64), :]), preferred_element_type=F32)
            for ri in range(2):
                y = res[:, 128 * ri:128 * ri + 128]
                if l2 == 3 and ri == 1 and isinstance(i.i, int) and i.i < 2:
                    y = pad_tail(y, i)
                uhat[2 * l2 + ri, :, pl.ds(r0, CB), :] = y.reshape(4, CB, 128)
            yield

    def c_mid(i):
        for k in range(CB // 8):
            rows = pl.ds(i.off(CB, 8 * k, 8), 8)
            krows = pl.ds(i.off(CB, 16 * (k // 2) + k % 2), 8, stride=2)
            uu = [_fft4([(uhat[2 * l2, b, rows, :], uhat[2 * l2 + 1, b, rows, :]) for l2 in range(4)], -1)
                  for b in range(4)]
            yy = [[None] * 4 for _ in range(4)]
            kmode = _DEV.get("kfft", 0)

            def khalf(dl, odd):
                kr = pl.ds(i.off(CB, 16 * (k // 2) + k % 2) + (zero if odd else 0), 8, stride=2)
                x = [(khat[2 * l2, dl, kr, :], khat[2 * l2 + 1, dl, kr, :]) for l2 in range(4)]
                if not odd:
                    s0 = (x[0][0] + x[2][0], x[0][1] + x[2][1])
                    s1 = (x[1][0] + x[3][0], x[1][1] + x[3][1])
                    return {0: (s0[0] + s1[0], s0[1] + s1[1]), 2: (s0[0] - s1[0], s0[1] - s1[1])}
                d0 = (x[0][0] - x[2][0], x[0][1] - x[2][1])
                d1 = (x[1][0] - x[3][0], x[1][1] - x[3][1])
                return {1: (d0[0] + d1[1], d0[1] - d1[0]), 3: (d0[0] - d1[1], d0[1] + d1[0])}

            def acc(pp, m, t):
                pp[m] = t if pp[m] is None else (pp[m][0] + t[0], pp[m][1] + t[1])

            for odd in range(2):
                pps = {k2: [None] * 4 for k2 in (odd, odd + 2)}
                if kmode == 0:
                    for k2 in pps:
                        for dl in range(3, -1, -1):
                            kk = (khat[2 * k2, dl, krows, :], khat[2 * k2 + 1, dl, krows, :])
                            for m in range(3, dl - 1, -1):
                                acc(pps[k2], m, _cmul(*uu[m - dl][k2], *kk))
                elif kmode == 1:
                    for dl in range(3, -1, -1):
                        kk = khalf(dl, odd)
                        for k2 in pps:
                            for m in range(3, dl - 1, -1):
                                acc(pps[k2], m, _cmul(*uu[m - dl][k2], *kk[k2]))
                else:
                    kk = [khalf(dl, odd) for dl in range(4)]
                    for k2 in pps:
                        for m in range(3, -1, -1):
                            for b in range(m, -1, -1):
                                acc(pps[k2], m, _cmul(*uu[b][k2], *kk[m - b][k2]))
                for k2, pp in pps.items():
                    for m in range(3, -1, -1):
                        yy[m][k2] = pp[0] if m == 0 else (pp[m][0] - pp[m - 1][1], pp[m][1] + pp[m - 1][0])
            un = i.off(CB // 8, k)
            for bp in range(2):
                ww = [_fft4(yy[m], 1) for m in (2 * bp, 2 * bp + 1)]
                for l2 in range(4):
                    for ri in range(2):
                        v = _pack2(ww[0][l2][ri], ww[1][l2][ri])
                        yhat[2 * l2 + ri, bp, un] = v
            ctok["mid"].append(v)
            yield

    def c_inv(i):
        u0 = i.off(CB // 8)
        r0 = i.off(2 * CB, 0, 8)
        for l2 in range(4):
            for ri in range(2):
                lhs = yhat[2 * l2 + ri, :, pl.ds(u0, CB // 8)].reshape(2 * CB, 128)
                lhs = _bf(pin_lhs(lhs) if ri == 0 else lhs)
                y = lax.dot_general(lhs, _bf(fpk[l2, pl.ds(slow_zero(i), 64), pl.ds(128 * ri, 128)]), _NT, preferred_element_type=F32)
                if l2 == 3 and ri == 1:
                    y = pad_tail(y, i)
                ybuf[2 * l2 + ri, :, pl.ds(r0, 2 * CB), :] = y.reshape(2, 2 * CB, 128)
            yield

    def c_elt(i):
        for k in range(CB // 16):
            hr = pl.ds(i.off(CB // 2, 8 * k, 8), 8)
            sk = [skip[pl.ds(i.off(CB, 16 * k + e), 8, stride=2), :] for e in range(2)]
            for b in range(4):
                o = []
                for l2 in range(4):
                    xn = _unpack2(xnp[4 * l2 + b, hr, :])
                    xx = _unpack2(xp[4 * l2 + b, hr, :])
                    ss, v = [], []
                    for e in range(2):
                        yr = pl.ds(i.off(2 * CB, 32 * k + 2 * e + b % 2), 8, stride=4)
                        ss.append(ybuf[2 * l2, b // 2, yr, :] + ybuf[2 * l2 + 1, b // 2, yr, :] + xn[e] * sk[e])
                        v.append(xx[e] + ss[e] * _silu(xn[e]))
                    spk[4 * l2 + b, hr, :] = _pack2(*ss)
                    o.append(_pack2(*v))
                p = _butterfly(o)
                for j in range(4):
                    opk[4 * b + j, hr, :] = p[j]
            yield

    def c_top(i):
        k0, k1 = topk[i.off(0, 0)], topk[i.off(0, 1)]
        mx = jnp.max(jnp.max(jnp.maximum(k0, k1), axis=0, keepdims=True), axis=1, keepdims=True)
        topk[i.off(0, 0)] = jnp.where(k0 == mx, 0.0, k0)
        topk[i.off(0, 1)] = jnp.where(k1 == mx, 0.0, k1)
        topk[i.off(0, 2)] = jnp.where(sub8 == i.idx(), mx, topk[i.off(0, 2)])
        yield

    def c_first(i):
        if _DEV.get("toplast", 1):
            yield
            yield from c_fwd(i)
            yield from c_top(i)
        else:
            yield from c_top(i)
            yield from c_fwd(i)

    c_pro, c_loop, c_tail = _pipeline([c_first, c_mid, c_inv, c_elt], NB, newz, reset=c_reset,
                                      weave=_DEV.get("cweave", [1] * (CB // 8) + [3] * (CB // 16) + [0, 0, 0, 2, 2, 0, 0, 2, 2]))
    def first_fwd():
        i = _Idx(0, 0)
        for _ in c_fwd(i):
            pass
        for _ in c_top(i):
            pass

    if _DEV.get("only") != "C":
        ops = {"G": b_gather_direct, "s": b_stat, "d": b_dot, "n": b_norm,
               "a": lambda k: a_tail[k](), "f": lambda k: first_fwd()}
        for blk in _DEV.get("bplan", "a0G0G1 a1G2G3d0d1s0s1 s2s3n0n1d2d3 n2n3f0").split():
            block(*[lambda k=k: ops[blk[k]](int(blk[k + 1])) for k in range(0, len(blk), 2)])
    if _DEV.get("only") == "B":
        return bail([cp_g, cp_u] + cp_d)
    for fn in c_pro[1:]:
        block(fn)
    c_loop()
    if _DEV.get("only") in ("C", "ABC"):
        return bail([cp_g, cp_u] + cp_d)

    sel = pltpu.bitcast(topk[2], I32) - jnp.int32(0x00800000)
    mono = (sel >> 11) - 32768
    r_sel = pltpu.bitcast((mono ^ ((mono >> 31) & jnp.int32(0x7FFF))) << 16, F32)
    gate_r = _rbf(jax.nn.sigmoid(r_sel))
    posv[...] = 2047 - (sel & 2047)
    tok = [posv[c, 0] for c in range(C)]
    nat = [(t >> 7, t & 127) for t in tok]
    prm = []
    for t in tok:
        l2, l1 = t & 3, (t >> 2) & 127
        prm.append((4 * l2 + (t >> 9), 32 * ((l1 >> 5) ^ l2) + (l1 & 31)))

    def extract(src, k):
        for c, (tp, pp) in enumerate(prm):
            sh = (c - pp) & 127
            for u in range(NU):
                pltpu.store(cols.at[k, pl.ds(8 * u, 8), :], pltpu.roll(src[tp, pl.ds(8 * u, 8), :], sh, 1),
                            mask=lane8 == c)

    for c, (tp, pp) in enumerate(prm):
        ohb[c] = jnp.where(jnp.logical_and(sub8 == c // 2, lane8 == pp), jnp.int32(0x3F80 << (16 * (c % 2))), 0)

    def take_rows():
        for c, (tp, pp) in enumerate(prm):
            xsel_ref[c] = lax.dot_general(_bf(ohb[c]), _bf(xnp[tp]), _NT, preferred_element_type=F32)[:8]

    if _DEV.get("t1", 1) == 0:
        block(c_tail[0], take_rows)
        block(c_tail[1])
    else:
        block(c_tail[0])
        block(c_tail[1], take_rows)

    def o_gather(us):
        for j in range(4):
            pat = pats[4 + j]
            for b in range(4):
                for u in us:
                    v = _gather(opk[4 * b + j, zrow(u), :], pat)
                    og[4 * b + j, pl.ds(8 * u, 8), :] = v
                    o_store(u, v, pl.ds(512 * b + 128 * j, 128))

    def o_store(u, v, col):
        obuf[pl.ds(16 * u, 8), col] = _bf(v[0:4])
        obuf[pl.ds(16 * u + 8, 8), col] = _bf(pltpu.roll(v, 4, 0)[0:4])

    bits = jnp.int32(0)
    for c in range(C):
        bits = bits | (jnp.int32(1) << nat[c][0])

    def out_tiles(routed, a, n, op):
        for t in range(16):
            @pl.when(((bits >> t) & 1) == routed)
            def _():
                col = pl.ds(128 * t, 128)
                op(pltpu.make_async_copy(obuf.at[pl.ds(a, n), col], out_hbm.at[pl.ds(a, n), col], sem_out))

    late = _DEV.get("late", {2: (0, 384), 4: (384, 192)})

    u1, u2 = _DEV.get("u1", 12), _DEV.get("u2", 28)
    cp_g.wait()
    c_tail[2]()
    xsel = xsel_ref[0]
    for c in range(1, C):
        xsel = xsel + xsel_ref[c]
    xsel_b = jnp.concatenate([xsel, jnp.zeros((8, D), F32)], axis=0).astype(BF16)
    ga = _rbf(jnp.dot(xsel_b, wg[...], preferred_element_type=F32)[:8])
    ga = _rbf(ga * _rbf(jax.nn.sigmoid(ga)))
    extract(xp, 0)
    o_gather(range(u1))
    cp_u.wait()
    up = _rbf(jnp.dot(xsel_b, wu[...], preferred_element_type=F32)[:8])
    extract(spk, 1)
    o_gather(range(u1, u2))
    hh = jnp.concatenate([ga * up, jnp.zeros((8, F), F32)], axis=0).astype(BF16)
    pr = (r128 & (-16)) + 2 * (r128 & 7) + ((r128 >> 3) & 1)
    perm = jnp.where(pr == c128, 1.0, 0.0).astype(BF16)

    def patch(q, y):
        a, n = wd_rows[q]
        z = _rbf(xsel[:8, a:a + n] + _rbf(_rbf(y[:8]) * gate_r[:, :1]))
        g = z * _rbf(jax.nn.sigmoid(z))
        g = jnp.concatenate([g, jnp.zeros((120, n), F32)], axis=0).astype(BF16)
        gt = lax.dot_general(perm[:n, :n], g, _NT, preferred_element_type=F32)
        us = range(a // 16, (a + n) // 16)
        zz = newz()
        for u in us:
            hr = pl.ds(pl.multiple_of(zz + 8 * u, 8), 8)
            xx, ss = _unpack2(cols[0, hr, :]), _unpack2(cols[1, hr, :])
            r0 = 16 * u - a
            w = _pack2(*[xx[e] + _rbf(ss[e] * gt[r0 + 8 * e:r0 + 8 * e + 8]) for e in range(2)])
            for c, (tn, pn) in enumerate(nat):
                tt = 4 * (tn >> 2) + (tn & 3)
                pltpu.store(og.at[tt, pl.ds(8 * u, 8), :], pltpu.roll(w, (pn - c) & 127, 1), mask=lane8 == pn)
        for c, (tn, pn) in enumerate(nat):
            for u in us:
                o_store(u, og[tn, pl.ds(8 * u, 8), :], pl.ds(pl.multiple_of(tn * 128, 128), 128))
        if q in late:
            out_tiles(1, *late[q], lambda cp: cp.start())

    if u2 == NU:
        out_tiles(0, 0, D, lambda cp: cp.start())
    prev = None
    for q, (a, n) in enumerate(wd_rows):
        for k in waits.get(q, ()):
            cp_d[k].wait()
        if prev is not None and q in waits:
            patch(*prev)
            prev = None
        y = lax.dot_general(hh, wd[pl.ds(a, n), :], _NT, preferred_element_type=F32)
        if q == 0:
            o_gather(range(u2, NU))
        if prev is not None:
            patch(*prev)
        prev = (q, y)
        if q == 0 and u2 < NU:
            out_tiles(0, 0, D, lambda cp: cp.start())
    patch(*prev)
    pltpu.make_async_copy(obuf, out_hbm, sem_out).wait()


def _scratch():
    return [
        pltpu.VMEM((D, L), BF16),
        pltpu.VMEM((6, D, N), BF16),
        pltpu.VMEM((D,), BF16),
        pltpu.VMEM((D,), BF16),
        pltpu.VMEM((D,), BF16),
        pltpu.VMEM((D, F), BF16),
        pltpu.VMEM((D, F), BF16),
        pltpu.VMEM((D, F), BF16),
        pltpu.VMEM((4, 64, 256), U32),
        pltpu.VMEM((_NPAT, 8, 128), I32),
        pltpu.VMEM((D, 128), F32),
        pltpu.VMEM((D, 128), F32),
        pltpu.VMEM((5, 2 * D, 128), I32),
        pltpu.VMEM((5, 2 * D, 128), I32),
        pltpu.VMEM((8, 2 * D, 128), I32),
        pltpu.VMEM((8, 2 * D, 128), I32),
        pltpu.VMEM((2, 4 * D, 128), F32),
        pltpu.VMEM((8, 4, D, 128), F32),
        pltpu.VMEM((16, D // 2, 128), I32),
        pltpu.VMEM((16, D // 2, 128), I32),
        pltpu.VMEM((8, 4, D, 128), F32),
        pltpu.VMEM((8, 2, D // 8, 8, 128), I32),
        pltpu.VMEM((8, 2, 2 * D, 128), F32),
        pltpu.VMEM((16, D // 2, 128), I32),
        pltpu.VMEM((3, 8, 128), F32),
        pltpu.VMEM((8, 128), I32),
        pltpu.VMEM((8, D), I32),
        pltpu.VMEM((8, 128), F32),
        pltpu.VMEM((C, 8, 128), I32),
        pltpu.VMEM((C, 8, D), F32),
        pltpu.VMEM((2, D // 2, 128), I32),
        pltpu.VMEM((16, D // 2, 128), I32),
        pltpu.VMEM((16, D // 2, 128), I32),
        pltpu.VMEM((D, L), BF16),
        pltpu.SemaphoreType.DMA((6 + len(_DEV.get("waits", {0: 0})),)),
        pltpu.SemaphoreType.DMA,
    ] + [pltpu.VMEM((4, D // 2, 128), I32)] * 8 + [pltpu.VMEM((4, 24, 128), F32)] * 4


@jax.jit
def pallas_recurrent_scan__ssm_conv_s4__moe_arch_mod__prompt_kernel(
    A_u: jax.Array,
    A_A_re: jax.Array,
    A_A_im: jax.Array,
    A_B_re: jax.Array,
    A_B_im: jax.Array,
    A_C_re: jax.Array,
    A_C_im: jax.Array,
    A_log_dt: jax.Array,
    A_Dskip: jax.Array,
    B_x: jax.Array,
    B_w_r: jax.Array,
    B_w_gate: jax.Array,
    B_w_up: jax.Array,
    B_w_down: jax.Array,
):
    hbm = pl.BlockSpec(memory_space=pltpu.HBM)
    out = pl.pallas_call(
        _kernel,
        out_shape=jax.ShapeDtypeStruct((D, L), BF16),
        in_specs=[hbm] * 15,
        out_specs=hbm,
        scratch_shapes=_scratch(),
        compiler_params=pltpu.CompilerParams(vmem_limit_bytes=110 * 1024 * 1024),
        name="s4_mod",
    )(A_u[0].T, A_A_re, A_A_im, A_B_re, A_B_im, A_C_re, A_C_im, A_log_dt, A_Dskip, B_w_r,
      B_w_gate, B_w_up, B_w_down.T, jnp.asarray(_FPK), jnp.asarray(_PATS))
    return out.T[None]
```

```python
import numpy as np
import jax
import jax.numpy as jnp
from jax import lax
import jax.experimental.pallas as pl
import jax.experimental.pallas.tpu as pltpu

L, D, N, F, C = 2048, 576, 128, 4608, 8
NU = D // 16
CB = 64
NB = D // CB
CO = 32
NO = D // CO
UA = 4
F32, BF16, I32, U32 = jnp.float32, jnp.bfloat16, jnp.int32, jnp.uint32
EPS = 1e-5
_DEV = {}


def _bf16_round_np(x):
    u = np.asarray(x, np.float32).view(np.uint32).astype(np.uint64)
    r = ((u + 0x7FFF + ((u >> 16) & 1)) >> 16) << 16
    return r.astype(np.uint32)


_LROUND = _bf16_round_np(np.arange(L)).view(np.float32).astype(np.int64)
_HI = [(1, 3, 516, 1032), (5, 7, 520, 1288), (4, 260, 772, 1544), (8, 264, 776, 1800), (2, 6, 258, 262)]


def _lane_l1(l2):
    p = np.arange(128)
    return 32 * ((p // 32) ^ l2) + p % 32


def _comp_q():
    t = np.arange(8)[:, None]
    lane = np.arange(128)[None, :]
    return ((lane - 8 - 7 * (t % 4)) % 16) // 4


def _make_tables():
    lane = np.arange(128)
    lo = 8 * (4 * (lane // 16) + lane % 4)
    tab = [dict(), dict()]
    amask = np.zeros(128, bool)
    for q in range(5):
        for e in range(4):
            for par in range(2):
                t = 4 * par + e
                for h in range(2):
                    src = lane[(lane // 4) % 4 == 2 * h + par]
                    dst = (src + (4 * (q % 4) - 8 * h + 8) + 7 * t) % 128
                    assert np.all(_comp_q()[t, dst] == q % 4)
                    sid = e if q < 4 else 4 + e // 2
                    for sl, dl_ in zip(src, dst):
                        ent = (sid, int(dl_))
                        assert tab[par].setdefault(_HI[q][e] + int(lo[sl]), ent) == ent
                    if q == 4 and e % 2 == 1:
                        amask[dst % 16 + 16 * np.arange(8)[:, None]] = True
    pats = []
    for j in range(4):
        pats.append(np.tile(4 * (lane % 32) + ((lane // 32) ^ j), (8, 1)))
    for j in range(4):
        pats.append(np.tile(32 * ((lane % 4) ^ j) + lane // 4, (8, 1)))
    npat0 = len(pats)
    tiles, tile_of = [], {}
    for dl in range(4):
        for l2 in range(4):
            v = _LROUND[512 * dl + 4 * lane + l2]
            key = tuple(v.tolist())
            if key in tile_of:
                tile_of[dl, l2] = tile_of[key]
                continue
            sid = np.array([tab[0][x][0] if x else -1 for x in v])
            ln = np.array([[tab[s8 % 2][x][1] if x else 0 for x in v] for s8 in range(8)])
            steps = []
            for s in sorted(set(sid.tolist()), key=lambda s: -(sid == s).sum()):
                lanes = np.nonzero(sid == s)[0]
                if s < 0:
                    steps.append((-1, None, lanes))
                    continue
                care = sid == s
                kk = None
                for k in range(npat0, len(pats)):
                    oldp, oldc, olds = pats[k]
                    both = care & oldc
                    if olds == s and np.array_equal(oldp[:, both], ln[:, both]):
                        pats[k] = (np.where(care, ln, oldp), care | oldc, s)
                        kk = k
                        break
                if kk is None:
                    pats.append((np.where(care, ln, 0), care, s))
                    kk = len(pats) - 1
                steps.append((s, kk, lanes))
            tiles.append(steps)
            tile_of[key] = tile_of[dl, l2] = len(tiles) - 1
    pats = np.stack([p if k < npat0 else p[0] for k, p in enumerate(pats)]).astype(np.int32)
    tile_of = {k: v for k, v in tile_of.items() if len(k) == 2}
    m = np.arange(128)
    fw = np.zeros((4, 128, 256), np.float64)
    for l2 in range(4):
        t = 4 * _lane_l1(l2) + l2
        th = 2 * np.pi * (2 * m[None, :] + 0.5) * t[:, None] / 1024
        fw[l2, :, :128] = np.cos(th)
        fw[l2, :, 128:] = -np.sin(th)
    fb = _bf16_round_np(fw) >> 16
    fpk = (fb[:, 0::2, :] | (fb[:, 1::2, :] << 16)).astype(np.uint32)
    masks = np.stack([_comp_q() & 1, _comp_q() >> 1, np.tile(amask, (8, 1))]).astype(np.int32)
    return tiles, tile_of, np.concatenate([pats, masks]), fpk


_TILES, _TILE_OF, _PATS, _FPK = _make_tables()
_NPAT = _PATS.shape[0]
_NT_K = len(_TILES)


def _cmul(ar, ai, br, bi):
    return ar * br - ai * bi, ar * bi + ai * br


def _sincos(b):
    magic = jnp.float32(12582912.0)
    t = b * jnp.float32(2.0 / np.pi) + magic
    k = t - magic
    ki = pltpu.bitcast(t, I32)
    r = b - k * jnp.float32(1.5703125)
    r = r - k * jnp.float32(0.0004837512969970703)
    r = r - k * jnp.float32(7.549790126404332e-08)
    u = r * r
    ps = (jnp.float32(-0.0001958295761141926) * u + jnp.float32(0.008332725614309311)) * u \
        + jnp.float32(-0.166666641831398)
    sn = r + (r * u) * ps
    pc = ((jnp.float32(2.437065268168226e-05) * u + jnp.float32(-0.0013886778615415096)) * u
          + jnp.float32(0.04166663438081741)) * u + jnp.float32(-0.5)
    cs = pc * u + jnp.float32(1.0)
    odd = (ki & 1) == 1
    s1 = jnp.where(odd, cs, sn)
    c1 = jnp.where(odd, sn, cs)
    sign = jnp.int32(-2147483648)
    s1 = pltpu.bitcast(pltpu.bitcast(s1, I32) ^ ((ki << 30) & sign), F32)
    c1 = pltpu.bitcast(pltpu.bitcast(c1, I32) ^ (((ki + 1) << 30) & sign), F32)
    return s1, c1


def _gather(x, idx):
    return jnp.take_along_axis(x, idx, axis=1, mode="promise_in_bounds")


def _lanes_mask(lanes):
    lane = lax.broadcasted_iota(I32, (8, 128), 1)
    lanes = sorted(int(x) for x in lanes)
    runs, start, prev = [], lanes[0], lanes[0]
    for x in lanes[1:]:
        if x != prev + 1:
            runs.append((start, prev))
            start = x
        prev = x
    runs.append((start, prev))
    m = None
    for a, b in runs:
        t = (lane == a) if a == b else jnp.logical_and(lane >= a, lane <= b)
        m = t if m is None else jnp.logical_or(m, t)
    return m


def _butterfly(p):
    lane = lax.broadcasted_iota(I32, p[0].shape, 1)
    b0 = (lane & 32) != 0
    b1 = (lane & 64) != 0
    t = [jnp.where(b0, p[k ^ 1], p[k]) for k in range(4)]
    return [jnp.where(b1, t[k ^ 2], t[k]) for k in range(4)]


def _fft4(x, sgn):
    (ar, ai), (br, bi), (cr, ci), (dr, di) = x
    s0r, s0i, d0r, d0i = ar + cr, ai + ci, ar - cr, ai - ci
    s1r, s1i, d1r, d1i = br + dr, bi + di, br - dr, bi - di
    y0 = (s0r + s1r, s0i + s1i)
    y2 = (s0r - s1r, s0i - s1i)
    p = (d0r - d1i, d0i + d1r)
    m = (d0r + d1i, d0i - d1r)
    return [y0, p, y2, m] if sgn > 0 else [y0, m, y2, p]


def _silu(z):
    h = z * jnp.float32(0.5)
    return h + h * jnp.tanh(h)


def _rbf(x):
    return x.astype(BF16).astype(F32)


def _pack2(a, b):
    p = pltpu.pack_elementwise([a, b], packed_dtype=BF16)
    return p if p.dtype == I32 else pltpu.bitcast(p, I32)


def _unpack2(x):
    return [pltpu.unpack_elementwise(x, index=i, packed_dtype=BF16, unpacked_dtype=F32) for i in range(2)]


def _bf(x):
    return pltpu.bitcast(x, BF16)


_NT = (((1,), (1,)), ((), ()))


class _Idx:
    def __init__(self, i, lag, z=None):
        self.i, self.lag, self.z = i, lag, z

    def off(self, stride, const=0, align=None):
        c = const - self.lag * stride
        if isinstance(self.i, int):
            if self.z is None:
                return self.i * stride + c
            v = self.z + (self.i * stride + c)
        else:
            v = self.i * stride + c
        return pl.multiple_of(v, align) if align else v

    def idx(self):
        return self.i - self.lag


def _pipeline(stages, n, newz, weave=None, reset=None):
    ns = len(stages)

    def step(i, lo, hi):
        z = newz() if isinstance(i, int) else None
        gens = {k: stages[k](_Idx(i, k, z)) for k in range(lo, hi)}
        if reset is not None:
            reset()
        if callable(weave):
            weave(gens)
        else:
            for k in weave or ():
                if k in gens:
                    next(gens[k], None)
        for k in range(hi - 1, lo - 1, -1):
            for _ in gens[k]:
                pass

    def body(i, carry):
        step(i, 0, ns)
        return carry

    return ([lambda i=i: step(i, 0, i + 1) for i in range(ns - 1)],
            lambda: lax.fori_loop(ns - 1, n, body, 0),
            [lambda i=i: step(n + i, i + 1, ns) for i in range(ns - 1)])


def _run(fns):
    for fn in fns:
        fn()


def _kernel(x_hbm, are_hbm, aim_hbm, bre_hbm, bim_hbm, cre_hbm, cim_hbm, ldt_hbm, dsk_hbm, wr_hbm,
            wg_hbm, wu_hbm, wd_hbm, f_hbm, pat_hbm,
            out_hbm,
            xbuf, par, ldt, dsk, wr, wg, wu, wd, fpk, pats,
            dtcol, skip, hi_re, hi_im, lo_re, lo_im, comp, khat,
            xp, xnp, uhat, yhat, ybuf, spk, topk, posv, wr16b, wsum, ohb, xsel_ref, hbuf, hpk, cols, opk, og, obuf,
            sem_in, sem_out, *perb):
    xi, xg, stat = perb[0:4], perb[4:8], perb[8:12]
    p_hbm = (are_hbm, aim_hbm, bre_hbm, bim_hbm, cre_hbm, cim_hbm)
    r1 = 16 * UA
    small = [(ldt_hbm, ldt), (pat_hbm.at[pl.ds(0, 1)], pats.at[pl.ds(0, 1)]), (dsk_hbm, dsk)]
    small += [(h.at[pl.ds(0, r1)], par.at[i, pl.ds(0, r1)]) for i, h in enumerate(p_hbm)]
    small += [(h.at[pl.ds(r1, D - r1)], par.at[i, pl.ds(r1, D - r1)]) for i, h in enumerate(p_hbm)]
    small += [(pat_hbm.at[pl.ds(1, _NPAT - 1)], pats.at[pl.ds(1, _NPAT - 1)]), (f_hbm, fpk), (wr_hbm, wr)]
    cps = [pltpu.make_async_copy(s, d, sem_in.at[0 if i < 3 else 1 if i < 9 else 2])
           for i, (s, d) in enumerate(small)]
    ns = 3
    cp_x = pltpu.make_async_copy(x_hbm, xbuf, sem_in.at[ns])
    cp_g = pltpu.make_async_copy(wg_hbm, wg, sem_in.at[ns + 1])
    cp_u = pltpu.make_async_copy(wu_hbm, wu, sem_in.at[ns + 2])
    wd_rows = [(0, 128), (128, 128), (256, 128), (384, 128), (512, 64)]
    waits = _DEV.get("waits", {0: (0, 1, 2, 3), 4: (4,)})
    wd_grp = {k: g for g, ks in enumerate(waits.values()) for k in ks}
    cp_d = [pltpu.make_async_copy(wd_hbm.at[pl.ds(a, n)], wd.at[pl.ds(a, n)], sem_in.at[ns + 3 + wd_grp[i]])
            for i, (a, n) in enumerate(wd_rows)]
    if _DEV.get("only"):
        cp_g, cp_u, cp_d = None, None, []
    for cp in cps + [cp_x, cp_g, cp_u] + cp_d:
        if cp is not None:
            cp.start()

    for cp in cps[:3]:
        cp.wait()
    r128 = lax.broadcasted_iota(I32, (128, 128), 0)
    c128 = lax.broadcasted_iota(I32, (128, 128), 1)
    eye = jnp.where(r128 == c128, 1.0, 0.0).astype(BF16)
    dt_row = jnp.exp(ldt[...].astype(F32).reshape(1, D)).astype(BF16)
    dsk_row = dsk[...].reshape(1, D)
    for t in range(5):
        n = min(128, D - 128 * t)
        for row, dst in ((dt_row, dtcol), (dsk_row, skip)):
            b = jnp.broadcast_to(row[:, 128 * t:128 * t + n], (128, n))
            dst[pl.ds(128 * t, n), :] = lax.dot_general(eye[:n, :n], b, _NT, preferred_element_type=F32)

    sub8 = lax.broadcasted_iota(I32, (8, 128), 0)
    lane8 = lax.broadcasted_iota(I32, (8, 128), 1)
    zero = pats[0, 0, 0]
    zcount = [0]

    def newz():
        zcount[0] += 1
        return zero * (64 * zcount[0]) if _DEV.get("zpeel", 1) else None

    def block(*fns):
        if not _DEV.get("blocks", 1):
            return _run(fns)

        def body(k, carry):
            _run(fns)
            return carry

        lax.fori_loop(0, zero + 1, body, 0)

    def slow_zero(i):
        t = i.off(1) * zero if not isinstance(i.i, int) or i.z is None else i.z
        for _ in range(_DEV.get("slow", 0)):
            t = t * t
        return pl.multiple_of(t * 8, 8)

    def after(x, deps):
        never = pats[0] < 0
        d = None
        for v in deps:
            v = v if v.dtype == I32 else pltpu.bitcast(v, I32)
            d = v if d is None else d ^ v
        return jnp.where(never, d if x.dtype == I32 else pltpu.bitcast(d, x.dtype), x)

    def pad_tail(y, i):
        n = _DEV.get("pad", 16)
        if not n:
            return y
        m = y.shape[0]
        base = i.off(1)
        k = m - 8 * _DEV.get("padpos", 8)
        mid = after(y[k:k + 8], [pats[j % _NPAT] * (base + j) for j in range(n)])
        return jnp.concatenate([y[:k], mid, y[k + 8:]], axis=0)

    class Sched:
        tok, g, pre = {}, 0, []

        @classmethod
        def reset(cls):
            cls.tok, cls.g, cls.pre = {}, 0, []

        @classmethod
        def gate(cls, x):
            deps = cls.tok.pop(cls.g, [])
            cls.g += 1
            if not deps or not _DEV.get("gate", 1):
                return x
            return jnp.concatenate([after(x[:8], deps), after(x[8:], deps[-1:])], axis=0)

    slot = {h: (q, e) for q, ent in enumerate(_HI) for e, h in enumerate(ent)}

    def a_prep(i):
        gate = Sched.gate
        for u in range(UA):
            rows = pl.ds(i.off(16 * UA, 16 * u, 16), 16)
            ev = pl.ds(i.off(32 * UA, 32 * u), 16, stride=2)
            od = pl.ds(i.off(32 * UA, 32 * u + 1), 16, stride=2)
            dt = gate(dtcol[rows, :])
            al = dt * par[0, rows, :].astype(F32)
            be = dt * par[1, rows, :].astype(F32)
            cr, ci = _cmul(par[4, rows, :].astype(F32), par[5, rows, :].astype(F32),
                           par[2, rows, :].astype(F32), par[3, rows, :].astype(F32))
            dts = dt * jnp.float32(1.0 / 512)
            cr, ci = cr * dts, ci * dts
            k0 = jnp.sum(cr, axis=1, keepdims=True) * jnp.float32(512.0)
            skip[rows, :] = skip[rows, :] + k0
            yield cr
            s, c = _sincos(gate(be))
            yield c
            pw = {1: (c, s)}
            e = 1
            while e < 256:
                if e in (1, 16):
                    c = gate(c)
                c, s = (c - s) * (c + s), (c + c) * s
                e *= 2
                pw[e] = (c, s)
                if e in (16, 256):
                    yield c
            z = {}
            for e in (1, 8, 256):
                mag = jnp.exp(al * jnp.float32(e))
                c, s = pw[e]
                z[e] = (mag * c, mag * s)
            pend = {}

            def put(tab, q, ee, v):
                key = (tab[0] is hi_re, q, ee // 2)
                if key not in pend:
                    pend[key] = (ee % 2, v)
                    return
                w, o = pend.pop(key)
                lo_, hi_ = (o, v) if w == 0 else (v, o)
                dst = od if ee // 2 else ev
                tab[0][q, dst, :] = _pack2(lo_[0], hi_[0])
                tab[1][q, dst, :] = _pack2(lo_[1], hi_[1])

            h = (cr, ci)
            cnt = 0
            for e in range(1, 9):
                g, ee, m = h, e, z[1]
                while ee in slot:
                    if cnt % 4 == 0:
                        g = (gate(g[0]), g[1])
                    g = _cmul(*g, *m)
                    put((hi_re, hi_im), *slot[ee], g)
                    if ee == e:
                        h = g
                    ee, m = ee + 256, z[256]
                    cnt += 1
                    if cnt % 4 == 0:
                        yield g[0]
            w1 = (gate(z[8][0]), -z[8][1])
            v = [(jnp.ones((16, 128), F32), jnp.zeros((16, 128), F32)), w1]
            v.append(_cmul(*w1, *w1))
            v.append(_cmul(*v[2], *w1))
            w4 = _cmul(*v[2], *v[2])
            for j in range(8):
                for f in range(4):
                    put((lo_re, lo_im), j, f, v[f])
                yield v[3][0]
                if j < 7:
                    w4 = (gate(w4[0]), w4[1])
                    v = [w4 if (j == 0 and f == 0) else _cmul(*v[f], *w4) for f in range(4)]

    def a_gen(i):
        b0 = pats[_NPAT - 3] != 0
        b1 = pats[_NPAT - 2] != 0
        g0, gs = _DEV.get("g0", 13), _DEV.get("gs", None)
        rate = _DEV.get("rate", 0.9)
        for k in range(4 * UA):
            rows = pl.ds(i.off(32 * UA, 8 * k, 8), 8)
            lo = jnp.concatenate([lo_re[:, rows, :].reshape(64, 128), lo_im[:, rows, :].reshape(64, 128)], axis=1)
            h0 = hi_re[0, rows, :]
            if k % 2 == 0 and Sched.pre and _DEV.get("gate", 1):
                h0 = after(h0, Sched.pre)
                Sched.pre = []
            hi = jnp.concatenate([jnp.concatenate([h0, hi_re[1:5, rows, :].reshape(32, 128)], axis=0),
                                  hi_im[:, rows, :].reshape(40, 128)], axis=1)
            o = lax.dot_general(_bf(hi), _bf(lo), _NT, preferred_element_type=F32)
            for q in range(5):
                Sched.tok.setdefault(g0 + int(rate * (5 * (k // 2) + q)), []).append(o[16 * q + 8:16 * q + 16])
            for h in range(2):
                g = [pltpu.roll(o[16 * q + 8 * h:16 * q + 8 * h + 8], 4 * (q % 4) - 8 * h + 8, 1,
                                stride=7, stride_axis=0) for q in range(5)]
                dst = pl.ds(i.off(64 * UA, 16 * k + 8 * h, 8), 8)
                v = jnp.where(b1, jnp.where(b0, g[3], g[2]), jnp.where(b0, g[1], g[0]))
                comp[0, dst, :] = v
                comp[1, dst, :] = g[4]
                if gs is not None:
                    Sched.tok.setdefault(g0 + gs + int(rate * (5 * (k // 2) + 4)), []).append(v)
            if k % 2 == 1:
                yield

    def a_exp(i):
        bm = pats[_NPAT - 1] != 0
        srcs = []
        for u in range(UA):
            def ld(a, e):
                return _pack2(comp[a, pl.ds(i.off(64 * UA, 64 * u + e), 8, stride=4), :],
                              comp[a, pl.ds(i.off(64 * UA, 64 * u + 32 + e), 8, stride=4), :])

            srcs.append([ld(0, e) for e in range(4)]
                        + [jnp.where(bm, ld(1, 2 * k + 1), ld(1, 2 * k)) for k in range(2)])
        cache = {}

        def gat(s, key):
            if key not in cache:
                pat = pats[key]
                cache[key] = [_gather(srcs[u][s], pat) for u in range(UA)]
            return cache[key]

        tiles = []
        for steps in _TILES:
            t = None
            for s, key, lanes in steps:
                v = [jnp.zeros((8, 128), I32)] * UA if s < 0 else gat(s, key)
                t = v if t is None else [jnp.where(_lanes_mask(lanes), v[u], t[u]) for u in range(UA)]
            tiles.append(t)
        yield
        for u0 in range(0, UA, 2):
            lhs = [_bf(jnp.concatenate([tiles[_TILE_OF[dl, l2]][u] for dl in range(4) for u in (u0, u0 + 1)], axis=0))
                   for l2 in range(4)]
            z0 = 0 if u0 == 0 else zero * 8

            def dots(ri):
                return [jnp.dot(lhs[l2], _bf(jnp.concatenate(
                    [fpk[l2, pl.ds(z0 + 16 * (j ^ l2), 16) if u0 == 0 else
                         pl.ds(pl.multiple_of(z0 + 16 * (j ^ l2), 8), 16), pl.ds(128 * ri, 128)]
                     for j in range(4)], axis=0)), preferred_element_type=F32) for l2 in range(4)]

            def store(k2, ri, v):
                khat[2 * k2 + ri, :, pl.ds(i.off(16 * UA, 16 * u0, 16), 32), :] = v.reshape(4, 32, 128)

            def toks(v, step0):
                g1 = _DEV.get("g0", 13) + int(_DEV.get("rate", 0.9) * 10 * UA) + _DEV.get("g1", 0)
                for j in range(8):
                    g = g1 + int(_DEV.get("rate2", 0.7) * (step0 + j))
                    Sched.tok.setdefault(g, []).append(v[16 * j + 8:16 * j + 16])

            re = dots(0)
            s0, d0r, s1, d1r = re[0] + re[2], re[0] - re[2], re[1] + re[3], re[1] - re[3]
            store(0, 0, s0 + s1)
            v = s0 - s1
            store(2, 0, v)
            toks(v, 8 * u0)
            im = dots(1)
            s0, d0i, s1, d1i = im[0] + im[2], im[0] - im[2], im[1] + im[3], im[1] - im[3]
            store(0, 1, s0 + s1)
            store(2, 1, s0 - s1)
            store(1, 0, d0r + d1i)
            store(1, 1, d0i - d1r)
            store(3, 0, d0r - d1i)
            v = d0i + d1r
            store(3, 1, v)
            toks(v, 8 * u0 + 8)
            yield

    def bail(cl):
        for cp in cl:
            if cp is not None:
                cp.wait()
        zr = pl.ds(pl.multiple_of(zero * 8, 8), 16)
        v = khat[zero, zero, zr, :] + skip[zr, :] + (spk[zero, zr, :] + opk[zero, zr, :] + xnp[zero, zr, :] + xp[zero, zr, :]).astype(F32) + topk[zero][:1] + comp[zero, zr, :]
        v = v + (hi_re[zero, zr, :] + hi_im[zero, zr, :] + lo_re[zero, zr, :] + lo_im[zero, zr, :]).astype(F32)
        v = v + uhat[zero, zero, zr, :] + ybuf[zero, zero, zr, :] + yhat[zero, zero, zero][:1].astype(F32)
        obuf[pl.ds(0, 16), pl.ds(0, 128)] = v.astype(BF16)
        cp = pltpu.make_async_copy(obuf.at[pl.ds(0, 16)], out_hbm.at[pl.ds(0, 16)], sem_out)
        cp.start()
        cp.wait()

    if _DEV.get("only") == "C":
        a_tail = [lambda: None] * 2
    else:
        def a_weave(gens):
            if 2 in gens and _DEV.get("expfirst", 1):
                next(gens[2])
            if 0 in gens and 1 in gens:
                for n in _DEV.get("pre", (3, 5, 4)):
                    for _ in range(n):
                        v = next(gens[0])
                    Sched.pre = [v[:8], v[8:]]
                    next(gens[1])
            for k in (1, 2):
                if k in gens:
                    for _ in gens[k]:
                        pass
            if 0 in gens:
                for _ in gens[0]:
                    pass

        a_pro, a_loop, a_tail = _pipeline([a_prep, a_gen, a_exp], NU // UA, newz, reset=Sched.reset,
                                          weave=a_weave)
        for cp in cps[3:9]:
            cp.wait()
        if _DEV.get("only") == "0":
            return bail(cps[9:] + [cp_x])
        a_pro[0]()
        for cp in cps[9:]:
            cp.wait()
        a_pro[1]()
        a_loop()
    if _DEV.get("only") == "A":
        return bail([cp_x, cp_g, cp_u] + cp_d)

    cp_x.wait()

    def zrow(u):
        return pl.ds(pl.multiple_of(zero * 8 + 8 * u, 8), 8)

    def b_gather_direct(b):
        for j in range(4):
            pat = pats[j]
            for u in range(NU):
                v = pltpu.bitcast(xbuf[pl.ds(16 * u, 16), pl.ds(512 * b + 128 * j, 128)], I32)
                xg[b][j, pl.ds(8 * u, 8), :] = _gather(v, pat)

    def b_stat(b):
        for _ in b_stat_gen(b):
            pass

    def b_stat_gen(b):
        s2 = [jnp.zeros((8, 128), F32) for _ in range(4)]
        for u in range(NU):
            o = _butterfly([xg[b][j, zrow(u), :] for j in range(4)])
            for l2 in range(4):
                xp[4 * l2 + b, pl.ds(8 * u, 8), :] = o[l2]
                e_, o_ = _unpack2(o[l2])
                s2[l2] = s2[l2] + (e_ * e_ + o_ * o_)
            yield
        for l2 in range(4):
            stat[b][l2, pl.ds(16, 8), :] = s2[l2]

    def b_dot(b):
        lhs = _bf(wr16b[...])
        for j in range(4):
            stat[b][j, pl.ds(0, 16), :] = jnp.dot(lhs, _bf(xg[b][j, pl.ds(pl.multiple_of(zero * zero * 8, 8), D // 2), :]),
                                                  preferred_element_type=F32)

    def b_fin(b):
        st = []
        wxs = _butterfly([stat[b][j, zrow(0), :] for j in range(4)])
        sxs = _butterfly([stat[b][j, zrow(1), :] for j in range(4)])
        for l2 in range(4):
            wx, sx = wxs[l2], sxs[l2]
            m = sx * jnp.float32(1.0 / D)
            q = jnp.sum(stat[b][l2, zrow(2), :], axis=0, keepdims=True) * jnp.float32(1.0 / D)
            var = _rbf(jnp.maximum(q - m * m, 0.0))
            rs = 1.0 / _rbf(jnp.sqrt(_rbf(var + jnp.float32(EPS))))
            mb = _rbf(m)
            st.append((mb, rs))
            r = _rbf((wx - mb * wsum[...]) * rs)
            r = jnp.where(r == 0.0, 0.0, r)
            bits = pltpu.bitcast(r, I32)
            mono = ((bits ^ ((bits >> 31) & jnp.int32(0x7FFFFFFF))) >> 16) + 32768
            tok = 512 * b + 4 * (32 * ((lane8 >> 5) ^ l2) + (lane8 & 31)) + l2
            key = pltpu.bitcast((mono << 11) + (2047 - tok) + jnp.int32(0x00800000), F32)
            t = 4 * b + l2
            topk[t // 8] = key if t % 8 == 0 else jnp.where(sub8 == t % 8, key, topk[t // 8])
        return st

    def b_norm(b):
        st = b_fin(b)
        for us in (range(CB // 16), range(CB // 16, NU)):
            for l2 in range(4):
                mb, rs = st[l2]
                for u in us:
                    e_, o_ = _unpack2(xp[4 * l2 + b, zrow(u), :])
                    xnp[4 * l2 + b, pl.ds(8 * u, 8), :] = _pack2((e_ - mb) * rs, (o_ - mb) * rs)

    wrow = wr[...].reshape(1, D)
    wr16b[...] = pltpu.bitcast(jnp.concatenate([jnp.broadcast_to(wrow, (8, D)), jnp.ones((8, D), BF16)], axis=0), I32)
    wsum[...] = jnp.broadcast_to(jnp.sum(wrow.astype(F32), axis=1, keepdims=True), (8, 128))
    topk[2] = jnp.zeros((8, 128), F32)
    cols[...] = jnp.zeros(cols.shape, I32)

    ctok = {"mid": [], "n": 0, "elt": []}

    def c_reset():
        ctok["mid"], ctok["n"] = [], 0

    def pin_lhs(lhs):
        n = ctok["n"]
        ctok["n"] += 1
        nv = lhs.shape[0] // 8
        if n % 2 == 1 or not _DEV.get("cpin", 0):
            return lhs
        parts = [lhs[8 * j:8 * j + 8] for j in range(nv)]
        for k, tok in enumerate(ctok["mid"]):
            t = _DEV.get("cp0", 130) + _DEV.get("cp1", 128) * k - (n // 2) * nv * 16
            if 0 <= t < nv * 16:
                parts[t // 16] = after(parts[t // 16], [tok])
        return jnp.concatenate(parts, axis=0)

    def c_fwd(i):
        h0 = i.off(CB // 2, 0, 8)
        r0 = i.off(CB, 0, 8)
        for l2 in range(4):
            lhs = _bf(pin_lhs(xnp[pl.ds(4 * l2, 4), pl.ds(h0, CB // 2), :].reshape(2 * CB, 128)))
            res = jnp.dot(lhs, _bf(fpk[l2, pl.ds(slow_zero(i), 64), :]), preferred_element_type=F32)
            for ri in range(2):
                y = res[:, 128 * ri:128 * ri + 128]
                if l2 == 3 and ri == 1 and isinstance(i.i, int) and i.i < 2:
                    y = pad_tail(y, i)
                uhat[2 * l2 + ri, :, pl.ds(r0, CB), :] = y.reshape(4, CB, 128)
            yield

    def c_mid(i):
        for k in range(CB // 8):
            rows = pl.ds(i.off(CB, 8 * k, 8), 8)
            krows = pl.ds(i.off(CB, 16 * (k // 2) + k % 2), 8, stride=2)
            uu = [_fft4([(uhat[2 * l2, b, rows, :], uhat[2 * l2 + 1, b, rows, :]) for l2 in range(4)], -1)
                  for b in range(4)]
            yy = [[None] * 4 for _ in range(4)]
            kmode = _DEV.get("kfft", 0)

            def khalf(dl, odd):
                kr = pl.ds(i.off(CB, 16 * (k // 2) + k % 2) + (zero if odd else 0), 8, stride=2)
                x = [(khat[2 * l2, dl, kr, :], khat[2 * l2 + 1, dl, kr, :]) for l2 in range(4)]
                if not odd:
                    s0 = (x[0][0] + x[2][0], x[0][1] + x[2][1])
                    s1 = (x[1][0] + x[3][0], x[1][1] + x[3][1])
                    return {0: (s0[0] + s1[0], s0[1] + s1[1]), 2: (s0[0] - s1[0], s0[1] - s1[1])}
                d0 = (x[0][0] - x[2][0], x[0][1] - x[2][1])
                d1 = (x[1][0] - x[3][0], x[1][1] - x[3][1])
                return {1: (d0[0] + d1[1], d0[1] - d1[0]), 3: (d0[0] - d1[1], d0[1] + d1[0])}

            def acc(pp, m, t):
                pp[m] = t if pp[m] is None else (pp[m][0] + t[0], pp[m][1] + t[1])

            for odd in range(2):
                pps = {k2: [None] * 4 for k2 in (odd, odd + 2)}
                if kmode == 0:
                    for k2 in pps:
                        for dl in range(3, -1, -1):
                            kk = (khat[2 * k2, dl, krows, :], khat[2 * k2 + 1, dl, krows, :])
                            for m in range(3, dl - 1, -1):
                                acc(pps[k2], m, _cmul(*uu[m - dl][k2], *kk))
                elif kmode == 1:
                    for dl in range(3, -1, -1):
                        kk = khalf(dl, odd)
                        for k2 in pps:
                            for m in range(3, dl - 1, -1):
                                acc(pps[k2], m, _cmul(*uu[m - dl][k2], *kk[k2]))
                else:
                    kk = [khalf(dl, odd) for dl in range(4)]
                    for k2 in pps:
                        for m in range(3, -1, -1):
                            for b in range(m, -1, -1):
                                acc(pps[k2], m, _cmul(*uu[b][k2], *kk[m - b][k2]))
                for k2, pp in pps.items():
                    for m in range(3, -1, -1):
                        yy[m][k2] = pp[0] if m == 0 else (pp[m][0] - pp[m - 1][1], pp[m][1] + pp[m - 1][0])
            un = i.off(CB // 8, k)
            for bp in range(2):
                ww = [_fft4(yy[m], 1) for m in (2 * bp, 2 * bp + 1)]
                for l2 in range(4):
                    for ri in range(2):
                        v = _pack2(ww[0][l2][ri], ww[1][l2][ri])
                        yhat[2 * l2 + ri, bp, un] = v
            ctok["mid"].append(v)
            yield

    def c_inv(i):
        u0 = i.off(CB // 8)
        r0 = i.off(2 * CB, 0, 8)
        for l2 in range(4):
            for ri in range(2):
                lhs = yhat[2 * l2 + ri, :, pl.ds(u0, CB // 8)].reshape(2 * CB, 128)
                lhs = _bf(pin_lhs(lhs) if ri == 0 else lhs)
                y = lax.dot_general(lhs, _bf(fpk[l2, pl.ds(slow_zero(i), 64), pl.ds(128 * ri, 128)]), _NT, preferred_element_type=F32)
                if l2 == 3 and ri == 1:
                    y = pad_tail(y, i)
                ybuf[2 * l2 + ri, :, pl.ds(r0, 2 * CB), :] = y.reshape(2, 2 * CB, 128)
            yield

    def c_elt(i):
        for k in range(CB // 16):
            hr = pl.ds(i.off(CB // 2, 8 * k, 8), 8)
            sk = [skip[pl.ds(i.off(CB, 16 * k + e), 8, stride=2), :] for e in range(2)]
            for b in range(4):
                o = []
                for l2 in range(4):
                    w = xnp[4 * l2 + b, hr, :]
                    if ctok["elt"]:
                        w = after(w, ctok["elt"])
                    xn = _unpack2(w)
                    xx = _unpack2(xp[4 * l2 + b, hr, :])
                    ss, v = [], []
                    for e in range(2):
                        yr = pl.ds(i.off(2 * CB, 32 * k + 2 * e + b % 2), 8, stride=4)
                        ss.append(ybuf[2 * l2, b // 2, yr, :] + ybuf[2 * l2 + 1, b // 2, yr, :] + xn[e] * sk[e])
                        v.append(xx[e] + ss[e] * _silu(xn[e]))
                    spk[4 * l2 + b, hr, :] = _pack2(*ss)
                    o.append(_pack2(*v))
                p = _butterfly(o)
                for j in range(4):
                    opk[4 * b + j, hr, :] = p[j]
                yield

    def c_top(i):
        k0, k1 = topk[i.off(0, 0)], topk[i.off(0, 1)]
        mx = jnp.max(jnp.max(jnp.maximum(k0, k1), axis=0, keepdims=True), axis=1, keepdims=True)
        topk[i.off(0, 0)] = jnp.where(k0 == mx, 0.0, k0)
        topk[i.off(0, 1)] = jnp.where(k1 == mx, 0.0, k1)
        topk[i.off(0, 2)] = jnp.where(sub8 == i.idx(), mx, topk[i.off(0, 2)])
        yield

    def c_first(i):
        if _DEV.get("toplast", 1):
            yield
            yield from c_fwd(i)
            yield from c_top(i)
        else:
            yield from c_top(i)
            yield from c_fwd(i)

    c_pro, c_loop, c_tail = _pipeline([c_first, c_mid, c_inv, c_elt], NB, newz, reset=c_reset,
                                      weave=_DEV.get("cweave", [1] * (CB // 8) + [3] * (CB // 4) + [0, 0, 0, 2, 2, 0, 0, 2, 2]))
    def first_fwd():
        i = _Idx(0, 0)
        for _ in c_fwd(i):
            pass
        for _ in c_top(i):
            pass

    if _DEV.get("only") != "C":
        ops = {"G": b_gather_direct, "s": b_stat, "d": b_dot, "n": b_norm,
               "a": lambda k: a_tail[k](), "f": lambda k: first_fwd()}
        for blk in _DEV.get("bplan", "a0G0G1 a1G2G3d0d1s0s1 s2s3n0n1d2d3 n2n3f0").split():
            block(*[lambda k=k: ops[blk[k]](int(blk[k + 1])) for k in range(0, len(blk), 2)])
    if _DEV.get("only") == "B":
        return bail([cp_g, cp_u] + cp_d)
    for fn in c_pro[1:]:
        block(fn)
    c_loop()
    if _DEV.get("only") in ("C", "ABC"):
        return bail([cp_g, cp_u] + cp_d)

    sel = pltpu.bitcast(topk[2], I32) - jnp.int32(0x00800000)
    mono = (sel >> 11) - 32768
    r_sel = pltpu.bitcast((mono ^ ((mono >> 31) & jnp.int32(0x7FFF))) << 16, F32)
    gate_r = _rbf(jax.nn.sigmoid(r_sel))
    posv[...] = 2047 - (sel & 2047)
    tok = [posv[c, 0] for c in range(C)]
    nat = [(t >> 7, t & 127) for t in tok]
    prm = []
    for t in tok:
        l2, l1 = t & 3, (t >> 2) & 127
        prm.append((4 * l2 + (t >> 9), 32 * ((l1 >> 5) ^ l2) + (l1 & 31)))

    def extract(src, k):
        for c, (tp, pp) in enumerate(prm):
            sh = (c - pp) & 127
            for u in range(NU):
                pltpu.store(cols.at[k, pl.ds(8 * u, 8), :], pltpu.roll(src[tp, pl.ds(8 * u, 8), :], sh, 1),
                            mask=lane8 == c)

    for c, (tp, pp) in enumerate(prm):
        ohb[c] = jnp.where(jnp.logical_and(sub8 == c // 2, lane8 == pp), jnp.int32(0x3F80 << (16 * (c % 2))), 0)

    def take_rows():
        for c, (tp, pp) in enumerate(prm):
            xsel_ref[c] = lax.dot_general(_bf(ohb[c]), _bf(xnp[tp]), _NT, preferred_element_type=F32)[:8]

    def stages(*items):
        def run():
            z = newz()
            for fn, k in items:
                for _ in fn(_Idx(k, 0, z)):
                    pass
        return run

    e1, e2 = _DEV.get("e1", ()), _DEV.get("e2", (NB - 3,))
    block(stages((c_mid, NB - 1), *[(c_elt, k) for k in e1], (c_inv, NB - 2)))
    block(stages(*[(c_elt, k) for k in e2], (c_inv, NB - 1)), take_rows, lambda: extract(xp, 0))

    def o_gather(us):
        for j in range(4):
            pat = pats[4 + j]
            for b in range(4):
                for u in us:
                    v = _gather(opk[4 * b + j, pl.ds(8 * u, 8), :], pat)
                    og[4 * b + j, pl.ds(8 * u, 8), :] = v
                    o_store(u, v, pl.ds(512 * b + 128 * j, 128))

    def o_store(u, v, col):
        obuf[pl.ds(16 * u, 8), col] = _bf(v[0:4])
        obuf[pl.ds(16 * u + 8, 8), col] = _bf(pltpu.roll(v, 4, 0)[0:4])

    bits = jnp.int32(0)
    for c in range(C):
        bits = bits | (jnp.int32(1) << nat[c][0])

    def out_tiles(routed, a, n, op):
        for t in range(16):
            @pl.when(((bits >> t) & 1) == routed)
            def _():
                col = pl.ds(128 * t, 128)
                op(pltpu.make_async_copy(obuf.at[pl.ds(a, n), col], out_hbm.at[pl.ds(a, n), col], sem_out))

    late = _DEV.get("late", {2: (0, 384), 4: (384, 192)})

    u1, u2 = _DEV.get("u1", 28), NU

    def project(w, post, fill, frate):
        pend = []
        nt = F // 128
        lag = _DEV.get("flag", 0)
        done = 0
        for t in range(nt + lag):
            if t < nt:
                pend.append([jnp.dot(xsel_b[:, a:a + n], w[pl.ds(a, n), pl.ds(128 * t, 128)],
                                     preferred_element_type=F32)[:8] for a, n in wd_rows])
            if t >= lag:
                ps = pend.pop(0)
                v = _rbf((ps[0] + ps[1]) + (ps[2] + ps[3]) + ps[4])
                ctok["elt"] = [v]
                post(t - lag, v)
            while fill and done * nt < (t + 1) * len(fill) * frate and done < len(fill):
                fill[done]()
                done += 1
        for fn in fill[done:]:
            fn()
        ctok["elt"] = []

    def elt_pieces(ks):
        out = []
        for k in ks:
            g = c_elt(_Idx(k, 0))
            out += [lambda g=g: next(g, None)] * (CB // 4)
        return out

    def post_gate(t, ga):
        hbuf[:, pl.ds(128 * t, 128)] = _rbf(ga * _rbf(jax.nn.sigmoid(ga)))

    def post_up(t, up):
        h = hbuf[:, pl.ds(128 * t, 128)] * up
        hpk[:, pl.ds(128 * t, 128)] = pltpu.bitcast(
            jnp.concatenate([h, jnp.zeros((8, 128), F32)], axis=0).astype(BF16), I32)

    cp_g.wait()
    xsel = xsel_ref[0]
    for c in range(1, C):
        xsel = xsel + xsel_ref[c]
    xsel_b = jnp.concatenate([xsel, jnp.zeros((8, D), F32)], axis=0).astype(BF16)
    ks = [k for k in range(NB - 3, NB) if k not in e1 and k not in e2]
    ng = _DEV.get("ng", 2)
    project(wg, post_gate, elt_pieces(ks[:ng]), _DEV.get("fr1", 1.0))
    o_gather(range(u1))
    cp_u.wait()
    project(wu, post_up, elt_pieces(ks[ng:]), _DEV.get("fr2", 2.5))
    o_gather(range(u1, 32))
    o_gather(range(32, u2))
    extract(spk, 1)
    pr = (r128 & (-16)) + 2 * (r128 & 7) + ((r128 >> 3) & 1)
    perm = jnp.where(pr == c128, 1.0, 0.0).astype(BF16)

    def patch(q, y):
        a, n = wd_rows[q]
        z = _rbf(xsel[:8, a:a + n] + _rbf(_rbf(y[:8]) * gate_r[:, :1]))
        g = z * _rbf(jax.nn.sigmoid(z))
        g = jnp.concatenate([g, jnp.zeros((120, n), F32)], axis=0).astype(BF16)
        gt = lax.dot_general(perm[:n, :n], g, _NT, preferred_element_type=F32)
        us = range(a // 16, (a + n) // 16)
        zz = newz()
        for u in us:
            hr = pl.ds(pl.multiple_of(zz + 8 * u, 8), 8)
            xx, ss = _unpack2(cols[0, hr, :]), _unpack2(cols[1, hr, :])
            r0 = 16 * u - a
            w = _pack2(*[xx[e] + _rbf(ss[e] * gt[r0 + 8 * e:r0 + 8 * e + 8]) for e in range(2)])
            for c, (tn, pn) in enumerate(nat):
                tt = 4 * (tn >> 2) + (tn & 3)
                pltpu.store(og.at[tt, pl.ds(8 * u, 8), :], pltpu.roll(w, (pn - c) & 127, 1), mask=lane8 == pn)
        for c, (tn, pn) in enumerate(nat):
            for u in us:
                o_store(u, og[tn, pl.ds(8 * u, 8), :], pl.ds(pl.multiple_of(tn * 128, 128), 128))
        if q in late:
            out_tiles(1, *late[q], lambda cp: cp.start())

    if u2 == NU:
        out_tiles(0, 0, D, lambda cp: cp.start())
    prev = None
    for q, (a, n) in enumerate(wd_rows):
        for k in waits.get(q, ()):
            cp_d[k].wait()
        if prev is not None and q in waits:
            patch(*prev)
            prev = None
        y = lax.dot_general(_bf(hpk[...]), wd[pl.ds(a, n), :], _NT, preferred_element_type=F32)
        if q == 0:
            o_gather(range(u2, NU))
        if prev is not None:
            patch(*prev)
        prev = (q, y)
        if q == 0 and u2 < NU:
            out_tiles(0, 0, D, lambda cp: cp.start())
    patch(*prev)
    pltpu.make_async_copy(obuf, out_hbm, sem_out).wait()


def _scratch():
    return [
        pltpu.VMEM((D, L), BF16),
        pltpu.VMEM((6, D, N), BF16),
        pltpu.VMEM((D,), BF16),
        pltpu.VMEM((D,), BF16),
        pltpu.VMEM((D,), BF16),
        pltpu.VMEM((D, F), BF16),
        pltpu.VMEM((D, F), BF16),
        pltpu.VMEM((D, F), BF16),
        pltpu.VMEM((4, 64, 256), U32),
        pltpu.VMEM((_NPAT, 8, 128), I32),
        pltpu.VMEM((D, 128), F32),
        pltpu.VMEM((D, 128), F32),
        pltpu.VMEM((5, 2 * D, 128), I32),
        pltpu.VMEM((5, 2 * D, 128), I32),
        pltpu.VMEM((8, 2 * D, 128), I32),
        pltpu.VMEM((8, 2 * D, 128), I32),
        pltpu.VMEM((2, 4 * D, 128), F32),
        pltpu.VMEM((8, 4, D, 128), F32),
        pltpu.VMEM((16, D // 2, 128), I32),
        pltpu.VMEM((16, D // 2, 128), I32),
        pltpu.VMEM((8, 4, D, 128), F32),
        pltpu.VMEM((8, 2, D // 8, 8, 128), I32),
        pltpu.VMEM((8, 2, 2 * D, 128), F32),
        pltpu.VMEM((16, D // 2, 128), I32),
        pltpu.VMEM((3, 8, 128), F32),
        pltpu.VMEM((8, 128), I32),
        pltpu.VMEM((8, D), I32),
        pltpu.VMEM((8, 128), F32),
        pltpu.VMEM((C, 8, 128), I32),
        pltpu.VMEM((C, 8, D), F32),
        pltpu.VMEM((8, F), F32),
        pltpu.VMEM((8, F), I32),
        pltpu.VMEM((2, D // 2, 128), I32),
        pltpu.VMEM((16, D // 2, 128), I32),
        pltpu.VMEM((16, D // 2, 128), I32),
        pltpu.VMEM((D, L), BF16),
        pltpu.SemaphoreType.DMA((6 + len(_DEV.get("waits", {0: 0, 4: 0})),)),
        pltpu.SemaphoreType.DMA,
    ] + [pltpu.VMEM((4, D // 2, 128), I32)] * 8 + [pltpu.VMEM((4, 24, 128), F32)] * 4


@jax.jit
def pallas_recurrent_scan__ssm_conv_s4__moe_arch_mod__prompt_kernel(
    A_u: jax.Array,
    A_A_re: jax.Array,
    A_A_im: jax.Array,
    A_B_re: jax.Array,
    A_B_im: jax.Array,
    A_C_re: jax.Array,
    A_C_im: jax.Array,
    A_log_dt: jax.Array,
    A_Dskip: jax.Array,
    B_x: jax.Array,
    B_w_r: jax.Array,
    B_w_gate: jax.Array,
    B_w_up: jax.Array,
    B_w_down: jax.Array,
):
    hbm = pl.BlockSpec(memory_space=pltpu.HBM)
    out = pl.pallas_call(
        _kernel,
        out_shape=jax.ShapeDtypeStruct((D, L), BF16),
        in_specs=[hbm] * 15,
        out_specs=hbm,
        scratch_shapes=_scratch(),
        compiler_params=pltpu.CompilerParams(vmem_limit_bytes=110 * 1024 * 1024),
        name="s4_mod",
    )(A_u[0].T, A_A_re, A_A_im, A_B_re, A_B_im, A_C_re, A_C_im, A_log_dt, A_Dskip, B_w_r,
      B_w_gate, B_w_up, B_w_down.T, jnp.asarray(_FPK), jnp.asarray(_PATS))
    return out.T[None]
```

```python
import numpy as np
import jax
import jax.numpy as jnp
from jax import lax
import jax.experimental.pallas as pl
import jax.experimental.pallas.tpu as pltpu

L, D, N, F, C = 2048, 576, 128, 4608, 8
NU = D // 16
CB = 64
NB = D // CB
CO = 32
NO = D // CO
UA = 4
F32, BF16, I32, U32 = jnp.float32, jnp.bfloat16, jnp.int32, jnp.uint32
EPS = 1e-5
_DEV = {}


def _bf16_round_np(x):
    u = np.asarray(x, np.float32).view(np.uint32).astype(np.uint64)
    r = ((u + 0x7FFF + ((u >> 16) & 1)) >> 16) << 16
    return r.astype(np.uint32)


_LROUND = _bf16_round_np(np.arange(L)).view(np.float32).astype(np.int64)
_HI = [(1, 3, 516, 1032), (5, 7, 520, 1288), (4, 260, 772, 1544), (8, 264, 776, 1800), (2, 6, 258, 262)]


def _lane_l1(l2):
    p = np.arange(128)
    return 32 * ((p // 32) ^ l2) + p % 32


def _comp_q():
    t = np.arange(8)[:, None]
    lane = np.arange(128)[None, :]
    return ((lane - 8 - 7 * (t % 4)) % 16) // 4


def _make_tables():
    lane = np.arange(128)
    lo = 8 * (4 * (lane // 16) + lane % 4)
    tab = [dict(), dict()]
    amask = np.zeros(128, bool)
    for q in range(5):
        for e in range(4):
            for par in range(2):
                t = 4 * par + e
                for h in range(2):
                    src = lane[(lane // 4) % 4 == 2 * h + par]
                    dst = (src + (4 * (q % 4) - 8 * h + 8) + 7 * t) % 128
                    assert np.all(_comp_q()[t, dst] == q % 4)
                    sid = e if q < 4 else 4 + e // 2
                    for sl, dl_ in zip(src, dst):
                        ent = (sid, int(dl_))
                        assert tab[par].setdefault(_HI[q][e] + int(lo[sl]), ent) == ent
                    if q == 4 and e % 2 == 1:
                        amask[dst % 16 + 16 * np.arange(8)[:, None]] = True
    pats = []
    for j in range(4):
        pats.append(np.tile(4 * (lane % 32) + ((lane // 32) ^ j), (8, 1)))
    for j in range(4):
        pats.append(np.tile(32 * ((lane % 4) ^ j) + lane // 4, (8, 1)))
    npat0 = len(pats)
    tiles, tile_of = [], {}
    for dl in range(4):
        for l2 in range(4):
            v = _LROUND[512 * dl + 4 * lane + l2]
            key = tuple(v.tolist())
            if key in tile_of:
                tile_of[dl, l2] = tile_of[key]
                continue
            sid = np.array([tab[0][x][0] if x else -1 for x in v])
            ln = np.array([[tab[s8 % 2][x][1] if x else 0 for x in v] for s8 in range(8)])
            steps = []
            for s in sorted(set(sid.tolist()), key=lambda s: -(sid == s).sum()):
                lanes = np.nonzero(sid == s)[0]
                if s < 0:
                    steps.append((-1, None, lanes))
                    continue
                care = sid == s
                kk = None
                for k in range(npat0, len(pats)):
                    oldp, oldc, olds = pats[k]
                    both = care & oldc
                    if olds == s and np.array_equal(oldp[:, both], ln[:, both]):
                        pats[k] = (np.where(care, ln, oldp), care | oldc, s)
                        kk = k
                        break
                if kk is None:
                    pats.append((np.where(care, ln, 0), care, s))
                    kk = len(pats) - 1
                steps.append((s, kk, lanes))
            tiles.append(steps)
            tile_of[key] = tile_of[dl, l2] = len(tiles) - 1
    pats = np.stack([p if k < npat0 else p[0] for k, p in enumerate(pats)]).astype(np.int32)
    tile_of = {k: v for k, v in tile_of.items() if len(k) == 2}
    rows = np.concatenate([pats[:, :2].reshape(-1, 128), amask[None].astype(np.int32)])
    rows = np.concatenate([rows, np.zeros((-len(rows) % 8, 128), np.int32)])
    return tiles, tile_of, len(pats), rows


_TILES, _TILE_OF, _NGAT, _PROWS = _make_tables()
_NPAT = _NGAT + 3


def _cmul(ar, ai, br, bi):
    return ar * br - ai * bi, ar * bi + ai * br


def _sincos(b):
    magic = jnp.float32(12582912.0)
    t = b * jnp.float32(2.0 / np.pi) + magic
    k = t - magic
    ki = pltpu.bitcast(t, I32)
    r = b - k * jnp.float32(1.5703125)
    r = r - k * jnp.float32(0.0004837512969970703)
    r = r - k * jnp.float32(7.549790126404332e-08)
    u = r * r
    ps = (jnp.float32(-0.0001958295761141926) * u + jnp.float32(0.008332725614309311)) * u \
        + jnp.float32(-0.166666641831398)
    sn = r + (r * u) * ps
    pc = ((jnp.float32(2.437065268168226e-05) * u + jnp.float32(-0.0013886778615415096)) * u
          + jnp.float32(0.04166663438081741)) * u + jnp.float32(-0.5)
    cs = pc * u + jnp.float32(1.0)
    odd = (ki & 1) == 1
    s1 = jnp.where(odd, cs, sn)
    c1 = jnp.where(odd, sn, cs)
    sign = jnp.int32(-2147483648)
    s1 = pltpu.bitcast(pltpu.bitcast(s1, I32) ^ ((ki << 30) & sign), F32)
    c1 = pltpu.bitcast(pltpu.bitcast(c1, I32) ^ (((ki + 1) << 30) & sign), F32)
    return s1, c1


def _gather(x, idx):
    return jnp.take_along_axis(x, idx, axis=1, mode="promise_in_bounds")


def _lanes_mask(lanes):
    lane = lax.broadcasted_iota(I32, (8, 128), 1)
    lanes = sorted(int(x) for x in lanes)
    runs, start, prev = [], lanes[0], lanes[0]
    for x in lanes[1:]:
        if x != prev + 1:
            runs.append((start, prev))
            start = x
        prev = x
    runs.append((start, prev))
    m = None
    for a, b in runs:
        t = (lane == a) if a == b else jnp.logical_and(lane >= a, lane <= b)
        m = t if m is None else jnp.logical_or(m, t)
    return m


def _butterfly(p):
    lane = lax.broadcasted_iota(I32, p[0].shape, 1)
    b0 = (lane & 32) != 0
    b1 = (lane & 64) != 0
    t = [jnp.where(b0, p[k ^ 1], p[k]) for k in range(4)]
    return [jnp.where(b1, t[k ^ 2], t[k]) for k in range(4)]


def _fft4(x, sgn):
    (ar, ai), (br, bi), (cr, ci), (dr, di) = x
    s0r, s0i, d0r, d0i = ar + cr, ai + ci, ar - cr, ai - ci
    s1r, s1i, d1r, d1i = br + dr, bi + di, br - dr, bi - di
    y0 = (s0r + s1r, s0i + s1i)
    y2 = (s0r - s1r, s0i - s1i)
    p = (d0r - d1i, d0i + d1r)
    m = (d0r + d1i, d0i - d1r)
    return [y0, p, y2, m] if sgn > 0 else [y0, m, y2, p]


def _silu(z):
    h = z * jnp.float32(0.5)
    return h + h * jnp.tanh(h)


def _rbf(x):
    return x.astype(BF16).astype(F32)


def _pack2(a, b):
    p = pltpu.pack_elementwise([a, b], packed_dtype=BF16)
    return p if p.dtype == I32 else pltpu.bitcast(p, I32)


def _unpack2(x):
    return [pltpu.unpack_elementwise(x, index=i, packed_dtype=BF16, unpacked_dtype=F32) for i in range(2)]


def _bf(x):
    return pltpu.bitcast(x, BF16)


_NT = (((1,), (1,)), ((), ()))


class _Idx:
    def __init__(self, i, lag, z=None):
        self.i, self.lag, self.z = i, lag, z

    def off(self, stride, const=0, align=None):
        c = const - self.lag * stride
        if isinstance(self.i, int):
            if self.z is None:
                return self.i * stride + c
            v = self.z + (self.i * stride + c)
        else:
            v = self.i * stride + c
        return pl.multiple_of(v, align) if align else v

    def idx(self):
        return self.i - self.lag


def _pipeline(stages, n, newz, weave=None, reset=None):
    ns = len(stages)

    def step(i, lo, hi):
        z = newz() if isinstance(i, int) else None
        gens = {k: stages[k](_Idx(i, k, z)) for k in range(lo, hi)}
        if reset is not None:
            reset()
        if callable(weave):
            weave(gens)
        else:
            for k in weave or ():
                if k in gens:
                    next(gens[k], None)
        for k in range(hi - 1, lo - 1, -1):
            for _ in gens[k]:
                pass

    def body(i, carry):
        step(i, 0, ns)
        return carry

    return ([lambda i=i: step(i, 0, i + 1) for i in range(ns - 1)],
            lambda: lax.fori_loop(ns - 1, n, body, 0),
            [lambda i=i: step(n + i, i + 1, ns) for i in range(ns - 1)])


def _run(fns):
    for fn in fns:
        fn()


def _kernel(x_hbm, are_hbm, aim_hbm, bre_hbm, bim_hbm, cre_hbm, cim_hbm, ldt_hbm, dsk_hbm, wr_hbm,
            wg_hbm, wu_hbm, wd_hbm, pat_hbm,
            out_hbm,
            xbuf, par, ldt, dsk, wr, wg, wu, wd, fpk, prow, pats,
            dtcol, skip, hi_re, hi_im, lo_re, lo_im, comp, khat,
            xp, xnp, uhat, yhat, ybuf, spk, topk, posv, wr16b, wsum, ohb, xsel_ref, hbuf, hpk, cols, opk, og, obuf,
            sem_in, sem_out, *perb):
    xi, xg, stat = perb[0:4], perb[4:8], perb[8:12]
    p_hbm = (are_hbm, aim_hbm, bre_hbm, bim_hbm, cre_hbm, cim_hbm)
    r1 = 16 * UA
    small = [(ldt_hbm, ldt), (pat_hbm, prow), (dsk_hbm, dsk)]
    small += [(h.at[pl.ds(0, r1)], par.at[i, pl.ds(0, r1)]) for i, h in enumerate(p_hbm)]
    small += [(h.at[pl.ds(r1, D - r1)], par.at[i, pl.ds(r1, D - r1)]) for i, h in enumerate(p_hbm)]
    small += [(wr_hbm, wr)]
    cps = [pltpu.make_async_copy(s, d, sem_in.at[0 if i < 3 else 1 if i < 9 else 2])
           for i, (s, d) in enumerate(small)]
    ns = 3
    cp_x = pltpu.make_async_copy(x_hbm, xbuf, sem_in.at[ns])
    cp_g = pltpu.make_async_copy(wg_hbm, wg, sem_in.at[ns + 1])
    cp_u = pltpu.make_async_copy(wu_hbm, wu, sem_in.at[ns + 2])
    wd_rows = [(0, 128), (128, 128), (256, 128), (384, 128), (512, 64)]
    waits = _DEV.get("waits", {0: (0, 1, 2, 3, 4)})
    wd_grp = {k: g for g, ks in enumerate(waits.values()) for k in ks}
    cp_d = [pltpu.make_async_copy(wd_hbm.at[pl.ds(a, n)], wd.at[pl.ds(a, n)], sem_in.at[ns + 3 + wd_grp[i]])
            for i, (a, n) in enumerate(wd_rows)]
    if _DEV.get("only"):
        cp_g, cp_u, cp_d = None, None, []
    for cp in cps + [cp_x, cp_g, cp_u] + cp_d:
        if cp is not None:
            cp.start()

    sub8 = lax.broadcasted_iota(I32, (8, 128), 0)
    lane8 = lax.broadcasted_iota(I32, (8, 128), 1)
    for l2 in range(4):
        for g in range(8):
            cs = []
            for e in range(2):
                p = 16 * g + 2 * sub8 + e
                t = 4 * (32 * ((p >> 5) ^ l2) + (p & 31)) + l2
                n = ((4 * lane8 + 1) * t) & 2047
                cs.append(_sincos(n.astype(F32) * jnp.float32(-2.0 * np.pi / 2048)))
            fpk[l2, pl.ds(8 * g, 8), pl.ds(0, 128)] = _pack2(cs[0][1], cs[1][1])
            fpk[l2, pl.ds(8 * g, 8), pl.ds(128, 128)] = _pack2(cs[0][0], cs[1][0])

    for cp in cps[:3]:
        cp.wait()
    for k in range(_NGAT):
        pats[k] = jnp.where((sub8 & 1) == 1, jnp.broadcast_to(prow[pl.ds(2 * k + 1, 1), :], (8, 128)),
                            jnp.broadcast_to(prow[pl.ds(2 * k, 1), :], (8, 128)))
    cq = ((lane8 - 8 - 7 * (sub8 & 3)) & 15) >> 2
    pats[_NGAT] = cq & 1
    pats[_NGAT + 1] = cq >> 1
    pats[_NGAT + 2] = jnp.broadcast_to(prow[pl.ds(2 * _NGAT, 1), :], (8, 128))
    r128 = lax.broadcasted_iota(I32, (128, 128), 0)
    c128 = lax.broadcasted_iota(I32, (128, 128), 1)
    eye = jnp.where(r128 == c128, 1.0, 0.0).astype(BF16)
    dt_row = jnp.exp(ldt[...].astype(F32).reshape(1, D)).astype(BF16)
    dsk_row = dsk[...].reshape(1, D)
    for t in range(5):
        n = min(128, D - 128 * t)
        for row, dst in ((dt_row, dtcol), (dsk_row, skip)):
            b = jnp.broadcast_to(row[:, 128 * t:128 * t + n], (128, n))
            dst[pl.ds(128 * t, n), :] = lax.dot_general(eye[:n, :n], b, _NT, preferred_element_type=F32)

    zero = prow[0, 0]
    zcount = [0]

    def newz():
        zcount[0] += 1
        return zero * (64 * zcount[0]) if _DEV.get("zpeel", 1) else None

    def block(*fns):
        if not _DEV.get("blocks", 1):
            return _run(fns)

        def body(k, carry):
            _run(fns)
            return carry

        lax.fori_loop(0, zero + 1, body, 0)

    def slow_zero(i):
        t = i.off(1) * zero if not isinstance(i.i, int) or i.z is None else i.z
        for _ in range(_DEV.get("slow", 0)):
            t = t * t
        return pl.multiple_of(t * 8, 8)

    def after(x, deps):
        never = pats[0] < 0
        d = None
        for v in deps:
            v = v if v.dtype == I32 else pltpu.bitcast(v, I32)
            d = v if d is None else d ^ v
        return jnp.where(never, d if x.dtype == I32 else pltpu.bitcast(d, x.dtype), x)

    def pad_tail(y, i):
        n = _DEV.get("pad", 16)
        if not n:
            return y
        m = y.shape[0]
        base = i.off(1)
        k = m - 8 * _DEV.get("padpos", 8)
        mid = after(y[k:k + 8], [pats[j % _NPAT] * (base + j) for j in range(n)])
        return jnp.concatenate([y[:k], mid, y[k + 8:]], axis=0)

    class Sched:
        tok, g, pre = {}, 0, []

        @classmethod
        def reset(cls):
            cls.tok, cls.g, cls.pre = {}, 0, []

        @classmethod
        def gate(cls, x):
            deps = cls.tok.pop(cls.g, [])
            cls.g += 1
            if not deps or not _DEV.get("gate", 1):
                return x
            return jnp.concatenate([after(x[:8], deps), after(x[8:], deps[-1:])], axis=0)

    slot = {h: (q, e) for q, ent in enumerate(_HI) for e, h in enumerate(ent)}

    def a_prep(i):
        gate = Sched.gate
        for u in range(UA):
            rows = pl.ds(i.off(16 * UA, 16 * u, 16), 16)
            ev = pl.ds(i.off(32 * UA, 32 * u), 16, stride=2)
            od = pl.ds(i.off(32 * UA, 32 * u + 1), 16, stride=2)
            dt = gate(dtcol[rows, :])
            al = dt * par[0, rows, :].astype(F32)
            be = dt * par[1, rows, :].astype(F32)
            cr, ci = _cmul(par[4, rows, :].astype(F32), par[5, rows, :].astype(F32),
                           par[2, rows, :].astype(F32), par[3, rows, :].astype(F32))
            dts = dt * jnp.float32(1.0 / 512)
            cr, ci = cr * dts, ci * dts
            k0 = jnp.sum(cr, axis=1, keepdims=True) * jnp.float32(512.0)
            skip[rows, :] = skip[rows, :] + k0
            yield cr
            s, c = _sincos(gate(be))
            yield c
            pw = {1: (c, s)}
            e = 1
            while e < 256:
                if e in (1, 16):
                    c = gate(c)
                c, s = (c - s) * (c + s), (c + c) * s
                e *= 2
                pw[e] = (c, s)
                if e in (16, 256):
                    yield c
            z = {}
            for e in (1, 8, 256):
                mag = jnp.exp(al * jnp.float32(e))
                c, s = pw[e]
                z[e] = (mag * c, mag * s)
            pend = {}

            def put(tab, q, ee, v):
                key = (tab[0] is hi_re, q, ee // 2)
                if key not in pend:
                    pend[key] = (ee % 2, v)
                    return
                w, o = pend.pop(key)
                lo_, hi_ = (o, v) if w == 0 else (v, o)
                dst = od if ee // 2 else ev
                tab[0][q, dst, :] = _pack2(lo_[0], hi_[0])
                tab[1][q, dst, :] = _pack2(lo_[1], hi_[1])

            h = (cr, ci)
            cnt = 0
            for e in range(1, 9):
                g, ee, m = h, e, z[1]
                while ee in slot:
                    if cnt % 4 == 0:
                        g = (gate(g[0]), g[1])
                    g = _cmul(*g, *m)
                    put((hi_re, hi_im), *slot[ee], g)
                    if ee == e:
                        h = g
                    ee, m = ee + 256, z[256]
                    cnt += 1
                    if cnt % 4 == 0:
                        yield g[0]
            w1 = (gate(z[8][0]), -z[8][1])
            v = [(jnp.ones((16, 128), F32), jnp.zeros((16, 128), F32)), w1]
            v.append(_cmul(*w1, *w1))
            v.append(_cmul(*v[2], *w1))
            w4 = _cmul(*v[2], *v[2])
            for j in range(8):
                for f in range(4):
                    put((lo_re, lo_im), j, f, v[f])
                yield v[3][0]
                if j < 7:
                    w4 = (gate(w4[0]), w4[1])
                    v = [w4 if (j == 0 and f == 0) else _cmul(*v[f], *w4) for f in range(4)]

    def a_gen(i):
        b0 = pats[_NPAT - 3] != 0
        b1 = pats[_NPAT - 2] != 0
        g0, gs = _DEV.get("g0", 13), _DEV.get("gs", None)
        rate = _DEV.get("rate", 0.9)
        for k in range(4 * UA):
            rows = pl.ds(i.off(32 * UA, 8 * k, 8), 8)
            lo = jnp.concatenate([lo_re[:, rows, :].reshape(64, 128), lo_im[:, rows, :].reshape(64, 128)], axis=1)
            h0 = hi_re[0, rows, :]
            if k % 2 == 0 and Sched.pre and _DEV.get("gate", 1):
                h0 = after(h0, Sched.pre)
                Sched.pre = []
            hi = jnp.concatenate([jnp.concatenate([h0, hi_re[1:5, rows, :].reshape(32, 128)], axis=0),
                                  hi_im[:, rows, :].reshape(40, 128)], axis=1)
            o = lax.dot_general(_bf(hi), _bf(lo), _NT, preferred_element_type=F32)
            for q in range(5):
                Sched.tok.setdefault(g0 + int(rate * (5 * (k // 2) + q)), []).append(o[16 * q + 8:16 * q + 16])
            for h in range(2):
                g = [pltpu.roll(o[16 * q + 8 * h:16 * q + 8 * h + 8], 4 * (q % 4) - 8 * h + 8, 1,
                                stride=7, stride_axis=0) for q in range(5)]
                dst = pl.ds(i.off(64 * UA, 16 * k + 8 * h, 8), 8)
                v = jnp.where(b1, jnp.where(b0, g[3], g[2]), jnp.where(b0, g[1], g[0]))
                comp[0, dst, :] = v
                comp[1, dst, :] = g[4]
                if gs is not None:
                    Sched.tok.setdefault(g0 + gs + int(rate * (5 * (k // 2) + 4)), []).append(v)
            if k % 2 == 1:
                yield

    def a_exp(i):
        bm = pats[_NPAT - 1] != 0
        srcs = []
        for u in range(UA):
            def ld(a, e):
                return _pack2(comp[a, pl.ds(i.off(64 * UA, 64 * u + e), 8, stride=4), :],
                              comp[a, pl.ds(i.off(64 * UA, 64 * u + 32 + e), 8, stride=4), :])

            srcs.append([ld(0, e) for e in range(4)]
                        + [jnp.where(bm, ld(1, 2 * k + 1), ld(1, 2 * k)) for k in range(2)])
        cache = {}

        def gat(s, key):
            if key not in cache:
                pat = pats[key]
                cache[key] = [_gather(srcs[u][s], pat) for u in range(UA)]
            return cache[key]

        tiles = []
        for steps in _TILES:
            t = None
            for s, key, lanes in steps:
                v = [jnp.zeros((8, 128), I32)] * UA if s < 0 else gat(s, key)
                t = v if t is None else [jnp.where(_lanes_mask(lanes), v[u], t[u]) for u in range(UA)]
            tiles.append(t)
        yield
        for u0 in range(0, UA, 2):
            lhs = [_bf(jnp.concatenate([tiles[_TILE_OF[dl, l2]][u] for dl in range(4) for u in (u0, u0 + 1)], axis=0))
                   for l2 in range(4)]
            z0 = 0 if u0 == 0 else zero * 8

            def dots(ri):
                return [jnp.dot(lhs[l2], _bf(jnp.concatenate(
                    [fpk[l2, pl.ds(z0 + 16 * (j ^ l2), 16) if u0 == 0 else
                         pl.ds(pl.multiple_of(z0 + 16 * (j ^ l2), 8), 16), pl.ds(128 * ri, 128)]
                     for j in range(4)], axis=0)), preferred_element_type=F32) for l2 in range(4)]

            def store(k2, ri, v):
                khat[2 * k2 + ri, :, pl.ds(i.off(16 * UA, 16 * u0, 16), 32), :] = v.reshape(4, 32, 128)

            def toks(v, step0):
                g1 = _DEV.get("g0", 13) + int(_DEV.get("rate", 0.9) * 10 * UA) + _DEV.get("g1", 0)
                for j in range(8):
                    g = g1 + int(_DEV.get("rate2", 0.7) * (step0 + j))
                    Sched.tok.setdefault(g, []).append(v[16 * j + 8:16 * j + 16])

            re = dots(0)
            s0, d0r, s1, d1r = re[0] + re[2], re[0] - re[2], re[1] + re[3], re[1] - re[3]
            store(0, 0, s0 + s1)
            v = s0 - s1
            store(2, 0, v)
            toks(v, 8 * u0)
            im = dots(1)
            s0, d0i, s1, d1i = im[0] + im[2], im[0] - im[2], im[1] + im[3], im[1] - im[3]
            store(0, 1, s0 + s1)
            store(2, 1, s0 - s1)
            store(1, 0, d0r + d1i)
            store(1, 1, d0i - d1r)
            store(3, 0, d0r - d1i)
            v = d0i + d1r
            store(3, 1, v)
            toks(v, 8 * u0 + 8)
            yield

    def bail(cl):
        for cp in cl:
            if cp is not None:
                cp.wait()
        zr = pl.ds(pl.multiple_of(zero * 8, 8), 16)
        v = khat[zero, zero, zr, :] + skip[zr, :] + (spk[zero, zr, :] + opk[zero, zr, :] + xnp[zero, zr, :] + xp[zero, zr, :]).astype(F32) + topk[zero][:1] + comp[zero, zr, :]
        v = v + (hi_re[zero, zr, :] + hi_im[zero, zr, :] + lo_re[zero, zr, :] + lo_im[zero, zr, :]).astype(F32)
        v = v + uhat[zero, zero, zr, :] + ybuf[zero, zero, zr, :] + yhat[zero, zero, zero][:1].astype(F32)
        obuf[pl.ds(0, 16), pl.ds(0, 128)] = v.astype(BF16)
        cp = pltpu.make_async_copy(obuf.at[pl.ds(0, 16)], out_hbm.at[pl.ds(0, 16)], sem_out)
        cp.start()
        cp.wait()

    if _DEV.get("only") == "C":
        a_tail = [lambda: None] * 2
    else:
        def a_weave(gens):
            if 2 in gens and _DEV.get("expfirst", 1):
                next(gens[2])
            if 0 in gens and 1 in gens:
                for n in _DEV.get("pre", (3, 5, 4)):
                    for _ in range(n):
                        v = next(gens[0])
                    Sched.pre = [v[:8], v[8:]]
                    next(gens[1])
            for k in (1, 2):
                if k in gens:
                    for _ in gens[k]:
                        pass
            if 0 in gens:
                for _ in gens[0]:
                    pass

        a_pro, a_loop, a_tail = _pipeline([a_prep, a_gen, a_exp], NU // UA, newz, reset=Sched.reset,
                                          weave=a_weave)
        for cp in cps[3:9]:
            cp.wait()
        if _DEV.get("only") == "0":
            return bail(cps[9:] + [cp_x])
        a_pro[0]()
        for cp in cps[9:]:
            cp.wait()
        a_pro[1]()
        a_loop()
    if _DEV.get("only") == "A":
        return bail([cp_x, cp_g, cp_u] + cp_d)

    cp_x.wait()

    def zrow(u):
        return pl.ds(pl.multiple_of(zero * 8 + 8 * u, 8), 8)

    def b_gather_direct(b):
        for j in range(4):
            pat = pats[j]
            for u in range(NU):
                v = pltpu.bitcast(xbuf[pl.ds(16 * u, 16), pl.ds(512 * b + 128 * j, 128)], I32)
                xg[b][j, pl.ds(8 * u, 8), :] = _gather(v, pat)

    def b_stat(b):
        for _ in b_stat_gen(b):
            pass

    def b_stat_gen(b):
        s2 = [jnp.zeros((8, 128), F32) for _ in range(4)]
        for u in range(NU):
            o = _butterfly([xg[b][j, zrow(u), :] for j in range(4)])
            for l2 in range(4):
                xp[4 * l2 + b, pl.ds(8 * u, 8), :] = o[l2]
                e_, o_ = _unpack2(o[l2])
                s2[l2] = s2[l2] + (e_ * e_ + o_ * o_)
            yield
        for l2 in range(4):
            stat[b][l2, pl.ds(16, 8), :] = s2[l2]

    def b_dot(b):
        lhs = _bf(wr16b[...])
        for j in range(4):
            stat[b][j, pl.ds(0, 16), :] = jnp.dot(lhs, _bf(xg[b][j, pl.ds(pl.multiple_of(zero * zero * 8, 8), D // 2), :]),
                                                  preferred_element_type=F32)

    def b_fin(b):
        st = []
        wxs = _butterfly([stat[b][j, zrow(0), :] for j in range(4)])
        sxs = _butterfly([stat[b][j, zrow(1), :] for j in range(4)])
        for l2 in range(4):
            wx, sx = wxs[l2], sxs[l2]
            m = sx * jnp.float32(1.0 / D)
            q = jnp.sum(stat[b][l2, zrow(2), :], axis=0, keepdims=True) * jnp.float32(1.0 / D)
            var = _rbf(jnp.maximum(q - m * m, 0.0))
            rs = 1.0 / _rbf(jnp.sqrt(_rbf(var + jnp.float32(EPS))))
            mb = _rbf(m)
            st.append((mb, rs))
            r = _rbf((wx - mb * wsum[...]) * rs)
            r = jnp.where(r == 0.0, 0.0, r)
            bits = pltpu.bitcast(r, I32)
            mono = ((bits ^ ((bits >> 31) & jnp.int32(0x7FFFFFFF))) >> 16) + 32768
            tok = 512 * b + 4 * (32 * ((lane8 >> 5) ^ l2) + (lane8 & 31)) + l2
            key = pltpu.bitcast((mono << 11) + (2047 - tok) + jnp.int32(0x00800000), F32)
            t = 4 * b + l2
            topk[t // 8] = key if t % 8 == 0 else jnp.where(sub8 == t % 8, key, topk[t // 8])
        return st

    def b_norm(b):
        st = b_fin(b)
        for us in (range(CB // 16), range(CB // 16, NU)):
            for l2 in range(4):
                mb, rs = st[l2]
                for u in us:
                    e_, o_ = _unpack2(xp[4 * l2 + b, zrow(u), :])
                    xnp[4 * l2 + b, pl.ds(8 * u, 8), :] = _pack2((e_ - mb) * rs, (o_ - mb) * rs)

    wrow = wr[...].reshape(1, D)
    wr16b[...] = pltpu.bitcast(jnp.concatenate([jnp.broadcast_to(wrow, (8, D)), jnp.ones((8, D), BF16)], axis=0), I32)
    wsum[...] = jnp.broadcast_to(jnp.sum(wrow.astype(F32), axis=1, keepdims=True), (8, 128))
    topk[2] = jnp.zeros((8, 128), F32)
    cols[...] = jnp.zeros(cols.shape, I32)

    ctok = {"mid": [], "n": 0, "elt": []}

    def c_reset():
        ctok["mid"], ctok["n"] = [], 0

    def pin_lhs(lhs):
        n = ctok["n"]
        ctok["n"] += 1
        nv = lhs.shape[0] // 8
        if n % 2 == 1 or not _DEV.get("cpin", 0):
            return lhs
        parts = [lhs[8 * j:8 * j + 8] for j in range(nv)]
        for k, tok in enumerate(ctok["mid"]):
            t = _DEV.get("cp0", 130) + _DEV.get("cp1", 128) * k - (n // 2) * nv * 16
            if 0 <= t < nv * 16:
                parts[t // 16] = after(parts[t // 16], [tok])
        return jnp.concatenate(parts, axis=0)

    def c_fwd(i):
        h0 = i.off(CB // 2, 0, 8)
        r0 = i.off(CB, 0, 8)
        for l2 in range(4):
            lhs = _bf(pin_lhs(xnp[pl.ds(4 * l2, 4), pl.ds(h0, CB // 2), :].reshape(2 * CB, 128)))
            res = jnp.dot(lhs, _bf(fpk[l2, pl.ds(slow_zero(i), 64), :]), preferred_element_type=F32)
            for ri in range(2):
                y = res[:, 128 * ri:128 * ri + 128]
                if l2 == 3 and ri == 1 and isinstance(i.i, int) and i.i < 2:
                    y = pad_tail(y, i)
                uhat[2 * l2 + ri, :, pl.ds(r0, CB), :] = y.reshape(4, CB, 128)
            yield

    def c_mid(i):
        for k in range(CB // 8):
            rows = pl.ds(i.off(CB, 8 * k, 8), 8)
            krows = pl.ds(i.off(CB, 16 * (k // 2) + k % 2), 8, stride=2)
            uu = [_fft4([(uhat[2 * l2, b, rows, :], uhat[2 * l2 + 1, b, rows, :]) for l2 in range(4)], -1)
                  for b in range(4)]
            yy = [[None] * 4 for _ in range(4)]
            kmode = _DEV.get("kfft", 0)

            def khalf(dl, odd):
                kr = pl.ds(i.off(CB, 16 * (k // 2) + k % 2) + (zero if odd else 0), 8, stride=2)
                x = [(khat[2 * l2, dl, kr, :], khat[2 * l2 + 1, dl, kr, :]) for l2 in range(4)]
                if not odd:
                    s0 = (x[0][0] + x[2][0], x[0][1] + x[2][1])
                    s1 = (x[1][0] + x[3][0], x[1][1] + x[3][1])
                    return {0: (s0[0] + s1[0], s0[1] + s1[1]), 2: (s0[0] - s1[0], s0[1] - s1[1])}
                d0 = (x[0][0] - x[2][0], x[0][1] - x[2][1])
                d1 = (x[1][0] - x[3][0], x[1][1] - x[3][1])
                return {1: (d0[0] + d1[1], d0[1] - d1[0]), 3: (d0[0] - d1[1], d0[1] + d1[0])}

            def acc(pp, m, t):
                pp[m] = t if pp[m] is None else (pp[m][0] + t[0], pp[m][1] + t[1])

            for odd in range(2):
                pps = {k2: [None] * 4 for k2 in (odd, odd + 2)}
                if kmode == 0:
                    for k2 in pps:
                        for dl in range(3, -1, -1):
                            kk = (khat[2 * k2, dl, krows, :], khat[2 * k2 + 1, dl, krows, :])
                            for m in range(3, dl - 1, -1):
                                acc(pps[k2], m, _cmul(*uu[m - dl][k2], *kk))
                elif kmode == 1:
                    for dl in range(3, -1, -1):
                        kk = khalf(dl, odd)
                        for k2 in pps:
                            for m in range(3, dl - 1, -1):
                                acc(pps[k2], m, _cmul(*uu[m - dl][k2], *kk[k2]))
                else:
                    kk = [khalf(dl, odd) for dl in range(4)]
                    for k2 in pps:
                        for m in range(3, -1, -1):
                            for b in range(m, -1, -1):
                                acc(pps[k2], m, _cmul(*uu[b][k2], *kk[m - b][k2]))
                for k2, pp in pps.items():
                    for m in range(3, -1, -1):
                        yy[m][k2] = pp[0] if m == 0 else (pp[m][0] - pp[m - 1][1], pp[m][1] + pp[m - 1][0])
            un = i.off(CB // 8, k)
            for bp in range(2):
                ww = [_fft4(yy[m], 1) for m in (2 * bp, 2 * bp + 1)]
                for l2 in range(4):
                    for ri in range(2):
                        v = _pack2(ww[0][l2][ri], ww[1][l2][ri])
                        yhat[2 * l2 + ri, bp, un] = v
            ctok["mid"].append(v)
            yield

    def c_inv(i):
        u0 = i.off(CB // 8)
        r0 = i.off(2 * CB, 0, 8)
        for l2 in range(4):
            for ri in range(2):
                lhs = yhat[2 * l2 + ri, :, pl.ds(u0, CB // 8)].reshape(2 * CB, 128)
                lhs = _bf(pin_lhs(lhs) if ri == 0 else lhs)
                y = lax.dot_general(lhs, _bf(fpk[l2, pl.ds(slow_zero(i), 64), pl.ds(128 * ri, 128)]), _NT, preferred_element_type=F32)
                if l2 == 3 and ri == 1:
                    y = pad_tail(y, i)
                ybuf[2 * l2 + ri, :, pl.ds(r0, 2 * CB), :] = y.reshape(2, 2 * CB, 128)
            yield

    def c_elt(i):
        for k in range(CB // 16):
            hr = pl.ds(i.off(CB // 2, 8 * k, 8), 8)
            sk = [skip[pl.ds(i.off(CB, 16 * k + e), 8, stride=2), :] for e in range(2)]
            for b in range(4):
                o = []
                for l2 in range(4):
                    w = xnp[4 * l2 + b, hr, :]
                    if ctok["elt"]:
                        w = after(w, ctok["elt"])
                    xn = _unpack2(w)
                    xx = _unpack2(xp[4 * l2 + b, hr, :])
                    ss, v = [], []
                    for e in range(2):
                        yr = pl.ds(i.off(2 * CB, 32 * k + 2 * e + b % 2), 8, stride=4)
                        ss.append(ybuf[2 * l2, b // 2, yr, :] + ybuf[2 * l2 + 1, b // 2, yr, :] + xn[e] * sk[e])
                        v.append(xx[e] + ss[e] * _silu(xn[e]))
                    spk[4 * l2 + b, hr, :] = _pack2(*ss)
                    o.append(_pack2(*v))
                p = _butterfly(o)
                for j in range(4):
                    opk[4 * b + j, hr, :] = p[j]
                yield

    def c_top(i):
        k0, k1 = topk[i.off(0, 0)], topk[i.off(0, 1)]
        mx = jnp.max(jnp.max(jnp.maximum(k0, k1), axis=0, keepdims=True), axis=1, keepdims=True)
        topk[i.off(0, 0)] = jnp.where(k0 == mx, 0.0, k0)
        topk[i.off(0, 1)] = jnp.where(k1 == mx, 0.0, k1)
        topk[i.off(0, 2)] = jnp.where(sub8 == i.idx(), mx, topk[i.off(0, 2)])
        yield

    def c_first(i):
        if _DEV.get("toplast", 1):
            yield
            yield from c_fwd(i)
            yield from c_top(i)
        else:
            yield from c_top(i)
            yield from c_fwd(i)

    c_pro, c_loop, c_tail = _pipeline([c_first, c_mid, c_inv, c_elt], NB, newz, reset=c_reset,
                                      weave=_DEV.get("cweave", [1] * (CB // 8) + [3] * (CB // 4) + [0, 0, 0, 2, 2, 0, 0, 2, 2]))
    def first_fwd():
        i = _Idx(0, 0)
        for _ in c_fwd(i):
            pass
        for _ in c_top(i):
            pass

    if _DEV.get("only") != "C":
        ops = {"G": b_gather_direct, "s": b_stat, "d": b_dot, "n": b_norm,
               "a": lambda k: a_tail[k](), "f": lambda k: first_fwd()}
        for blk in _DEV.get("bplan", "a0G0G1 a1G2G3d0d1s0s1 s2s3n0n1d2d3 n2n3f0").split():
            block(*[lambda k=k: ops[blk[k]](int(blk[k + 1])) for k in range(0, len(blk), 2)])
    if _DEV.get("only") == "B":
        return bail([cp_g, cp_u] + cp_d)
    for fn in c_pro[1:]:
        block(fn)
    c_loop()
    if _DEV.get("only") in ("C", "ABC"):
        return bail([cp_g, cp_u] + cp_d)

    sel = pltpu.bitcast(topk[2], I32) - jnp.int32(0x00800000)
    mono = (sel >> 11) - 32768
    r_sel = pltpu.bitcast((mono ^ ((mono >> 31) & jnp.int32(0x7FFF))) << 16, F32)
    gate_r = _rbf(jax.nn.sigmoid(r_sel))
    posv[...] = 2047 - (sel & 2047)
    tok = [posv[c, 0] for c in range(C)]
    nat = [(t >> 7, t & 127) for t in tok]
    prm = []
    for t in tok:
        l2, l1 = t & 3, (t >> 2) & 127
        prm.append((4 * l2 + (t >> 9), 32 * ((l1 >> 5) ^ l2) + (l1 & 31)))

    def extract(src, k):
        for c, (tp, pp) in enumerate(prm):
            sh = (c - pp) & 127
            for u in range(NU):
                pltpu.store(cols.at[k, pl.ds(8 * u, 8), :], pltpu.roll(src[tp, pl.ds(8 * u, 8), :], sh, 1),
                            mask=lane8 == c)

    for c, (tp, pp) in enumerate(prm):
        ohb[c] = jnp.where(jnp.logical_and(sub8 == c // 2, lane8 == pp), jnp.int32(0x3F80 << (16 * (c % 2))), 0)

    def take_rows():
        for c, (tp, pp) in enumerate(prm):
            xsel_ref[c] = lax.dot_general(_bf(ohb[c]), _bf(xnp[tp]), _NT, preferred_element_type=F32)[:8]

    def stages(*items):
        def run():
            z = newz()
            for fn, k in items:
                for _ in fn(_Idx(k, 0, z)):
                    pass
        return run

    e1, e2 = _DEV.get("e1", ()), _DEV.get("e2", (NB - 3,))
    block(stages((c_mid, NB - 1), *[(c_elt, k) for k in e1], (c_inv, NB - 2)))
    block(stages(*[(c_elt, k) for k in e2], (c_inv, NB - 1)), take_rows, lambda: extract(xp, 0))

    def o_gather(us):
        for j in range(4):
            pat = pats[4 + j]
            for b in range(4):
                for u in us:
                    v = _gather(opk[4 * b + j, pl.ds(8 * u, 8), :], pat)
                    og[4 * b + j, pl.ds(8 * u, 8), :] = v
                    o_store(u, v, pl.ds(512 * b + 128 * j, 128))

    def o_store(u, v, col):
        obuf[pl.ds(16 * u, 8), col] = _bf(v[0:4])
        obuf[pl.ds(16 * u + 8, 8), col] = _bf(pltpu.roll(v, 4, 0)[0:4])

    bits = jnp.int32(0)
    for c in range(C):
        bits = bits | (jnp.int32(1) << nat[c][0])

    def out_tiles(routed, a, n, op):
        for t in range(16):
            @pl.when(((bits >> t) & 1) == routed)
            def _():
                col = pl.ds(128 * t, 128)
                op(pltpu.make_async_copy(obuf.at[pl.ds(a, n), col], out_hbm.at[pl.ds(a, n), col], sem_out))

    late = _DEV.get("late", {2: (0, 384), 4: (384, 192)})

    u1, u2 = _DEV.get("u1", 28), NU

    def project(w, post, fill, frate):
        pend = []
        nt = F // 128
        lag = _DEV.get("flag", 0)
        done = 0
        for t in range(nt + lag):
            if t < nt:
                pend.append([jnp.dot(xsel_b[:, a:a + n], w[pl.ds(a, n), pl.ds(128 * t, 128)],
                                     preferred_element_type=F32)[:8] for a, n in wd_rows])
            if t >= lag:
                ps = pend.pop(0)
                v = _rbf((ps[0] + ps[1]) + (ps[2] + ps[3]) + ps[4])
                ctok["elt"] = [v]
                post(t - lag, v)
            while fill and done * nt < (t + 1) * len(fill) * frate and done < len(fill):
                fill[done]()
                done += 1
        for fn in fill[done:]:
            fn()
        ctok["elt"] = []

    def elt_pieces(ks):
        out = []
        for k in ks:
            g = c_elt(_Idx(k, 0))
            out += [lambda g=g: next(g, None)] * (CB // 4)
        return out

    def post_gate(t, ga):
        hbuf[:, pl.ds(128 * t, 128)] = _rbf(ga * _rbf(jax.nn.sigmoid(ga)))

    def post_up(t, up):
        h = hbuf[:, pl.ds(128 * t, 128)] * up
        hpk[:, pl.ds(128 * t, 128)] = pltpu.bitcast(
            jnp.concatenate([h, jnp.zeros((8, 128), F32)], axis=0).astype(BF16), I32)

    cp_g.wait()
    xsel = xsel_ref[0]
    for c in range(1, C):
        xsel = xsel + xsel_ref[c]
    xsel_b = jnp.concatenate([xsel, jnp.zeros((8, D), F32)], axis=0).astype(BF16)
    ks = [k for k in range(NB - 3, NB) if k not in e1 and k not in e2]
    ng = _DEV.get("ng", 2)
    project(wg, post_gate, elt_pieces(ks[:ng]), _DEV.get("fr1", 1.0))
    o_gather(range(u1))
    cp_u.wait()
    project(wu, post_up, elt_pieces(ks[ng:]), _DEV.get("fr2", 2.5))
    o_gather(range(u1, 32))
    o_gather(range(32, u2))
    extract(spk, 1)
    pr = (r128 & (-16)) + 2 * (r128 & 7) + ((r128 >> 3) & 1)
    perm = jnp.where(pr == c128, 1.0, 0.0).astype(BF16)

    def patch(q, y):
        a, n = wd_rows[q]
        z = _rbf(xsel[:8, a:a + n] + _rbf(_rbf(y[:8]) * gate_r[:, :1]))
        g = z * _rbf(jax.nn.sigmoid(z))
        g = jnp.concatenate([g, jnp.zeros((120, n), F32)], axis=0).astype(BF16)
        gt = lax.dot_general(perm[:n, :n], g, _NT, preferred_element_type=F32)
        us = range(a // 16, (a + n) // 16)
        zz = newz()
        for u in us:
            hr = pl.ds(pl.multiple_of(zz + 8 * u, 8), 8)
            xx, ss = _unpack2(cols[0, hr, :]), _unpack2(cols[1, hr, :])
            r0 = 16 * u - a
            w = _pack2(*[xx[e] + _rbf(ss[e] * gt[r0 + 8 * e:r0 + 8 * e + 8]) for e in range(2)])
            for c, (tn, pn) in enumerate(nat):
                tt = 4 * (tn >> 2) + (tn & 3)
                pltpu.store(og.at[tt, pl.ds(8 * u, 8), :], pltpu.roll(w, (pn - c) & 127, 1), mask=lane8 == pn)
        for c, (tn, pn) in enumerate(nat):
            for u in us:
                o_store(u, og[tn, pl.ds(8 * u, 8), :], pl.ds(pl.multiple_of(tn * 128, 128), 128))
        if q in late:
            out_tiles(1, *late[q], lambda cp: cp.start())

    if u2 == NU:
        out_tiles(0, 0, D, lambda cp: cp.start())
    prev = None
    for q, (a, n) in enumerate(wd_rows):
        for k in waits.get(q, ()):
            cp_d[k].wait()
        if prev is not None and q in waits:
            patch(*prev)
            prev = None
        y = lax.dot_general(_bf(hpk[...]), wd[pl.ds(a, n), :], _NT, preferred_element_type=F32)
        if q == 0:
            o_gather(range(u2, NU))
        if prev is not None:
            patch(*prev)
        prev = (q, y)
        if q == 0 and u2 < NU:
            out_tiles(0, 0, D, lambda cp: cp.start())
    patch(*prev)
    pltpu.make_async_copy(obuf, out_hbm, sem_out).wait()


def _scratch():
    return [
        pltpu.VMEM((D, L), BF16),
        pltpu.VMEM((6, D, N), BF16),
        pltpu.VMEM((D,), BF16),
        pltpu.VMEM((D,), BF16),
        pltpu.VMEM((D,), BF16),
        pltpu.VMEM((D, F), BF16),
        pltpu.VMEM((D, F), BF16),
        pltpu.VMEM((D, F), BF16),
        pltpu.VMEM((4, 64, 256), I32),
        pltpu.VMEM(_PROWS.shape, I32),
        pltpu.VMEM((_NPAT, 8, 128), I32),
        pltpu.VMEM((D, 128), F32),
        pltpu.VMEM((D, 128), F32),
        pltpu.VMEM((5, 2 * D, 128), I32),
        pltpu.VMEM((5, 2 * D, 128), I32),
        pltpu.VMEM((8, 2 * D, 128), I32),
        pltpu.VMEM((8, 2 * D, 128), I32),
        pltpu.VMEM((2, 4 * D, 128), F32),
        pltpu.VMEM((8, 4, D, 128), F32),
        pltpu.VMEM((16, D // 2, 128), I32),
        pltpu.VMEM((16, D // 2, 128), I32),
        pltpu.VMEM((8, 4, D, 128), F32),
        pltpu.VMEM((8, 2, D // 8, 8, 128), I32),
        pltpu.VMEM((8, 2, 2 * D, 128), F32),
        pltpu.VMEM((16, D // 2, 128), I32),
        pltpu.VMEM((3, 8, 128), F32),
        pltpu.VMEM((8, 128), I32),
        pltpu.VMEM((8, D), I32),
        pltpu.VMEM((8, 128), F32),
        pltpu.VMEM((C, 8, 128), I32),
        pltpu.VMEM((C, 8, D), F32),
        pltpu.VMEM((8, F), F32),
        pltpu.VMEM((8, F), I32),
        pltpu.VMEM((2, D // 2, 128), I32),
        pltpu.VMEM((16, D // 2, 128), I32),
        pltpu.VMEM((16, D // 2, 128), I32),
        pltpu.VMEM((D, L), BF16),
        pltpu.SemaphoreType.DMA((6 + len(_DEV.get("waits", {0: 0})),)),
        pltpu.SemaphoreType.DMA,
    ] + [pltpu.VMEM((4, D // 2, 128), I32)] * 8 + [pltpu.VMEM((4, 24, 128), F32)] * 4


@jax.jit
def pallas_recurrent_scan__ssm_conv_s4__moe_arch_mod__prompt_kernel(
    A_u: jax.Array,
    A_A_re: jax.Array,
    A_A_im: jax.Array,
    A_B_re: jax.Array,
    A_B_im: jax.Array,
    A_C_re: jax.Array,
    A_C_im: jax.Array,
    A_log_dt: jax.Array,
    A_Dskip: jax.Array,
    B_x: jax.Array,
    B_w_r: jax.Array,
    B_w_gate: jax.Array,
    B_w_up: jax.Array,
    B_w_down: jax.Array,
):
    hbm = pl.BlockSpec(memory_space=pltpu.HBM)
    out = pl.pallas_call(
        _kernel,
        out_shape=jax.ShapeDtypeStruct((D, L), BF16),
        in_specs=[hbm] * 14,
        out_specs=hbm,
        scratch_shapes=_scratch(),
        compiler_params=pltpu.CompilerParams(vmem_limit_bytes=110 * 1024 * 1024),
        name="s4_mod",
    )(A_u[0].T, A_A_re, A_A_im, A_B_re, A_B_im, A_C_re, A_C_im, A_log_dt, A_Dskip, B_w_r,
      B_w_gate, B_w_up, B_w_down.T, jnp.asarray(_PROWS))
    return out.T[None]
```

```python
import numpy as np
import jax
import jax.numpy as jnp
from jax import lax
import jax.experimental.pallas as pl
import jax.experimental.pallas.tpu as pltpu

L, D, N, F, C = 2048, 576, 128, 4608, 8
NU = D // 16
CB = 64
NB = D // CB
CO = 32
NO = D // CO
UA = 4
F32, BF16, I32, U32 = jnp.float32, jnp.bfloat16, jnp.int32, jnp.uint32
EPS = 1e-5
_DEV = {}


def _bf16_round_np(x):
    u = np.asarray(x, np.float32).view(np.uint32).astype(np.uint64)
    r = ((u + 0x7FFF + ((u >> 16) & 1)) >> 16) << 16
    return r.astype(np.uint32)


_LROUND = _bf16_round_np(np.arange(L)).view(np.float32).astype(np.int64)
_HI = [(1, 3, 516, 1032), (5, 7, 520, 1288), (4, 260, 772, 1544), (8, 264, 776, 1800), (2, 6, 258, 262)]


def _lane_l1(l2):
    p = np.arange(128)
    return 32 * ((p // 32) ^ l2) + p % 32


def _comp_q():
    t = np.arange(8)[:, None]
    lane = np.arange(128)[None, :]
    return ((lane - 8 - 7 * (t % 4)) % 16) // 4


def _make_tables():
    lane = np.arange(128)
    lo = 8 * (4 * (lane // 16) + lane % 4)
    tab = [dict(), dict()]
    amask = np.zeros(128, bool)
    for q in range(5):
        for e in range(4):
            for par in range(2):
                t = 4 * par + e
                for h in range(2):
                    src = lane[(lane // 4) % 4 == 2 * h + par]
                    dst = (src + (4 * (q % 4) - 8 * h + 8) + 7 * t) % 128
                    assert np.all(_comp_q()[t, dst] == q % 4)
                    sid = e if q < 4 else 4 + e // 2
                    for sl, dl_ in zip(src, dst):
                        ent = (sid, int(dl_))
                        assert tab[par].setdefault(_HI[q][e] + int(lo[sl]), ent) == ent
                    if q == 4 and e % 2 == 1:
                        amask[dst % 16 + 16 * np.arange(8)[:, None]] = True
    pats = []
    for j in range(4):
        pats.append(np.tile(4 * (lane % 32) + ((lane // 32) ^ j), (8, 1)))
    for j in range(4):
        pats.append(np.tile(32 * ((lane % 4) ^ j) + lane // 4, (8, 1)))
    npat0 = len(pats)
    tiles, tile_of = [], {}
    for dl in range(4):
        for l2 in range(4):
            v = _LROUND[512 * dl + 4 * lane + l2]
            key = tuple(v.tolist())
            if key in tile_of:
                tile_of[dl, l2] = tile_of[key]
                continue
            sid = np.array([tab[0][x][0] if x else -1 for x in v])
            ln = np.array([[tab[s8 % 2][x][1] if x else 0 for x in v] for s8 in range(8)])
            steps = []
            for s in sorted(set(sid.tolist()), key=lambda s: -(sid == s).sum()):
                lanes = np.nonzero(sid == s)[0]
                if s < 0:
                    steps.append((-1, None, lanes))
                    continue
                care = sid == s
                kk = None
                for k in range(npat0, len(pats)):
                    oldp, oldc, olds = pats[k]
                    both = care & oldc
                    if olds == s and np.array_equal(oldp[:, both], ln[:, both]):
                        pats[k] = (np.where(care, ln, oldp), care | oldc, s)
                        kk = k
                        break
                if kk is None:
                    pats.append((np.where(care, ln, 0), care, s))
                    kk = len(pats) - 1
                steps.append((s, kk, lanes))
            tiles.append(steps)
            tile_of[key] = tile_of[dl, l2] = len(tiles) - 1
    pats = np.stack([p if k < npat0 else p[0] for k, p in enumerate(pats)]).astype(np.int32)
    tile_of = {k: v for k, v in tile_of.items() if len(k) == 2}
    rows = np.concatenate([pats[:, :2].reshape(-1, 128), amask[None].astype(np.int32)])
    rows = np.concatenate([rows, np.zeros((-len(rows) % 8, 128), np.int32)])
    return tiles, tile_of, len(pats), rows


_TILES, _TILE_OF, _NGAT, _PROWS = _make_tables()
_NPAT = _NGAT + 3


def _cmul(ar, ai, br, bi):
    return ar * br - ai * bi, ar * bi + ai * br


def _sincos(b):
    magic = jnp.float32(12582912.0)
    t = b * jnp.float32(2.0 / np.pi) + magic
    k = t - magic
    ki = pltpu.bitcast(t, I32)
    r = b - k * jnp.float32(1.5703125)
    r = r - k * jnp.float32(0.0004837512969970703)
    r = r - k * jnp.float32(7.549790126404332e-08)
    u = r * r
    ps = (jnp.float32(-0.0001958295761141926) * u + jnp.float32(0.008332725614309311)) * u \
        + jnp.float32(-0.166666641831398)
    sn = r + (r * u) * ps
    pc = ((jnp.float32(2.437065268168226e-05) * u + jnp.float32(-0.0013886778615415096)) * u
          + jnp.float32(0.04166663438081741)) * u + jnp.float32(-0.5)
    cs = pc * u + jnp.float32(1.0)
    odd = (ki & 1) == 1
    s1 = jnp.where(odd, cs, sn)
    c1 = jnp.where(odd, sn, cs)
    sign = jnp.int32(-2147483648)
    s1 = pltpu.bitcast(pltpu.bitcast(s1, I32) ^ ((ki << 30) & sign), F32)
    c1 = pltpu.bitcast(pltpu.bitcast(c1, I32) ^ (((ki + 1) << 30) & sign), F32)
    return s1, c1


def _gather(x, idx):
    return jnp.take_along_axis(x, idx, axis=1, mode="promise_in_bounds")


def _lanes_mask(lanes):
    lane = lax.broadcasted_iota(I32, (8, 128), 1)
    lanes = sorted(int(x) for x in lanes)
    runs, start, prev = [], lanes[0], lanes[0]
    for x in lanes[1:]:
        if x != prev + 1:
            runs.append((start, prev))
            start = x
        prev = x
    runs.append((start, prev))
    m = None
    for a, b in runs:
        t = (lane == a) if a == b else jnp.logical_and(lane >= a, lane <= b)
        m = t if m is None else jnp.logical_or(m, t)
    return m


def _butterfly(p):
    lane = lax.broadcasted_iota(I32, p[0].shape, 1)
    b0 = (lane & 32) != 0
    b1 = (lane & 64) != 0
    t = [jnp.where(b0, p[k ^ 1], p[k]) for k in range(4)]
    return [jnp.where(b1, t[k ^ 2], t[k]) for k in range(4)]


def _fft4(x, sgn):
    (ar, ai), (br, bi), (cr, ci), (dr, di) = x
    s0r, s0i, d0r, d0i = ar + cr, ai + ci, ar - cr, ai - ci
    s1r, s1i, d1r, d1i = br + dr, bi + di, br - dr, bi - di
    y0 = (s0r + s1r, s0i + s1i)
    y2 = (s0r - s1r, s0i - s1i)
    p = (d0r - d1i, d0i + d1r)
    m = (d0r + d1i, d0i - d1r)
    return [y0, p, y2, m] if sgn > 0 else [y0, m, y2, p]


def _silu(z):
    h = z * jnp.float32(0.5)
    return h + h * jnp.tanh(h)


def _rbf(x):
    return x.astype(BF16).astype(F32)


def _pack2(a, b):
    p = pltpu.pack_elementwise([a, b], packed_dtype=BF16)
    return p if p.dtype == I32 else pltpu.bitcast(p, I32)


def _unpack2(x):
    return [pltpu.unpack_elementwise(x, index=i, packed_dtype=BF16, unpacked_dtype=F32) for i in range(2)]


def _bf(x):
    return pltpu.bitcast(x, BF16)


_NT = (((1,), (1,)), ((), ()))


class _Idx:
    def __init__(self, i, lag, z=None):
        self.i, self.lag, self.z = i, lag, z

    def off(self, stride, const=0, align=None):
        c = const - self.lag * stride
        if isinstance(self.i, int):
            if self.z is None:
                return self.i * stride + c
            v = self.z + (self.i * stride + c)
        else:
            v = self.i * stride + c
        return pl.multiple_of(v, align) if align else v

    def idx(self):
        return self.i - self.lag


def _pipeline(stages, n, newz, weave=None, reset=None):
    ns = len(stages)

    def step(i, lo, hi):
        z = newz() if isinstance(i, int) else None
        gens = {k: stages[k](_Idx(i, k, z)) for k in range(lo, hi)}
        if reset is not None:
            reset()
        if callable(weave):
            weave(gens)
        else:
            for k in weave or ():
                if k in gens:
                    next(gens[k], None)
        for k in range(hi - 1, lo - 1, -1):
            for _ in gens[k]:
                pass

    def body(i, carry):
        step(i, 0, ns)
        return carry

    return ([lambda i=i: step(i, 0, i + 1) for i in range(ns - 1)],
            lambda: lax.fori_loop(ns - 1, n, body, 0),
            [lambda i=i: step(n + i, i + 1, ns) for i in range(ns - 1)])


def _run(fns):
    for fn in fns:
        fn()


def _kernel(x_hbm, are_hbm, aim_hbm, bre_hbm, bim_hbm, cre_hbm, cim_hbm, ldt_hbm, dsk_hbm, wr_hbm,
            wg_hbm, wu_hbm, wd_hbm, pat_hbm,
            out_hbm,
            xbuf, par, ldt, dsk, wr, wg, wu, wd, fpk, prow, pats,
            dtcol, skip, hi_re, hi_im, lo_re, lo_im, comp, khat,
            xp, xnp, uhat, yhat, ybuf, spk, topk, posv, wr16b, wsum, ohb, xsel_ref, hbuf, hpk, cols, opk, og, obuf,
            sem_in, sem_out, sem_bar, *perb):
    xi, xg, stat = perb[0:4], perb[4:8], perb[8:12]
    p_hbm = (are_hbm, aim_hbm, bre_hbm, bim_hbm, cre_hbm, cim_hbm)
    r1 = 16 * UA
    small = [(ldt_hbm, ldt), (pat_hbm, prow), (dsk_hbm, dsk)]
    small += [(h.at[pl.ds(0, r1)], par.at[i, pl.ds(0, r1)]) for i, h in enumerate(p_hbm)]
    small += [(h.at[pl.ds(r1, D - r1)], par.at[i, pl.ds(r1, D - r1)]) for i, h in enumerate(p_hbm)]
    small += [(wr_hbm, wr)]
    cps = [pltpu.make_async_copy(s, d, sem_in.at[0 if i < 3 else 1 if i < 9 else 2])
           for i, (s, d) in enumerate(small)]
    ns = 3
    cp_x = pltpu.make_async_copy(x_hbm, xbuf, sem_in.at[ns])
    cp_g = pltpu.make_async_copy(wg_hbm, wg, sem_in.at[ns + 1])
    cp_u = pltpu.make_async_copy(wu_hbm, wu, sem_in.at[ns + 2])
    wd_rows = [(0, 128), (128, 128), (256, 128), (384, 128), (512, 64)]
    waits = _DEV.get("waits", {0: (0, 1, 2), 3: (3, 4)})
    wd_grp = {k: g for g, ks in enumerate(waits.values()) for k in ks}
    cp_d = [pltpu.make_async_copy(wd_hbm.at[pl.ds(a, n)], wd.at[pl.ds(a, n)], sem_in.at[ns + 3 + wd_grp[i]])
            for i, (a, n) in enumerate(wd_rows)]
    cp_bar = pltpu.make_async_copy(pat_hbm.at[pl.ds(0, 8)], posv, sem_bar) if _DEV.get("bar", 1) else None
    if _DEV.get("only"):
        cp_g, cp_u, cp_d, cp_bar = None, None, [], None
    for cp in cps + [cp_x, cp_g, cp_u] + cp_d:
        if cp is not None:
            cp.start()

    sub8 = lax.broadcasted_iota(I32, (8, 128), 0)
    lane8 = lax.broadcasted_iota(I32, (8, 128), 1)
    for l2 in range(4):
        for g in range(8):
            cs = []
            for e in range(2):
                p = 16 * g + 2 * sub8 + e
                t = 4 * (32 * ((p >> 5) ^ l2) + (p & 31)) + l2
                n = ((4 * lane8 + 1) * t) & 2047
                cs.append(_sincos(n.astype(F32) * jnp.float32(-2.0 * np.pi / 2048)))
            fpk[l2, pl.ds(8 * g, 8), pl.ds(0, 128)] = _pack2(cs[0][1], cs[1][1])
            fpk[l2, pl.ds(8 * g, 8), pl.ds(128, 128)] = _pack2(cs[0][0], cs[1][0])

    for cp in cps[:3]:
        cp.wait()
    for k in range(_NGAT):
        pats[k] = jnp.where((sub8 & 1) == 1, jnp.broadcast_to(prow[pl.ds(2 * k + 1, 1), :], (8, 128)),
                            jnp.broadcast_to(prow[pl.ds(2 * k, 1), :], (8, 128)))
    cq = ((lane8 - 8 - 7 * (sub8 & 3)) & 15) >> 2
    pats[_NGAT] = cq & 1
    pats[_NGAT + 1] = cq >> 1
    pats[_NGAT + 2] = jnp.broadcast_to(prow[pl.ds(2 * _NGAT, 1), :], (8, 128))
    r128 = lax.broadcasted_iota(I32, (128, 128), 0)
    c128 = lax.broadcasted_iota(I32, (128, 128), 1)
    eye = jnp.where(r128 == c128, 1.0, 0.0).astype(BF16)
    dt_row = jnp.exp(ldt[...].astype(F32).reshape(1, D)).astype(BF16)
    dsk_row = dsk[...].reshape(1, D)
    for t in range(5):
        n = min(128, D - 128 * t)
        for row, dst in ((dt_row, dtcol), (dsk_row, skip)):
            b = jnp.broadcast_to(row[:, 128 * t:128 * t + n], (128, n))
            dst[pl.ds(128 * t, n), :] = lax.dot_general(eye[:n, :n], b, _NT, preferred_element_type=F32)

    zero = prow[0, 0]
    zcount = [0]

    def newz():
        zcount[0] += 1
        return zero * (64 * zcount[0]) if _DEV.get("zpeel", 1) else None

    def block(*fns):
        if not _DEV.get("blocks", 1):
            return _run(fns)

        def body(k, carry):
            _run(fns)
            return carry

        lax.fori_loop(0, zero + 1, body, 0)

    def slow_zero(i):
        t = i.off(1) * zero if not isinstance(i.i, int) or i.z is None else i.z
        for _ in range(_DEV.get("slow", 0)):
            t = t * t
        return pl.multiple_of(t * 8, 8)

    def after(x, deps):
        never = pats[0] < 0
        d = None
        for v in deps:
            v = v if v.dtype == I32 else pltpu.bitcast(v, I32)
            d = v if d is None else d ^ v
        return jnp.where(never, d if x.dtype == I32 else pltpu.bitcast(d, x.dtype), x)

    def pad_tail(y, i):
        n = _DEV.get("pad", 16)
        if not n:
            return y
        m = y.shape[0]
        base = i.off(1)
        k = m - 8 * _DEV.get("padpos", 8)
        mid = after(y[k:k + 8], [pats[j % _NPAT] * (base + j) for j in range(n)])
        return jnp.concatenate([y[:k], mid, y[k + 8:]], axis=0)

    class Sched:
        tok, g, pre = {}, 0, []

        @classmethod
        def reset(cls):
            cls.tok, cls.g, cls.pre = {}, 0, []

        @classmethod
        def gate(cls, x):
            deps = cls.tok.pop(cls.g, [])
            cls.g += 1
            if not deps or not _DEV.get("gate", 1):
                return x
            return jnp.concatenate([after(x[:8], deps), after(x[8:], deps[-1:])], axis=0)

    slot = {h: (q, e) for q, ent in enumerate(_HI) for e, h in enumerate(ent)}

    def a_prep(i):
        gate = Sched.gate
        for u in range(UA):
            rows = pl.ds(i.off(16 * UA, 16 * u, 16), 16)
            ev = pl.ds(i.off(32 * UA, 32 * u), 16, stride=2)
            od = pl.ds(i.off(32 * UA, 32 * u + 1), 16, stride=2)
            dt = gate(dtcol[rows, :])
            al = dt * par[0, rows, :].astype(F32)
            be = dt * par[1, rows, :].astype(F32)
            cr, ci = _cmul(par[4, rows, :].astype(F32), par[5, rows, :].astype(F32),
                           par[2, rows, :].astype(F32), par[3, rows, :].astype(F32))
            dts = dt * jnp.float32(1.0 / 512)
            cr, ci = cr * dts, ci * dts
            k0 = jnp.sum(cr, axis=1, keepdims=True) * jnp.float32(512.0)
            skip[rows, :] = skip[rows, :] + k0
            yield cr
            s, c = _sincos(gate(be))
            yield c
            pw = {1: (c, s)}
            e = 1
            while e < 256:
                if e in (1, 16):
                    c = gate(c)
                c, s = (c - s) * (c + s), (c + c) * s
                e *= 2
                pw[e] = (c, s)
                if e in (16, 256):
                    yield c
            z = {}
            for e in (1, 8, 256):
                mag = jnp.exp(al * jnp.float32(e))
                c, s = pw[e]
                z[e] = (mag * c, mag * s)
            pend = {}

            def put(tab, q, ee, v):
                key = (tab[0] is hi_re, q, ee // 2)
                if key not in pend:
                    pend[key] = (ee % 2, v)
                    return
                w, o = pend.pop(key)
                lo_, hi_ = (o, v) if w == 0 else (v, o)
                dst = od if ee // 2 else ev
                tab[0][q, dst, :] = _pack2(lo_[0], hi_[0])
                tab[1][q, dst, :] = _pack2(lo_[1], hi_[1])

            h = (cr, ci)
            cnt = 0
            for e in range(1, 9):
                g, ee, m = h, e, z[1]
                while ee in slot:
                    if cnt % 4 == 0:
                        g = (gate(g[0]), g[1])
                    g = _cmul(*g, *m)
                    put((hi_re, hi_im), *slot[ee], g)
                    if ee == e:
                        h = g
                    ee, m = ee + 256, z[256]
                    cnt += 1
                    if cnt % 4 == 0:
                        yield g[0]
            w1 = (gate(z[8][0]), -z[8][1])
            v = [(jnp.ones((16, 128), F32), jnp.zeros((16, 128), F32)), w1]
            v.append(_cmul(*w1, *w1))
            v.append(_cmul(*v[2], *w1))
            w4 = _cmul(*v[2], *v[2])
            for j in range(8):
                for f in range(4):
                    put((lo_re, lo_im), j, f, v[f])
                yield v[3][0]
                if j < 7:
                    w4 = (gate(w4[0]), w4[1])
                    v = [w4 if (j == 0 and f == 0) else _cmul(*v[f], *w4) for f in range(4)]

    def a_gen(i):
        b0 = pats[_NPAT - 3] != 0
        b1 = pats[_NPAT - 2] != 0
        g0, gs = _DEV.get("g0", 13), _DEV.get("gs", None)
        rate = _DEV.get("rate", 0.9)
        for k in range(4 * UA):
            rows = pl.ds(i.off(32 * UA, 8 * k, 8), 8)
            lo = jnp.concatenate([lo_re[:, rows, :].reshape(64, 128), lo_im[:, rows, :].reshape(64, 128)], axis=1)
            h0 = hi_re[0, rows, :]
            if k % 2 == 0 and Sched.pre and _DEV.get("gate", 1):
                h0 = after(h0, Sched.pre)
                Sched.pre = []
            hi = jnp.concatenate([jnp.concatenate([h0, hi_re[1:5, rows, :].reshape(32, 128)], axis=0),
                                  hi_im[:, rows, :].reshape(40, 128)], axis=1)
            o = lax.dot_general(_bf(hi), _bf(lo), _NT, preferred_element_type=F32)
            for q in range(5):
                Sched.tok.setdefault(g0 + int(rate * (5 * (k // 2) + q)), []).append(o[16 * q + 8:16 * q + 16])
            for h in range(2):
                g = [pltpu.roll(o[16 * q + 8 * h:16 * q + 8 * h + 8], 4 * (q % 4) - 8 * h + 8, 1,
                                stride=7, stride_axis=0) for q in range(5)]
                dst = pl.ds(i.off(64 * UA, 16 * k + 8 * h, 8), 8)
                v = jnp.where(b1, jnp.where(b0, g[3], g[2]), jnp.where(b0, g[1], g[0]))
                comp[0, dst, :] = v
                comp[1, dst, :] = g[4]
                if gs is not None:
                    Sched.tok.setdefault(g0 + gs + int(rate * (5 * (k // 2) + 4)), []).append(v)
            if k % 2 == 1:
                yield

    def a_exp(i):
        bm = pats[_NPAT - 1] != 0
        srcs = []
        for u in range(UA):
            def ld(a, e):
                return _pack2(comp[a, pl.ds(i.off(64 * UA, 64 * u + e), 8, stride=4), :],
                              comp[a, pl.ds(i.off(64 * UA, 64 * u + 32 + e), 8, stride=4), :])

            srcs.append([ld(0, e) for e in range(4)]
                        + [jnp.where(bm, ld(1, 2 * k + 1), ld(1, 2 * k)) for k in range(2)])
        cache = {}

        def gat(s, key):
            if key not in cache:
                pat = pats[key]
                cache[key] = [_gather(srcs[u][s], pat) for u in range(UA)]
            return cache[key]

        tiles = []
        for steps in _TILES:
            t = None
            for s, key, lanes in steps:
                v = [jnp.zeros((8, 128), I32)] * UA if s < 0 else gat(s, key)
                t = v if t is None else [jnp.where(_lanes_mask(lanes), v[u], t[u]) for u in range(UA)]
            tiles.append(t)
        yield
        for u0 in range(0, UA, 2):
            lhs = [_bf(jnp.concatenate([tiles[_TILE_OF[dl, l2]][u] for dl in range(4) for u in (u0, u0 + 1)], axis=0))
                   for l2 in range(4)]
            z0 = 0 if u0 == 0 else zero * 8

            def dots(ri):
                return [jnp.dot(lhs[l2], _bf(jnp.concatenate(
                    [fpk[l2, pl.ds(z0 + 16 * (j ^ l2), 16) if u0 == 0 else
                         pl.ds(pl.multiple_of(z0 + 16 * (j ^ l2), 8), 16), pl.ds(128 * ri, 128)]
                     for j in range(4)], axis=0)), preferred_element_type=F32) for l2 in range(4)]

            def store(k2, ri, v):
                khat[2 * k2 + ri, :, pl.ds(i.off(16 * UA, 16 * u0, 16), 32), :] = v.reshape(4, 32, 128)

            def toks(v, step0):
                g1 = _DEV.get("g0", 13) + int(_DEV.get("rate", 0.9) * 10 * UA) + _DEV.get("g1", 0)
                for j in range(8):
                    g = g1 + int(_DEV.get("rate2", 0.7) * (step0 + j))
                    Sched.tok.setdefault(g, []).append(v[16 * j + 8:16 * j + 16])

            re = dots(0)
            s0, d0r, s1, d1r = re[0] + re[2], re[0] - re[2], re[1] + re[3], re[1] - re[3]
            store(0, 0, s0 + s1)
            v = s0 - s1
            store(2, 0, v)
            toks(v, 8 * u0)
            im = dots(1)
            s0, d0i, s1, d1i = im[0] + im[2], im[0] - im[2], im[1] + im[3], im[1] - im[3]
            store(0, 1, s0 + s1)
            store(2, 1, s0 - s1)
            store(1, 0, d0r + d1i)
            store(1, 1, d0i - d1r)
            store(3, 0, d0r - d1i)
            v = d0i + d1r
            store(3, 1, v)
            toks(v, 8 * u0 + 8)
            yield

    def bail(cl):
        for cp in cl:
            if cp is not None:
                cp.wait()
        zr = pl.ds(pl.multiple_of(zero * 8, 8), 16)
        v = khat[zero, zero, zr, :] + skip[zr, :] + (spk[zero, zr, :] + opk[zero, zr, :] + xnp[zero, zr, :] + xp[zero, zr, :]).astype(F32) + topk[zero][:1] + comp[zero, zr, :]
        v = v + (hi_re[zero, zr, :] + hi_im[zero, zr, :] + lo_re[zero, zr, :] + lo_im[zero, zr, :]).astype(F32)
        v = v + uhat[zero, zero, zr, :] + ybuf[zero, zero, zr, :] + yhat[zero, zero, zero][:1].astype(F32)
        obuf[pl.ds(0, 16), pl.ds(0, 128)] = v.astype(BF16)
        cp = pltpu.make_async_copy(obuf.at[pl.ds(0, 16)], out_hbm.at[pl.ds(0, 16)], sem_out)
        cp.start()
        cp.wait()

    if _DEV.get("only") == "C":
        a_tail = [lambda: None] * 2
    else:
        def a_weave(gens):
            if 2 in gens and _DEV.get("expfirst", 1):
                next(gens[2])
            if 0 in gens and 1 in gens:
                for n in _DEV.get("pre", (3, 5, 4)):
                    for _ in range(n):
                        v = next(gens[0])
                    Sched.pre = [v[:8], v[8:]]
                    next(gens[1])
            for k in (1, 2):
                if k in gens:
                    for _ in gens[k]:
                        pass
            if 0 in gens:
                for _ in gens[0]:
                    pass

        a_pro, a_loop, a_tail = _pipeline([a_prep, a_gen, a_exp], NU // UA, newz, reset=Sched.reset,
                                          weave=a_weave)
        for cp in cps[3:9]:
            cp.wait()
        if _DEV.get("only") == "0":
            return bail(cps[9:] + [cp_x])
        a_pro[0]()
        for cp in cps[9:]:
            cp.wait()
        a_pro[1]()
        a_loop()
    if _DEV.get("only") == "A":
        return bail([cp_x, cp_g, cp_u] + cp_d)

    cp_x.wait()

    def zrow(u):
        return pl.ds(pl.multiple_of(zero * 8 + 8 * u, 8), 8)

    def b_gather_direct(b):
        for j in range(4):
            pat = pats[j]
            for u in range(NU):
                v = pltpu.bitcast(xbuf[pl.ds(16 * u, 16), pl.ds(512 * b + 128 * j, 128)], I32)
                xg[b][j, pl.ds(8 * u, 8), :] = _gather(v, pat)

    def b_stat(b):
        for _ in b_stat_gen(b):
            pass

    def b_stat_gen(b):
        s2 = [jnp.zeros((8, 128), F32) for _ in range(4)]
        for u in range(NU):
            o = _butterfly([xg[b][j, zrow(u), :] for j in range(4)])
            for l2 in range(4):
                xp[4 * l2 + b, pl.ds(8 * u, 8), :] = o[l2]
                e_, o_ = _unpack2(o[l2])
                s2[l2] = s2[l2] + (e_ * e_ + o_ * o_)
            yield
        for l2 in range(4):
            stat[b][l2, pl.ds(16, 8), :] = s2[l2]

    def b_dot(b):
        lhs = _bf(wr16b[...])
        for j in range(4):
            stat[b][j, pl.ds(0, 16), :] = jnp.dot(lhs, _bf(xg[b][j, pl.ds(pl.multiple_of(zero * zero * 8, 8), D // 2), :]),
                                                  preferred_element_type=F32)

    def b_fin(b):
        st = []
        wxs = _butterfly([stat[b][j, zrow(0), :] for j in range(4)])
        sxs = _butterfly([stat[b][j, zrow(1), :] for j in range(4)])
        for l2 in range(4):
            wx, sx = wxs[l2], sxs[l2]
            m = sx * jnp.float32(1.0 / D)
            q = jnp.sum(stat[b][l2, zrow(2), :], axis=0, keepdims=True) * jnp.float32(1.0 / D)
            var = _rbf(jnp.maximum(q - m * m, 0.0))
            rs = 1.0 / _rbf(jnp.sqrt(_rbf(var + jnp.float32(EPS))))
            mb = _rbf(m)
            st.append((mb, rs))
            r = _rbf((wx - mb * wsum[...]) * rs)
            r = jnp.where(r == 0.0, 0.0, r)
            bits = pltpu.bitcast(r, I32)
            mono = ((bits ^ ((bits >> 31) & jnp.int32(0x7FFFFFFF))) >> 16) + 32768
            tok = 512 * b + 4 * (32 * ((lane8 >> 5) ^ l2) + (lane8 & 31)) + l2
            key = pltpu.bitcast((mono << 11) + (2047 - tok) + jnp.int32(0x00800000), F32)
            t = 4 * b + l2
            topk[t // 8] = key if t % 8 == 0 else jnp.where(sub8 == t % 8, key, topk[t // 8])
        return st

    def b_norm(b):
        st = b_fin(b)
        for us in (range(CB // 16), range(CB // 16, NU)):
            for l2 in range(4):
                mb, rs = st[l2]
                for u in us:
                    e_, o_ = _unpack2(xp[4 * l2 + b, zrow(u), :])
                    xnp[4 * l2 + b, pl.ds(8 * u, 8), :] = _pack2((e_ - mb) * rs, (o_ - mb) * rs)

    wrow = wr[...].reshape(1, D)
    wr16b[...] = pltpu.bitcast(jnp.concatenate([jnp.broadcast_to(wrow, (8, D)), jnp.ones((8, D), BF16)], axis=0), I32)
    wsum[...] = jnp.broadcast_to(jnp.sum(wrow.astype(F32), axis=1, keepdims=True), (8, 128))
    topk[2] = jnp.zeros((8, 128), F32)
    cols[...] = jnp.zeros(cols.shape, I32)

    ctok = {"mid": [], "n": 0, "elt": []}

    def c_reset():
        ctok["mid"], ctok["n"] = [], 0

    def pin_lhs(lhs):
        n = ctok["n"]
        ctok["n"] += 1
        nv = lhs.shape[0] // 8
        if n % 2 == 1 or not _DEV.get("cpin", 0):
            return lhs
        parts = [lhs[8 * j:8 * j + 8] for j in range(nv)]
        for k, tok in enumerate(ctok["mid"]):
            t = _DEV.get("cp0", 130) + _DEV.get("cp1", 128) * k - (n // 2) * nv * 16
            if 0 <= t < nv * 16:
                parts[t // 16] = after(parts[t // 16], [tok])
        return jnp.concatenate(parts, axis=0)

    def c_fwd(i):
        h0 = i.off(CB // 2, 0, 8)
        r0 = i.off(CB, 0, 8)
        for l2 in range(4):
            lhs = _bf(pin_lhs(xnp[pl.ds(4 * l2, 4), pl.ds(h0, CB // 2), :].reshape(2 * CB, 128)))
            res = jnp.dot(lhs, _bf(fpk[l2, pl.ds(slow_zero(i), 64), :]), preferred_element_type=F32)
            for ri in range(2):
                y = res[:, 128 * ri:128 * ri + 128]
                if l2 == 3 and ri == 1 and isinstance(i.i, int) and i.i < 2:
                    y = pad_tail(y, i)
                uhat[2 * l2 + ri, :, pl.ds(r0, CB), :] = y.reshape(4, CB, 128)
            yield

    def c_mid(i):
        for k in range(CB // 8):
            rows = pl.ds(i.off(CB, 8 * k, 8), 8)
            krows = pl.ds(i.off(CB, 16 * (k // 2) + k % 2), 8, stride=2)
            uu = [_fft4([(uhat[2 * l2, b, rows, :], uhat[2 * l2 + 1, b, rows, :]) for l2 in range(4)], -1)
                  for b in range(4)]
            yy = [[None] * 4 for _ in range(4)]
            kmode = _DEV.get("kfft", 0)

            def khalf(dl, odd):
                kr = pl.ds(i.off(CB, 16 * (k // 2) + k % 2) + (zero if odd else 0), 8, stride=2)
                x = [(khat[2 * l2, dl, kr, :], khat[2 * l2 + 1, dl, kr, :]) for l2 in range(4)]
                if not odd:
                    s0 = (x[0][0] + x[2][0], x[0][1] + x[2][1])
                    s1 = (x[1][0] + x[3][0], x[1][1] + x[3][1])
                    return {0: (s0[0] + s1[0], s0[1] + s1[1]), 2: (s0[0] - s1[0], s0[1] - s1[1])}
                d0 = (x[0][0] - x[2][0], x[0][1] - x[2][1])
                d1 = (x[1][0] - x[3][0], x[1][1] - x[3][1])
                return {1: (d0[0] + d1[1], d0[1] - d1[0]), 3: (d0[0] - d1[1], d0[1] + d1[0])}

            def acc(pp, m, t):
                pp[m] = t if pp[m] is None else (pp[m][0] + t[0], pp[m][1] + t[1])

            for odd in range(2):
                pps = {k2: [None] * 4 for k2 in (odd, odd + 2)}
                if kmode == 0:
                    for k2 in pps:
                        for dl in range(3, -1, -1):
                            kk = (khat[2 * k2, dl, krows, :], khat[2 * k2 + 1, dl, krows, :])
                            for m in range(3, dl - 1, -1):
                                acc(pps[k2], m, _cmul(*uu[m - dl][k2], *kk))
                elif kmode == 1:
                    for dl in range(3, -1, -1):
                        kk = khalf(dl, odd)
                        for k2 in pps:
                            for m in range(3, dl - 1, -1):
                                acc(pps[k2], m, _cmul(*uu[m - dl][k2], *kk[k2]))
                else:
                    kk = [khalf(dl, odd) for dl in range(4)]
                    for k2 in pps:
                        for m in range(3, -1, -1):
                            for b in range(m, -1, -1):
                                acc(pps[k2], m, _cmul(*uu[b][k2], *kk[m - b][k2]))
                for k2, pp in pps.items():
                    for m in range(3, -1, -1):
                        yy[m][k2] = pp[0] if m == 0 else (pp[m][0] - pp[m - 1][1], pp[m][1] + pp[m - 1][0])
            un = i.off(CB // 8, k)
            for bp in range(2):
                ww = [_fft4(yy[m], 1) for m in (2 * bp, 2 * bp + 1)]
                for l2 in range(4):
                    for ri in range(2):
                        v = _pack2(ww[0][l2][ri], ww[1][l2][ri])
                        yhat[2 * l2 + ri, bp, un] = v
            ctok["mid"].append(v)
            yield

    def c_inv(i):
        u0 = i.off(CB // 8)
        r0 = i.off(2 * CB, 0, 8)
        for l2 in range(4):
            for ri in range(2):
                lhs = yhat[2 * l2 + ri, :, pl.ds(u0, CB // 8)].reshape(2 * CB, 128)
                lhs = _bf(pin_lhs(lhs) if ri == 0 else lhs)
                y = lax.dot_general(lhs, _bf(fpk[l2, pl.ds(slow_zero(i), 64), pl.ds(128 * ri, 128)]), _NT, preferred_element_type=F32)
                if l2 == 3 and ri == 1:
                    y = pad_tail(y, i)
                ybuf[2 * l2 + ri, :, pl.ds(r0, 2 * CB), :] = y.reshape(2, 2 * CB, 128)
            yield

    def c_elt(i):
        for k in range(CB // 16):
            hr = pl.ds(i.off(CB // 2, 8 * k, 8), 8)
            sk = [skip[pl.ds(i.off(CB, 16 * k + e), 8, stride=2), :] for e in range(2)]
            for b in range(4):
                o = []
                for l2 in range(4):
                    w = xnp[4 * l2 + b, hr, :]
                    if ctok["elt"]:
                        w = after(w, ctok["elt"])
                    xn = _unpack2(w)
                    xx = _unpack2(xp[4 * l2 + b, hr, :])
                    ss, v = [], []
                    for e in range(2):
                        yr = pl.ds(i.off(2 * CB, 32 * k + 2 * e + b % 2), 8, stride=4)
                        ss.append(ybuf[2 * l2, b // 2, yr, :] + ybuf[2 * l2 + 1, b // 2, yr, :] + xn[e] * sk[e])
                        v.append(xx[e] + ss[e] * _silu(xn[e]))
                    spk[4 * l2 + b, hr, :] = _pack2(*ss)
                    o.append(_pack2(*v))
                p = _butterfly(o)
                for j in range(4):
                    opk[4 * b + j, hr, :] = p[j]
                yield

    def c_top(i):
        k0, k1 = topk[i.off(0, 0)], topk[i.off(0, 1)]
        mx = jnp.max(jnp.max(jnp.maximum(k0, k1), axis=0, keepdims=True), axis=1, keepdims=True)
        topk[i.off(0, 0)] = jnp.where(k0 == mx, 0.0, k0)
        topk[i.off(0, 1)] = jnp.where(k1 == mx, 0.0, k1)
        topk[i.off(0, 2)] = jnp.where(sub8 == i.idx(), mx, topk[i.off(0, 2)])
        yield

    def c_first(i):
        if _DEV.get("toplast", 1):
            yield
            yield from c_fwd(i)
            yield from c_top(i)
        else:
            yield from c_top(i)
            yield from c_fwd(i)

    c_pro, c_loop, c_tail = _pipeline([c_first, c_mid, c_inv, c_elt], NB, newz, reset=c_reset,
                                      weave=_DEV.get("cweave", [1] * (CB // 8) + [3] * (CB // 4) + [0, 0, 0, 2, 2, 0, 0, 2, 2]))
    def first_fwd():
        i = _Idx(0, 0)
        for _ in c_fwd(i):
            pass
        for _ in c_top(i):
            pass

    if _DEV.get("only") != "C":
        ops = {"G": b_gather_direct, "s": b_stat, "d": b_dot, "n": b_norm,
               "a": lambda k: a_tail[k](), "f": lambda k: first_fwd()}
        for blk in _DEV.get("bplan", "a0G0G1 a1G2G3d0d1s0s1 s2s3n0n1d2d3 n2n3f0").split():
            block(*[lambda k=k: ops[blk[k]](int(blk[k + 1])) for k in range(0, len(blk), 2)])
    if _DEV.get("only") == "B":
        return bail([cp_g, cp_u] + cp_d)
    for fn in c_pro[1:]:
        block(fn)
    c_loop()
    if _DEV.get("only") in ("C", "ABC"):
        return bail([cp_g, cp_u] + cp_d)

    sel = pltpu.bitcast(topk[2], I32) - jnp.int32(0x00800000)
    mono = (sel >> 11) - 32768
    r_sel = pltpu.bitcast((mono ^ ((mono >> 31) & jnp.int32(0x7FFF))) << 16, F32)
    gate_r = _rbf(jax.nn.sigmoid(r_sel))
    posv[...] = 2047 - (sel & 2047)
    tok = [posv[c, 0] for c in range(C)]
    nat = [(t >> 7, t & 127) for t in tok]
    prm = []
    for t in tok:
        l2, l1 = t & 3, (t >> 2) & 127
        prm.append((4 * l2 + (t >> 9), 32 * ((l1 >> 5) ^ l2) + (l1 & 31)))

    def extract(src, k):
        for c, (tp, pp) in enumerate(prm):
            sh = (c - pp) & 127
            for u in range(NU):
                pltpu.store(cols.at[k, pl.ds(8 * u, 8), :], pltpu.roll(src[tp, pl.ds(8 * u, 8), :], sh, 1),
                            mask=lane8 == c)

    for c, (tp, pp) in enumerate(prm):
        ohb[c] = jnp.where(jnp.logical_and(sub8 == c // 2, lane8 == pp), jnp.int32(0x3F80 << (16 * (c % 2))), 0)

    def take_rows():
        for c, (tp, pp) in enumerate(prm):
            xsel_ref[c] = lax.dot_general(_bf(ohb[c]), _bf(xnp[tp]), _NT, preferred_element_type=F32)[:8]

    def stages(*items):
        def run():
            z = newz()
            for fn, k in items:
                for _ in fn(_Idx(k, 0, z)):
                    pass
        return run

    e1, e2 = _DEV.get("e1", ()), _DEV.get("e2", (NB - 3,))
    block(stages((c_mid, NB - 1), *[(c_elt, k) for k in e1], (c_inv, NB - 2)))
    block(stages(*[(c_elt, k) for k in e2], (c_inv, NB - 1)), take_rows, lambda: extract(xp, 0))

    def o_gather(us):
        for j in range(4):
            pat = pats[4 + j]
            for b in range(4):
                for u in us:
                    v = _gather(opk[4 * b + j, pl.ds(8 * u, 8), :], pat)
                    og[4 * b + j, pl.ds(8 * u, 8), :] = v
                    o_store(u, v, pl.ds(512 * b + 128 * j, 128))

    def o_store(u, v, col):
        obuf[pl.ds(16 * u, 8), col] = _bf(v[0:4])
        obuf[pl.ds(16 * u + 8, 8), col] = _bf(pltpu.roll(v, 4, 0)[0:4])

    bits = jnp.int32(0)
    for c in range(C):
        bits = bits | (jnp.int32(1) << nat[c][0])

    if cp_bar is not None:
        cp_bar.start()

    def out_tiles(routed, a, n, op):
        for t in range(16):
            @pl.when(((bits >> t) & 1) == routed)
            def _():
                col = pl.ds(128 * t, 128)
                op(pltpu.make_async_copy(obuf.at[pl.ds(a, n), col], out_hbm.at[pl.ds(a, n), col], sem_out))

    late = _DEV.get("late", {1: (0, 256), 3: (256, 256), 4: (512, 64)})

    u1, u2 = _DEV.get("u1", 28), NU

    def project(w, post, fill, frate):
        pend = []
        nt = F // 128
        lag = _DEV.get("flag", 0)
        done = 0
        for t in range(nt + lag):
            if t < nt:
                pend.append([jnp.dot(xsel_b[:, a:a + n], w[pl.ds(a, n), pl.ds(128 * t, 128)],
                                     preferred_element_type=F32)[:8] for a, n in wd_rows])
            if t >= lag:
                ps = pend.pop(0)
                v = _rbf((ps[0] + ps[1]) + (ps[2] + ps[3]) + ps[4])
                ctok["elt"] = [v]
                post(t - lag, v)
            while fill and done * nt < (t + 1) * len(fill) * frate and done < len(fill):
                fill[done]()
                done += 1
        for fn in fill[done:]:
            fn()
        ctok["elt"] = []

    def elt_pieces(ks):
        out = []
        for k in ks:
            g = c_elt(_Idx(k, 0))
            out += [lambda g=g: next(g, None)] * (CB // 4)
        return out

    def post_gate(t, ga):
        hbuf[:, pl.ds(128 * t, 128)] = _rbf(ga * _rbf(jax.nn.sigmoid(ga)))

    def post_up(t, up):
        h = hbuf[:, pl.ds(128 * t, 128)] * up
        hpk[:, pl.ds(128 * t, 128)] = pltpu.bitcast(
            jnp.concatenate([h, jnp.zeros((8, 128), F32)], axis=0).astype(BF16), I32)

    cp_g.wait()
    xsel = xsel_ref[0]
    for c in range(1, C):
        xsel = xsel + xsel_ref[c]
    xsel_b = jnp.concatenate([xsel, jnp.zeros((8, D), F32)], axis=0).astype(BF16)
    ks = [k for k in range(NB - 3, NB) if k not in e1 and k not in e2]
    ng = _DEV.get("ng", 2)
    project(wg, post_gate, elt_pieces(ks[:ng]), _DEV.get("fr1", 1.0))
    o_gather(range(u1))
    cp_u.wait()
    project(wu, post_up, elt_pieces(ks[ng:]), _DEV.get("fr2", 2.5))
    o_gather(range(u1, 32))
    o_gather(range(32, u2))
    extract(spk, 1)
    pr = (r128 & (-16)) + 2 * (r128 & 7) + ((r128 >> 3) & 1)
    perm = jnp.where(pr == c128, 1.0, 0.0).astype(BF16)

    def patch(q, y):
        a, n = wd_rows[q]
        z = _rbf(xsel[:8, a:a + n] + _rbf(_rbf(y[:8]) * gate_r[:, :1]))
        g = z * _rbf(jax.nn.sigmoid(z))
        g = jnp.concatenate([g, jnp.zeros((120, n), F32)], axis=0).astype(BF16)
        gt = lax.dot_general(perm[:n, :n], g, _NT, preferred_element_type=F32)
        us = range(a // 16, (a + n) // 16)
        zz = newz()
        for u in us:
            hr = pl.ds(pl.multiple_of(zz + 8 * u, 8), 8)
            xx, ss = _unpack2(cols[0, hr, :]), _unpack2(cols[1, hr, :])
            r0 = 16 * u - a
            w = _pack2(*[xx[e] + _rbf(ss[e] * gt[r0 + 8 * e:r0 + 8 * e + 8]) for e in range(2)])
            for c, (tn, pn) in enumerate(nat):
                tt = 4 * (tn >> 2) + (tn & 3)
                pltpu.store(og.at[tt, pl.ds(8 * u, 8), :], pltpu.roll(w, (pn - c) & 127, 1), mask=lane8 == pn)
        for c, (tn, pn) in enumerate(nat):
            for u in us:
                v = og[tn, pl.ds(8 * u, 8), :]
                o_store(u, v, pl.ds(pl.multiple_of(tn * 128, 128), 128))
        if q in late:
            out_tiles(1, *late[q], lambda cp: cp.start())

    if u2 == NU:
        out_tiles(0, 0, D, lambda cp: cp.start())
    prev = None
    for q, (a, n) in enumerate(wd_rows):
        for k in waits.get(q, ()):
            cp_d[k].wait()
        if prev is not None and q in waits:
            patch(*prev)
            prev = None
        y = lax.dot_general(_bf(hpk[...]), wd[pl.ds(a, n), :], _NT, preferred_element_type=F32)
        if q == 0:
            o_gather(range(u2, NU))
        if prev is not None:
            patch(*prev)
        prev = (q, y)
        if q == 0 and u2 < NU:
            out_tiles(0, 0, D, lambda cp: cp.start())
    if _DEV.get("bar", 1):
        cp_bar.wait()
    patch(*prev)
    pltpu.make_async_copy(obuf, out_hbm, sem_out).wait()


def _scratch():
    return [
        pltpu.VMEM((D, L), BF16),
        pltpu.VMEM((6, D, N), BF16),
        pltpu.VMEM((D,), BF16),
        pltpu.VMEM((D,), BF16),
        pltpu.VMEM((D,), BF16),
        pltpu.VMEM((D, F), BF16),
        pltpu.VMEM((D, F), BF16),
        pltpu.VMEM((D, F), BF16),
        pltpu.VMEM((4, 64, 256), I32),
        pltpu.VMEM(_PROWS.shape, I32),
        pltpu.VMEM((_NPAT, 8, 128), I32),
        pltpu.VMEM((D, 128), F32),
        pltpu.VMEM((D, 128), F32),
        pltpu.VMEM((5, 2 * D, 128), I32),
        pltpu.VMEM((5, 2 * D, 128), I32),
        pltpu.VMEM((8, 2 * D, 128), I32),
        pltpu.VMEM((8, 2 * D, 128), I32),
        pltpu.VMEM((2, 4 * D, 128), F32),
        pltpu.VMEM((8, 4, D, 128), F32),
        pltpu.VMEM((16, D // 2, 128), I32),
        pltpu.VMEM((16, D // 2, 128), I32),
        pltpu.VMEM((8, 4, D, 128), F32),
        pltpu.VMEM((8, 2, D // 8, 8, 128), I32),
        pltpu.VMEM((8, 2, 2 * D, 128), F32),
        pltpu.VMEM((16, D // 2, 128), I32),
        pltpu.VMEM((3, 8, 128), F32),
        pltpu.VMEM((8, 128), I32),
        pltpu.VMEM((8, D), I32),
        pltpu.VMEM((8, 128), F32),
        pltpu.VMEM((C, 8, 128), I32),
        pltpu.VMEM((C, 8, D), F32),
        pltpu.VMEM((8, F), F32),
        pltpu.VMEM((8, F), I32),
        pltpu.VMEM((2, D // 2, 128), I32),
        pltpu.VMEM((16, D // 2, 128), I32),
        pltpu.VMEM((16, D // 2, 128), I32),
        pltpu.VMEM((D, L), BF16),
        pltpu.SemaphoreType.DMA((6 + len(_DEV.get("waits", {0: 0, 1: 0})),)),
        pltpu.SemaphoreType.DMA,
        pltpu.SemaphoreType.DMA,
    ] + [pltpu.VMEM((4, D // 2, 128), I32)] * 8 + [pltpu.VMEM((4, 24, 128), F32)] * 4


@jax.jit
def pallas_recurrent_scan__ssm_conv_s4__moe_arch_mod__prompt_kernel(
    A_u: jax.Array,
    A_A_re: jax.Array,
    A_A_im: jax.Array,
    A_B_re: jax.Array,
    A_B_im: jax.Array,
    A_C_re: jax.Array,
    A_C_im: jax.Array,
    A_log_dt: jax.Array,
    A_Dskip: jax.Array,
    B_x: jax.Array,
    B_w_r: jax.Array,
    B_w_gate: jax.Array,
    B_w_up: jax.Array,
    B_w_down: jax.Array,
):
    hbm = pl.BlockSpec(memory_space=pltpu.HBM)
    out = pl.pallas_call(
        _kernel,
        out_shape=jax.ShapeDtypeStruct((D, L), BF16),
        in_specs=[hbm] * 14,
        out_specs=hbm,
        scratch_shapes=_scratch(),
        compiler_params=pltpu.CompilerParams(vmem_limit_bytes=110 * 1024 * 1024),
        name="s4_mod",
    )(A_u[0].T, A_A_re, A_A_im, A_B_re, A_B_im, A_C_re, A_C_im, A_log_dt, A_Dskip, B_w_r,
      B_w_gate, B_w_up, B_w_down.T, jnp.asarray(_PROWS))
    return out.T[None]
```

```python
import numpy as np
import jax
import jax.numpy as jnp
from jax import lax
import jax.experimental.pallas as pl
import jax.experimental.pallas.tpu as pltpu

L, D, N, F, C = 2048, 576, 128, 4608, 8
NU = D // 16
CB = 64
NB = D // CB
CO = 32
NO = D // CO
UA = 4
F32, BF16, I32, U32 = jnp.float32, jnp.bfloat16, jnp.int32, jnp.uint32
EPS = 1e-5
_DEV = {}


def _bf16_round_np(x):
    u = np.asarray(x, np.float32).view(np.uint32).astype(np.uint64)
    r = ((u + 0x7FFF + ((u >> 16) & 1)) >> 16) << 16
    return r.astype(np.uint32)


_LROUND = _bf16_round_np(np.arange(L)).view(np.float32).astype(np.int64)
_HI = [(1, 3, 516, 1032), (5, 7, 520, 1288), (4, 260, 772, 1544), (8, 264, 776, 1800), (2, 6, 258, 262)]


def _lane_l1(l2):
    p = np.arange(128)
    return 32 * ((p // 32) ^ l2) + p % 32


def _comp_q():
    t = np.arange(8)[:, None]
    lane = np.arange(128)[None, :]
    return ((lane - 8 - 7 * (t % 4)) % 16) // 4


def _make_tables():
    lane = np.arange(128)
    lo = 8 * (4 * (lane // 16) + lane % 4)
    tab = [dict(), dict()]
    amask = np.zeros(128, bool)
    for q in range(5):
        for e in range(4):
            for par in range(2):
                t = 4 * par + e
                for h in range(2):
                    src = lane[(lane // 4) % 4 == 2 * h + par]
                    dst = (src + (4 * (q % 4) - 8 * h + 8) + 7 * t) % 128
                    assert np.all(_comp_q()[t, dst] == q % 4)
                    sid = e if q < 4 else 4 + e // 2
                    for sl, dl_ in zip(src, dst):
                        ent = (sid, int(dl_))
                        assert tab[par].setdefault(_HI[q][e] + int(lo[sl]), ent) == ent
                    if q == 4 and e % 2 == 1:
                        amask[dst % 16 + 16 * np.arange(8)[:, None]] = True
    pats = []
    for j in range(4):
        pats.append(np.tile(4 * (lane % 32) + ((lane // 32) ^ j), (8, 1)))
    for j in range(4):
        pats.append(np.tile(32 * ((lane % 4) ^ j) + lane // 4, (8, 1)))
    npat0 = len(pats)
    tiles, tile_of = [], {}
    for dl in range(4):
        for l2 in range(4):
            v = _LROUND[512 * dl + 4 * lane + l2]
            key = tuple(v.tolist())
            if key in tile_of:
                tile_of[dl, l2] = tile_of[key]
                continue
            sid = np.array([tab[0][x][0] if x else -1 for x in v])
            ln = np.array([[tab[s8 % 2][x][1] if x else 0 for x in v] for s8 in range(8)])
            steps = []
            for s in sorted(set(sid.tolist()), key=lambda s: -(sid == s).sum()):
                lanes = np.nonzero(sid == s)[0]
                if s < 0:
                    steps.append((-1, None, lanes))
                    continue
                care = sid == s
                kk = None
                for k in range(npat0, len(pats)):
                    oldp, oldc, olds = pats[k]
                    both = care & oldc
                    if olds == s and np.array_equal(oldp[:, both], ln[:, both]):
                        pats[k] = (np.where(care, ln, oldp), care | oldc, s)
                        kk = k
                        break
                if kk is None:
                    pats.append((np.where(care, ln, 0), care, s))
                    kk = len(pats) - 1
                steps.append((s, kk, lanes))
            tiles.append(steps)
            tile_of[key] = tile_of[dl, l2] = len(tiles) - 1
    pats = np.stack([p if k < npat0 else p[0] for k, p in enumerate(pats)]).astype(np.int32)
    tile_of = {k: v for k, v in tile_of.items() if len(k) == 2}
    rows = np.concatenate([pats[:, :2].reshape(-1, 128), amask[None].astype(np.int32)])
    rows = np.concatenate([rows, np.zeros((-len(rows) % 8, 128), np.int32)])
    return tiles, tile_of, len(pats), rows


_TILES, _TILE_OF, _NGAT, _PROWS = _make_tables()
_NPAT = _NGAT + 3


def _cmul(ar, ai, br, bi):
    return ar * br - ai * bi, ar * bi + ai * br


def _sincos(b):
    magic = jnp.float32(12582912.0)
    t = b * jnp.float32(2.0 / np.pi) + magic
    k = t - magic
    ki = pltpu.bitcast(t, I32)
    r = b - k * jnp.float32(1.5703125)
    r = r - k * jnp.float32(0.0004837512969970703)
    r = r - k * jnp.float32(7.549790126404332e-08)
    u = r * r
    ps = (jnp.float32(-0.0001958295761141926) * u + jnp.float32(0.008332725614309311)) * u \
        + jnp.float32(-0.166666641831398)
    sn = r + (r * u) * ps
    pc = ((jnp.float32(2.437065268168226e-05) * u + jnp.float32(-0.0013886778615415096)) * u
          + jnp.float32(0.04166663438081741)) * u + jnp.float32(-0.5)
    cs = pc * u + jnp.float32(1.0)
    odd = (ki & 1) == 1
    s1 = jnp.where(odd, cs, sn)
    c1 = jnp.where(odd, sn, cs)
    sign = jnp.int32(-2147483648)
    s1 = pltpu.bitcast(pltpu.bitcast(s1, I32) ^ ((ki << 30) & sign), F32)
    c1 = pltpu.bitcast(pltpu.bitcast(c1, I32) ^ (((ki + 1) << 30) & sign), F32)
    return s1, c1


def _gather(x, idx):
    return jnp.take_along_axis(x, idx, axis=1, mode="promise_in_bounds")


def _lanes_mask(lanes):
    lane = lax.broadcasted_iota(I32, (8, 128), 1)
    lanes = sorted(int(x) for x in lanes)
    runs, start, prev = [], lanes[0], lanes[0]
    for x in lanes[1:]:
        if x != prev + 1:
            runs.append((start, prev))
            start = x
        prev = x
    runs.append((start, prev))
    m = None
    for a, b in runs:
        t = (lane == a) if a == b else jnp.logical_and(lane >= a, lane <= b)
        m = t if m is None else jnp.logical_or(m, t)
    return m


def _butterfly(p):
    lane = lax.broadcasted_iota(I32, p[0].shape, 1)
    b0 = (lane & 32) != 0
    b1 = (lane & 64) != 0
    t = [jnp.where(b0, p[k ^ 1], p[k]) for k in range(4)]
    return [jnp.where(b1, t[k ^ 2], t[k]) for k in range(4)]


def _fft4(x, sgn):
    (ar, ai), (br, bi), (cr, ci), (dr, di) = x
    s0r, s0i, d0r, d0i = ar + cr, ai + ci, ar - cr, ai - ci
    s1r, s1i, d1r, d1i = br + dr, bi + di, br - dr, bi - di
    y0 = (s0r + s1r, s0i + s1i)
    y2 = (s0r - s1r, s0i - s1i)
    p = (d0r - d1i, d0i + d1r)
    m = (d0r + d1i, d0i - d1r)
    return [y0, p, y2, m] if sgn > 0 else [y0, m, y2, p]


def _silu(z):
    h = z * jnp.float32(0.5)
    return h + h * jnp.tanh(h)


def _rbf(x):
    return x.astype(BF16).astype(F32)


def _pack2(a, b):
    p = pltpu.pack_elementwise([a, b], packed_dtype=BF16)
    return p if p.dtype == I32 else pltpu.bitcast(p, I32)


def _unpack2(x):
    return [pltpu.unpack_elementwise(x, index=i, packed_dtype=BF16, unpacked_dtype=F32) for i in range(2)]


def _bf(x):
    return pltpu.bitcast(x, BF16)


_NT = (((1,), (1,)), ((), ()))


class _Idx:
    def __init__(self, i, lag, z=None):
        self.i, self.lag, self.z = i, lag, z

    def off(self, stride, const=0, align=None):
        c = const - self.lag * stride
        if isinstance(self.i, int):
            if self.z is None:
                return self.i * stride + c
            v = self.z + (self.i * stride + c)
        else:
            v = self.i * stride + c
        return pl.multiple_of(v, align) if align else v

    def idx(self):
        return self.i - self.lag


def _pipeline(stages, n, newz, weave=None, reset=None):
    ns = len(stages)

    def step(i, lo, hi):
        z = newz() if isinstance(i, int) else None
        gens = {k: stages[k](_Idx(i, k, z)) for k in range(lo, hi)}
        if reset is not None:
            reset()
        if callable(weave):
            weave(gens)
        else:
            for k in weave or ():
                if k in gens:
                    next(gens[k], None)
        for k in range(hi - 1, lo - 1, -1):
            for _ in gens[k]:
                pass

    def body(i, carry):
        step(i, 0, ns)
        return carry

    return ([lambda i=i: step(i, 0, i + 1) for i in range(ns - 1)],
            lambda: lax.fori_loop(ns - 1, n, body, 0),
            [lambda i=i: step(n + i, i + 1, ns) for i in range(ns - 1)])


def _run(fns):
    for fn in fns:
        fn()


def _kernel(x_hbm, are_hbm, aim_hbm, bre_hbm, bim_hbm, cre_hbm, cim_hbm, ldt_hbm, dsk_hbm, wr_hbm,
            wg_hbm, wu_hbm, wd_hbm, pat_hbm,
            out_hbm,
            xbuf, par, ldt, dsk, wr, wg, wu, wd, fpk, prow, pats,
            dtcol, skip, hi_re, hi_im, lo_re, lo_im, comp, khat,
            xp, xnp, uhat, yhat, ybuf, spk, topk, posv, wr16b, wsum, ohb, xsel_ref, hbuf, hpk, cols, opk, og, obuf,
            sem_in, sem_out, sem_bar, *perb):
    xi, xg, stat = perb[0:4], perb[4:8], perb[8:12]
    p_hbm = (are_hbm, aim_hbm, bre_hbm, bim_hbm, cre_hbm, cim_hbm)
    r1 = 16 * UA
    small = [(ldt_hbm, ldt), (pat_hbm, prow), (dsk_hbm, dsk)]
    small += [(h.at[pl.ds(0, r1)], par.at[i, pl.ds(0, r1)]) for i, h in enumerate(p_hbm)]
    small += [(h.at[pl.ds(r1, D - r1)], par.at[i, pl.ds(r1, D - r1)]) for i, h in enumerate(p_hbm)]
    small += [(wr_hbm, wr)]
    cps = [pltpu.make_async_copy(s, d, sem_in.at[0 if i < 3 else 1 if i < 9 else 2])
           for i, (s, d) in enumerate(small)]
    ns = 3
    cp_x = pltpu.make_async_copy(x_hbm, xbuf, sem_in.at[ns])
    cp_g = pltpu.make_async_copy(wg_hbm, wg, sem_in.at[ns + 1])
    cp_u = pltpu.make_async_copy(wu_hbm, wu, sem_in.at[ns + 2])
    k_rows = [(0, 128), (128, 128), (256, 128), (384, 128), (512, 64)]
    wd_rows = _DEV.get("wdr", k_rows)
    waits = _DEV.get("waits", {0: (0, 1, 2), 3: (3, 4)})
    wd_grp = {k: g for g, ks in enumerate(waits.values()) for k in ks}
    cp_d = [pltpu.make_async_copy(wd_hbm.at[pl.ds(a, n)], wd.at[pl.ds(a, n)], sem_in.at[ns + 3 + wd_grp[i]])
            for i, (a, n) in enumerate(wd_rows)]
    cp_bar = pltpu.make_async_copy(pat_hbm.at[pl.ds(0, 8)], posv, sem_bar) if _DEV.get("bar", 1) else None
    if _DEV.get("only"):
        cp_g, cp_u, cp_d, cp_bar = None, None, [], None
    for cp in cps + [cp_x, cp_g, cp_u] + cp_d:
        if cp is not None:
            cp.start()

    sub8 = lax.broadcasted_iota(I32, (8, 128), 0)
    lane8 = lax.broadcasted_iota(I32, (8, 128), 1)
    for l2 in range(4):
        for g in range(8):
            cs = []
            for e in range(2):
                p = 16 * g + 2 * sub8 + e
                t = 4 * (32 * ((p >> 5) ^ l2) + (p & 31)) + l2
                n = ((4 * lane8 + 1) * t) & 2047
                cs.append(_sincos(n.astype(F32) * jnp.float32(-2.0 * np.pi / 2048)))
            fpk[l2, pl.ds(8 * g, 8), pl.ds(0, 128)] = _pack2(cs[0][1], cs[1][1])
            fpk[l2, pl.ds(8 * g, 8), pl.ds(128, 128)] = _pack2(cs[0][0], cs[1][0])

    for cp in cps[:3]:
        cp.wait()
    for k in range(_NGAT):
        pats[k] = jnp.where((sub8 & 1) == 1, jnp.broadcast_to(prow[pl.ds(2 * k + 1, 1), :], (8, 128)),
                            jnp.broadcast_to(prow[pl.ds(2 * k, 1), :], (8, 128)))
    cq = ((lane8 - 8 - 7 * (sub8 & 3)) & 15) >> 2
    pats[_NGAT] = cq & 1
    pats[_NGAT + 1] = cq >> 1
    pats[_NGAT + 2] = jnp.broadcast_to(prow[pl.ds(2 * _NGAT, 1), :], (8, 128))
    r128 = lax.broadcasted_iota(I32, (128, 128), 0)
    c128 = lax.broadcasted_iota(I32, (128, 128), 1)
    eye = jnp.where(r128 == c128, 1.0, 0.0).astype(BF16)
    dt_row = jnp.exp(ldt[...].astype(F32).reshape(1, D)).astype(BF16)
    dsk_row = dsk[...].reshape(1, D)
    for t in range(5):
        n = min(128, D - 128 * t)
        for row, dst in ((dt_row, dtcol), (dsk_row, skip)):
            b = jnp.broadcast_to(row[:, 128 * t:128 * t + n], (128, n))
            dst[pl.ds(128 * t, n), :] = lax.dot_general(eye[:n, :n], b, _NT, preferred_element_type=F32)

    zero = prow[0, 0]
    zcount = [0]

    def newz():
        zcount[0] += 1
        return zero * (64 * zcount[0]) if _DEV.get("zpeel", 1) else None

    def block(*fns):
        if not _DEV.get("blocks", 1):
            return _run(fns)

        def body(k, carry):
            _run(fns)
            return carry

        lax.fori_loop(0, zero + 1, body, 0)

    def slow_zero(i):
        t = i.off(1) * zero if not isinstance(i.i, int) or i.z is None else i.z
        for _ in range(_DEV.get("slow", 0)):
            t = t * t
        return pl.multiple_of(t * 8, 8)

    def after(x, deps):
        never = pats[0] < 0
        d = None
        for v in deps:
            v = v if v.dtype == I32 else pltpu.bitcast(v, I32)
            d = v if d is None else d ^ v
        return jnp.where(never, d if x.dtype == I32 else pltpu.bitcast(d, x.dtype), x)

    def pad_tail(y, i):
        n = _DEV.get("pad", 16)
        if not n:
            return y
        m = y.shape[0]
        base = i.off(1)
        k = m - 8 * _DEV.get("padpos", 8)
        mid = after(y[k:k + 8], [pats[j % _NPAT] * (base + j) for j in range(n)])
        return jnp.concatenate([y[:k], mid, y[k + 8:]], axis=0)

    class Sched:
        tok, g, pre = {}, 0, []

        @classmethod
        def reset(cls):
            cls.tok, cls.g, cls.pre = {}, 0, []

        @classmethod
        def gate(cls, x):
            deps = cls.tok.pop(cls.g, [])
            cls.g += 1
            if not deps or not _DEV.get("gate", 1):
                return x
            return jnp.concatenate([after(x[:8], deps), after(x[8:], deps[-1:])], axis=0)

    slot = {h: (q, e) for q, ent in enumerate(_HI) for e, h in enumerate(ent)}

    def a_prep(i):
        gate = Sched.gate
        for u in range(UA):
            rows = pl.ds(i.off(16 * UA, 16 * u, 16), 16)
            ev = pl.ds(i.off(32 * UA, 32 * u), 16, stride=2)
            od = pl.ds(i.off(32 * UA, 32 * u + 1), 16, stride=2)
            dt = gate(dtcol[rows, :])
            al = dt * par[0, rows, :].astype(F32)
            be = dt * par[1, rows, :].astype(F32)
            cr, ci = _cmul(par[4, rows, :].astype(F32), par[5, rows, :].astype(F32),
                           par[2, rows, :].astype(F32), par[3, rows, :].astype(F32))
            dts = dt * jnp.float32(1.0 / 512)
            cr, ci = cr * dts, ci * dts
            k0 = jnp.sum(cr, axis=1, keepdims=True) * jnp.float32(512.0)
            skip[rows, :] = skip[rows, :] + k0
            yield cr
            s, c = _sincos(gate(be))
            yield c
            pw = {1: (c, s)}
            e = 1
            while e < 256:
                if e in (1, 16):
                    c = gate(c)
                c, s = (c - s) * (c + s), (c + c) * s
                e *= 2
                pw[e] = (c, s)
                if e in (16, 256):
                    yield c
            z = {}
            for e in (1, 8, 256):
                mag = jnp.exp(al * jnp.float32(e))
                c, s = pw[e]
                z[e] = (mag * c, mag * s)
            pend = {}

            def put(tab, q, ee, v):
                key = (tab[0] is hi_re, q, ee // 2)
                if key not in pend:
                    pend[key] = (ee % 2, v)
                    return
                w, o = pend.pop(key)
                lo_, hi_ = (o, v) if w == 0 else (v, o)
                dst = od if ee // 2 else ev
                tab[0][q, dst, :] = _pack2(lo_[0], hi_[0])
                tab[1][q, dst, :] = _pack2(lo_[1], hi_[1])

            h = (cr, ci)
            cnt = 0
            for e in range(1, 9):
                g, ee, m = h, e, z[1]
                while ee in slot:
                    if cnt % 4 == 0:
                        g = (gate(g[0]), g[1])
                    g = _cmul(*g, *m)
                    put((hi_re, hi_im), *slot[ee], g)
                    if ee == e:
                        h = g
                    ee, m = ee + 256, z[256]
                    cnt += 1
                    if cnt % 4 == 0:
                        yield g[0]
            w1 = (gate(z[8][0]), -z[8][1])
            v = [(jnp.ones((16, 128), F32), jnp.zeros((16, 128), F32)), w1]
            v.append(_cmul(*w1, *w1))
            v.append(_cmul(*v[2], *w1))
            w4 = _cmul(*v[2], *v[2])
            for j in range(8):
                for f in range(4):
                    put((lo_re, lo_im), j, f, v[f])
                yield v[3][0]
                if j < 7:
                    w4 = (gate(w4[0]), w4[1])
                    v = [w4 if (j == 0 and f == 0) else _cmul(*v[f], *w4) for f in range(4)]

    def a_gen(i):
        b0 = pats[_NPAT - 3] != 0
        b1 = pats[_NPAT - 2] != 0
        g0, gs = _DEV.get("g0", 13), _DEV.get("gs", None)
        rate = _DEV.get("rate", 0.9)
        for k in range(4 * UA):
            rows = pl.ds(i.off(32 * UA, 8 * k, 8), 8)
            lo = jnp.concatenate([lo_re[:, rows, :].reshape(64, 128), lo_im[:, rows, :].reshape(64, 128)], axis=1)
            h0 = hi_re[0, rows, :]
            if k % 2 == 0 and Sched.pre and _DEV.get("gate", 1):
                h0 = after(h0, Sched.pre)
                Sched.pre = []
            hi = jnp.concatenate([jnp.concatenate([h0, hi_re[1:5, rows, :].reshape(32, 128)], axis=0),
                                  hi_im[:, rows, :].reshape(40, 128)], axis=1)
            o = lax.dot_general(_bf(hi), _bf(lo), _NT, preferred_element_type=F32)
            for q in range(5):
                Sched.tok.setdefault(g0 + int(rate * (5 * (k // 2) + q)), []).append(o[16 * q + 8:16 * q + 16])
            for h in range(2):
                g = [pltpu.roll(o[16 * q + 8 * h:16 * q + 8 * h + 8], 4 * (q % 4) - 8 * h + 8, 1,
                                stride=7, stride_axis=0) for q in range(5)]
                dst = pl.ds(i.off(64 * UA, 16 * k + 8 * h, 8), 8)
                v = jnp.where(b1, jnp.where(b0, g[3], g[2]), jnp.where(b0, g[1], g[0]))
                comp[0, dst, :] = v
                comp[1, dst, :] = g[4]
                if gs is not None:
                    Sched.tok.setdefault(g0 + gs + int(rate * (5 * (k // 2) + 4)), []).append(v)
            if k % 2 == 1:
                yield

    def a_exp(i):
        bm = pats[_NPAT - 1] != 0
        srcs = []
        for u in range(UA):
            def ld(a, e):
                return _pack2(comp[a, pl.ds(i.off(64 * UA, 64 * u + e), 8, stride=4), :],
                              comp[a, pl.ds(i.off(64 * UA, 64 * u + 32 + e), 8, stride=4), :])

            srcs.append([ld(0, e) for e in range(4)]
                        + [jnp.where(bm, ld(1, 2 * k + 1), ld(1, 2 * k)) for k in range(2)])
        cache = {}

        def gat(s, key):
            if key not in cache:
                pat = pats[key]
                cache[key] = [_gather(srcs[u][s], pat) for u in range(UA)]
            return cache[key]

        tiles = []
        for steps in _TILES:
            t = None
            for s, key, lanes in steps:
                v = [jnp.zeros((8, 128), I32)] * UA if s < 0 else gat(s, key)
                t = v if t is None else [jnp.where(_lanes_mask(lanes), v[u], t[u]) for u in range(UA)]
            tiles.append(t)
        yield
        for u0 in range(0, UA, 2):
            lhs = [_bf(jnp.concatenate([tiles[_TILE_OF[dl, l2]][u] for dl in range(4) for u in (u0, u0 + 1)], axis=0))
                   for l2 in range(4)]
            z0 = 0 if u0 == 0 else zero * 8

            def dots(ri):
                return [jnp.dot(lhs[l2], _bf(jnp.concatenate(
                    [fpk[l2, pl.ds(z0 + 16 * (j ^ l2), 16) if u0 == 0 else
                         pl.ds(pl.multiple_of(z0 + 16 * (j ^ l2), 8), 16), pl.ds(128 * ri, 128)]
                     for j in range(4)], axis=0)), preferred_element_type=F32) for l2 in range(4)]

            def store(k2, ri, v):
                khat[2 * k2 + ri, :, pl.ds(i.off(16 * UA, 16 * u0, 16), 32), :] = v.reshape(4, 32, 128)

            def toks(v, step0):
                g1 = _DEV.get("g0", 13) + int(_DEV.get("rate", 0.9) * 10 * UA) + _DEV.get("g1", 0)
                for j in range(8):
                    g = g1 + int(_DEV.get("rate2", 0.7) * (step0 + j))
                    Sched.tok.setdefault(g, []).append(v[16 * j + 8:16 * j + 16])

            re = dots(0)
            s0, d0r, s1, d1r = re[0] + re[2], re[0] - re[2], re[1] + re[3], re[1] - re[3]
            store(0, 0, s0 + s1)
            v = s0 - s1
            store(2, 0, v)
            toks(v, 8 * u0)
            im = dots(1)
            s0, d0i, s1, d1i = im[0] + im[2], im[0] - im[2], im[1] + im[3], im[1] - im[3]
            store(0, 1, s0 + s1)
            store(2, 1, s0 - s1)
            store(1, 0, d0r + d1i)
            store(1, 1, d0i - d1r)
            store(3, 0, d0r - d1i)
            v = d0i + d1r
            store(3, 1, v)
            toks(v, 8 * u0 + 8)
            yield

    def bail(cl):
        for cp in cl:
            if cp is not None:
                cp.wait()
        zr = pl.ds(pl.multiple_of(zero * 8, 8), 16)
        v = khat[zero, zero, zr, :] + skip[zr, :] + (spk[zero, zr, :] + opk[zero, zr, :] + xnp[zero, zr, :] + xp[zero, zr, :]).astype(F32) + topk[zero][:1] + comp[zero, zr, :]
        v = v + (hi_re[zero, zr, :] + hi_im[zero, zr, :] + lo_re[zero, zr, :] + lo_im[zero, zr, :]).astype(F32)
        v = v + uhat[zero, zero, zr, :] + ybuf[zero, zero, zr, :] + yhat[zero, zero, zero][:1].astype(F32)
        obuf[pl.ds(0, 16), pl.ds(0, 128)] = v.astype(BF16)
        cp = pltpu.make_async_copy(obuf.at[pl.ds(0, 16)], out_hbm.at[pl.ds(0, 16)], sem_out)
        cp.start()
        cp.wait()

    if _DEV.get("only") == "C":
        a_tail = [lambda: None] * 2
    else:
        def a_weave(gens):
            if 2 in gens and _DEV.get("expfirst", 1):
                next(gens[2])
            if 0 in gens and 1 in gens:
                for n in _DEV.get("pre", (3, 5, 4)):
                    for _ in range(n):
                        v = next(gens[0])
                    Sched.pre = [v[:8], v[8:]]
                    next(gens[1])
            for k in (1, 2):
                if k in gens:
                    for _ in gens[k]:
                        pass
            if 0 in gens:
                for _ in gens[0]:
                    pass

        a_pro, a_loop, a_tail = _pipeline([a_prep, a_gen, a_exp], NU // UA, newz, reset=Sched.reset,
                                          weave=a_weave)
        for cp in cps[3:9]:
            cp.wait()
        if _DEV.get("only") == "0":
            return bail(cps[9:] + [cp_x])
        a_pro[0]()
        for cp in cps[9:]:
            cp.wait()
        a_pro[1]()
        a_loop()
    if _DEV.get("only") == "A":
        return bail([cp_x, cp_g, cp_u] + cp_d)

    cp_x.wait()

    def zrow(u):
        return pl.ds(pl.multiple_of(zero * 8 + 8 * u, 8), 8)

    def b_gather_direct(b):
        for j in range(4):
            pat = pats[j]
            for u in range(NU):
                v = pltpu.bitcast(xbuf[pl.ds(16 * u, 16), pl.ds(512 * b + 128 * j, 128)], I32)
                xg[b][j, pl.ds(8 * u, 8), :] = _gather(v, pat)

    def b_stat(b):
        for _ in b_stat_gen(b):
            pass

    def b_stat_gen(b):
        s2 = [jnp.zeros((8, 128), F32) for _ in range(4)]
        for u in range(NU):
            o = _butterfly([xg[b][j, zrow(u), :] for j in range(4)])
            for l2 in range(4):
                xp[4 * l2 + b, pl.ds(8 * u, 8), :] = o[l2]
                e_, o_ = _unpack2(o[l2])
                s2[l2] = s2[l2] + (e_ * e_ + o_ * o_)
            yield
        for l2 in range(4):
            stat[b][l2, pl.ds(16, 8), :] = s2[l2]

    def b_dot(b):
        lhs = _bf(wr16b[...])
        for j in range(4):
            stat[b][j, pl.ds(0, 16), :] = jnp.dot(lhs, _bf(xg[b][j, pl.ds(pl.multiple_of(zero * zero * 8, 8), D // 2), :]),
                                                  preferred_element_type=F32)

    def b_fin(b):
        st = []
        wxs = _butterfly([stat[b][j, zrow(0), :] for j in range(4)])
        sxs = _butterfly([stat[b][j, zrow(1), :] for j in range(4)])
        for l2 in range(4):
            wx, sx = wxs[l2], sxs[l2]
            m = sx * jnp.float32(1.0 / D)
            q = jnp.sum(stat[b][l2, zrow(2), :], axis=0, keepdims=True) * jnp.float32(1.0 / D)
            var = _rbf(jnp.maximum(q - m * m, 0.0))
            rs = 1.0 / _rbf(jnp.sqrt(_rbf(var + jnp.float32(EPS))))
            mb = _rbf(m)
            st.append((mb, rs))
            r = _rbf((wx - mb * wsum[...]) * rs)
            r = jnp.where(r == 0.0, 0.0, r)
            bits = pltpu.bitcast(r, I32)
            mono = ((bits ^ ((bits >> 31) & jnp.int32(0x7FFFFFFF))) >> 16) + 32768
            tok = 512 * b + 4 * (32 * ((lane8 >> 5) ^ l2) + (lane8 & 31)) + l2
            key = pltpu.bitcast((mono << 11) + (2047 - tok) + jnp.int32(0x00800000), F32)
            t = 4 * b + l2
            topk[t // 8] = key if t % 8 == 0 else jnp.where(sub8 == t % 8, key, topk[t // 8])
        return st

    def b_norm(b):
        st = b_fin(b)
        for us in (range(CB // 16), range(CB // 16, NU)):
            for l2 in range(4):
                mb, rs = st[l2]
                for u in us:
                    e_, o_ = _unpack2(xp[4 * l2 + b, zrow(u), :])
                    xnp[4 * l2 + b, pl.ds(8 * u, 8), :] = _pack2((e_ - mb) * rs, (o_ - mb) * rs)

    wrow = wr[...].reshape(1, D)
    wr16b[...] = pltpu.bitcast(jnp.concatenate([jnp.broadcast_to(wrow, (8, D)), jnp.ones((8, D), BF16)], axis=0), I32)
    wsum[...] = jnp.broadcast_to(jnp.sum(wrow.astype(F32), axis=1, keepdims=True), (8, 128))
    topk[2] = jnp.zeros((8, 128), F32)
    cols[...] = jnp.zeros(cols.shape, I32)

    ctok = {"mid": [], "n": 0, "elt": []}

    def c_reset():
        ctok["mid"], ctok["n"] = [], 0

    def pin_lhs(lhs):
        n = ctok["n"]
        ctok["n"] += 1
        nv = lhs.shape[0] // 8
        if n % 2 == 1 or not _DEV.get("cpin", 0):
            return lhs
        parts = [lhs[8 * j:8 * j + 8] for j in range(nv)]
        for k, tok in enumerate(ctok["mid"]):
            t = _DEV.get("cp0", 130) + _DEV.get("cp1", 128) * k - (n // 2) * nv * 16
            if 0 <= t < nv * 16:
                parts[t // 16] = after(parts[t // 16], [tok])
        return jnp.concatenate(parts, axis=0)

    def c_fwd(i):
        h0 = i.off(CB // 2, 0, 8)
        r0 = i.off(CB, 0, 8)
        for l2 in range(4):
            lhs = _bf(pin_lhs(xnp[pl.ds(4 * l2, 4), pl.ds(h0, CB // 2), :].reshape(2 * CB, 128)))
            res = jnp.dot(lhs, _bf(fpk[l2, pl.ds(slow_zero(i), 64), :]), preferred_element_type=F32)
            for ri in range(2):
                y = res[:, 128 * ri:128 * ri + 128]
                if l2 == 3 and ri == 1 and isinstance(i.i, int) and i.i < 2:
                    y = pad_tail(y, i)
                uhat[2 * l2 + ri, :, pl.ds(r0, CB), :] = y.reshape(4, CB, 128)
            yield

    def c_mid(i):
        for k in range(CB // 8):
            rows = pl.ds(i.off(CB, 8 * k, 8), 8)
            krows = pl.ds(i.off(CB, 16 * (k // 2) + k % 2), 8, stride=2)
            uu = [_fft4([(uhat[2 * l2, b, rows, :], uhat[2 * l2 + 1, b, rows, :]) for l2 in range(4)], -1)
                  for b in range(4)]
            yy = [[None] * 4 for _ in range(4)]
            kmode = _DEV.get("kfft", 0)

            def khalf(dl, odd):
                kr = pl.ds(i.off(CB, 16 * (k // 2) + k % 2) + (zero if odd else 0), 8, stride=2)
                x = [(khat[2 * l2, dl, kr, :], khat[2 * l2 + 1, dl, kr, :]) for l2 in range(4)]
                if not odd:
                    s0 = (x[0][0] + x[2][0], x[0][1] + x[2][1])
                    s1 = (x[1][0] + x[3][0], x[1][1] + x[3][1])
                    return {0: (s0[0] + s1[0], s0[1] + s1[1]), 2: (s0[0] - s1[0], s0[1] - s1[1])}
                d0 = (x[0][0] - x[2][0], x[0][1] - x[2][1])
                d1 = (x[1][0] - x[3][0], x[1][1] - x[3][1])
                return {1: (d0[0] + d1[1], d0[1] - d1[0]), 3: (d0[0] - d1[1], d0[1] + d1[0])}

            def acc(pp, m, t):
                pp[m] = t if pp[m] is None else (pp[m][0] + t[0], pp[m][1] + t[1])

            for odd in range(2):
                pps = {k2: [None] * 4 for k2 in (odd, odd + 2)}
                if kmode == 0:
                    for k2 in pps:
                        for dl in range(3, -1, -1):
                            kk = (khat[2 * k2, dl, krows, :], khat[2 * k2 + 1, dl, krows, :])
                            for m in range(3, dl - 1, -1):
                                acc(pps[k2], m, _cmul(*uu[m - dl][k2], *kk))
                elif kmode == 1:
                    for dl in range(3, -1, -1):
                        kk = khalf(dl, odd)
                        for k2 in pps:
                            for m in range(3, dl - 1, -1):
                                acc(pps[k2], m, _cmul(*uu[m - dl][k2], *kk[k2]))
                else:
                    kk = [khalf(dl, odd) for dl in range(4)]
                    for k2 in pps:
                        for m in range(3, -1, -1):
                            for b in range(m, -1, -1):
                                acc(pps[k2], m, _cmul(*uu[b][k2], *kk[m - b][k2]))
                for k2, pp in pps.items():
                    for m in range(3, -1, -1):
                        yy[m][k2] = pp[0] if m == 0 else (pp[m][0] - pp[m - 1][1], pp[m][1] + pp[m - 1][0])
            un = i.off(CB // 8, k)
            for bp in range(2):
                ww = [_fft4(yy[m], 1) for m in (2 * bp, 2 * bp + 1)]
                for l2 in range(4):
                    for ri in range(2):
                        v = _pack2(ww[0][l2][ri], ww[1][l2][ri])
                        yhat[2 * l2 + ri, bp, un] = v
            ctok["mid"].append(v)
            yield

    def c_inv(i):
        u0 = i.off(CB // 8)
        r0 = i.off(2 * CB, 0, 8)
        for l2 in range(4):
            for ri in range(2):
                lhs = yhat[2 * l2 + ri, :, pl.ds(u0, CB // 8)].reshape(2 * CB, 128)
                lhs = _bf(pin_lhs(lhs) if ri == 0 else lhs)
                y = lax.dot_general(lhs, _bf(fpk[l2, pl.ds(slow_zero(i), 64), pl.ds(128 * ri, 128)]), _NT, preferred_element_type=F32)
                if l2 == 3 and ri == 1 and isinstance(i.i, int):
                    y = pad_tail(y, i)
                ybuf[2 * l2 + ri, :, pl.ds(r0, 2 * CB), :] = y.reshape(2, 2 * CB, 128)
            yield

    def c_elt(i):
        for k in range(CB // 16):
            hr = pl.ds(i.off(CB // 2, 8 * k, 8), 8)
            sk = [skip[pl.ds(i.off(CB, 16 * k + e), 8, stride=2), :] for e in range(2)]
            for b in range(4):
                o = []
                for l2 in range(4):
                    w = xnp[4 * l2 + b, hr, :]
                    if ctok["elt"]:
                        w = after(w, ctok["elt"])
                    xn = _unpack2(w)
                    xx = _unpack2(xp[4 * l2 + b, hr, :])
                    ss, v = [], []
                    for e in range(2):
                        yr = pl.ds(i.off(2 * CB, 32 * k + 2 * e + b % 2), 8, stride=4)
                        ss.append(ybuf[2 * l2, b // 2, yr, :] + ybuf[2 * l2 + 1, b // 2, yr, :] + xn[e] * sk[e])
                        v.append(xx[e] + ss[e] * _silu(xn[e]))
                    spk[4 * l2 + b, hr, :] = _pack2(*ss)
                    o.append(_pack2(*v))
                p = _butterfly(o)
                for j in range(4):
                    opk[4 * b + j, hr, :] = p[j]
                yield

    def c_top(i):
        k0, k1 = topk[i.off(0, 0)], topk[i.off(0, 1)]
        mx = jnp.max(jnp.max(jnp.maximum(k0, k1), axis=0, keepdims=True), axis=1, keepdims=True)
        topk[i.off(0, 0)] = jnp.where(k0 == mx, 0.0, k0)
        topk[i.off(0, 1)] = jnp.where(k1 == mx, 0.0, k1)
        topk[i.off(0, 2)] = jnp.where(sub8 == i.idx(), mx, topk[i.off(0, 2)])
        yield

    def c_first(i):
        if _DEV.get("toplast", 1):
            yield
            yield from c_fwd(i)
            yield from c_top(i)
        else:
            yield from c_top(i)
            yield from c_fwd(i)

    c_pro, c_loop, c_tail = _pipeline([c_first, c_mid, c_inv, c_elt], NB, newz, reset=c_reset,
                                      weave=_DEV.get("cweave", [1] * (CB // 8) + [3] * (CB // 4) + [0, 0, 0, 2, 2, 0, 0, 2, 2]))
    def first_fwd():
        i = _Idx(0, 0)
        for _ in c_fwd(i):
            pass
        for _ in c_top(i):
            pass

    if _DEV.get("only") != "C":
        ops = {"G": b_gather_direct, "s": b_stat, "d": b_dot, "n": b_norm,
               "a": lambda k: a_tail[k](), "f": lambda k: first_fwd()}
        for blk in _DEV.get("bplan", "a0G0G1 a1G2G3d0d1s0s1 s2s3n0n1d2d3 n2n3f0").split():
            block(*[lambda k=k: ops[blk[k]](int(blk[k + 1])) for k in range(0, len(blk), 2)])
    if _DEV.get("only") == "B":
        return bail([cp_g, cp_u] + cp_d)
    for fn in c_pro[1:]:
        block(fn)
    c_loop()
    if _DEV.get("only") in ("C", "ABC"):
        return bail([cp_g, cp_u] + cp_d)

    sel = pltpu.bitcast(topk[2], I32) - jnp.int32(0x00800000)
    mono = (sel >> 11) - 32768
    r_sel = pltpu.bitcast((mono ^ ((mono >> 31) & jnp.int32(0x7FFF))) << 16, F32)
    gate_r = _rbf(jax.nn.sigmoid(r_sel))
    posv[...] = 2047 - (sel & 2047)
    tok = [posv[c, 0] for c in range(C)]
    nat = [(t >> 7, t & 127) for t in tok]
    prm = []
    for t in tok:
        l2, l1 = t & 3, (t >> 2) & 127
        prm.append((4 * l2 + (t >> 9), 32 * ((l1 >> 5) ^ l2) + (l1 & 31)))

    def extract(src, k):
        for c, (tp, pp) in enumerate(prm):
            sh = (c - pp) & 127
            for u in range(NU):
                pltpu.store(cols.at[k, pl.ds(8 * u, 8), :], pltpu.roll(src[tp, pl.ds(8 * u, 8), :], sh, 1),
                            mask=lane8 == c)

    for c, (tp, pp) in enumerate(prm):
        ohb[c] = jnp.where(jnp.logical_and(sub8 == c // 2, lane8 == pp), jnp.int32(0x3F80 << (16 * (c % 2))), 0)

    def take_rows():
        for c, (tp, pp) in enumerate(prm):
            xsel_ref[c] = lax.dot_general(_bf(ohb[c]), _bf(xnp[tp]), _NT, preferred_element_type=F32)[:8]

    def stages(*items):
        def run():
            z = newz()
            for fn, k in items:
                for _ in fn(_Idx(k, 0, z)):
                    pass
        return run

    e1, e2 = _DEV.get("e1", ()), _DEV.get("e2", (NB - 3,))
    block(stages((c_mid, NB - 1), *[(c_elt, k) for k in e1], (c_inv, NB - 2)))
    block(stages(*[(c_elt, k) for k in e2], (c_inv, NB - 1)), take_rows, lambda: extract(xp, 0))

    def o_gather(us):
        for j in range(4):
            pat = pats[4 + j]
            for b in range(4):
                for u in us:
                    v = _gather(opk[4 * b + j, pl.ds(8 * u, 8), :], pat)
                    og[4 * b + j, pl.ds(8 * u, 8), :] = v
                    o_store(u, v, pl.ds(512 * b + 128 * j, 128))

    def o_store(u, v, col):
        obuf[pl.ds(16 * u, 8), col] = _bf(v[0:4])
        obuf[pl.ds(16 * u + 8, 8), col] = _bf(pltpu.roll(v, 4, 0)[0:4])

    bits = jnp.int32(0)
    for c in range(C):
        bits = bits | (jnp.int32(1) << nat[c][0])

    if cp_bar is not None:
        cp_bar.start()

    def out_tiles(routed, a, n, op):
        for t in range(16):
            @pl.when(((bits >> t) & 1) == routed)
            def _():
                col = pl.ds(128 * t, 128)
                op(pltpu.make_async_copy(obuf.at[pl.ds(a, n), col], out_hbm.at[pl.ds(a, n), col], sem_out))

    late = _DEV.get("late", {1: (0, 256), 3: (256, 256), 4: (512, 64)})

    u1, u2 = _DEV.get("u1", 28), NU

    def project(w, post, fill, frate):
        pend = []
        nt = F // 128
        lag = _DEV.get("flag", 0)
        done = 0
        for t in range(nt + lag):
            if t < nt:
                pend.append([jnp.dot(xsel_b[:, a:a + n], w[pl.ds(a, n), pl.ds(128 * t, 128)],
                                     preferred_element_type=F32)[:8] for a, n in k_rows])
            if t >= lag:
                ps = pend.pop(0)
                v = _rbf((ps[0] + ps[1]) + (ps[2] + ps[3]) + ps[4])
                ctok["elt"] = [v]
                post(t - lag, v)
            while fill and done * nt < (t + 1) * len(fill) * frate and done < len(fill):
                fill[done]()
                done += 1
        for fn in fill[done:]:
            fn()
        ctok["elt"] = []

    def elt_pieces(ks):
        out = []
        for k in ks:
            g = c_elt(_Idx(k, 0))
            out += [lambda g=g: next(g, None)] * (CB // 4)
        return out

    def post_gate(t, ga):
        hbuf[:, pl.ds(128 * t, 128)] = _rbf(ga * _rbf(jax.nn.sigmoid(ga)))

    def post_up(t, up):
        h = hbuf[:, pl.ds(128 * t, 128)] * up
        hpk[:, pl.ds(128 * t, 128)] = pltpu.bitcast(
            jnp.concatenate([h, jnp.zeros((8, 128), F32)], axis=0).astype(BF16), I32)

    cp_g.wait()
    xsel = xsel_ref[0]
    for c in range(1, C):
        xsel = xsel + xsel_ref[c]
    xsel_b = jnp.concatenate([xsel, jnp.zeros((8, D), F32)], axis=0).astype(BF16)
    ks = [k for k in range(NB - 3, NB) if k not in e1 and k not in e2]
    ng = _DEV.get("ng", 2)
    project(wg, post_gate, elt_pieces(ks[:ng]), _DEV.get("fr1", 1.0))
    o_gather(range(u1))
    cp_u.wait()
    project(wu, post_up, elt_pieces(ks[ng:]), _DEV.get("fr2", 2.5))
    o_gather(range(u1, 32))
    o_gather(range(32, u2))
    extract(spk, 1)
    pr = (r128 & (-16)) + 2 * (r128 & 7) + ((r128 >> 3) & 1)
    perm = jnp.where(pr == c128, 1.0, 0.0).astype(BF16)

    def patch(q, y):
        a, n = wd_rows[q]
        z = _rbf(xsel[:8, a:a + n] + _rbf(_rbf(y[:8]) * gate_r[:, :1]))
        g = z * _rbf(jax.nn.sigmoid(z))
        g = jnp.concatenate([g, jnp.zeros((120, n), F32)], axis=0).astype(BF16)
        gt = lax.dot_general(perm[:n, :n], g, _NT, preferred_element_type=F32)
        us = range(a // 16, (a + n) // 16)
        zz = newz()
        for u in us:
            hr = pl.ds(pl.multiple_of(zz + 8 * u, 8), 8)
            xx, ss = _unpack2(cols[0, hr, :]), _unpack2(cols[1, hr, :])
            r0 = 16 * u - a
            w = _pack2(*[xx[e] + _rbf(ss[e] * gt[r0 + 8 * e:r0 + 8 * e + 8]) for e in range(2)])
            for c, (tn, pn) in enumerate(nat):
                tt = 4 * (tn >> 2) + (tn & 3)
                pltpu.store(og.at[tt, pl.ds(8 * u, 8), :], pltpu.roll(w, (pn - c) & 127, 1), mask=lane8 == pn)
        for c, (tn, pn) in enumerate(nat):
            for u in us:
                v = og[tn, pl.ds(8 * u, 8), :]
                o_store(u, v, pl.ds(pl.multiple_of(tn * 128, 128), 128))
        if q in late:
            out_tiles(1, *late[q], lambda cp: cp.start())

    out_tiles(0, 0, D, lambda cp: cp.start())
    def down(q, f0, f1):
        a, n = wd_rows[q]
        return lax.dot_general(_bf(hpk[:, pl.ds(f0, f1 - f0)]), wd[pl.ds(a, n), pl.ds(f0, f1 - f0)], _NT,
                               preferred_element_type=F32)[:8]

    prev = None
    for q in range(len(wd_rows)):
        for k in waits.get(q, ()):
            cp_d[k].wait()
        fs = 0 if q in waits else 128 * _DEV.get("fs", {1: 10, 2: 10, 4: 20})[q]
        y0 = down(q, 0, fs) if fs else None
        if prev is not None:
            patch(*prev)
        y = down(q, fs, F)
        prev = (q, y if y0 is None else y0 + y)
    if _DEV.get("bar", 1):
        cp_bar.wait()
    patch(*prev)
    pltpu.make_async_copy(obuf, out_hbm, sem_out).wait()


def _scratch():
    return [
        pltpu.VMEM((D, L), BF16),
        pltpu.VMEM((6, D, N), BF16),
        pltpu.VMEM((D,), BF16),
        pltpu.VMEM((D,), BF16),
        pltpu.VMEM((D,), BF16),
        pltpu.VMEM((D, F), BF16),
        pltpu.VMEM((D, F), BF16),
        pltpu.VMEM((D, F), BF16),
        pltpu.VMEM((4, 64, 256), I32),
        pltpu.VMEM(_PROWS.shape, I32),
        pltpu.VMEM((_NPAT, 8, 128), I32),
        pltpu.VMEM((D, 128), F32),
        pltpu.VMEM((D, 128), F32),
        pltpu.VMEM((5, 2 * D, 128), I32),
        pltpu.VMEM((5, 2 * D, 128), I32),
        pltpu.VMEM((8, 2 * D, 128), I32),
        pltpu.VMEM((8, 2 * D, 128), I32),
        pltpu.VMEM((2, 4 * D, 128), F32),
        pltpu.VMEM((8, 4, D, 128), F32),
        pltpu.VMEM((16, D // 2, 128), I32),
        pltpu.VMEM((16, D // 2, 128), I32),
        pltpu.VMEM((8, 4, D, 128), F32),
        pltpu.VMEM((8, 2, D // 8, 8, 128), I32),
        pltpu.VMEM((8, 2, 2 * D, 128), F32),
        pltpu.VMEM((16, D // 2, 128), I32),
        pltpu.VMEM((3, 8, 128), F32),
        pltpu.VMEM((8, 128), I32),
        pltpu.VMEM((8, D), I32),
        pltpu.VMEM((8, 128), F32),
        pltpu.VMEM((C, 8, 128), I32),
        pltpu.VMEM((C, 8, D), F32),
        pltpu.VMEM((8, F), F32),
        pltpu.VMEM((8, F), I32),
        pltpu.VMEM((2, D // 2, 128), I32),
        pltpu.VMEM((16, D // 2, 128), I32),
        pltpu.VMEM((16, D // 2, 128), I32),
        pltpu.VMEM((D, L), BF16),
        pltpu.SemaphoreType.DMA((6 + len(_DEV.get("waits", {0: 0, 1: 0})),)),
        pltpu.SemaphoreType.DMA,
        pltpu.SemaphoreType.DMA,
    ] + [pltpu.VMEM((4, D // 2, 128), I32)] * 8 + [pltpu.VMEM((4, 24, 128), F32)] * 4


@jax.jit
def pallas_recurrent_scan__ssm_conv_s4__moe_arch_mod__prompt_kernel(
    A_u: jax.Array,
    A_A_re: jax.Array,
    A_A_im: jax.Array,
    A_B_re: jax.Array,
    A_B_im: jax.Array,
    A_C_re: jax.Array,
    A_C_im: jax.Array,
    A_log_dt: jax.Array,
    A_Dskip: jax.Array,
    B_x: jax.Array,
    B_w_r: jax.Array,
    B_w_gate: jax.Array,
    B_w_up: jax.Array,
    B_w_down: jax.Array,
):
    hbm = pl.BlockSpec(memory_space=pltpu.HBM)
    out = pl.pallas_call(
        _kernel,
        out_shape=jax.ShapeDtypeStruct((D, L), BF16),
        in_specs=[hbm] * 14,
        out_specs=hbm,
        scratch_shapes=_scratch(),
        compiler_params=pltpu.CompilerParams(vmem_limit_bytes=110 * 1024 * 1024),
        name="s4_mod",
    )(A_u[0].T, A_A_re, A_A_im, A_B_re, A_B_im, A_C_re, A_C_im, A_log_dt, A_Dskip, B_w_r,
      B_w_gate, B_w_up, B_w_down.T, jnp.asarray(_PROWS))
    return out.T[None]
```

```python
import numpy as np
import jax
import jax.numpy as jnp
from jax import lax
import jax.experimental.pallas as pl
import jax.experimental.pallas.tpu as pltpu

L, D, N, F, C = 2048, 576, 128, 4608, 8
NU = D // 16
CB = 64
NB = D // CB
UA = 4
F32, BF16, I32 = jnp.float32, jnp.bfloat16, jnp.int32
EPS = 1e-5


def _bf16_round_np(x):
    u = np.asarray(x, np.float32).view(np.uint32).astype(np.uint64)
    r = ((u + 0x7FFF + ((u >> 16) & 1)) >> 16) << 16
    return r.astype(np.uint32)


_LROUND = _bf16_round_np(np.arange(L)).view(np.float32).astype(np.int64)
_HI = [(1, 3, 516, 1032), (5, 7, 520, 1288), (4, 260, 772, 1544), (8, 264, 776, 1800), (2, 6, 258, 262)]


def _comp_q():
    t = np.arange(8)[:, None]
    lane = np.arange(128)[None, :]
    return ((lane - 8 - 7 * (t % 4)) % 16) // 4


def _make_tables():
    lane = np.arange(128)
    lo = 8 * (4 * (lane // 16) + lane % 4)
    tab = [dict(), dict()]
    amask = np.zeros(128, bool)
    for q in range(5):
        for e in range(4):
            for par in range(2):
                t = 4 * par + e
                for h in range(2):
                    src = lane[(lane // 4) % 4 == 2 * h + par]
                    dst = (src + (4 * (q % 4) - 8 * h + 8) + 7 * t) % 128
                    assert np.all(_comp_q()[t, dst] == q % 4)
                    sid = e if q < 4 else 4 + e // 2
                    for sl, dl_ in zip(src, dst):
                        ent = (sid, int(dl_))
                        assert tab[par].setdefault(_HI[q][e] + int(lo[sl]), ent) == ent
                    if q == 4 and e % 2 == 1:
                        amask[dst % 16 + 16 * np.arange(8)[:, None]] = True
    pats = []
    for j in range(4):
        pats.append(np.tile(4 * (lane % 32) + ((lane // 32) ^ j), (8, 1)))
    for j in range(4):
        pats.append(np.tile(32 * ((lane % 4) ^ j) + lane // 4, (8, 1)))
    npat0 = len(pats)
    tiles, tile_of = [], {}
    for dl in range(4):
        for l2 in range(4):
            v = _LROUND[512 * dl + 4 * lane + l2]
            key = tuple(v.tolist())
            if key in tile_of:
                tile_of[dl, l2] = tile_of[key]
                continue
            sid = np.array([tab[0][x][0] if x else -1 for x in v])
            ln = np.array([[tab[s8 % 2][x][1] if x else 0 for x in v] for s8 in range(8)])
            steps = []
            for s in sorted(set(sid.tolist()), key=lambda s: -(sid == s).sum()):
                lanes = np.nonzero(sid == s)[0]
                if s < 0:
                    steps.append((-1, None, lanes))
                    continue
                care = sid == s
                kk = None
                for k in range(npat0, len(pats)):
                    oldp, oldc, olds = pats[k]
                    both = care & oldc
                    if olds == s and np.array_equal(oldp[:, both], ln[:, both]):
                        pats[k] = (np.where(care, ln, oldp), care | oldc, s)
                        kk = k
                        break
                if kk is None:
                    pats.append((np.where(care, ln, 0), care, s))
                    kk = len(pats) - 1
                steps.append((s, kk, lanes))
            tiles.append(steps)
            tile_of[key] = tile_of[dl, l2] = len(tiles) - 1
    pats = np.stack([p if k < npat0 else p[0] for k, p in enumerate(pats)]).astype(np.int32)
    tile_of = {k: v for k, v in tile_of.items() if len(k) == 2}
    rows = np.concatenate([pats[:, :2].reshape(-1, 128), amask[None].astype(np.int32)])
    rows = np.concatenate([rows, np.zeros((-len(rows) % 8, 128), np.int32)])
    return tiles, tile_of, len(pats), rows


_TILES, _TILE_OF, _NGAT, _PROWS = _make_tables()
_NPAT = _NGAT + 3


def _cmul(ar, ai, br, bi):
    return ar * br - ai * bi, ar * bi + ai * br


def _sincos(b):
    magic = jnp.float32(12582912.0)
    t = b * jnp.float32(2.0 / np.pi) + magic
    k = t - magic
    ki = pltpu.bitcast(t, I32)
    r = b - k * jnp.float32(1.5703125)
    r = r - k * jnp.float32(0.0004837512969970703)
    r = r - k * jnp.float32(7.549790126404332e-08)
    u = r * r
    ps = (jnp.float32(-0.0001958295761141926) * u + jnp.float32(0.008332725614309311)) * u \
        + jnp.float32(-0.166666641831398)
    sn = r + (r * u) * ps
    pc = ((jnp.float32(2.437065268168226e-05) * u + jnp.float32(-0.0013886778615415096)) * u
          + jnp.float32(0.04166663438081741)) * u + jnp.float32(-0.5)
    cs = pc * u + jnp.float32(1.0)
    odd = (ki & 1) == 1
    s1 = jnp.where(odd, cs, sn)
    c1 = jnp.where(odd, sn, cs)
    sign = jnp.int32(-2147483648)
    s1 = pltpu.bitcast(pltpu.bitcast(s1, I32) ^ ((ki << 30) & sign), F32)
    c1 = pltpu.bitcast(pltpu.bitcast(c1, I32) ^ (((ki + 1) << 30) & sign), F32)
    return s1, c1


def _gather(x, idx):
    return jnp.take_along_axis(x, idx, axis=1, mode="promise_in_bounds")


def _lanes_mask(lanes):
    lane = lax.broadcasted_iota(I32, (8, 128), 1)
    lanes = sorted(int(x) for x in lanes)
    runs, start, prev = [], lanes[0], lanes[0]
    for x in lanes[1:]:
        if x != prev + 1:
            runs.append((start, prev))
            start = x
        prev = x
    runs.append((start, prev))
    m = None
    for a, b in runs:
        t = (lane == a) if a == b else jnp.logical_and(lane >= a, lane <= b)
        m = t if m is None else jnp.logical_or(m, t)
    return m


def _butterfly(p):
    lane = lax.broadcasted_iota(I32, p[0].shape, 1)
    b0 = (lane & 32) != 0
    b1 = (lane & 64) != 0
    t = [jnp.where(b0, p[k ^ 1], p[k]) for k in range(4)]
    return [jnp.where(b1, t[k ^ 2], t[k]) for k in range(4)]


def _fft4(x, sgn):
    (ar, ai), (br, bi), (cr, ci), (dr, di) = x
    s0r, s0i, d0r, d0i = ar + cr, ai + ci, ar - cr, ai - ci
    s1r, s1i, d1r, d1i = br + dr, bi + di, br - dr, bi - di
    y0 = (s0r + s1r, s0i + s1i)
    y2 = (s0r - s1r, s0i - s1i)
    p = (d0r - d1i, d0i + d1r)
    m = (d0r + d1i, d0i - d1r)
    return [y0, p, y2, m] if sgn > 0 else [y0, m, y2, p]


def _silu(z):
    h = z * jnp.float32(0.5)
    return h + h * jnp.tanh(h)


def _rbf(x):
    return x.astype(BF16).astype(F32)


def _pack2(a, b):
    p = pltpu.pack_elementwise([a, b], packed_dtype=BF16)
    return p if p.dtype == I32 else pltpu.bitcast(p, I32)


def _unpack2(x):
    return [pltpu.unpack_elementwise(x, index=i, packed_dtype=BF16, unpacked_dtype=F32) for i in range(2)]


def _bf(x):
    return pltpu.bitcast(x, BF16)


_NT = (((1,), (1,)), ((), ()))


class _Idx:
    def __init__(self, i, lag, z=None):
        self.i, self.lag, self.z = i, lag, z

    def off(self, stride, const=0, align=None):
        c = const - self.lag * stride
        if isinstance(self.i, int):
            if self.z is None:
                return self.i * stride + c
            v = self.z + (self.i * stride + c)
        else:
            v = self.i * stride + c
        return pl.multiple_of(v, align) if align else v

    def idx(self):
        return self.i - self.lag


def _pipeline(stages, n, newz, weave=None, reset=None):
    ns = len(stages)

    def step(i, lo, hi):
        z = newz() if isinstance(i, int) else None
        gens = {k: stages[k](_Idx(i, k, z)) for k in range(lo, hi)}
        if reset is not None:
            reset()
        if callable(weave):
            weave(gens)
        else:
            for k in weave or ():
                if k in gens:
                    next(gens[k], None)
        for k in range(hi - 1, lo - 1, -1):
            for _ in gens[k]:
                pass

    def body(i, carry):
        step(i, 0, ns)
        return carry

    return ([lambda i=i: step(i, 0, i + 1) for i in range(ns - 1)],
            lambda: lax.fori_loop(ns - 1, n, body, 0),
            [lambda i=i: step(n + i, i + 1, ns) for i in range(ns - 1)])


def _kernel(x_hbm, are_hbm, aim_hbm, bre_hbm, bim_hbm, cre_hbm, cim_hbm, ldt_hbm, dsk_hbm, wr_hbm,
            wg_hbm, wu_hbm, wd_hbm, pat_hbm,
            out_hbm,
            xbuf, par, ldt, dsk, wr, wg, wu, wd, fpk, prow, pats,
            dtcol, skip, hi_re, hi_im, lo_re, lo_im, comp, khat,
            xp, xnp, uhat, yhat, ybuf, spk, topk, posv, wr16b, wsum, ohb, xsel_ref, hbuf, hpk, cols, opk, og, obuf,
            sem_in, sem_out, sem_bar, *perb):
    xg, stat = perb[0:4], perb[4:8]
    p_hbm = (are_hbm, aim_hbm, bre_hbm, bim_hbm, cre_hbm, cim_hbm)
    r1 = 16 * UA
    small = [(ldt_hbm, ldt), (pat_hbm, prow), (dsk_hbm, dsk)]
    small += [(h.at[pl.ds(0, r1)], par.at[i, pl.ds(0, r1)]) for i, h in enumerate(p_hbm)]
    small += [(h.at[pl.ds(r1, D - r1)], par.at[i, pl.ds(r1, D - r1)]) for i, h in enumerate(p_hbm)]
    small += [(wr_hbm, wr)]
    cps = [pltpu.make_async_copy(s, d, sem_in.at[0 if i < 3 else 1 if i < 9 else 2])
           for i, (s, d) in enumerate(small)]
    ns = 3
    cp_x = pltpu.make_async_copy(x_hbm, xbuf, sem_in.at[ns])
    cp_g = pltpu.make_async_copy(wg_hbm, wg, sem_in.at[ns + 1])
    cp_u = pltpu.make_async_copy(wu_hbm, wu, sem_in.at[ns + 2])
    chunks = [(0, 128), (128, 128), (256, 128), (384, 128), (512, 64)]
    cp_d = [pltpu.make_async_copy(wd_hbm.at[pl.ds(a, n)], wd.at[pl.ds(a, n)], sem_in.at[ns + 3 + q // 3])
            for q, (a, n) in enumerate(chunks)]
    cp_bar = pltpu.make_async_copy(pat_hbm.at[pl.ds(0, 8)], posv, sem_bar)
    for cp in cps + [cp_x, cp_g, cp_u] + cp_d:
        cp.start()

    sub8 = lax.broadcasted_iota(I32, (8, 128), 0)
    lane8 = lax.broadcasted_iota(I32, (8, 128), 1)
    for l2 in range(4):
        for g in range(8):
            cs = []
            for e in range(2):
                p = 16 * g + 2 * sub8 + e
                t = 4 * (32 * ((p >> 5) ^ l2) + (p & 31)) + l2
                n = ((4 * lane8 + 1) * t) & 2047
                cs.append(_sincos(n.astype(F32) * jnp.float32(-2.0 * np.pi / 2048)))
            fpk[l2, pl.ds(8 * g, 8), pl.ds(0, 128)] = _pack2(cs[0][1], cs[1][1])
            fpk[l2, pl.ds(8 * g, 8), pl.ds(128, 128)] = _pack2(cs[0][0], cs[1][0])

    for cp in cps[:3]:
        cp.wait()
    for k in range(_NGAT):
        pats[k] = jnp.where((sub8 & 1) == 1, jnp.broadcast_to(prow[pl.ds(2 * k + 1, 1), :], (8, 128)),
                            jnp.broadcast_to(prow[pl.ds(2 * k, 1), :], (8, 128)))
    cq = ((lane8 - 8 - 7 * (sub8 & 3)) & 15) >> 2
    pats[_NGAT] = cq & 1
    pats[_NGAT + 1] = cq >> 1
    pats[_NGAT + 2] = jnp.broadcast_to(prow[pl.ds(2 * _NGAT, 1), :], (8, 128))
    r128 = lax.broadcasted_iota(I32, (128, 128), 0)
    c128 = lax.broadcasted_iota(I32, (128, 128), 1)
    eye = jnp.where(r128 == c128, 1.0, 0.0).astype(BF16)
    dt_row = jnp.exp(ldt[...].astype(F32).reshape(1, D)).astype(BF16)
    dsk_row = dsk[...].reshape(1, D)
    for t in range(5):
        n = min(128, D - 128 * t)
        for row, dst in ((dt_row, dtcol), (dsk_row, skip)):
            b = jnp.broadcast_to(row[:, 128 * t:128 * t + n], (128, n))
            dst[pl.ds(128 * t, n), :] = lax.dot_general(eye[:n, :n], b, _NT, preferred_element_type=F32)

    zero = prow[0, 0]
    zcount = [0]

    def newz():
        zcount[0] += 1
        return zero * (64 * zcount[0])

    def block(*fns):
        def body(k, carry):
            for fn in fns:
                fn()
            return carry

        lax.fori_loop(0, zero + 1, body, 0)

    def step_zero(i):
        t = i.off(1) * zero if not isinstance(i.i, int) or i.z is None else i.z
        return pl.multiple_of(t * 8, 8)

    def after(x, deps):
        never = pats[0] < 0
        d = None
        for v in deps:
            v = v if v.dtype == I32 else pltpu.bitcast(v, I32)
            d = v if d is None else d ^ v
        return jnp.where(never, d if x.dtype == I32 else pltpu.bitcast(d, x.dtype), x)

    def pad_tail(y, i):
        n, k = 16, y.shape[0] - 64
        base = i.off(1)
        mid = after(y[k:k + 8], [pats[j % _NPAT] * (base + j) for j in range(n)])
        return jnp.concatenate([y[:k], mid, y[k + 8:]], axis=0)

    class Sched:
        tok, g, pre = {}, 0, []

        @classmethod
        def reset(cls):
            cls.tok, cls.g, cls.pre = {}, 0, []

        @classmethod
        def gate(cls, x):
            deps = cls.tok.pop(cls.g, [])
            cls.g += 1
            if not deps:
                return x
            return jnp.concatenate([after(x[:8], deps), after(x[8:], deps[-1:])], axis=0)

    slot = {h: (q, e) for q, ent in enumerate(_HI) for e, h in enumerate(ent)}

    def a_prep(i):
        gate = Sched.gate
        for u in range(UA):
            rows = pl.ds(i.off(16 * UA, 16 * u, 16), 16)
            ev = pl.ds(i.off(32 * UA, 32 * u), 16, stride=2)
            od = pl.ds(i.off(32 * UA, 32 * u + 1), 16, stride=2)
            dt = gate(dtcol[rows, :])
            al = dt * par[0, rows, :].astype(F32)
            be = dt * par[1, rows, :].astype(F32)
            cr, ci = _cmul(par[4, rows, :].astype(F32), par[5, rows, :].astype(F32),
                           par[2, rows, :].astype(F32), par[3, rows, :].astype(F32))
            dts = dt * jnp.float32(1.0 / 512)
            cr, ci = cr * dts, ci * dts
            k0 = jnp.sum(cr, axis=1, keepdims=True) * jnp.float32(512.0)
            skip[rows, :] = skip[rows, :] + k0
            yield cr
            s, c = _sincos(gate(be))
            yield c
            pw = {1: (c, s)}
            e = 1
            while e < 256:
                if e in (1, 16):
                    c = gate(c)
                c, s = (c - s) * (c + s), (c + c) * s
                e *= 2
                pw[e] = (c, s)
                if e in (16, 256):
                    yield c
            z = {}
            for e in (1, 8, 256):
                mag = jnp.exp(al * jnp.float32(e))
                c, s = pw[e]
                z[e] = (mag * c, mag * s)
            pend = {}

            def put(tab, q, ee, v):
                key = (tab[0] is hi_re, q, ee // 2)
                if key not in pend:
                    pend[key] = (ee % 2, v)
                    return
                w, o = pend.pop(key)
                lo_, hi_ = (o, v) if w == 0 else (v, o)
                dst = od if ee // 2 else ev
                tab[0][q, dst, :] = _pack2(lo_[0], hi_[0])
                tab[1][q, dst, :] = _pack2(lo_[1], hi_[1])

            h = (cr, ci)
            cnt = 0
            for e in range(1, 9):
                g, ee, m = h, e, z[1]
                while ee in slot:
                    if cnt % 4 == 0:
                        g = (gate(g[0]), g[1])
                    g = _cmul(*g, *m)
                    put((hi_re, hi_im), *slot[ee], g)
                    if ee == e:
                        h = g
                    ee, m = ee + 256, z[256]
                    cnt += 1
                    if cnt % 4 == 0:
                        yield g[0]
            w1 = (gate(z[8][0]), -z[8][1])
            v = [(jnp.ones((16, 128), F32), jnp.zeros((16, 128), F32)), w1]
            v.append(_cmul(*w1, *w1))
            v.append(_cmul(*v[2], *w1))
            w4 = _cmul(*v[2], *v[2])
            for j in range(8):
                for f in range(4):
                    put((lo_re, lo_im), j, f, v[f])
                yield v[3][0]
                if j < 7:
                    w4 = (gate(w4[0]), w4[1])
                    v = [w4 if (j == 0 and f == 0) else _cmul(*v[f], *w4) for f in range(4)]

    def a_gen(i):
        b0 = pats[_NPAT - 3] != 0
        b1 = pats[_NPAT - 2] != 0
        for k in range(4 * UA):
            rows = pl.ds(i.off(32 * UA, 8 * k, 8), 8)
            lo = jnp.concatenate([lo_re[:, rows, :].reshape(64, 128), lo_im[:, rows, :].reshape(64, 128)], axis=1)
            h0 = hi_re[0, rows, :]
            if k % 2 == 0 and Sched.pre:
                h0 = after(h0, Sched.pre)
                Sched.pre = []
            hi = jnp.concatenate([jnp.concatenate([h0, hi_re[1:5, rows, :].reshape(32, 128)], axis=0),
                                  hi_im[:, rows, :].reshape(40, 128)], axis=1)
            o = lax.dot_general(_bf(hi), _bf(lo), _NT, preferred_element_type=F32)
            for q in range(5):
                Sched.tok.setdefault(13 + int(0.9 * (5 * (k // 2) + q)), []).append(o[16 * q + 8:16 * q + 16])
            for h in range(2):
                g = [pltpu.roll(o[16 * q + 8 * h:16 * q + 8 * h + 8], 4 * (q % 4) - 8 * h + 8, 1,
                                stride=7, stride_axis=0) for q in range(5)]
                dst = pl.ds(i.off(64 * UA, 16 * k + 8 * h, 8), 8)
                comp[0, dst, :] = jnp.where(b1, jnp.where(b0, g[3], g[2]), jnp.where(b0, g[1], g[0]))
                comp[1, dst, :] = g[4]
            if k % 2 == 1:
                yield

    def a_exp(i):
        bm = pats[_NPAT - 1] != 0
        srcs = []
        for u in range(UA):
            def ld(a, e):
                return _pack2(comp[a, pl.ds(i.off(64 * UA, 64 * u + e), 8, stride=4), :],
                              comp[a, pl.ds(i.off(64 * UA, 64 * u + 32 + e), 8, stride=4), :])

            srcs.append([ld(0, e) for e in range(4)]
                        + [jnp.where(bm, ld(1, 2 * k + 1), ld(1, 2 * k)) for k in range(2)])
        cache = {}

        def gat(s, key):
            if key not in cache:
                pat = pats[key]
                cache[key] = [_gather(srcs[u][s], pat) for u in range(UA)]
            return cache[key]

        tiles = []
        for steps in _TILES:
            t = None
            for s, key, lanes in steps:
                v = [jnp.zeros((8, 128), I32)] * UA if s < 0 else gat(s, key)
                t = v if t is None else [jnp.where(_lanes_mask(lanes), v[u], t[u]) for u in range(UA)]
            tiles.append(t)
        yield
        for u0 in range(0, UA, 2):
            lhs = [_bf(jnp.concatenate([tiles[_TILE_OF[dl, l2]][u] for dl in range(4) for u in (u0, u0 + 1)], axis=0))
                   for l2 in range(4)]
            z0 = 0 if u0 == 0 else zero * 8

            def dots(ri):
                return [jnp.dot(lhs[l2], _bf(jnp.concatenate(
                    [fpk[l2, pl.ds(z0 + 16 * (j ^ l2), 16) if u0 == 0 else
                         pl.ds(pl.multiple_of(z0 + 16 * (j ^ l2), 8), 16), pl.ds(128 * ri, 128)]
                     for j in range(4)], axis=0)), preferred_element_type=F32) for l2 in range(4)]

            def store(k2, ri, v):
                khat[2 * k2 + ri, :, pl.ds(i.off(16 * UA, 16 * u0, 16), 32), :] = v.reshape(4, 32, 128)

            def toks(v, step0):
                for j in range(8):
                    g = 13 + 9 * UA + int(0.7 * (step0 + j))
                    Sched.tok.setdefault(g, []).append(v[16 * j + 8:16 * j + 16])

            re = dots(0)
            s0, d0r, s1, d1r = re[0] + re[2], re[0] - re[2], re[1] + re[3], re[1] - re[3]
            store(0, 0, s0 + s1)
            v = s0 - s1
            store(2, 0, v)
            toks(v, 8 * u0)
            im = dots(1)
            s0, d0i, s1, d1i = im[0] + im[2], im[0] - im[2], im[1] + im[3], im[1] - im[3]
            store(0, 1, s0 + s1)
            store(2, 1, s0 - s1)
            store(1, 0, d0r + d1i)
            store(1, 1, d0i - d1r)
            store(3, 0, d0r - d1i)
            v = d0i + d1r
            store(3, 1, v)
            toks(v, 8 * u0 + 8)
            yield

    def a_weave(gens):
        if 2 in gens:
            next(gens[2])
        if 0 in gens and 1 in gens:
            for n in (3, 5, 4):
                for _ in range(n):
                    v = next(gens[0])
                Sched.pre = [v[:8], v[8:]]
                next(gens[1])
        for k in (1, 2, 0):
            if k in gens:
                for _ in gens[k]:
                    pass

    a_pro, a_loop, a_tail = _pipeline([a_prep, a_gen, a_exp], NU // UA, newz, reset=Sched.reset, weave=a_weave)
    for cp in cps[3:9]:
        cp.wait()
    a_pro[0]()
    for cp in cps[9:]:
        cp.wait()
    a_pro[1]()
    a_loop()

    cp_x.wait()

    def zrow(u):
        return pl.ds(pl.multiple_of(zero * 8 + 8 * u, 8), 8)

    def b_gather(b):
        for j in range(4):
            pat = pats[j]
            for u in range(NU):
                v = pltpu.bitcast(xbuf[pl.ds(16 * u, 16), pl.ds(512 * b + 128 * j, 128)], I32)
                xg[b][j, pl.ds(8 * u, 8), :] = _gather(v, pat)

    def b_stat(b):
        s2 = [jnp.zeros((8, 128), F32) for _ in range(4)]
        for u in range(NU):
            o = _butterfly([xg[b][j, zrow(u), :] for j in range(4)])
            for l2 in range(4):
                xp[4 * l2 + b, pl.ds(8 * u, 8), :] = o[l2]
                e_, o_ = _unpack2(o[l2])
                s2[l2] = s2[l2] + (e_ * e_ + o_ * o_)
        for l2 in range(4):
            stat[b][l2, pl.ds(16, 8), :] = s2[l2]

    def b_dot(b):
        lhs = _bf(wr16b[...])
        for j in range(4):
            rows = pl.ds(pl.multiple_of(zero * zero * 8, 8), D // 2)
            stat[b][j, pl.ds(0, 16), :] = jnp.dot(lhs, _bf(xg[b][j, rows, :]), preferred_element_type=F32)

    def b_fin(b):
        st = []
        wxs = _butterfly([stat[b][j, zrow(0), :] for j in range(4)])
        sxs = _butterfly([stat[b][j, zrow(1), :] for j in range(4)])
        for l2 in range(4):
            wx, sx = wxs[l2], sxs[l2]
            m = sx * jnp.float32(1.0 / D)
            q = jnp.sum(stat[b][l2, zrow(2), :], axis=0, keepdims=True) * jnp.float32(1.0 / D)
            var = _rbf(jnp.maximum(q - m * m, 0.0))
            rs = 1.0 / _rbf(jnp.sqrt(_rbf(var + jnp.float32(EPS))))
            mb = _rbf(m)
            st.append((mb, rs))
            r = _rbf((wx - mb * wsum[...]) * rs)
            r = jnp.where(r == 0.0, 0.0, r)
            bits = pltpu.bitcast(r, I32)
            mono = ((bits ^ ((bits >> 31) & jnp.int32(0x7FFFFFFF))) >> 16) + 32768
            tok = 512 * b + 4 * (32 * ((lane8 >> 5) ^ l2) + (lane8 & 31)) + l2
            key = pltpu.bitcast((mono << 11) + (2047 - tok) + jnp.int32(0x00800000), F32)
            t = 4 * b + l2
            topk[t // 8] = key if t % 8 == 0 else jnp.where(sub8 == t % 8, key, topk[t // 8])
        return st

    def b_norm(b):
        st = b_fin(b)
        for us in (range(CB // 16), range(CB // 16, NU)):
            for l2 in range(4):
                mb, rs = st[l2]
                for u in us:
                    e_, o_ = _unpack2(xp[4 * l2 + b, zrow(u), :])
                    xnp[4 * l2 + b, pl.ds(8 * u, 8), :] = _pack2((e_ - mb) * rs, (o_ - mb) * rs)

    wrow = wr[...].reshape(1, D)
    wr16b[...] = pltpu.bitcast(jnp.concatenate([jnp.broadcast_to(wrow, (8, D)), jnp.ones((8, D), BF16)], axis=0), I32)
    wsum[...] = jnp.broadcast_to(jnp.sum(wrow.astype(F32), axis=1, keepdims=True), (8, 128))
    topk[2] = jnp.zeros((8, 128), F32)
    cols[...] = jnp.zeros(cols.shape, I32)

    elt_dep = []

    def c_fwd(i):
        h0 = i.off(CB // 2, 0, 8)
        r0 = i.off(CB, 0, 8)
        for l2 in range(4):
            lhs = _bf(xnp[pl.ds(4 * l2, 4), pl.ds(h0, CB // 2), :].reshape(2 * CB, 128))
            res = jnp.dot(lhs, _bf(fpk[l2, pl.ds(step_zero(i), 64), :]), preferred_element_type=F32)
            for ri in range(2):
                y = res[:, 128 * ri:128 * ri + 128]
                if l2 == 3 and ri == 1 and isinstance(i.i, int) and i.i < 2:
                    y = pad_tail(y, i)
                uhat[2 * l2 + ri, :, pl.ds(r0, CB), :] = y.reshape(4, CB, 128)
            yield

    def c_mid(i):
        for k in range(CB // 8):
            rows = pl.ds(i.off(CB, 8 * k, 8), 8)
            krows = pl.ds(i.off(CB, 16 * (k // 2) + k % 2), 8, stride=2)
            uu = [_fft4([(uhat[2 * l2, b, rows, :], uhat[2 * l2 + 1, b, rows, :]) for l2 in range(4)], -1)
                  for b in range(4)]
            yy = [[None] * 4 for _ in range(4)]
            for k2s in ((0, 2), (1, 3)):
                pps = {k2: [None] * 4 for k2 in k2s}
                for k2, pp in pps.items():
                    for dl in range(3, -1, -1):
                        kk = (khat[2 * k2, dl, krows, :], khat[2 * k2 + 1, dl, krows, :])
                        for m in range(3, dl - 1, -1):
                            t = _cmul(*uu[m - dl][k2], *kk)
                            pp[m] = t if pp[m] is None else (pp[m][0] + t[0], pp[m][1] + t[1])
                for k2, pp in pps.items():
                    for m in range(3, -1, -1):
                        yy[m][k2] = pp[0] if m == 0 else (pp[m][0] - pp[m - 1][1], pp[m][1] + pp[m - 1][0])
            un = i.off(CB // 8, k)
            for bp in range(2):
                ww = [_fft4(yy[m], 1) for m in (2 * bp, 2 * bp + 1)]
                for l2 in range(4):
                    for ri in range(2):
                        yhat[2 * l2 + ri, bp, un] = _pack2(ww[0][l2][ri], ww[1][l2][ri])
            yield

    def c_inv(i):
        u0 = i.off(CB // 8)
        r0 = i.off(2 * CB, 0, 8)
        for l2 in range(4):
            for ri in range(2):
                lhs = _bf(yhat[2 * l2 + ri, :, pl.ds(u0, CB // 8)].reshape(2 * CB, 128))
                y = lax.dot_general(lhs, _bf(fpk[l2, pl.ds(step_zero(i), 64), pl.ds(128 * ri, 128)]), _NT,
                                    preferred_element_type=F32)
                if l2 == 3 and ri == 1 and isinstance(i.i, int):
                    y = pad_tail(y, i)
                ybuf[2 * l2 + ri, :, pl.ds(r0, 2 * CB), :] = y.reshape(2, 2 * CB, 128)
            yield

    def c_elt(i):
        for k in range(CB // 16):
            hr = pl.ds(i.off(CB // 2, 8 * k, 8), 8)
            sk = [skip[pl.ds(i.off(CB, 16 * k + e), 8, stride=2), :] for e in range(2)]
            for b in range(4):
                o = []
                for l2 in range(4):
                    w = xnp[4 * l2 + b, hr, :]
                    if elt_dep:
                        w = after(w, elt_dep)
                    xn = _unpack2(w)
                    xx = _unpack2(xp[4 * l2 + b, hr, :])
                    ss, v = [], []
                    for e in range(2):
                        yr = pl.ds(i.off(2 * CB, 32 * k + 2 * e + b % 2), 8, stride=4)
                        ss.append(ybuf[2 * l2, b // 2, yr, :] + ybuf[2 * l2 + 1, b // 2, yr, :] + xn[e] * sk[e])
                        v.append(xx[e] + ss[e] * _silu(xn[e]))
                    spk[4 * l2 + b, hr, :] = _pack2(*ss)
                    o.append(_pack2(*v))
                p = _butterfly(o)
                for j in range(4):
                    opk[4 * b + j, hr, :] = p[j]
                yield

    def c_top(i):
        k0, k1 = topk[i.off(0, 0)], topk[i.off(0, 1)]
        mx = jnp.max(jnp.max(jnp.maximum(k0, k1), axis=0, keepdims=True), axis=1, keepdims=True)
        topk[i.off(0, 0)] = jnp.where(k0 == mx, 0.0, k0)
        topk[i.off(0, 1)] = jnp.where(k1 == mx, 0.0, k1)
        topk[i.off(0, 2)] = jnp.where(sub8 == i.idx(), mx, topk[i.off(0, 2)])
        yield

    def c_first(i):
        yield from c_fwd(i)
        yield from c_top(i)

    c_pro, c_loop, _ = _pipeline([c_first, c_mid, c_inv, c_elt], NB, newz,
                                 weave=[1] * (CB // 8) + [3] * (CB // 4) + [0, 0, 2, 2, 0, 0, 2, 2])

    def first_fwd():
        for _ in c_first(_Idx(0, 0)):
            pass

    def each(fn, *bs):
        return [lambda b=b: fn(b) for b in bs]

    block(a_tail[0], *each(b_gather, 0, 1))
    block(a_tail[1], *each(b_gather, 2, 3), *each(b_dot, 0, 1), *each(b_stat, 0, 1))
    block(*each(b_stat, 2, 3), *each(b_norm, 0, 1), *each(b_dot, 2, 3))
    block(*each(b_norm, 2, 3), first_fwd)
    block(c_pro[1])
    block(c_pro[2])
    c_loop()

    sel = pltpu.bitcast(topk[2], I32) - jnp.int32(0x00800000)
    mono = (sel >> 11) - 32768
    r_sel = pltpu.bitcast((mono ^ ((mono >> 31) & jnp.int32(0x7FFF))) << 16, F32)
    gate_r = _rbf(jax.nn.sigmoid(r_sel))
    posv[...] = 2047 - (sel & 2047)
    tok = [posv[c, 0] for c in range(C)]
    nat = [(t >> 7, t & 127) for t in tok]
    prm = []
    for t in tok:
        l2, l1 = t & 3, (t >> 2) & 127
        prm.append((4 * l2 + (t >> 9), 32 * ((l1 >> 5) ^ l2) + (l1 & 31)))

    def extract(src, k):
        for c, (tp, pp) in enumerate(prm):
            sh = (c - pp) & 127
            for u in range(NU):
                pltpu.store(cols.at[k, pl.ds(8 * u, 8), :], pltpu.roll(src[tp, pl.ds(8 * u, 8), :], sh, 1),
                            mask=lane8 == c)

    for c, (tp, pp) in enumerate(prm):
        ohb[c] = jnp.where(jnp.logical_and(sub8 == c // 2, lane8 == pp), jnp.int32(0x3F80 << (16 * (c % 2))), 0)

    def take_rows():
        for c, (tp, pp) in enumerate(prm):
            xsel_ref[c] = lax.dot_general(_bf(ohb[c]), _bf(xnp[tp]), _NT, preferred_element_type=F32)[:8]

    def stages(*items):
        def run():
            z = newz()
            for fn, k in items:
                for _ in fn(_Idx(k, 0, z)):
                    pass
        return run

    block(stages((c_mid, NB - 1), (c_inv, NB - 2)))
    block(stages((c_elt, NB - 3), (c_inv, NB - 1)), take_rows, lambda: extract(xp, 0))

    def o_gather(us):
        for j in range(4):
            pat = pats[4 + j]
            for b in range(4):
                for u in us:
                    v = _gather(opk[4 * b + j, pl.ds(8 * u, 8), :], pat)
                    og[4 * b + j, pl.ds(8 * u, 8), :] = v
                    o_store(u, v, pl.ds(512 * b + 128 * j, 128))

    def o_store(u, v, col):
        obuf[pl.ds(16 * u, 8), col] = _bf(v[0:4])
        obuf[pl.ds(16 * u + 8, 8), col] = _bf(pltpu.roll(v, 4, 0)[0:4])

    bits = jnp.int32(0)
    for c in range(C):
        bits = bits | (jnp.int32(1) << nat[c][0])

    cp_bar.start()

    def send(routed, a, n):
        for t in range(16):
            @pl.when(((bits >> t) & 1) == routed)
            def _():
                col = pl.ds(128 * t, 128)
                pltpu.make_async_copy(obuf.at[pl.ds(a, n), col], out_hbm.at[pl.ds(a, n), col], sem_out).start()

    late = {1: (0, 256), 3: (256, 256), 4: (512, 64)}

    def project(w, post, ks):
        fill = [g for k in ks for g in [c_elt(_Idx(k, 0))] * (CB // 4)]
        nt, done = F // 128, 0
        for t in range(nt):
            ps = [jnp.dot(xsel_b[:, a:a + n], w[pl.ds(a, n), pl.ds(128 * t, 128)],
                          preferred_element_type=F32)[:8] for a, n in chunks]
            v = _rbf((ps[0] + ps[1]) + (ps[2] + ps[3]) + ps[4])
            elt_dep[:] = [v]
            post(t, v)
            while done * nt < (t + 1) * len(fill):
                next(fill[done], None)
                done += 1
        elt_dep.clear()

    def post_gate(t, ga):
        hbuf[:, pl.ds(128 * t, 128)] = _rbf(ga * _rbf(jax.nn.sigmoid(ga)))

    def post_up(t, up):
        h = hbuf[:, pl.ds(128 * t, 128)] * up
        hpk[:, pl.ds(128 * t, 128)] = pltpu.bitcast(
            jnp.concatenate([h, jnp.zeros((8, 128), F32)], axis=0).astype(BF16), I32)

    cp_g.wait()
    xsel = xsel_ref[0]
    for c in range(1, C):
        xsel = xsel + xsel_ref[c]
    xsel_b = jnp.concatenate([xsel, jnp.zeros((8, D), F32)], axis=0).astype(BF16)
    project(wg, post_gate, (NB - 2, NB - 1))
    o_gather(range(28))
    cp_u.wait()
    project(wu, post_up, ())
    o_gather(range(28, 32))
    o_gather(range(32, NU))
    extract(spk, 1)
    pr = (r128 & (-16)) + 2 * (r128 & 7) + ((r128 >> 3) & 1)
    perm = jnp.where(pr == c128, 1.0, 0.0).astype(BF16)

    def patch(q, y):
        a, n = chunks[q]
        z = _rbf(xsel[:8, a:a + n] + _rbf(_rbf(y[:8]) * gate_r[:, :1]))
        g = z * _rbf(jax.nn.sigmoid(z))
        g = jnp.concatenate([g, jnp.zeros((120, n), F32)], axis=0).astype(BF16)
        gt = lax.dot_general(perm[:n, :n], g, _NT, preferred_element_type=F32)
        us = range(a // 16, (a + n) // 16)
        zz = newz()
        for u in us:
            hr = pl.ds(pl.multiple_of(zz + 8 * u, 8), 8)
            xx, ss = _unpack2(cols[0, hr, :]), _unpack2(cols[1, hr, :])
            r0 = 16 * u - a
            w = _pack2(*[xx[e] + _rbf(ss[e] * gt[r0 + 8 * e:r0 + 8 * e + 8]) for e in range(2)])
            for c, (tn, pn) in enumerate(nat):
                tt = 4 * (tn >> 2) + (tn & 3)
                pltpu.store(og.at[tt, pl.ds(8 * u, 8), :], pltpu.roll(w, (pn - c) & 127, 1), mask=lane8 == pn)
        for c, (tn, pn) in enumerate(nat):
            for u in us:
                v = og[tn, pl.ds(8 * u, 8), :]
                o_store(u, v, pl.ds(pl.multiple_of(tn * 128, 128), 128))
        if q in late:
            send(1, *late[q])

    send(0, 0, D)
    def down(q, f0, f1):
        a, n = chunks[q]
        return lax.dot_general(_bf(hpk[:, pl.ds(f0, f1 - f0)]), wd[pl.ds(a, n), pl.ds(f0, f1 - f0)], _NT,
                               preferred_element_type=F32)[:8]

    prev = None
    for q, fs in enumerate((0, 1280, 1280, 0, 2560)):
        if q % 3 == 0:
            for cp in cp_d[q:q + 3]:
                cp.wait()
        y0 = down(q, 0, fs) if fs else None
        if prev is not None:
            patch(*prev)
        y = down(q, fs, F)
        prev = (q, y if y0 is None else y0 + y)
    cp_bar.wait()
    patch(*prev)
    pltpu.make_async_copy(obuf, out_hbm, sem_out).wait()


def _scratch():
    return [
        pltpu.VMEM((D, L), BF16),
        pltpu.VMEM((6, D, N), BF16),
        pltpu.VMEM((D,), BF16),
        pltpu.VMEM((D,), BF16),
        pltpu.VMEM((D,), BF16),
        pltpu.VMEM((D, F), BF16),
        pltpu.VMEM((D, F), BF16),
        pltpu.VMEM((D, F), BF16),
        pltpu.VMEM((4, 64, 256), I32),
        pltpu.VMEM(_PROWS.shape, I32),
        pltpu.VMEM((_NPAT, 8, 128), I32),
        pltpu.VMEM((D, 128), F32),
        pltpu.VMEM((D, 128), F32),
        pltpu.VMEM((5, 2 * D, 128), I32),
        pltpu.VMEM((5, 2 * D, 128), I32),
        pltpu.VMEM((8, 2 * D, 128), I32),
        pltpu.VMEM((8, 2 * D, 128), I32),
        pltpu.VMEM((2, 4 * D, 128), F32),
        pltpu.VMEM((8, 4, D, 128), F32),
        pltpu.VMEM((16, D // 2, 128), I32),
        pltpu.VMEM((16, D // 2, 128), I32),
        pltpu.VMEM((8, 4, D, 128), F32),
        pltpu.VMEM((8, 2, D // 8, 8, 128), I32),
        pltpu.VMEM((8, 2, 2 * D, 128), F32),
        pltpu.VMEM((16, D // 2, 128), I32),
        pltpu.VMEM((3, 8, 128), F32),
        pltpu.VMEM((8, 128), I32),
        pltpu.VMEM((8, D), I32),
        pltpu.VMEM((8, 128), F32),
        pltpu.VMEM((C, 8, 128), I32),
        pltpu.VMEM((C, 8, D), F32),
        pltpu.VMEM((8, F), F32),
        pltpu.VMEM((8, F), I32),
        pltpu.VMEM((2, D // 2, 128), I32),
        pltpu.VMEM((16, D // 2, 128), I32),
        pltpu.VMEM((16, D // 2, 128), I32),
        pltpu.VMEM((D, L), BF16),
        pltpu.SemaphoreType.DMA((8,)),
        pltpu.SemaphoreType.DMA,
        pltpu.SemaphoreType.DMA,
    ] + [pltpu.VMEM((4, D // 2, 128), I32)] * 4 + [pltpu.VMEM((4, 24, 128), F32)] * 4


@jax.jit
def pallas_recurrent_scan__ssm_conv_s4__moe_arch_mod__prompt_kernel(
    A_u: jax.Array,
    A_A_re: jax.Array,
    A_A_im: jax.Array,
    A_B_re: jax.Array,
    A_B_im: jax.Array,
    A_C_re: jax.Array,
    A_C_im: jax.Array,
    A_log_dt: jax.Array,
    A_Dskip: jax.Array,
    B_x: jax.Array,
    B_w_r: jax.Array,
    B_w_gate: jax.Array,
    B_w_up: jax.Array,
    B_w_down: jax.Array,
):
    hbm = pl.BlockSpec(memory_space=pltpu.HBM)
    out = pl.pallas_call(
        _kernel,
        out_shape=jax.ShapeDtypeStruct((D, L), BF16),
        in_specs=[hbm] * 14,
        out_specs=hbm,
        scratch_shapes=_scratch(),
        compiler_params=pltpu.CompilerParams(vmem_limit_bytes=110 * 1024 * 1024),
        name="s4_mod",
    )(A_u[0].T, A_A_re, A_A_im, A_B_re, A_B_im, A_C_re, A_C_im, A_log_dt, A_Dskip, B_w_r,
      B_w_gate, B_w_up, B_w_down.T, jnp.asarray(_PROWS))
    return out.T[None]
```

```python
import numpy as np
import jax
import jax.numpy as jnp
from jax import lax
import jax.experimental.pallas as pl
import jax.experimental.pallas.tpu as pltpu

L, D, N, F, C = 2048, 576, 128, 4608, 8
NU = D // 16
CB = 64
NB = D // CB
UA = 4
F32, BF16, I32 = jnp.float32, jnp.bfloat16, jnp.int32
EPS = 1e-5


def _bf16_round_np(x):
    u = np.asarray(x, np.float32).view(np.uint32).astype(np.uint64)
    r = ((u + 0x7FFF + ((u >> 16) & 1)) >> 16) << 16
    return r.astype(np.uint32)


_LROUND = _bf16_round_np(np.arange(L)).view(np.float32).astype(np.int64)
_HI = [(1, 3, 516, 1032), (5, 7, 520, 1288), (4, 260, 772, 1544), (8, 264, 776, 1800), (2, 6, 258, 262)]


def _comp_q():
    t = np.arange(8)[:, None]
    lane = np.arange(128)[None, :]
    return ((lane - 8 - 7 * (t % 4)) % 16) // 4


def _make_tables():
    lane = np.arange(128)
    lo = 8 * (4 * (lane // 16) + lane % 4)
    tab = [dict(), dict()]
    amask = np.zeros(128, bool)
    for q in range(5):
        for e in range(4):
            for par in range(2):
                t = 4 * par + e
                for h in range(2):
                    src = lane[(lane // 4) % 4 == 2 * h + par]
                    dst = (src + (4 * (q % 4) - 8 * h + 8) + 7 * t) % 128
                    assert np.all(_comp_q()[t, dst] == q % 4)
                    sid = e if q < 4 else 4 + e // 2
                    for sl, dl_ in zip(src, dst):
                        ent = (sid, int(dl_))
                        assert tab[par].setdefault(_HI[q][e] + int(lo[sl]), ent) == ent
                    if q == 4 and e % 2 == 1:
                        amask[dst % 16 + 16 * np.arange(8)[:, None]] = True
    pats = []
    for j in range(4):
        pats.append(np.tile(4 * (lane % 32) + ((lane // 32) ^ j), (8, 1)))
    for j in range(4):
        pats.append(np.tile(32 * ((lane % 4) ^ j) + lane // 4, (8, 1)))
    npat0 = len(pats)
    tiles, tile_of = [], {}
    for dl in range(4):
        for l2 in range(4):
            v = _LROUND[512 * dl + 4 * lane + l2]
            key = tuple(v.tolist())
            if key in tile_of:
                tile_of[dl, l2] = tile_of[key]
                continue
            sid = np.array([tab[0][x][0] if x else -1 for x in v])
            ln = np.array([[tab[s8 % 2][x][1] if x else 0 for x in v] for s8 in range(8)])
            steps = []
            for s in sorted(set(sid.tolist()), key=lambda s: -(sid == s).sum()):
                lanes = np.nonzero(sid == s)[0]
                if s < 0:
                    steps.append((-1, None, lanes))
                    continue
                care = sid == s
                kk = None
                for k in range(npat0, len(pats)):
                    oldp, oldc, olds = pats[k]
                    both = care & oldc
                    if olds == s and np.array_equal(oldp[:, both], ln[:, both]):
                        pats[k] = (np.where(care, ln, oldp), care | oldc, s)
                        kk = k
                        break
                if kk is None:
                    pats.append((np.where(care, ln, 0), care, s))
                    kk = len(pats) - 1
                steps.append((s, kk, lanes))
            tiles.append(steps)
            tile_of[key] = tile_of[dl, l2] = len(tiles) - 1
    pats = np.stack([p if k < npat0 else p[0] for k, p in enumerate(pats)]).astype(np.int32)
    tile_of = {k: v for k, v in tile_of.items() if len(k) == 2}
    rows = np.concatenate([pats[:, :2].reshape(-1, 128), amask[None].astype(np.int32)])
    rows = np.concatenate([rows, np.zeros((-len(rows) % 8, 128), np.int32)])
    return tiles, tile_of, len(pats), rows


_TILES, _TILE_OF, _NGAT, _PROWS = _make_tables()
_NPAT = _NGAT + 3


def _cmul(ar, ai, br, bi):
    return ar * br - ai * bi, ar * bi + ai * br


def _sincos(b):
    magic = jnp.float32(12582912.0)
    t = b * jnp.float32(2.0 / np.pi) + magic
    k = t - magic
    ki = pltpu.bitcast(t, I32)
    r = b - k * jnp.float32(1.5703125)
    r = r - k * jnp.float32(0.0004837512969970703)
    r = r - k * jnp.float32(7.549790126404332e-08)
    u = r * r
    ps = (jnp.float32(-0.0001958295761141926) * u + jnp.float32(0.008332725614309311)) * u \
        + jnp.float32(-0.166666641831398)
    sn = r + (r * u) * ps
    pc = ((jnp.float32(2.437065268168226e-05) * u + jnp.float32(-0.0013886778615415096)) * u
          + jnp.float32(0.04166663438081741)) * u + jnp.float32(-0.5)
    cs = pc * u + jnp.float32(1.0)
    odd = (ki & 1) == 1
    s1 = jnp.where(odd, cs, sn)
    c1 = jnp.where(odd, sn, cs)
    sign = jnp.int32(-2147483648)
    s1 = pltpu.bitcast(pltpu.bitcast(s1, I32) ^ ((ki << 30) & sign), F32)
    c1 = pltpu.bitcast(pltpu.bitcast(c1, I32) ^ (((ki + 1) << 30) & sign), F32)
    return s1, c1


def _gather(x, idx):
    return jnp.take_along_axis(x, idx, axis=1, mode="promise_in_bounds")


def _lanes_mask(lanes):
    lane = lax.broadcasted_iota(I32, (8, 128), 1)
    lanes = sorted(int(x) for x in lanes)
    runs, start, prev = [], lanes[0], lanes[0]
    for x in lanes[1:]:
        if x != prev + 1:
            runs.append((start, prev))
            start = x
        prev = x
    runs.append((start, prev))
    m = None
    for a, b in runs:
        t = (lane == a) if a == b else jnp.logical_and(lane >= a, lane <= b)
        m = t if m is None else jnp.logical_or(m, t)
    return m


def _butterfly(p):
    lane = lax.broadcasted_iota(I32, p[0].shape, 1)
    b0 = (lane & 32) != 0
    b1 = (lane & 64) != 0
    t = [jnp.where(b0, p[k ^ 1], p[k]) for k in range(4)]
    return [jnp.where(b1, t[k ^ 2], t[k]) for k in range(4)]


def _fft4(x, sgn):
    (ar, ai), (br, bi), (cr, ci), (dr, di) = x
    s0r, s0i, d0r, d0i = ar + cr, ai + ci, ar - cr, ai - ci
    s1r, s1i, d1r, d1i = br + dr, bi + di, br - dr, bi - di
    y0 = (s0r + s1r, s0i + s1i)
    y2 = (s0r - s1r, s0i - s1i)
    p = (d0r - d1i, d0i + d1r)
    m = (d0r + d1i, d0i - d1r)
    return [y0, p, y2, m] if sgn > 0 else [y0, m, y2, p]


def _silu(z):
    h = z * jnp.float32(0.5)
    return h + h * jnp.tanh(h)


def _rbf(x):
    return x.astype(BF16).astype(F32)


def _pack2(a, b):
    p = pltpu.pack_elementwise([a, b], packed_dtype=BF16)
    return p if p.dtype == I32 else pltpu.bitcast(p, I32)


def _unpack2(x):
    return [pltpu.unpack_elementwise(x, index=i, packed_dtype=BF16, unpacked_dtype=F32) for i in range(2)]


def _bf(x):
    return pltpu.bitcast(x, BF16)


_NT = (((1,), (1,)), ((), ()))


class _Idx:
    def __init__(self, i, lag, z=None):
        self.i, self.lag, self.z = i, lag, z

    def off(self, stride, const=0, align=None):
        c = const - self.lag * stride
        if isinstance(self.i, int):
            if self.z is None:
                return self.i * stride + c
            v = self.z + (self.i * stride + c)
        else:
            v = self.i * stride + c
        return pl.multiple_of(v, align) if align else v

    def idx(self):
        return self.i - self.lag


def _pipeline(stages, n, newz, weave=None, reset=None):
    ns = len(stages)

    def step(i, lo, hi):
        z = newz() if isinstance(i, int) else None
        gens = {k: stages[k](_Idx(i, k, z)) for k in range(lo, hi)}
        if reset is not None:
            reset()
        if callable(weave):
            weave(gens)
        else:
            for k in weave or ():
                if k in gens:
                    next(gens[k], None)
        for k in range(hi - 1, lo - 1, -1):
            for _ in gens[k]:
                pass

    def body(i, carry):
        step(i, 0, ns)
        return carry

    return ([lambda i=i: step(i, 0, i + 1) for i in range(ns - 1)],
            lambda: lax.fori_loop(ns - 1, n, body, 0),
            [lambda i=i: step(n + i, i + 1, ns) for i in range(ns - 1)])


def _kernel(x_hbm, are_hbm, aim_hbm, bre_hbm, bim_hbm, cre_hbm, cim_hbm, ldt_hbm, dsk_hbm, wr_hbm,
            wg_hbm, wu_hbm, wd_hbm, pat_hbm,
            out_hbm,
            xbuf, par, ldt, dsk, wr, wg, wu, wd, fpk, prow, pats,
            dtcol, skip, hi_re, hi_im, lo_re, lo_im, comp, khat,
            xp, xnp, uhat, yhat, ybuf, spk, topk, posv, wr16b, wsum, ohb, xsel_ref, hbuf, hpk, cols, opk, og, obuf,
            sem_in, sem_out, sem_bar, *perb):
    xg, stat = perb[0:4], perb[4:8]
    p_hbm = (are_hbm, aim_hbm, bre_hbm, bim_hbm, cre_hbm, cim_hbm)
    r1 = 16 * UA
    small = [(ldt_hbm, ldt), (pat_hbm, prow), (dsk_hbm, dsk)]
    for a, n in ((0, r1), (r1, r1), (2 * r1, D - 2 * r1)):
        small += [(h.at[pl.ds(a, n)], par.at[i, pl.ds(a, n)]) for i, h in enumerate(p_hbm)]
    small += [(wr_hbm, wr)]
    cps = [pltpu.make_async_copy(s, d, sem_in.at[min((i + 3) // 6, 3)]) for i, (s, d) in enumerate(small)]
    ns = 4
    cp_x = pltpu.make_async_copy(x_hbm, xbuf, sem_in.at[ns])
    cp_g = pltpu.make_async_copy(wg_hbm, wg, sem_in.at[ns + 1])
    cp_u = pltpu.make_async_copy(wu_hbm, wu, sem_in.at[ns + 2])
    chunks = [(0, 128), (128, 128), (256, 128), (384, 128), (512, 64)]
    cp_d = [pltpu.make_async_copy(wd_hbm.at[pl.ds(a, n)], wd.at[pl.ds(a, n)], sem_in.at[ns + 3 + q // 3])
            for q, (a, n) in enumerate(chunks)]
    cp_bar = pltpu.make_async_copy(pat_hbm.at[pl.ds(0, 8)], posv, sem_bar)
    for cp in cps + [cp_x, cp_g, cp_u] + cp_d:
        cp.start()

    sub8 = lax.broadcasted_iota(I32, (8, 128), 0)
    lane8 = lax.broadcasted_iota(I32, (8, 128), 1)
    for l2 in range(4):
        for g in range(8):
            cs = []
            for e in range(2):
                p = 16 * g + 2 * sub8 + e
                t = 4 * (32 * ((p >> 5) ^ l2) + (p & 31)) + l2
                n = ((4 * lane8 + 1) * t) & 2047
                cs.append(_sincos(n.astype(F32) * jnp.float32(-2.0 * np.pi / 2048)))
            fpk[l2, pl.ds(8 * g, 8), pl.ds(0, 128)] = _pack2(cs[0][1], cs[1][1])
            fpk[l2, pl.ds(8 * g, 8), pl.ds(128, 128)] = _pack2(cs[0][0], cs[1][0])

    for cp in cps[:3]:
        cp.wait()
    for k in range(_NGAT):
        pats[k] = jnp.where((sub8 & 1) == 1, jnp.broadcast_to(prow[pl.ds(2 * k + 1, 1), :], (8, 128)),
                            jnp.broadcast_to(prow[pl.ds(2 * k, 1), :], (8, 128)))
    cq = ((lane8 - 8 - 7 * (sub8 & 3)) & 15) >> 2
    pats[_NGAT] = cq & 1
    pats[_NGAT + 1] = cq >> 1
    pats[_NGAT + 2] = jnp.broadcast_to(prow[pl.ds(2 * _NGAT, 1), :], (8, 128))
    r128 = lax.broadcasted_iota(I32, (128, 128), 0)
    c128 = lax.broadcasted_iota(I32, (128, 128), 1)
    eye = jnp.where(r128 == c128, 1.0, 0.0).astype(BF16)
    dt_row = jnp.exp(ldt[...].astype(F32).reshape(1, D)).astype(BF16)
    dsk_row = dsk[...].reshape(1, D)
    for t in range(5):
        n = min(128, D - 128 * t)
        for row, dst in ((dt_row, dtcol), (dsk_row, skip)):
            b = jnp.broadcast_to(row[:, 128 * t:128 * t + n], (128, n))
            dst[pl.ds(128 * t, n), :] = lax.dot_general(eye[:n, :n], b, _NT, preferred_element_type=F32)

    zero = prow[0, 0]
    zcount = [0]

    def newz():
        zcount[0] += 1
        return zero * (64 * zcount[0])

    def block(*fns):
        def body(k, carry):
            for fn in fns:
                fn()
            return carry

        lax.fori_loop(0, zero + 1, body, 0)

    def step_zero(i):
        t = i.off(1) * zero if not isinstance(i.i, int) or i.z is None else i.z
        return pl.multiple_of(t * 8, 8)

    def after(x, deps):
        never = pats[0] < 0
        d = None
        for v in deps:
            v = v if v.dtype == I32 else pltpu.bitcast(v, I32)
            d = v if d is None else d ^ v
        return jnp.where(never, d if x.dtype == I32 else pltpu.bitcast(d, x.dtype), x)

    def pad_tail(y, i):
        n, k = 16, y.shape[0] - 64
        base = i.off(1)
        mid = after(y[k:k + 8], [pats[j % _NPAT] * (base + j) for j in range(n)])
        return jnp.concatenate([y[:k], mid, y[k + 8:]], axis=0)

    class Sched:
        tok, g, pre = {}, 0, []

        @classmethod
        def reset(cls):
            cls.tok, cls.g, cls.pre = {}, 0, []

        @classmethod
        def gate(cls, x):
            deps = cls.tok.pop(cls.g, [])
            cls.g += 1
            if not deps:
                return x
            return jnp.concatenate([after(x[:8], deps), after(x[8:], deps[-1:])], axis=0)

    slot = {h: (q, e) for q, ent in enumerate(_HI) for e, h in enumerate(ent)}

    def a_prep(i):
        gate = Sched.gate
        for u in range(UA):
            rows = pl.ds(i.off(16 * UA, 16 * u, 16), 16)
            ev = pl.ds(i.off(32 * UA, 32 * u), 16, stride=2)
            od = pl.ds(i.off(32 * UA, 32 * u + 1), 16, stride=2)
            dt = gate(dtcol[rows, :])
            al = dt * par[0, rows, :].astype(F32)
            be = dt * par[1, rows, :].astype(F32)
            cr, ci = _cmul(par[4, rows, :].astype(F32), par[5, rows, :].astype(F32),
                           par[2, rows, :].astype(F32), par[3, rows, :].astype(F32))
            dts = dt * jnp.float32(1.0 / 512)
            cr, ci = cr * dts, ci * dts
            k0 = jnp.sum(cr, axis=1, keepdims=True) * jnp.float32(512.0)
            skip[rows, :] = skip[rows, :] + k0
            yield cr
            s, c = _sincos(gate(be))
            yield c
            pw = {1: (c, s)}
            e = 1
            while e < 256:
                if e in (1, 16):
                    c = gate(c)
                c, s = (c - s) * (c + s), (c + c) * s
                e *= 2
                pw[e] = (c, s)
                if e in (16, 256):
                    yield c
            z = {}
            for e in (1, 8, 256):
                mag = jnp.exp(al * jnp.float32(e))
                c, s = pw[e]
                z[e] = (mag * c, mag * s)
            pend = {}

            def put(tab, q, ee, v):
                key = (tab[0] is hi_re, q, ee // 2)
                if key not in pend:
                    pend[key] = (ee % 2, v)
                    return
                w, o = pend.pop(key)
                lo_, hi_ = (o, v) if w == 0 else (v, o)
                dst = od if ee // 2 else ev
                tab[0][q, dst, :] = _pack2(lo_[0], hi_[0])
                tab[1][q, dst, :] = _pack2(lo_[1], hi_[1])

            h = (cr, ci)
            cnt = 0
            for e in range(1, 9):
                g, ee, m = h, e, z[1]
                while ee in slot:
                    if cnt % 4 == 0:
                        g = (gate(g[0]), g[1])
                    g = _cmul(*g, *m)
                    put((hi_re, hi_im), *slot[ee], g)
                    if ee == e:
                        h = g
                    ee, m = ee + 256, z[256]
                    cnt += 1
                    if cnt % 4 == 0:
                        yield g[0]
            w1 = (gate(z[8][0]), -z[8][1])
            v = [(jnp.ones((16, 128), F32), jnp.zeros((16, 128), F32)), w1]
            v.append(_cmul(*w1, *w1))
            v.append(_cmul(*v[2], *w1))
            w4 = _cmul(*v[2], *v[2])
            for j in range(8):
                for f in range(4):
                    put((lo_re, lo_im), j, f, v[f])
                yield v[3][0]
                if j < 7:
                    w4 = (gate(w4[0]), w4[1])
                    v = [w4 if (j == 0 and f == 0) else _cmul(*v[f], *w4) for f in range(4)]

    def a_gen(i):
        b0 = pats[_NPAT - 3] != 0
        b1 = pats[_NPAT - 2] != 0
        for k in range(4 * UA):
            rows = pl.ds(i.off(32 * UA, 8 * k, 8), 8)
            lo = jnp.concatenate([lo_re[:, rows, :].reshape(64, 128), lo_im[:, rows, :].reshape(64, 128)], axis=1)
            h0 = hi_re[0, rows, :]
            if k % 2 == 0 and Sched.pre:
                h0 = after(h0, Sched.pre)
                Sched.pre = []
            hi = jnp.concatenate([jnp.concatenate([h0, hi_re[1:5, rows, :].reshape(32, 128)], axis=0),
                                  hi_im[:, rows, :].reshape(40, 128)], axis=1)
            o = lax.dot_general(_bf(hi), _bf(lo), _NT, preferred_element_type=F32)
            for q in range(5):
                Sched.tok.setdefault(13 + int(0.9 * (5 * (k // 2) + q)), []).append(o[16 * q + 8:16 * q + 16])
            for h in range(2):
                g = [pltpu.roll(o[16 * q + 8 * h:16 * q + 8 * h + 8], 4 * (q % 4) - 8 * h + 8, 1,
                                stride=7, stride_axis=0) for q in range(5)]
                dst = pl.ds(i.off(64 * UA, 16 * k + 8 * h, 8), 8)
                comp[0, dst, :] = jnp.where(b1, jnp.where(b0, g[3], g[2]), jnp.where(b0, g[1], g[0]))
                comp[1, dst, :] = g[4]
            if k % 2 == 1:
                yield

    def a_exp(i):
        bm = pats[_NPAT - 1] != 0
        srcs = []
        for u in range(UA):
            def ld(a, e):
                return _pack2(comp[a, pl.ds(i.off(64 * UA, 64 * u + e), 8, stride=4), :],
                              comp[a, pl.ds(i.off(64 * UA, 64 * u + 32 + e), 8, stride=4), :])

            srcs.append([ld(0, e) for e in range(4)]
                        + [jnp.where(bm, ld(1, 2 * k + 1), ld(1, 2 * k)) for k in range(2)])
        cache = {}

        def gat(s, key):
            if key not in cache:
                pat = pats[key]
                cache[key] = [_gather(srcs[u][s], pat) for u in range(UA)]
            return cache[key]

        tiles = []
        for steps in _TILES:
            t = None
            for s, key, lanes in steps:
                v = [jnp.zeros((8, 128), I32)] * UA if s < 0 else gat(s, key)
                t = v if t is None else [jnp.where(_lanes_mask(lanes), v[u], t[u]) for u in range(UA)]
            tiles.append(t)
        yield
        for u0 in range(0, UA, 2):
            lhs = [_bf(jnp.concatenate([tiles[_TILE_OF[dl, l2]][u] for dl in range(4) for u in (u0, u0 + 1)], axis=0))
                   for l2 in range(4)]
            z0 = 0 if u0 == 0 else zero * 8

            def dots(ri):
                return [jnp.dot(lhs[l2], _bf(jnp.concatenate(
                    [fpk[l2, pl.ds(z0 + 16 * (j ^ l2), 16) if u0 == 0 else
                         pl.ds(pl.multiple_of(z0 + 16 * (j ^ l2), 8), 16), pl.ds(128 * ri, 128)]
                     for j in range(4)], axis=0)), preferred_element_type=F32) for l2 in range(4)]

            def store(k2, ri, v):
                khat[2 * k2 + ri, :, pl.ds(i.off(16 * UA, 16 * u0, 16), 32), :] = v.reshape(4, 32, 128)

            def toks(v, step0):
                for j in range(8):
                    g = 13 + 9 * UA + int(0.7 * (step0 + j))
                    Sched.tok.setdefault(g, []).append(v[16 * j + 8:16 * j + 16])

            re = dots(0)
            s0, d0r, s1, d1r = re[0] + re[2], re[0] - re[2], re[1] + re[3], re[1] - re[3]
            store(0, 0, s0 + s1)
            v = s0 - s1
            store(2, 0, v)
            toks(v, 8 * u0)
            im = dots(1)
            s0, d0i, s1, d1i = im[0] + im[2], im[0] - im[2], im[1] + im[3], im[1] - im[3]
            store(0, 1, s0 + s1)
            store(2, 1, s0 - s1)
            store(1, 0, d0r + d1i)
            store(1, 1, d0i - d1r)
            store(3, 0, d0r - d1i)
            v = d0i + d1r
            store(3, 1, v)
            toks(v, 8 * u0 + 8)
            yield

    def a_weave(gens):
        if 2 in gens:
            next(gens[2])
        if 0 in gens and 1 in gens:
            for n in (3, 5, 4):
                for _ in range(n):
                    v = next(gens[0])
                Sched.pre = [v[:8], v[8:]]
                next(gens[1])
        for k in (1, 2, 0):
            if k in gens:
                for _ in gens[k]:
                    pass

    a_pro, a_loop, a_tail = _pipeline([a_prep, a_gen, a_exp], NU // UA, newz, reset=Sched.reset, weave=a_weave)
    for cp in cps[3:9]:
        cp.wait()
    a_pro[0]()
    for cp in cps[9:15]:
        cp.wait()
    a_pro[1]()
    for cp in cps[15:]:
        cp.wait()
    a_loop()

    cp_x.wait()

    def zrow(u):
        return pl.ds(pl.multiple_of(zero * 8 + 8 * u, 8), 8)

    def b_gather(b):
        for j in range(4):
            pat = pats[j]
            for u in range(NU):
                v = pltpu.bitcast(xbuf[pl.ds(16 * u, 16), pl.ds(512 * b + 128 * j, 128)], I32)
                xg[b][j, pl.ds(8 * u, 8), :] = _gather(v, pat)

    def b_stat(b):
        s2 = [jnp.zeros((8, 128), F32) for _ in range(4)]
        for u in range(NU):
            o = _butterfly([xg[b][j, zrow(u), :] for j in range(4)])
            for l2 in range(4):
                xp[4 * l2 + b, pl.ds(8 * u, 8), :] = o[l2]
                e_, o_ = _unpack2(o[l2])
                s2[l2] = s2[l2] + (e_ * e_ + o_ * o_)
        for l2 in range(4):
            stat[b][l2, pl.ds(16, 8), :] = s2[l2]

    def b_dot(b):
        lhs = _bf(wr16b[...])
        for j in range(4):
            rows = pl.ds(pl.multiple_of(zero * zero * 8, 8), D // 2)
            stat[b][j, pl.ds(0, 16), :] = jnp.dot(lhs, _bf(xg[b][j, rows, :]), preferred_element_type=F32)

    def b_fin(b):
        st = []
        wxs = _butterfly([stat[b][j, zrow(0), :] for j in range(4)])
        sxs = _butterfly([stat[b][j, zrow(1), :] for j in range(4)])
        for l2 in range(4):
            wx, sx = wxs[l2], sxs[l2]
            m = sx * jnp.float32(1.0 / D)
            q = jnp.sum(stat[b][l2, zrow(2), :], axis=0, keepdims=True) * jnp.float32(1.0 / D)
            var = _rbf(jnp.maximum(q - m * m, 0.0))
            rs = 1.0 / _rbf(jnp.sqrt(_rbf(var + jnp.float32(EPS))))
            mb = _rbf(m)
            st.append((mb, rs))
            r = _rbf((wx - mb * wsum[...]) * rs)
            r = jnp.where(r == 0.0, 0.0, r)
            bits = pltpu.bitcast(r, I32)
            mono = ((bits ^ ((bits >> 31) & jnp.int32(0x7FFFFFFF))) >> 16) + 32768
            tok = 512 * b + 4 * (32 * ((lane8 >> 5) ^ l2) + (lane8 & 31)) + l2
            key = pltpu.bitcast((mono << 11) + (2047 - tok) + jnp.int32(0x00800000), F32)
            t = 4 * b + l2
            topk[t // 8] = key if t % 8 == 0 else jnp.where(sub8 == t % 8, key, topk[t // 8])
        return st

    def b_norm(b):
        st = b_fin(b)
        for us in (range(CB // 16), range(CB // 16, NU)):
            for l2 in range(4):
                mb, rs = st[l2]
                for u in us:
                    e_, o_ = _unpack2(xp[4 * l2 + b, zrow(u), :])
                    xnp[4 * l2 + b, pl.ds(8 * u, 8), :] = _pack2((e_ - mb) * rs, (o_ - mb) * rs)

    wrow = wr[...].reshape(1, D)
    wr16b[...] = pltpu.bitcast(jnp.concatenate([jnp.broadcast_to(wrow, (8, D)), jnp.ones((8, D), BF16)], axis=0), I32)
    wsum[...] = jnp.broadcast_to(jnp.sum(wrow.astype(F32), axis=1, keepdims=True), (8, 128))
    topk[2] = jnp.zeros((8, 128), F32)
    cols[...] = jnp.zeros(cols.shape, I32)

    elt_dep = []

    def c_fwd(i):
        h0 = i.off(CB // 2, 0, 8)
        r0 = i.off(CB, 0, 8)
        for l2 in range(4):
            lhs = _bf(xnp[pl.ds(4 * l2, 4), pl.ds(h0, CB // 2), :].reshape(2 * CB, 128))
            res = jnp.dot(lhs, _bf(fpk[l2, pl.ds(step_zero(i), 64), :]), preferred_element_type=F32)
            for ri in range(2):
                y = res[:, 128 * ri:128 * ri + 128]
                if l2 == 3 and ri == 1 and isinstance(i.i, int) and i.i < 2:
                    y = pad_tail(y, i)
                uhat[2 * l2 + ri, :, pl.ds(r0, CB), :] = y.reshape(4, CB, 128)
            yield

    def c_mid(i):
        for k in range(CB // 8):
            rows = pl.ds(i.off(CB, 8 * k, 8), 8)
            krows = pl.ds(i.off(CB, 16 * (k // 2) + k % 2), 8, stride=2)
            uu = [_fft4([(uhat[2 * l2, b, rows, :], uhat[2 * l2 + 1, b, rows, :]) for l2 in range(4)], -1)
                  for b in range(4)]
            yy = [[None] * 4 for _ in range(4)]
            for k2s in ((0, 2), (1, 3)):
                pps = {k2: [None] * 4 for k2 in k2s}
                for k2, pp in pps.items():
                    for dl in range(3, -1, -1):
                        kk = (khat[2 * k2, dl, krows, :], khat[2 * k2 + 1, dl, krows, :])
                        for m in range(3, dl - 1, -1):
                            t = _cmul(*uu[m - dl][k2], *kk)
                            pp[m] = t if pp[m] is None else (pp[m][0] + t[0], pp[m][1] + t[1])
                for k2, pp in pps.items():
                    for m in range(3, -1, -1):
                        yy[m][k2] = pp[0] if m == 0 else (pp[m][0] - pp[m - 1][1], pp[m][1] + pp[m - 1][0])
            un = i.off(CB // 8, k)
            for bp in range(2):
                ww = [_fft4(yy[m], 1) for m in (2 * bp, 2 * bp + 1)]
                for l2 in range(4):
                    for ri in range(2):
                        yhat[2 * l2 + ri, bp, un] = _pack2(ww[0][l2][ri], ww[1][l2][ri])
            yield

    def c_inv(i):
        u0 = i.off(CB // 8)
        r0 = i.off(2 * CB, 0, 8)
        for l2 in range(4):
            for ri in range(2):
                lhs = _bf(yhat[2 * l2 + ri, :, pl.ds(u0, CB // 8)].reshape(2 * CB, 128))
                y = lax.dot_general(lhs, _bf(fpk[l2, pl.ds(step_zero(i), 64), pl.ds(128 * ri, 128)]), _NT,
                                    preferred_element_type=F32)
                if l2 == 3 and ri == 1 and isinstance(i.i, int):
                    y = pad_tail(y, i)
                ybuf[2 * l2 + ri, :, pl.ds(r0, 2 * CB), :] = y.reshape(2, 2 * CB, 128)
            yield

    def c_elt(i):
        for k in range(CB // 16):
            hr = pl.ds(i.off(CB // 2, 8 * k, 8), 8)
            sk = [skip[pl.ds(i.off(CB, 16 * k + e), 8, stride=2), :] for e in range(2)]
            for b in range(4):
                o = []
                for l2 in range(4):
                    w = xnp[4 * l2 + b, hr, :]
                    if elt_dep:
                        w = after(w, elt_dep)
                    xn = _unpack2(w)
                    xx = _unpack2(xp[4 * l2 + b, hr, :])
                    ss, v = [], []
                    for e in range(2):
                        yr = pl.ds(i.off(2 * CB, 32 * k + 2 * e + b % 2), 8, stride=4)
                        ss.append(ybuf[2 * l2, b // 2, yr, :] + ybuf[2 * l2 + 1, b // 2, yr, :] + xn[e] * sk[e])
                        v.append(xx[e] + ss[e] * _silu(xn[e]))
                    spk[4 * l2 + b, hr, :] = _pack2(*ss)
                    o.append(_pack2(*v))
                p = _butterfly(o)
                for j in range(4):
                    opk[4 * b + j, hr, :] = p[j]
                yield

    def c_top(i):
        k0, k1 = topk[i.off(0, 0)], topk[i.off(0, 1)]
        mx = jnp.max(jnp.max(jnp.maximum(k0, k1), axis=0, keepdims=True), axis=1, keepdims=True)
        topk[i.off(0, 0)] = jnp.where(k0 == mx, 0.0, k0)
        topk[i.off(0, 1)] = jnp.where(k1 == mx, 0.0, k1)
        topk[i.off(0, 2)] = jnp.where(sub8 == i.idx(), mx, topk[i.off(0, 2)])
        yield

    def c_first(i):
        yield from c_fwd(i)
        yield from c_top(i)

    c_pro, c_loop, _ = _pipeline([c_first, c_mid, c_inv, c_elt], NB, newz,
                                 weave=[1] * (CB // 8) + [3] * (CB // 4) + [0, 0, 2, 2, 0, 0, 2, 2])

    def first_fwd():
        for _ in c_first(_Idx(0, 0)):
            pass

    def each(fn, *bs):
        return [lambda b=b: fn(b) for b in bs]

    block(a_tail[0], *each(b_gather, 0, 1))
    block(a_tail[1], *each(b_gather, 2, 3), *each(b_dot, 0, 1), *each(b_stat, 0, 1))
    block(*each(b_stat, 2, 3), *each(b_norm, 0, 1), *each(b_dot, 2, 3))
    block(*each(b_norm, 2, 3), first_fwd)
    block(c_pro[1])
    block(c_pro[2])
    c_loop()

    sel = pltpu.bitcast(topk[2], I32) - jnp.int32(0x00800000)
    mono = (sel >> 11) - 32768
    r_sel = pltpu.bitcast((mono ^ ((mono >> 31) & jnp.int32(0x7FFF))) << 16, F32)
    gate_r = _rbf(jax.nn.sigmoid(r_sel))
    posv[...] = 2047 - (sel & 2047)
    tok = [posv[c, 0] for c in range(C)]
    nat = [(t >> 7, t & 127) for t in tok]
    prm = []
    for t in tok:
        l2, l1 = t & 3, (t >> 2) & 127
        prm.append((4 * l2 + (t >> 9), 32 * ((l1 >> 5) ^ l2) + (l1 & 31)))

    def extract(src, k):
        for c, (tp, pp) in enumerate(prm):
            sh = (c - pp) & 127
            for u in range(NU):
                pltpu.store(cols.at[k, pl.ds(8 * u, 8), :], pltpu.roll(src[tp, pl.ds(8 * u, 8), :], sh, 1),
                            mask=lane8 == c)

    for c, (tp, pp) in enumerate(prm):
        ohb[c] = jnp.where(jnp.logical_and(sub8 == c // 2, lane8 == pp), jnp.int32(0x3F80 << (16 * (c % 2))), 0)

    def take_rows():
        for c, (tp, pp) in enumerate(prm):
            xsel_ref[c] = lax.dot_general(_bf(ohb[c]), _bf(xnp[tp]), _NT, preferred_element_type=F32)[:8]

    def stages(*items):
        def run():
            z = newz()
            for fn, k in items:
                for _ in fn(_Idx(k, 0, z)):
                    pass
        return run

    block(stages((c_mid, NB - 1), (c_inv, NB - 2)))
    block(stages((c_elt, NB - 3), (c_inv, NB - 1)), take_rows, lambda: extract(xp, 0))

    def o_gather(us):
        for j in range(4):
            pat = pats[4 + j]
            for b in range(4):
                for u in us:
                    v = _gather(opk[4 * b + j, pl.ds(8 * u, 8), :], pat)
                    og[4 * b + j, pl.ds(8 * u, 8), :] = v
                    o_store(u, v, pl.ds(512 * b + 128 * j, 128))

    def o_store(u, v, col):
        obuf[pl.ds(16 * u, 8), col] = _bf(v[0:4])
        obuf[pl.ds(16 * u + 8, 8), col] = _bf(pltpu.roll(v, 4, 0)[0:4])

    bits = jnp.int32(0)
    for c in range(C):
        bits = bits | (jnp.int32(1) << nat[c][0])

    cp_bar.start()

    def send(routed, a, n):
        for t in range(16):
            @pl.when(((bits >> t) & 1) == routed)
            def _():
                col = pl.ds(128 * t, 128)
                pltpu.make_async_copy(obuf.at[pl.ds(a, n), col], out_hbm.at[pl.ds(a, n), col], sem_out).start()

    late = {1: (0, 256), 3: (256, 256), 4: (512, 64)}

    def project(w, post, ks):
        fill = [g for k in ks for g in [c_elt(_Idx(k, 0))] * (CB // 4)]
        nt, done = F // 128, 0
        for t in range(nt):
            ps = [jnp.dot(xsel_b[:, a:a + n], w[pl.ds(a, n), pl.ds(128 * t, 128)],
                          preferred_element_type=F32)[:8] for a, n in chunks]
            v = _rbf((ps[0] + ps[1]) + (ps[2] + ps[3]) + ps[4])
            elt_dep[:] = [v]
            post(t, v)
            while done * nt < (t + 1) * len(fill):
                next(fill[done], None)
                done += 1
        elt_dep.clear()

    def post_gate(t, ga):
        hbuf[:, pl.ds(128 * t, 128)] = _rbf(ga * _rbf(jax.nn.sigmoid(ga)))

    def post_up(t, up):
        h = hbuf[:, pl.ds(128 * t, 128)] * up
        hpk[:, pl.ds(128 * t, 128)] = pltpu.bitcast(
            jnp.concatenate([h, jnp.zeros((8, 128), F32)], axis=0).astype(BF16), I32)

    cp_g.wait()
    xsel = xsel_ref[0]
    for c in range(1, C):
        xsel = xsel + xsel_ref[c]
    xsel_b = jnp.concatenate([xsel, jnp.zeros((8, D), F32)], axis=0).astype(BF16)
    project(wg, post_gate, (NB - 2, NB - 1))
    o_gather(range(28))
    cp_u.wait()
    project(wu, post_up, ())
    o_gather(range(28, 32))
    o_gather(range(32, NU))
    extract(spk, 1)
    pr = (r128 & (-16)) + 2 * (r128 & 7) + ((r128 >> 3) & 1)
    perm = jnp.where(pr == c128, 1.0, 0.0).astype(BF16)

    def patch(q, y):
        a, n = chunks[q]
        z = _rbf(xsel[:8, a:a + n] + _rbf(_rbf(y[:8]) * gate_r[:, :1]))
        g = z * _rbf(jax.nn.sigmoid(z))
        g = jnp.concatenate([g, jnp.zeros((120, n), F32)], axis=0).astype(BF16)
        gt = lax.dot_general(perm[:n, :n], g, _NT, preferred_element_type=F32)
        us = range(a // 16, (a + n) // 16)
        zz = newz()
        for u in us:
            hr = pl.ds(pl.multiple_of(zz + 8 * u, 8), 8)
            xx, ss = _unpack2(cols[0, hr, :]), _unpack2(cols[1, hr, :])
            r0 = 16 * u - a
            w = _pack2(*[xx[e] + _rbf(ss[e] * gt[r0 + 8 * e:r0 + 8 * e + 8]) for e in range(2)])
            for c, (tn, pn) in enumerate(nat):
                tt = 4 * (tn >> 2) + (tn & 3)
                pltpu.store(og.at[tt, pl.ds(8 * u, 8), :], pltpu.roll(w, (pn - c) & 127, 1), mask=lane8 == pn)
        for c, (tn, pn) in enumerate(nat):
            for u in us:
                v = og[tn, pl.ds(8 * u, 8), :]
                o_store(u, v, pl.ds(pl.multiple_of(tn * 128, 128), 128))
        if q in late:
            send(1, *late[q])

    send(0, 0, D)
    def down(q, f0, f1):
        a, n = chunks[q]
        return lax.dot_general(_bf(hpk[:, pl.ds(f0, f1 - f0)]), wd[pl.ds(a, n), pl.ds(f0, f1 - f0)], _NT,
                               preferred_element_type=F32)[:8]

    prev = None
    for q, fs in enumerate((0, 1280, 1280, 0, 2560)):
        if q % 3 == 0:
            for cp in cp_d[q:q + 3]:
                cp.wait()
        y0 = down(q, 0, fs) if fs else None
        if prev is not None:
            patch(*prev)
        y = down(q, fs, F)
        prev = (q, y if y0 is None else y0 + y)
    cp_bar.wait()
    patch(*prev)
    pltpu.make_async_copy(obuf, out_hbm, sem_out).wait()


def _scratch():
    return [
        pltpu.VMEM((D, L), BF16),
        pltpu.VMEM((6, D, N), BF16),
        pltpu.VMEM((D,), BF16),
        pltpu.VMEM((D,), BF16),
        pltpu.VMEM((D,), BF16),
        pltpu.VMEM((D, F), BF16),
        pltpu.VMEM((D, F), BF16),
        pltpu.VMEM((D, F), BF16),
        pltpu.VMEM((4, 64, 256), I32),
        pltpu.VMEM(_PROWS.shape, I32),
        pltpu.VMEM((_NPAT, 8, 128), I32),
        pltpu.VMEM((D, 128), F32),
        pltpu.VMEM((D, 128), F32),
        pltpu.VMEM((5, 2 * D, 128), I32),
        pltpu.VMEM((5, 2 * D, 128), I32),
        pltpu.VMEM((8, 2 * D, 128), I32),
        pltpu.VMEM((8, 2 * D, 128), I32),
        pltpu.VMEM((2, 4 * D, 128), F32),
        pltpu.VMEM((8, 4, D, 128), F32),
        pltpu.VMEM((16, D // 2, 128), I32),
        pltpu.VMEM((16, D // 2, 128), I32),
        pltpu.VMEM((8, 4, D, 128), F32),
        pltpu.VMEM((8, 2, D // 8, 8, 128), I32),
        pltpu.VMEM((8, 2, 2 * D, 128), F32),
        pltpu.VMEM((16, D // 2, 128), I32),
        pltpu.VMEM((3, 8, 128), F32),
        pltpu.VMEM((8, 128), I32),
        pltpu.VMEM((8, D), I32),
        pltpu.VMEM((8, 128), F32),
        pltpu.VMEM((C, 8, 128), I32),
        pltpu.VMEM((C, 8, D), F32),
        pltpu.VMEM((8, F), F32),
        pltpu.VMEM((8, F), I32),
        pltpu.VMEM((2, D // 2, 128), I32),
        pltpu.VMEM((16, D // 2, 128), I32),
        pltpu.VMEM((16, D // 2, 128), I32),
        pltpu.VMEM((D, L), BF16),
        pltpu.SemaphoreType.DMA((9,)),
        pltpu.SemaphoreType.DMA,
        pltpu.SemaphoreType.DMA,
    ] + [pltpu.VMEM((4, D // 2, 128), I32)] * 4 + [pltpu.VMEM((4, 24, 128), F32)] * 4


@jax.jit
def pallas_recurrent_scan__ssm_conv_s4__moe_arch_mod__prompt_kernel(
    A_u: jax.Array,
    A_A_re: jax.Array,
    A_A_im: jax.Array,
    A_B_re: jax.Array,
    A_B_im: jax.Array,
    A_C_re: jax.Array,
    A_C_im: jax.Array,
    A_log_dt: jax.Array,
    A_Dskip: jax.Array,
    B_x: jax.Array,
    B_w_r: jax.Array,
    B_w_gate: jax.Array,
    B_w_up: jax.Array,
    B_w_down: jax.Array,
):
    hbm = pl.BlockSpec(memory_space=pltpu.HBM)
    out = pl.pallas_call(
        _kernel,
        out_shape=jax.ShapeDtypeStruct((D, L), BF16),
        in_specs=[hbm] * 14,
        out_specs=hbm,
        scratch_shapes=_scratch(),
        compiler_params=pltpu.CompilerParams(vmem_limit_bytes=110 * 1024 * 1024),
        name="s4_mod",
    )(A_u[0].T, A_A_re, A_A_im, A_B_re, A_B_im, A_C_re, A_C_im, A_log_dt, A_Dskip, B_w_r,
      B_w_gate, B_w_up, B_w_down.T, jnp.asarray(_PROWS))
    return out.T[None]
```

```python
import numpy as np
import jax
import jax.numpy as jnp
from jax import lax
import jax.experimental.pallas as pl
import jax.experimental.pallas.tpu as pltpu

L, D, N, F, C = 2048, 576, 128, 4608, 8
NU = D // 16
CB = 64
NB = D // CB
FG0 = 3
UA = 4
F32, BF16, I32 = jnp.float32, jnp.bfloat16, jnp.int32
EPS = 1e-5


def _bf16_round_np(x):
    u = np.asarray(x, np.float32).view(np.uint32).astype(np.uint64)
    r = ((u + 0x7FFF + ((u >> 16) & 1)) >> 16) << 16
    return r.astype(np.uint32)


_LROUND = _bf16_round_np(np.arange(L)).view(np.float32).astype(np.int64)
_HI = [(1, 3, 516, 1032), (5, 7, 520, 1288), (4, 260, 772, 1544), (8, 264, 776, 1800), (2, 6, 258, 262)]


def _comp_q():
    t = np.arange(8)[:, None]
    lane = np.arange(128)[None, :]
    return ((lane - 8 - 7 * (t % 4)) % 16) // 4


def _make_tables():
    lane = np.arange(128)
    lo = 8 * (4 * (lane // 16) + lane % 4)
    tab = [dict(), dict()]
    amask = np.zeros(128, bool)
    for q in range(5):
        for e in range(4):
            for par in range(2):
                t = 4 * par + e
                for h in range(2):
                    src = lane[(lane // 4) % 4 == 2 * h + par]
                    dst = (src + (4 * (q % 4) - 8 * h + 8) + 7 * t) % 128
                    assert np.all(_comp_q()[t, dst] == q % 4)
                    sid = e if q < 4 else 4 + e // 2
                    for sl, dl_ in zip(src, dst):
                        ent = (sid, int(dl_))
                        assert tab[par].setdefault(_HI[q][e] + int(lo[sl]), ent) == ent
                    if q == 4 and e % 2 == 1:
                        amask[dst % 16 + 16 * np.arange(8)[:, None]] = True
    pats = []
    for j in range(4):
        pats.append(np.tile(4 * (lane % 32) + ((lane // 32) ^ j), (8, 1)))
    for j in range(4):
        pats.append(np.tile(32 * ((lane % 4) ^ j) + lane // 4, (8, 1)))
    npat0 = len(pats)
    tiles, tile_of = [], {}
    for dl in range(4):
        for l2 in range(4):
            v = _LROUND[512 * dl + 4 * lane + l2]
            key = tuple(v.tolist())
            if key in tile_of:
                tile_of[dl, l2] = tile_of[key]
                continue
            sid = np.array([tab[0][x][0] if x else -1 for x in v])
            ln = np.array([[tab[s8 % 2][x][1] if x else 0 for x in v] for s8 in range(8)])
            steps = []
            for s in sorted(set(sid.tolist()), key=lambda s: -(sid == s).sum()):
                lanes = np.nonzero(sid == s)[0]
                if s < 0:
                    steps.append((-1, None, lanes))
                    continue
                care = sid == s
                kk = None
                for k in range(npat0, len(pats)):
                    oldp, oldc, olds = pats[k]
                    both = care & oldc
                    if olds == s and np.array_equal(oldp[:, both], ln[:, both]):
                        pats[k] = (np.where(care, ln, oldp), care | oldc, s)
                        kk = k
                        break
                if kk is None:
                    pats.append((np.where(care, ln, 0), care, s))
                    kk = len(pats) - 1
                steps.append((s, kk, lanes))
            tiles.append(steps)
            tile_of[key] = tile_of[dl, l2] = len(tiles) - 1
    pats = np.stack([p if k < npat0 else p[0] for k, p in enumerate(pats)]).astype(np.int32)
    tile_of = {k: v for k, v in tile_of.items() if len(k) == 2}
    rows = np.concatenate([pats[:, :2].reshape(-1, 128), amask[None].astype(np.int32)])
    rows = np.concatenate([rows, np.zeros((-len(rows) % 8, 128), np.int32)])
    return tiles, tile_of, len(pats), rows


_TILES, _TILE_OF, _NGAT, _PROWS = _make_tables()
_NPAT = _NGAT + 3


def _cmul(ar, ai, br, bi):
    return ar * br - ai * bi, ar * bi + ai * br


def _sincos(b):
    magic = jnp.float32(12582912.0)
    t = b * jnp.float32(2.0 / np.pi) + magic
    k = t - magic
    ki = pltpu.bitcast(t, I32)
    r = b - k * jnp.float32(1.5703125)
    r = r - k * jnp.float32(0.0004837512969970703)
    r = r - k * jnp.float32(7.549790126404332e-08)
    u = r * r
    ps = (jnp.float32(-0.0001958295761141926) * u + jnp.float32(0.008332725614309311)) * u \
        + jnp.float32(-0.166666641831398)
    sn = r + (r * u) * ps
    pc = ((jnp.float32(2.437065268168226e-05) * u + jnp.float32(-0.0013886778615415096)) * u
          + jnp.float32(0.04166663438081741)) * u + jnp.float32(-0.5)
    cs = pc * u + jnp.float32(1.0)
    odd = (ki & 1) == 1
    s1 = jnp.where(odd, cs, sn)
    c1 = jnp.where(odd, sn, cs)
    sign = jnp.int32(-2147483648)
    s1 = pltpu.bitcast(pltpu.bitcast(s1, I32) ^ ((ki << 30) & sign), F32)
    c1 = pltpu.bitcast(pltpu.bitcast(c1, I32) ^ (((ki + 1) << 30) & sign), F32)
    return s1, c1


def _gather(x, idx):
    return jnp.take_along_axis(x, idx, axis=1, mode="promise_in_bounds")


def _lanes_mask(lanes):
    lane = lax.broadcasted_iota(I32, (8, 128), 1)
    lanes = sorted(int(x) for x in lanes)
    runs, start, prev = [], lanes[0], lanes[0]
    for x in lanes[1:]:
        if x != prev + 1:
            runs.append((start, prev))
            start = x
        prev = x
    runs.append((start, prev))
    m = None
    for a, b in runs:
        t = (lane == a) if a == b else jnp.logical_and(lane >= a, lane <= b)
        m = t if m is None else jnp.logical_or(m, t)
    return m


def _butterfly(p):
    lane = lax.broadcasted_iota(I32, p[0].shape, 1)
    b0 = (lane & 32) != 0
    b1 = (lane & 64) != 0
    t = [jnp.where(b0, p[k ^ 1], p[k]) for k in range(4)]
    return [jnp.where(b1, t[k ^ 2], t[k]) for k in range(4)]


def _fft4(x, sgn):
    (ar, ai), (br, bi), (cr, ci), (dr, di) = x
    s0r, s0i, d0r, d0i = ar + cr, ai + ci, ar - cr, ai - ci
    s1r, s1i, d1r, d1i = br + dr, bi + di, br - dr, bi - di
    y0 = (s0r + s1r, s0i + s1i)
    y2 = (s0r - s1r, s0i - s1i)
    p = (d0r - d1i, d0i + d1r)
    m = (d0r + d1i, d0i - d1r)
    return [y0, p, y2, m] if sgn > 0 else [y0, m, y2, p]


def _silu(z):
    h = z * jnp.float32(0.5)
    return h + h * jnp.tanh(h)


def _rbf(x):
    return x.astype(BF16).astype(F32)


def _pack2(a, b):
    p = pltpu.pack_elementwise([a, b], packed_dtype=BF16)
    return p if p.dtype == I32 else pltpu.bitcast(p, I32)


def _unpack2(x):
    return [pltpu.unpack_elementwise(x, index=i, packed_dtype=BF16, unpacked_dtype=F32) for i in range(2)]


def _bf(x):
    return pltpu.bitcast(x, BF16)


_NT = (((1,), (1,)), ((), ()))


class _Idx:
    def __init__(self, i, lag, z=None):
        self.i, self.lag, self.z = i, lag, z

    def off(self, stride, const=0, align=None):
        c = const - self.lag * stride
        if isinstance(self.i, int):
            if self.z is None:
                return self.i * stride + c
            v = self.z + (self.i * stride + c)
        else:
            v = self.i * stride + c
        return pl.multiple_of(v, align) if align else v

    def idx(self):
        return self.i - self.lag


def _pipeline(stages, n, newz, weave=None, reset=None):
    ns = len(stages)

    def step(i, lo, hi):
        z = newz() if isinstance(i, int) else None
        gens = {k: stages[k](_Idx(i, k, z)) for k in range(lo, hi)}
        if reset is not None:
            reset()
        if callable(weave):
            weave(gens)
        else:
            for k in weave or ():
                if k in gens:
                    next(gens[k], None)
        for k in range(hi - 1, lo - 1, -1):
            for _ in gens[k]:
                pass

    def body(i, carry):
        step(i, 0, ns)
        return carry

    return ([lambda i=i: step(i, 0, i + 1) for i in range(ns - 1)],
            lambda: lax.fori_loop(ns - 1, n, body, 0),
            [lambda i=i: step(n + i, i + 1, ns) for i in range(ns - 1)])


def _kernel(x_hbm, are_hbm, aim_hbm, bre_hbm, bim_hbm, cre_hbm, cim_hbm, ldt_hbm, dsk_hbm, wr_hbm,
            wg_hbm, wu_hbm, wd_hbm, pat_hbm,
            out_hbm,
            xbuf, par, ldt, dsk, wr, wg, wu, wd, fpk, prow, pats,
            dtcol, skip, hi_re, hi_im, lo_re, lo_im, comp, khat,
            xp, xnp, uhat, yhat, ybuf, spk, topk, posv, wr16b, wsum, ohb, xsel_ref, hbuf, hpk, cols, opk, og, obuf,
            sem_in, sem_out, sem_bar, *perb):
    xg, stat = perb[0:4], perb[4:8]
    p_hbm = (are_hbm, aim_hbm, bre_hbm, bim_hbm, cre_hbm, cim_hbm)
    r1 = 16 * UA
    small = [(ldt_hbm, ldt), (pat_hbm, prow)]
    for a, n in ((0, r1), (r1, r1), (2 * r1, D - 2 * r1)):
        small += [(h.at[pl.ds(a, n)], par.at[i, pl.ds(a, n)]) for i, h in enumerate(p_hbm)]
    small += [(wr_hbm, wr), (dsk_hbm, dsk)]
    cps = [pltpu.make_async_copy(s, d, sem_in.at[min((i + 4) // 6, 3)]) for i, (s, d) in enumerate(small)]
    ns = 4
    cp_x = pltpu.make_async_copy(x_hbm, xbuf, sem_in.at[ns])
    cp_g = pltpu.make_async_copy(wg_hbm, wg, sem_in.at[ns + 1])
    cp_u = pltpu.make_async_copy(wu_hbm, wu, sem_in.at[ns + 2])
    chunks = [(0, 128), (128, 128), (256, 128), (384, 128), (512, 64)]
    cp_d = [pltpu.make_async_copy(wd_hbm.at[pl.ds(a, n)], wd.at[pl.ds(a, n)], sem_in.at[ns + 3 + q // 3])
            for q, (a, n) in enumerate(chunks)]
    cp_bar = pltpu.make_async_copy(pat_hbm.at[pl.ds(0, 8)], posv, sem_bar)
    for cp in cps + [cp_x, cp_g, cp_u] + cp_d:
        cp.start()

    sub8 = lax.broadcasted_iota(I32, (8, 128), 0)
    lane8 = lax.broadcasted_iota(I32, (8, 128), 1)

    def dft_rows(l2):
        for g in range(8):
            cs = []
            for e in range(2):
                p = 16 * g + 2 * sub8 + e
                t = 4 * (32 * ((p >> 5) ^ l2) + (p & 31)) + l2
                n = ((4 * lane8 + 1) * t) & 2047
                cs.append(_sincos(n.astype(F32) * jnp.float32(-2.0 * np.pi / 2048)))
            fpk[l2, pl.ds(8 * g, 8), pl.ds(0, 128)] = _pack2(cs[0][1], cs[1][1])
            fpk[l2, pl.ds(8 * g, 8), pl.ds(128, 128)] = _pack2(cs[0][0], cs[1][0])

    for l2 in range(FG0):
        dft_rows(l2)

    for cp in cps[:2]:
        cp.wait()
    for l2 in range(FG0, 4):
        dft_rows(l2)
    for k in range(_NGAT):
        pats[k] = jnp.where((sub8 & 1) == 1, jnp.broadcast_to(prow[pl.ds(2 * k + 1, 1), :], (8, 128)),
                            jnp.broadcast_to(prow[pl.ds(2 * k, 1), :], (8, 128)))
    cq = ((lane8 - 8 - 7 * (sub8 & 3)) & 15) >> 2
    pats[_NGAT] = cq & 1
    pats[_NGAT + 1] = cq >> 1
    pats[_NGAT + 2] = jnp.broadcast_to(prow[pl.ds(2 * _NGAT, 1), :], (8, 128))
    r128 = lax.broadcasted_iota(I32, (128, 128), 0)
    c128 = lax.broadcasted_iota(I32, (128, 128), 1)

    def column(row):
        pk = pltpu.bitcast(jnp.broadcast_to(row, (8, D)), I32)
        lhs = []
        for u in range(NU):
            t = u // 8
            v = pk[:, 128 * t:128 * t + 128] if t < 4 else jnp.concatenate([pk[:, 512:], pk[:, 512:]], axis=1)
            c0 = 16 * (u % 8) + 2 * sub8
            lhs.append(jnp.where(lane8 == c0, lax.shift_right_logical(v, 16), jnp.where(lane8 == c0 + 1, v, 0)))
        ones = jnp.ones((128, 128), BF16)
        return jnp.concatenate([jnp.dot(_bf(jnp.concatenate(lhs[k:k + NU // 4], axis=0)), ones,
                                        preferred_element_type=F32) for k in range(0, NU, NU // 4)], axis=0)

    dtcol[...] = column(_rbf(jnp.exp(ldt[...].astype(F32).reshape(1, D))))

    zero = prow[0, 0]
    zcount = [0]

    def newz():
        zcount[0] += 1
        return zero * (64 * zcount[0])

    def block(*fns):
        def body(k, carry):
            for fn in fns:
                fn()
            return carry

        lax.fori_loop(0, zero + 1, body, 0)

    def step_zero(i):
        t = i.off(1) * zero if not isinstance(i.i, int) or i.z is None else i.z
        return pl.multiple_of(t * 8, 8)

    def after(x, deps):
        never = pats[0] < 0
        d = None
        for v in deps:
            v = v if v.dtype == I32 else pltpu.bitcast(v, I32)
            d = v if d is None else d ^ v
        return jnp.where(never, d if x.dtype == I32 else pltpu.bitcast(d, x.dtype), x)

    def pad_tail(y, i):
        n, k = 16, y.shape[0] - 64
        base = i.off(1)
        mid = after(y[k:k + 8], [pats[j % _NPAT] * (base + j) for j in range(n)])
        return jnp.concatenate([y[:k], mid, y[k + 8:]], axis=0)

    class Sched:
        tok, g, pre = {}, 0, []

        @classmethod
        def reset(cls):
            cls.tok, cls.g, cls.pre = {}, 0, []

        @classmethod
        def gate(cls, x):
            deps = cls.tok.pop(cls.g, [])
            cls.g += 1
            if not deps:
                return x
            return jnp.concatenate([after(x[:8], deps), after(x[8:], deps[-1:])], axis=0)

    slot = {h: (q, e) for q, ent in enumerate(_HI) for e, h in enumerate(ent)}

    def a_prep(i):
        gate = Sched.gate
        for u in range(UA):
            rows = pl.ds(i.off(16 * UA, 16 * u, 16), 16)
            ev = pl.ds(i.off(32 * UA, 32 * u), 16, stride=2)
            od = pl.ds(i.off(32 * UA, 32 * u + 1), 16, stride=2)
            dt = gate(dtcol[rows, :])
            al = dt * par[0, rows, :].astype(F32)
            be = dt * par[1, rows, :].astype(F32)
            cr, ci = _cmul(par[4, rows, :].astype(F32), par[5, rows, :].astype(F32),
                           par[2, rows, :].astype(F32), par[3, rows, :].astype(F32))
            dts = dt * jnp.float32(1.0 / 512)
            cr, ci = cr * dts, ci * dts
            k0 = jnp.sum(cr, axis=1, keepdims=True) * jnp.float32(512.0)
            skip[rows, :] = jnp.broadcast_to(k0, (16, 128))
            yield cr
            s, c = _sincos(gate(be))
            yield c
            pw = {1: (c, s)}
            e = 1
            while e < 256:
                if e in (1, 16):
                    c = gate(c)
                c, s = (c - s) * (c + s), (c + c) * s
                e *= 2
                pw[e] = (c, s)
                if e in (16, 256):
                    yield c
            z = {}
            for e in (1, 8, 256):
                mag = jnp.exp(al * jnp.float32(e))
                c, s = pw[e]
                z[e] = (mag * c, mag * s)
            pend = {}

            def put(tab, q, ee, v):
                key = (tab[0] is hi_re, q, ee // 2)
                if key not in pend:
                    pend[key] = (ee % 2, v)
                    return
                w, o = pend.pop(key)
                lo_, hi_ = (o, v) if w == 0 else (v, o)
                dst = od if ee // 2 else ev
                tab[0][q, dst, :] = _pack2(lo_[0], hi_[0])
                tab[1][q, dst, :] = _pack2(lo_[1], hi_[1])

            h = (cr, ci)
            cnt = 0
            for e in range(1, 9):
                g, ee, m = h, e, z[1]
                while ee in slot:
                    if cnt % 4 == 0:
                        g = (gate(g[0]), g[1])
                    g = _cmul(*g, *m)
                    put((hi_re, hi_im), *slot[ee], g)
                    if ee == e:
                        h = g
                    ee, m = ee + 256, z[256]
                    cnt += 1
                    if cnt % 4 == 0:
                        yield g[0]
            w1 = (gate(z[8][0]), -z[8][1])
            v = [(jnp.ones((16, 128), F32), jnp.zeros((16, 128), F32)), w1]
            v.append(_cmul(*w1, *w1))
            v.append(_cmul(*v[2], *w1))
            w4 = _cmul(*v[2], *v[2])
            for j in range(8):
                for f in range(4):
                    put((lo_re, lo_im), j, f, v[f])
                yield v[3][0]
                if j < 7:
                    w4 = (gate(w4[0]), w4[1])
                    v = [w4 if (j == 0 and f == 0) else _cmul(*v[f], *w4) for f in range(4)]

    def a_gen(i):
        b0 = pats[_NPAT - 3] != 0
        b1 = pats[_NPAT - 2] != 0
        for k in range(4 * UA):
            rows = pl.ds(i.off(32 * UA, 8 * k, 8), 8)
            lo = jnp.concatenate([lo_re[:, rows, :].reshape(64, 128), lo_im[:, rows, :].reshape(64, 128)], axis=1)
            h0 = hi_re[0, rows, :]
            if k % 2 == 0 and Sched.pre:
                h0 = after(h0, Sched.pre)
                Sched.pre = []
            hi = jnp.concatenate([jnp.concatenate([h0, hi_re[1:5, rows, :].reshape(32, 128)], axis=0),
                                  hi_im[:, rows, :].reshape(40, 128)], axis=1)
            o = lax.dot_general(_bf(hi), _bf(lo), _NT, preferred_element_type=F32)
            for q in range(5):
                Sched.tok.setdefault(13 + int(0.9 * (5 * (k // 2) + q)), []).append(o[16 * q + 8:16 * q + 16])
            for h in range(2):
                g = [pltpu.roll(o[16 * q + 8 * h:16 * q + 8 * h + 8], 4 * (q % 4) - 8 * h + 8, 1,
                                stride=7, stride_axis=0) for q in range(5)]
                dst = pl.ds(i.off(64 * UA, 16 * k + 8 * h, 8), 8)
                comp[0, dst, :] = jnp.where(b1, jnp.where(b0, g[3], g[2]), jnp.where(b0, g[1], g[0]))
                comp[1, dst, :] = g[4]
            if k % 2 == 1:
                yield

    def a_exp(i):
        bm = pats[_NPAT - 1] != 0
        srcs = []
        for u in range(UA):
            def ld(a, e):
                return _pack2(comp[a, pl.ds(i.off(64 * UA, 64 * u + e), 8, stride=4), :],
                              comp[a, pl.ds(i.off(64 * UA, 64 * u + 32 + e), 8, stride=4), :])

            srcs.append([ld(0, e) for e in range(4)]
                        + [jnp.where(bm, ld(1, 2 * k + 1), ld(1, 2 * k)) for k in range(2)])
        cache = {}

        def gat(s, key):
            if key not in cache:
                pat = pats[key]
                cache[key] = [_gather(srcs[u][s], pat) for u in range(UA)]
            return cache[key]

        tiles = []
        for steps in _TILES:
            t = None
            for s, key, lanes in steps:
                v = [jnp.zeros((8, 128), I32)] * UA if s < 0 else gat(s, key)
                t = v if t is None else [jnp.where(_lanes_mask(lanes), v[u], t[u]) for u in range(UA)]
            tiles.append(t)
        yield
        for u0 in range(0, UA, 2):
            lhs = [_bf(jnp.concatenate([tiles[_TILE_OF[dl, l2]][u] for dl in range(4) for u in (u0, u0 + 1)], axis=0))
                   for l2 in range(4)]
            z0 = 0 if u0 == 0 else zero * 8

            def dots(ri):
                return [jnp.dot(lhs[l2], _bf(jnp.concatenate(
                    [fpk[l2, pl.ds(z0 + 16 * (j ^ l2), 16) if u0 == 0 else
                         pl.ds(pl.multiple_of(z0 + 16 * (j ^ l2), 8), 16), pl.ds(128 * ri, 128)]
                     for j in range(4)], axis=0)), preferred_element_type=F32) for l2 in range(4)]

            def store(k2, ri, v):
                khat[2 * k2 + ri, :, pl.ds(i.off(16 * UA, 16 * u0, 16), 32), :] = v.reshape(4, 32, 128)

            def toks(v, step0):
                for j in range(8):
                    g = 13 + 9 * UA + int(0.7 * (step0 + j))
                    Sched.tok.setdefault(g, []).append(v[16 * j + 8:16 * j + 16])

            re = dots(0)
            s0, d0r, s1, d1r = re[0] + re[2], re[0] - re[2], re[1] + re[3], re[1] - re[3]
            store(0, 0, s0 + s1)
            v = s0 - s1
            store(2, 0, v)
            toks(v, 8 * u0)
            im = dots(1)
            s0, d0i, s1, d1i = im[0] + im[2], im[0] - im[2], im[1] + im[3], im[1] - im[3]
            store(0, 1, s0 + s1)
            store(2, 1, s0 - s1)
            store(1, 0, d0r + d1i)
            store(1, 1, d0i - d1r)
            store(3, 0, d0r - d1i)
            v = d0i + d1r
            store(3, 1, v)
            toks(v, 8 * u0 + 8)
            yield

    def a_weave(gens):
        if 2 in gens:
            next(gens[2])
        if 0 in gens and 1 in gens:
            for n in (3, 5, 4):
                for _ in range(n):
                    v = next(gens[0])
                Sched.pre = [v[:8], v[8:]]
                next(gens[1])
        for k in (1, 2, 0):
            if k in gens:
                for _ in gens[k]:
                    pass

    a_pro, a_loop, a_tail = _pipeline([a_prep, a_gen, a_exp], NU // UA, newz, reset=Sched.reset, weave=a_weave)
    for cp in cps[2:8]:
        cp.wait()
    a_pro[0]()
    for cp in cps[8:14]:
        cp.wait()
    a_pro[1]()
    for cp in cps[14:]:
        cp.wait()
    a_loop()

    cp_x.wait()

    def zrow(u):
        return pl.ds(pl.multiple_of(zero * 8 + 8 * u, 8), 8)

    def b_gather(b):
        for j in range(4):
            pat = pats[j]
            for u in range(NU):
                v = pltpu.bitcast(xbuf[pl.ds(16 * u, 16), pl.ds(512 * b + 128 * j, 128)], I32)
                xg[b][j, pl.ds(8 * u, 8), :] = _gather(v, pat)

    def b_stat(b):
        s2 = [jnp.zeros((8, 128), F32) for _ in range(4)]
        for u in range(NU):
            o = _butterfly([xg[b][j, zrow(u), :] for j in range(4)])
            for l2 in range(4):
                xp[4 * l2 + b, pl.ds(8 * u, 8), :] = o[l2]
                e_, o_ = _unpack2(o[l2])
                s2[l2] = s2[l2] + (e_ * e_ + o_ * o_)
        for l2 in range(4):
            stat[b][l2, pl.ds(16, 8), :] = s2[l2]

    def b_dot(b):
        lhs = _bf(wr16b[...])
        for j in range(4):
            rows = pl.ds(pl.multiple_of(zero * zero * 8, 8), D // 2)
            stat[b][j, pl.ds(0, 16), :] = jnp.dot(lhs, _bf(xg[b][j, rows, :]), preferred_element_type=F32)

    def b_fin(b):
        st = []
        wxs = _butterfly([stat[b][j, zrow(0), :] for j in range(4)])
        sxs = _butterfly([stat[b][j, zrow(1), :] for j in range(4)])
        for l2 in range(4):
            wx, sx = wxs[l2], sxs[l2]
            m = sx * jnp.float32(1.0 / D)
            q = jnp.sum(stat[b][l2, zrow(2), :], axis=0, keepdims=True) * jnp.float32(1.0 / D)
            var = _rbf(jnp.maximum(q - m * m, 0.0))
            rs = 1.0 / _rbf(jnp.sqrt(_rbf(var + jnp.float32(EPS))))
            mb = _rbf(m)
            st.append((mb, rs))
            r = _rbf((wx - mb * wsum[...]) * rs)
            r = jnp.where(r == 0.0, 0.0, r)
            bits = pltpu.bitcast(r, I32)
            mono = ((bits ^ ((bits >> 31) & jnp.int32(0x7FFFFFFF))) >> 16) + 32768
            tok = 512 * b + 4 * (32 * ((lane8 >> 5) ^ l2) + (lane8 & 31)) + l2
            key = pltpu.bitcast((mono << 11) + (2047 - tok) + jnp.int32(0x00800000), F32)
            t = 4 * b + l2
            topk[t // 8] = key if t % 8 == 0 else jnp.where(sub8 == t % 8, key, topk[t // 8])
        return st

    def b_norm(b):
        st = b_fin(b)
        for us in (range(CB // 16), range(CB // 16, NU)):
            for l2 in range(4):
                mb, rs = st[l2]
                for u in us:
                    e_, o_ = _unpack2(xp[4 * l2 + b, zrow(u), :])
                    xnp[4 * l2 + b, pl.ds(8 * u, 8), :] = _pack2((e_ - mb) * rs, (o_ - mb) * rs)

    wrow = wr[...].reshape(1, D)
    wr16b[...] = pltpu.bitcast(jnp.concatenate([jnp.broadcast_to(wrow, (8, D)), jnp.ones((8, D), BF16)], axis=0), I32)
    wsum[...] = jnp.broadcast_to(jnp.sum(wrow.astype(F32), axis=1, keepdims=True), (8, 128))
    topk[2] = jnp.zeros((8, 128), F32)
    cols[...] = jnp.zeros(cols.shape, I32)

    elt_dep = []

    def c_fwd(i):
        h0 = i.off(CB // 2, 0, 8)
        r0 = i.off(CB, 0, 8)
        for l2 in range(4):
            lhs = _bf(xnp[pl.ds(4 * l2, 4), pl.ds(h0, CB // 2), :].reshape(2 * CB, 128))
            res = jnp.dot(lhs, _bf(fpk[l2, pl.ds(step_zero(i), 64), :]), preferred_element_type=F32)
            for ri in range(2):
                y = res[:, 128 * ri:128 * ri + 128]
                if l2 == 3 and ri == 1 and isinstance(i.i, int) and i.i < 2:
                    y = pad_tail(y, i)
                uhat[2 * l2 + ri, :, pl.ds(r0, CB), :] = y.reshape(4, CB, 128)
            yield

    def c_mid(i):
        for k in range(CB // 8):
            rows = pl.ds(i.off(CB, 8 * k, 8), 8)
            krows = pl.ds(i.off(CB, 16 * (k // 2) + k % 2), 8, stride=2)
            uu = [_fft4([(uhat[2 * l2, b, rows, :], uhat[2 * l2 + 1, b, rows, :]) for l2 in range(4)], -1)
                  for b in range(4)]
            yy = [[None] * 4 for _ in range(4)]
            for k2s in ((0, 2), (1, 3)):
                pps = {k2: [None] * 4 for k2 in k2s}
                for k2, pp in pps.items():
                    for dl in range(3, -1, -1):
                        kk = (khat[2 * k2, dl, krows, :], khat[2 * k2 + 1, dl, krows, :])
                        for m in range(3, dl - 1, -1):
                            t = _cmul(*uu[m - dl][k2], *kk)
                            pp[m] = t if pp[m] is None else (pp[m][0] + t[0], pp[m][1] + t[1])
                for k2, pp in pps.items():
                    for m in range(3, -1, -1):
                        yy[m][k2] = pp[0] if m == 0 else (pp[m][0] - pp[m - 1][1], pp[m][1] + pp[m - 1][0])
            un = i.off(CB // 8, k)
            for bp in range(2):
                ww = [_fft4(yy[m], 1) for m in (2 * bp, 2 * bp + 1)]
                for l2 in range(4):
                    for ri in range(2):
                        yhat[2 * l2 + ri, bp, un] = _pack2(ww[0][l2][ri], ww[1][l2][ri])
            yield

    def c_inv(i):
        u0 = i.off(CB // 8)
        r0 = i.off(2 * CB, 0, 8)
        for l2 in range(4):
            for ri in range(2):
                lhs = _bf(yhat[2 * l2 + ri, :, pl.ds(u0, CB // 8)].reshape(2 * CB, 128))
                y = lax.dot_general(lhs, _bf(fpk[l2, pl.ds(step_zero(i), 64), pl.ds(128 * ri, 128)]), _NT,
                                    preferred_element_type=F32)
                if l2 == 3 and ri == 1 and isinstance(i.i, int):
                    y = pad_tail(y, i)
                ybuf[2 * l2 + ri, :, pl.ds(r0, 2 * CB), :] = y.reshape(2, 2 * CB, 128)
            yield

    def c_elt(i):
        for k in range(CB // 16):
            hr = pl.ds(i.off(CB // 2, 8 * k, 8), 8)
            sk = [skip[pl.ds(i.off(CB, 16 * k + e), 8, stride=2), :] for e in range(2)]
            for b in range(4):
                o = []
                for l2 in range(4):
                    w = xnp[4 * l2 + b, hr, :]
                    if elt_dep:
                        w = after(w, elt_dep)
                    xn = _unpack2(w)
                    xx = _unpack2(xp[4 * l2 + b, hr, :])
                    ss, v = [], []
                    for e in range(2):
                        yr = pl.ds(i.off(2 * CB, 32 * k + 2 * e + b % 2), 8, stride=4)
                        ss.append(ybuf[2 * l2, b // 2, yr, :] + ybuf[2 * l2 + 1, b // 2, yr, :] + xn[e] * sk[e])
                        v.append(xx[e] + ss[e] * _silu(xn[e]))
                    spk[4 * l2 + b, hr, :] = _pack2(*ss)
                    o.append(_pack2(*v))
                p = _butterfly(o)
                for j in range(4):
                    opk[4 * b + j, hr, :] = p[j]
                yield

    def c_top(i):
        k0, k1 = topk[i.off(0, 0)], topk[i.off(0, 1)]
        mx = jnp.max(jnp.max(jnp.maximum(k0, k1), axis=0, keepdims=True), axis=1, keepdims=True)
        topk[i.off(0, 0)] = jnp.where(k0 == mx, 0.0, k0)
        topk[i.off(0, 1)] = jnp.where(k1 == mx, 0.0, k1)
        topk[i.off(0, 2)] = jnp.where(sub8 == i.idx(), mx, topk[i.off(0, 2)])
        yield

    def c_first(i):
        yield from c_fwd(i)
        yield from c_top(i)

    c_pro, c_loop, _ = _pipeline([c_first, c_mid, c_inv, c_elt], NB, newz,
                                 weave=[1] * (CB // 8) + [3] * (CB // 4) + [0, 0, 2, 2, 0, 0, 2, 2])

    def first_fwd():
        for _ in c_first(_Idx(0, 0)):
            pass

    def each(fn, *bs):
        return [lambda b=b: fn(b) for b in bs]

    def add_dskip():
        skip[...] = skip[...] + column(dsk[...].astype(F32).reshape(1, D))

    block(a_tail[0], *each(b_gather, 0, 1))
    block(add_dskip, a_tail[1], *each(b_gather, 2, 3), *each(b_dot, 0, 1), *each(b_stat, 0, 1))
    block(*each(b_stat, 2, 3), *each(b_norm, 0, 1), *each(b_dot, 2, 3))
    block(*each(b_norm, 2, 3), first_fwd)
    block(c_pro[1])
    block(c_pro[2])
    c_loop()

    sel = pltpu.bitcast(topk[2], I32) - jnp.int32(0x00800000)
    mono = (sel >> 11) - 32768
    r_sel = pltpu.bitcast((mono ^ ((mono >> 31) & jnp.int32(0x7FFF))) << 16, F32)
    gate_r = _rbf(jax.nn.sigmoid(r_sel))
    posv[...] = 2047 - (sel & 2047)
    tok = [posv[c, 0] for c in range(C)]
    nat = [(t >> 7, t & 127) for t in tok]
    prm = []
    for t in tok:
        l2, l1 = t & 3, (t >> 2) & 127
        prm.append((4 * l2 + (t >> 9), 32 * ((l1 >> 5) ^ l2) + (l1 & 31)))

    def extract(src, k):
        for c, (tp, pp) in enumerate(prm):
            sh = (c - pp) & 127
            for u in range(NU):
                pltpu.store(cols.at[k, pl.ds(8 * u, 8), :], pltpu.roll(src[tp, pl.ds(8 * u, 8), :], sh, 1),
                            mask=lane8 == c)

    for c, (tp, pp) in enumerate(prm):
        ohb[c] = jnp.where(jnp.logical_and(sub8 == c // 2, lane8 == pp), jnp.int32(0x3F80 << (16 * (c % 2))), 0)

    def take_rows():
        for c, (tp, pp) in enumerate(prm):
            xsel_ref[c] = lax.dot_general(_bf(ohb[c]), _bf(xnp[tp]), _NT, preferred_element_type=F32)[:8]

    def stages(*items):
        def run():
            z = newz()
            for fn, k in items:
                for _ in fn(_Idx(k, 0, z)):
                    pass
        return run

    block(stages((c_mid, NB - 1), (c_inv, NB - 2)))
    block(stages((c_elt, NB - 3), (c_inv, NB - 1)), take_rows, lambda: extract(xp, 0))

    def o_gather(us):
        for j in range(4):
            pat = pats[4 + j]
            for b in range(4):
                for u in us:
                    v = _gather(opk[4 * b + j, pl.ds(8 * u, 8), :], pat)
                    og[4 * b + j, pl.ds(8 * u, 8), :] = v
                    o_store(u, v, pl.ds(512 * b + 128 * j, 128))

    def o_store(u, v, col):
        obuf[pl.ds(16 * u, 8), col] = _bf(v[0:4])
        obuf[pl.ds(16 * u + 8, 8), col] = _bf(pltpu.roll(v, 4, 0)[0:4])

    bits = jnp.int32(0)
    for c in range(C):
        bits = bits | (jnp.int32(1) << nat[c][0])

    cp_bar.start()

    def send(routed, a, n):
        for t in range(16):
            @pl.when(((bits >> t) & 1) == routed)
            def _():
                col = pl.ds(128 * t, 128)
                pltpu.make_async_copy(obuf.at[pl.ds(a, n), col], out_hbm.at[pl.ds(a, n), col], sem_out).start()

    late = {1: (0, 256), 3: (256, 256), 4: (512, 64)}

    def project(w, post, ks):
        fill = [g for k in ks for g in [c_elt(_Idx(k, 0))] * (CB // 4)]
        nt, done = F // 128, 0
        for t in range(nt):
            ps = [jnp.dot(xsel_b[:, a:a + n], w[pl.ds(a, n), pl.ds(128 * t, 128)],
                          preferred_element_type=F32)[:8] for a, n in chunks]
            v = _rbf((ps[0] + ps[1]) + (ps[2] + ps[3]) + ps[4])
            elt_dep[:] = [v]
            post(t, v)
            while done * nt < (t + 1) * len(fill):
                next(fill[done], None)
                done += 1
        elt_dep.clear()

    def post_gate(t, ga):
        hbuf[:, pl.ds(128 * t, 128)] = _rbf(ga * _rbf(jax.nn.sigmoid(ga)))

    def post_up(t, up):
        h = hbuf[:, pl.ds(128 * t, 128)] * up
        hpk[:, pl.ds(128 * t, 128)] = pltpu.bitcast(
            jnp.concatenate([h, jnp.zeros((8, 128), F32)], axis=0).astype(BF16), I32)

    cp_g.wait()
    xsel = xsel_ref[0]
    for c in range(1, C):
        xsel = xsel + xsel_ref[c]
    xsel_b = jnp.concatenate([xsel, jnp.zeros((8, D), F32)], axis=0).astype(BF16)
    project(wg, post_gate, (NB - 2, NB - 1))
    o_gather(range(28))
    cp_u.wait()
    project(wu, post_up, ())
    o_gather(range(28, 32))
    o_gather(range(32, NU))
    extract(spk, 1)
    pr = (r128 & (-16)) + 2 * (r128 & 7) + ((r128 >> 3) & 1)
    perm = jnp.where(pr == c128, 1.0, 0.0).astype(BF16)

    def patch(q, y):
        a, n = chunks[q]
        z = _rbf(xsel[:8, a:a + n] + _rbf(_rbf(y[:8]) * gate_r[:, :1]))
        g = z * _rbf(jax.nn.sigmoid(z))
        g = jnp.concatenate([g, jnp.zeros((120, n), F32)], axis=0).astype(BF16)
        gt = lax.dot_general(perm[:n, :n], g, _NT, preferred_element_type=F32)
        us = range(a // 16, (a + n) // 16)
        zz = newz()
        for u in us:
            hr = pl.ds(pl.multiple_of(zz + 8 * u, 8), 8)
            xx, ss = _unpack2(cols[0, hr, :]), _unpack2(cols[1, hr, :])
            r0 = 16 * u - a
            w = _pack2(*[xx[e] + _rbf(ss[e] * gt[r0 + 8 * e:r0 + 8 * e + 8]) for e in range(2)])
            for c, (tn, pn) in enumerate(nat):
                tt = 4 * (tn >> 2) + (tn & 3)
                pltpu.store(og.at[tt, pl.ds(8 * u, 8), :], pltpu.roll(w, (pn - c) & 127, 1), mask=lane8 == pn)
        for c, (tn, pn) in enumerate(nat):
            for u in us:
                v = og[tn, pl.ds(8 * u, 8), :]
                o_store(u, v, pl.ds(pl.multiple_of(tn * 128, 128), 128))
        if q in late:
            send(1, *late[q])

    send(0, 0, D)
    def down(q, f0, f1):
        a, n = chunks[q]
        return lax.dot_general(_bf(hpk[:, pl.ds(f0, f1 - f0)]), wd[pl.ds(a, n), pl.ds(f0, f1 - f0)], _NT,
                               preferred_element_type=F32)[:8]

    prev = None
    for q, fs in enumerate((0, 1280, 1280, 0, 2560)):
        if q % 3 == 0:
            for cp in cp_d[q:q + 3]:
                cp.wait()
        y0 = down(q, 0, fs) if fs else None
        if prev is not None:
            patch(*prev)
        y = down(q, fs, F)
        prev = (q, y if y0 is None else y0 + y)
    cp_bar.wait()
    patch(*prev)
    pltpu.make_async_copy(obuf, out_hbm, sem_out).wait()


def _scratch():
    return [
        pltpu.VMEM((D, L), BF16),
        pltpu.VMEM((6, D, N), BF16),
        pltpu.VMEM((D,), BF16),
        pltpu.VMEM((D,), BF16),
        pltpu.VMEM((D,), BF16),
        pltpu.VMEM((D, F), BF16),
        pltpu.VMEM((D, F), BF16),
        pltpu.VMEM((D, F), BF16),
        pltpu.VMEM((4, 64, 256), I32),
        pltpu.VMEM(_PROWS.shape, I32),
        pltpu.VMEM((_NPAT, 8, 128), I32),
        pltpu.VMEM((D, 128), F32),
        pltpu.VMEM((D, 128), F32),
        pltpu.VMEM((5, 2 * D, 128), I32),
        pltpu.VMEM((5, 2 * D, 128), I32),
        pltpu.VMEM((8, 2 * D, 128), I32),
        pltpu.VMEM((8, 2 * D, 128), I32),
        pltpu.VMEM((2, 4 * D, 128), F32),
        pltpu.VMEM((8, 4, D, 128), F32),
        pltpu.VMEM((16, D // 2, 128), I32),
        pltpu.VMEM((16, D // 2, 128), I32),
        pltpu.VMEM((8, 4, D, 128), F32),
        pltpu.VMEM((8, 2, D // 8, 8, 128), I32),
        pltpu.VMEM((8, 2, 2 * D, 128), F32),
        pltpu.VMEM((16, D // 2, 128), I32),
        pltpu.VMEM((3, 8, 128), F32),
        pltpu.VMEM((8, 128), I32),
        pltpu.VMEM((8, D), I32),
        pltpu.VMEM((8, 128), F32),
        pltpu.VMEM((C, 8, 128), I32),
        pltpu.VMEM((C, 8, D), F32),
        pltpu.VMEM((8, F), F32),
        pltpu.VMEM((8, F), I32),
        pltpu.VMEM((2, D // 2, 128), I32),
        pltpu.VMEM((16, D // 2, 128), I32),
        pltpu.VMEM((16, D // 2, 128), I32),
        pltpu.VMEM((D, L), BF16),
        pltpu.SemaphoreType.DMA((9,)),
        pltpu.SemaphoreType.DMA,
        pltpu.SemaphoreType.DMA,
    ] + [pltpu.VMEM((4, D // 2, 128), I32)] * 4 + [pltpu.VMEM((4, 24, 128), F32)] * 4


@jax.jit
def pallas_recurrent_scan__ssm_conv_s4__moe_arch_mod__prompt_kernel(
    A_u: jax.Array,
    A_A_re: jax.Array,
    A_A_im: jax.Array,
    A_B_re: jax.Array,
    A_B_im: jax.Array,
    A_C_re: jax.Array,
    A_C_im: jax.Array,
    A_log_dt: jax.Array,
    A_Dskip: jax.Array,
    B_x: jax.Array,
    B_w_r: jax.Array,
    B_w_gate: jax.Array,
    B_w_up: jax.Array,
    B_w_down: jax.Array,
):
    hbm = pl.BlockSpec(memory_space=pltpu.HBM)
    out = pl.pallas_call(
        _kernel,
        out_shape=jax.ShapeDtypeStruct((D, L), BF16),
        in_specs=[hbm] * 14,
        out_specs=hbm,
        scratch_shapes=_scratch(),
        compiler_params=pltpu.CompilerParams(vmem_limit_bytes=110 * 1024 * 1024),
        name="s4_mod",
    )(A_u[0].T, A_A_re, A_A_im, A_B_re, A_B_im, A_C_re, A_C_im, A_log_dt, A_Dskip, B_w_r,
      B_w_gate, B_w_up, B_w_down.T, jnp.asarray(_PROWS))
    return out.T[None]
```

```python
import numpy as np
import jax
import jax.numpy as jnp
from jax import lax
import jax.experimental.pallas as pl
import jax.experimental.pallas.tpu as pltpu

L, D, N, F, C = 2048, 576, 128, 4608, 8
NU = D // 16
CB = 64
NB = D // CB
FG0 = 3
UA = 4
F32, BF16, I32 = jnp.float32, jnp.bfloat16, jnp.int32
EPS = 1e-5


def _bf16_round_np(x):
    u = np.asarray(x, np.float32).view(np.uint32).astype(np.uint64)
    r = ((u + 0x7FFF + ((u >> 16) & 1)) >> 16) << 16
    return r.astype(np.uint32)


_LROUND = _bf16_round_np(np.arange(L)).view(np.float32).astype(np.int64)
_HI = [(1, 3, 516, 1032), (5, 7, 520, 1288), (4, 260, 772, 1544), (8, 264, 776, 1800), (2, 6, 258, 262)]


def _comp_q():
    t = np.arange(8)[:, None]
    lane = np.arange(128)[None, :]
    return ((lane - 8 - 7 * (t % 4)) % 16) // 4


def _make_tables():
    lane = np.arange(128)
    lo = 8 * (4 * (lane // 16) + lane % 4)
    tab = [dict(), dict()]
    amask = np.zeros(128, bool)
    for q in range(5):
        for e in range(4):
            for par in range(2):
                t = 4 * par + e
                for h in range(2):
                    src = lane[(lane // 4) % 4 == 2 * h + par]
                    dst = (src + (4 * (q % 4) - 8 * h + 8) + 7 * t) % 128
                    assert np.all(_comp_q()[t, dst] == q % 4)
                    sid = e if q < 4 else 4 + e // 2
                    for sl, dl_ in zip(src, dst):
                        ent = (sid, int(dl_))
                        assert tab[par].setdefault(_HI[q][e] + int(lo[sl]), ent) == ent
                    if q == 4 and e % 2 == 1:
                        amask[dst % 16 + 16 * np.arange(8)[:, None]] = True
    pats = []
    for j in range(4):
        pats.append(np.tile(4 * (lane % 32) + ((lane // 32) ^ j), (8, 1)))
    for j in range(4):
        pats.append(np.tile(32 * ((lane % 4) ^ j) + lane // 4, (8, 1)))
    npat0 = len(pats)
    tiles, tile_of = [], {}
    for dl in range(4):
        for l2 in range(4):
            v = _LROUND[512 * dl + 4 * lane + l2]
            key = tuple(v.tolist())
            if key in tile_of:
                tile_of[dl, l2] = tile_of[key]
                continue
            sid = np.array([tab[0][x][0] if x else -1 for x in v])
            ln = np.array([[tab[s8 % 2][x][1] if x else 0 for x in v] for s8 in range(8)])
            steps = []
            for s in sorted(set(sid.tolist()), key=lambda s: -(sid == s).sum()):
                lanes = np.nonzero(sid == s)[0]
                if s < 0:
                    steps.append((-1, None, lanes))
                    continue
                care = sid == s
                kk = None
                for k in range(npat0, len(pats)):
                    oldp, oldc, olds = pats[k]
                    both = care & oldc
                    if olds == s and np.array_equal(oldp[:, both], ln[:, both]):
                        pats[k] = (np.where(care, ln, oldp), care | oldc, s)
                        kk = k
                        break
                if kk is None:
                    pats.append((np.where(care, ln, 0), care, s))
                    kk = len(pats) - 1
                steps.append((s, kk, lanes))
            tiles.append(steps)
            tile_of[key] = tile_of[dl, l2] = len(tiles) - 1
    pats = np.stack([p if k < npat0 else p[0] for k, p in enumerate(pats)]).astype(np.int32)
    tile_of = {k: v for k, v in tile_of.items() if len(k) == 2}
    rows = np.concatenate([pats[:, :2].reshape(-1, 128), amask[None].astype(np.int32)])
    rows = np.concatenate([rows, np.zeros((-len(rows) % 8, 128), np.int32)])
    return tiles, tile_of, len(pats), rows


_TILES, _TILE_OF, _NGAT, _PROWS = _make_tables()
_NPAT = _NGAT + 3


def _cmul(ar, ai, br, bi):
    return ar * br - ai * bi, ar * bi + ai * br


def _sincos(b):
    magic = jnp.float32(12582912.0)
    t = b * jnp.float32(2.0 / np.pi) + magic
    k = t - magic
    ki = pltpu.bitcast(t, I32)
    r = b - k * jnp.float32(1.5703125)
    r = r - k * jnp.float32(0.0004837512969970703)
    r = r - k * jnp.float32(7.549790126404332e-08)
    u = r * r
    ps = (jnp.float32(-0.0001958295761141926) * u + jnp.float32(0.008332725614309311)) * u \
        + jnp.float32(-0.166666641831398)
    sn = r + (r * u) * ps
    pc = ((jnp.float32(2.437065268168226e-05) * u + jnp.float32(-0.0013886778615415096)) * u
          + jnp.float32(0.04166663438081741)) * u + jnp.float32(-0.5)
    cs = pc * u + jnp.float32(1.0)
    odd = (ki & 1) == 1
    s1 = jnp.where(odd, cs, sn)
    c1 = jnp.where(odd, sn, cs)
    sign = jnp.int32(-2147483648)
    s1 = pltpu.bitcast(pltpu.bitcast(s1, I32) ^ ((ki << 30) & sign), F32)
    c1 = pltpu.bitcast(pltpu.bitcast(c1, I32) ^ (((ki + 1) << 30) & sign), F32)
    return s1, c1


def _gather(x, idx):
    return jnp.take_along_axis(x, idx, axis=1, mode="promise_in_bounds")


def _lanes_mask(lanes):
    lane = lax.broadcasted_iota(I32, (8, 128), 1)
    lanes = sorted(int(x) for x in lanes)
    runs, start, prev = [], lanes[0], lanes[0]
    for x in lanes[1:]:
        if x != prev + 1:
            runs.append((start, prev))
            start = x
        prev = x
    runs.append((start, prev))
    m = None
    for a, b in runs:
        t = (lane == a) if a == b else jnp.logical_and(lane >= a, lane <= b)
        m = t if m is None else jnp.logical_or(m, t)
    return m


def _butterfly(p):
    lane = lax.broadcasted_iota(I32, p[0].shape, 1)
    b0 = (lane & 32) != 0
    b1 = (lane & 64) != 0
    t = [jnp.where(b0, p[k ^ 1], p[k]) for k in range(4)]
    return [jnp.where(b1, t[k ^ 2], t[k]) for k in range(4)]


def _fft4(x, sgn):
    (ar, ai), (br, bi), (cr, ci), (dr, di) = x
    s0r, s0i, d0r, d0i = ar + cr, ai + ci, ar - cr, ai - ci
    s1r, s1i, d1r, d1i = br + dr, bi + di, br - dr, bi - di
    y0 = (s0r + s1r, s0i + s1i)
    y2 = (s0r - s1r, s0i - s1i)
    p = (d0r - d1i, d0i + d1r)
    m = (d0r + d1i, d0i - d1r)
    return [y0, p, y2, m] if sgn > 0 else [y0, m, y2, p]


def _silu(z):
    h = z * jnp.float32(0.5)
    return h + h * jnp.tanh(h)


def _sigmoid(z):
    return jnp.tanh(z * jnp.float32(0.5)) * jnp.float32(0.5) + jnp.float32(0.5)


def _rbf(x):
    return x.astype(BF16).astype(F32)


def _pack2(a, b):
    p = pltpu.pack_elementwise([a, b], packed_dtype=BF16)
    return p if p.dtype == I32 else pltpu.bitcast(p, I32)


def _unpack2(x):
    return [pltpu.unpack_elementwise(x, index=i, packed_dtype=BF16, unpacked_dtype=F32) for i in range(2)]


def _bf(x):
    return pltpu.bitcast(x, BF16)


_NT = (((1,), (1,)), ((), ()))


class _Idx:
    def __init__(self, i, lag, z=None):
        self.i, self.lag, self.z = i, lag, z

    def off(self, stride, const=0, align=None):
        c = const - self.lag * stride
        if isinstance(self.i, int):
            if self.z is None:
                return self.i * stride + c
            v = self.z + (self.i * stride + c)
        else:
            v = self.i * stride + c
        return pl.multiple_of(v, align) if align else v

    def idx(self):
        return self.i - self.lag


def _pipeline(stages, n, newz, weave=None, reset=None):
    ns = len(stages)

    def step(i, lo, hi):
        z = newz() if isinstance(i, int) else None
        gens = {k: stages[k](_Idx(i, k, z)) for k in range(lo, hi)}
        if reset is not None:
            reset()
        if callable(weave):
            weave(gens)
        else:
            for k in weave or ():
                if k in gens:
                    next(gens[k], None)
        for k in range(hi - 1, lo - 1, -1):
            for _ in gens[k]:
                pass

    def body(i, carry):
        step(i, 0, ns)
        return carry

    return ([lambda i=i: step(i, 0, i + 1) for i in range(ns - 1)],
            lambda: lax.fori_loop(ns - 1, n, body, 0),
            [lambda i=i: step(n + i, i + 1, ns) for i in range(ns - 1)])


def _kernel(x_hbm, are_hbm, aim_hbm, bre_hbm, bim_hbm, cre_hbm, cim_hbm, ldt_hbm, dsk_hbm, wr_hbm,
            wg_hbm, wu_hbm, wd_hbm, pat_hbm,
            out_hbm,
            xbuf, par, ldt, dsk, wr, wg, wu, wd, fpk, prow, pats,
            dtcol, skip, hi_re, hi_im, lo_re, lo_im, comp, khat,
            xp, xnp, uhat, yhat, ybuf, spk, topk, posv, wr16b, wsum, ohb, xsel_ref, hbuf, hpk, cols, opk, og, obuf,
            sem_in, sem_out, sem_bar, *perb):
    xg, stat = perb[0:4], perb[4:8]
    p_hbm = (are_hbm, aim_hbm, bre_hbm, bim_hbm, cre_hbm, cim_hbm)
    r1 = 16 * UA
    small = [(ldt_hbm, ldt), (pat_hbm, prow)]
    for a, n in ((0, r1), (r1, r1), (2 * r1, D - 2 * r1)):
        small += [(h.at[pl.ds(a, n)], par.at[i, pl.ds(a, n)]) for i, h in enumerate(p_hbm)]
    small += [(wr_hbm, wr), (dsk_hbm, dsk)]
    cps = [pltpu.make_async_copy(s, d, sem_in.at[min((i + 4) // 6, 3)]) for i, (s, d) in enumerate(small)]
    ns = 4
    cp_x = pltpu.make_async_copy(x_hbm, xbuf, sem_in.at[ns])
    cp_g = pltpu.make_async_copy(wg_hbm, wg, sem_in.at[ns + 1])
    cp_u = pltpu.make_async_copy(wu_hbm, wu, sem_in.at[ns + 2])
    chunks = [(0, 128), (128, 128), (256, 128), (384, 128), (512, 64)]
    cp_d = [pltpu.make_async_copy(wd_hbm.at[pl.ds(a, n)], wd.at[pl.ds(a, n)], sem_in.at[ns + 3 + q // 3])
            for q, (a, n) in enumerate(chunks)]
    cp_bar = pltpu.make_async_copy(pat_hbm.at[pl.ds(0, 8)], posv, sem_bar)
    for cp in cps + [cp_x, cp_g, cp_u] + cp_d:
        cp.start()

    sub8 = lax.broadcasted_iota(I32, (8, 128), 0)
    lane8 = lax.broadcasted_iota(I32, (8, 128), 1)

    def dft_rows(l2):
        for g in range(8):
            cs = []
            for e in range(2):
                p = 16 * g + 2 * sub8 + e
                t = 4 * (32 * ((p >> 5) ^ l2) + (p & 31)) + l2
                n = ((4 * lane8 + 1) * t) & 2047
                cs.append(_sincos(n.astype(F32) * jnp.float32(-2.0 * np.pi / 2048)))
            fpk[l2, pl.ds(8 * g, 8), pl.ds(0, 128)] = _pack2(cs[0][1], cs[1][1])
            fpk[l2, pl.ds(8 * g, 8), pl.ds(128, 128)] = _pack2(cs[0][0], cs[1][0])

    for l2 in range(FG0):
        dft_rows(l2)

    for cp in cps[:2]:
        cp.wait()
    for l2 in range(FG0, 4):
        dft_rows(l2)
    for k in range(_NGAT):
        pats[k] = jnp.where((sub8 & 1) == 1, jnp.broadcast_to(prow[pl.ds(2 * k + 1, 1), :], (8, 128)),
                            jnp.broadcast_to(prow[pl.ds(2 * k, 1), :], (8, 128)))
    cq = ((lane8 - 8 - 7 * (sub8 & 3)) & 15) >> 2
    pats[_NGAT] = cq & 1
    pats[_NGAT + 1] = cq >> 1
    pats[_NGAT + 2] = jnp.broadcast_to(prow[pl.ds(2 * _NGAT, 1), :], (8, 128))
    r128 = lax.broadcasted_iota(I32, (128, 128), 0)
    c128 = lax.broadcasted_iota(I32, (128, 128), 1)

    def column(row):
        pk = pltpu.bitcast(jnp.broadcast_to(row, (8, D)), I32)
        lhs = []
        for u in range(NU):
            t = u // 8
            v = pk[:, 128 * t:128 * t + 128] if t < 4 else jnp.concatenate([pk[:, 512:], pk[:, 512:]], axis=1)
            c0 = 16 * (u % 8) + 2 * sub8
            lhs.append(jnp.where(lane8 == c0, lax.shift_right_logical(v, 16), jnp.where(lane8 == c0 + 1, v, 0)))
        ones = jnp.ones((128, 128), BF16)
        return jnp.concatenate([jnp.dot(_bf(jnp.concatenate(lhs[k:k + NU // 4], axis=0)), ones,
                                        preferred_element_type=F32) for k in range(0, NU, NU // 4)], axis=0)

    dtcol[...] = column(_rbf(jnp.exp(ldt[...].astype(F32).reshape(1, D))))

    zero = prow[0, 0]
    zcount = [0]

    def newz():
        zcount[0] += 1
        return zero * (64 * zcount[0])

    def block(*fns):
        def body(k, carry):
            for fn in fns:
                fn()
            return carry

        lax.fori_loop(0, zero + 1, body, 0)

    def step_zero(i):
        t = i.off(1) * zero if not isinstance(i.i, int) or i.z is None else i.z
        return pl.multiple_of(t * 8, 8)

    def after(x, deps):
        never = pats[0] < 0
        d = None
        for v in deps:
            v = v if v.dtype == I32 else pltpu.bitcast(v, I32)
            d = v if d is None else d ^ v
        return jnp.where(never, d if x.dtype == I32 else pltpu.bitcast(d, x.dtype), x)

    def pad_tail(y, i):
        n, k = 16, y.shape[0] - 64
        base = i.off(1)
        mid = after(y[k:k + 8], [pats[j % _NPAT] * (base + j) for j in range(n)])
        return jnp.concatenate([y[:k], mid, y[k + 8:]], axis=0)

    class Sched:
        tok, g, pre = {}, 0, []

        @classmethod
        def reset(cls):
            cls.tok, cls.g, cls.pre = {}, 0, []

        @classmethod
        def gate(cls, x):
            deps = cls.tok.pop(cls.g, [])
            cls.g += 1
            if not deps:
                return x
            return jnp.concatenate([after(x[:8], deps), after(x[8:], deps[-1:])], axis=0)

    slot = {h: (q, e) for q, ent in enumerate(_HI) for e, h in enumerate(ent)}

    def a_prep(i):
        gate = Sched.gate
        for u in range(UA):
            rows = pl.ds(i.off(16 * UA, 16 * u, 16), 16)
            ev = pl.ds(i.off(32 * UA, 32 * u), 16, stride=2)
            od = pl.ds(i.off(32 * UA, 32 * u + 1), 16, stride=2)
            dt = gate(dtcol[rows, :])
            al = dt * par[0, rows, :].astype(F32)
            be = dt * par[1, rows, :].astype(F32)
            cr, ci = _cmul(par[4, rows, :].astype(F32), par[5, rows, :].astype(F32),
                           par[2, rows, :].astype(F32), par[3, rows, :].astype(F32))
            dts = dt * jnp.float32(1.0 / 512)
            cr, ci = cr * dts, ci * dts
            k0 = jnp.sum(cr, axis=1, keepdims=True) * jnp.float32(512.0)
            skip[rows, :] = jnp.broadcast_to(k0, (16, 128))
            yield cr
            s, c = _sincos(gate(be))
            yield c
            pw = {1: (c, s)}
            e = 1
            while e < 256:
                if e in (1, 16):
                    c = gate(c)
                c, s = (c - s) * (c + s), (c + c) * s
                e *= 2
                pw[e] = (c, s)
                if e in (16, 256):
                    yield c
            z = {}
            for e in (1, 8, 256):
                mag = jnp.exp(al * jnp.float32(e))
                c, s = pw[e]
                z[e] = (mag * c, mag * s)
            pend = {}

            def put(tab, q, ee, v):
                key = (tab[0] is hi_re, q, ee // 2)
                if key not in pend:
                    pend[key] = (ee % 2, v)
                    return
                w, o = pend.pop(key)
                lo_, hi_ = (o, v) if w == 0 else (v, o)
                dst = od if ee // 2 else ev
                tab[0][q, dst, :] = _pack2(lo_[0], hi_[0])
                tab[1][q, dst, :] = _pack2(lo_[1], hi_[1])

            h = (cr, ci)
            cnt = 0
            for e in range(1, 9):
                g, ee, m = h, e, z[1]
                while ee in slot:
                    if cnt % 4 == 0:
                        g = (gate(g[0]), g[1])
                    g = _cmul(*g, *m)
                    put((hi_re, hi_im), *slot[ee], g)
                    if ee == e:
                        h = g
                    ee, m = ee + 256, z[256]
                    cnt += 1
                    if cnt % 4 == 0:
                        yield g[0]
            w1 = (gate(z[8][0]), -z[8][1])
            v = [(jnp.ones((16, 128), F32), jnp.zeros((16, 128), F32)), w1]
            v.append(_cmul(*w1, *w1))
            v.append(_cmul(*v[2], *w1))
            w4 = _cmul(*v[2], *v[2])
            for j in range(8):
                for f in range(4):
                    put((lo_re, lo_im), j, f, v[f])
                yield v[3][0]
                if j < 7:
                    w4 = (gate(w4[0]), w4[1])
                    v = [w4 if (j == 0 and f == 0) else _cmul(*v[f], *w4) for f in range(4)]

    def a_gen(i):
        b0 = pats[_NPAT - 3] != 0
        b1 = pats[_NPAT - 2] != 0
        for k in range(4 * UA):
            rows = pl.ds(i.off(32 * UA, 8 * k, 8), 8)
            lo = jnp.concatenate([lo_re[:, rows, :].reshape(64, 128), lo_im[:, rows, :].reshape(64, 128)], axis=1)
            h0 = hi_re[0, rows, :]
            if k % 2 == 0 and Sched.pre:
                h0 = after(h0, Sched.pre)
                Sched.pre = []
            hi = jnp.concatenate([jnp.concatenate([h0, hi_re[1:5, rows, :].reshape(32, 128)], axis=0),
                                  hi_im[:, rows, :].reshape(40, 128)], axis=1)
            o = lax.dot_general(_bf(hi), _bf(lo), _NT, preferred_element_type=F32)
            for q in range(5):
                Sched.tok.setdefault(13 + int(0.9 * (5 * (k // 2) + q)), []).append(o[16 * q + 8:16 * q + 16])
            for h in range(2):
                g = [pltpu.roll(o[16 * q + 8 * h:16 * q + 8 * h + 8], 4 * (q % 4) - 8 * h + 8, 1,
                                stride=7, stride_axis=0) for q in range(5)]
                dst = pl.ds(i.off(64 * UA, 16 * k + 8 * h, 8), 8)
                comp[0, dst, :] = jnp.where(b1, jnp.where(b0, g[3], g[2]), jnp.where(b0, g[1], g[0]))
                comp[1, dst, :] = g[4]
            if k % 2 == 1:
                yield

    def a_exp(i):
        bm = pats[_NPAT - 1] != 0
        srcs = []
        for u in range(UA):
            def ld(a, e):
                return _pack2(comp[a, pl.ds(i.off(64 * UA, 64 * u + e), 8, stride=4), :],
                              comp[a, pl.ds(i.off(64 * UA, 64 * u + 32 + e), 8, stride=4), :])

            srcs.append([ld(0, e) for e in range(4)]
                        + [jnp.where(bm, ld(1, 2 * k + 1), ld(1, 2 * k)) for k in range(2)])
        cache = {}

        def gat(s, key):
            if key not in cache:
                pat = pats[key]
                cache[key] = [_gather(srcs[u][s], pat) for u in range(UA)]
            return cache[key]

        tiles = []
        for steps in _TILES:
            t = None
            for s, key, lanes in steps:
                v = [jnp.zeros((8, 128), I32)] * UA if s < 0 else gat(s, key)
                t = v if t is None else [jnp.where(_lanes_mask(lanes), v[u], t[u]) for u in range(UA)]
            tiles.append(t)
        yield
        for u0 in range(0, UA, 2):
            lhs = [_bf(jnp.concatenate([tiles[_TILE_OF[dl, l2]][u] for dl in range(4) for u in (u0, u0 + 1)], axis=0))
                   for l2 in range(4)]
            z0 = 0 if u0 == 0 else zero * 8

            def dots(ri):
                return [jnp.dot(lhs[l2], _bf(jnp.concatenate(
                    [fpk[l2, pl.ds(z0 + 16 * (j ^ l2), 16) if u0 == 0 else
                         pl.ds(pl.multiple_of(z0 + 16 * (j ^ l2), 8), 16), pl.ds(128 * ri, 128)]
                     for j in range(4)], axis=0)), preferred_element_type=F32) for l2 in range(4)]

            def store(k2, ri, v):
                khat[2 * k2 + ri, :, pl.ds(i.off(16 * UA, 16 * u0, 16), 32), :] = v.reshape(4, 32, 128)

            def toks(v, step0):
                for j in range(8):
                    g = 13 + 9 * UA + int(0.7 * (step0 + j))
                    Sched.tok.setdefault(g, []).append(v[16 * j + 8:16 * j + 16])

            re = dots(0)
            s0, d0r, s1, d1r = re[0] + re[2], re[0] - re[2], re[1] + re[3], re[1] - re[3]
            store(0, 0, s0 + s1)
            v = s0 - s1
            store(2, 0, v)
            toks(v, 8 * u0)
            im = dots(1)
            s0, d0i, s1, d1i = im[0] + im[2], im[0] - im[2], im[1] + im[3], im[1] - im[3]
            store(0, 1, s0 + s1)
            store(2, 1, s0 - s1)
            store(1, 0, d0r + d1i)
            store(1, 1, d0i - d1r)
            store(3, 0, d0r - d1i)
            v = d0i + d1r
            store(3, 1, v)
            toks(v, 8 * u0 + 8)
            yield

    def a_weave(gens):
        if 2 in gens:
            next(gens[2])
        if 0 in gens and 1 in gens:
            for n in (3, 5, 4):
                for _ in range(n):
                    v = next(gens[0])
                Sched.pre = [v[:8], v[8:]]
                next(gens[1])
        for k in (1, 2, 0):
            if k in gens:
                for _ in gens[k]:
                    pass

    a_pro, a_loop, a_tail = _pipeline([a_prep, a_gen, a_exp], NU // UA, newz, reset=Sched.reset, weave=a_weave)
    for cp in cps[2:8]:
        cp.wait()
    a_pro[0]()
    for cp in cps[8:14]:
        cp.wait()
    a_pro[1]()
    for cp in cps[14:]:
        cp.wait()
    a_loop()

    cp_x.wait()

    def zrow(u):
        return pl.ds(pl.multiple_of(zero * 8 + 8 * u, 8), 8)

    def b_gather(b):
        for j in range(4):
            pat = pats[j]
            for u in range(NU):
                v = pltpu.bitcast(xbuf[pl.ds(16 * u, 16), pl.ds(512 * b + 128 * j, 128)], I32)
                xg[b][j, pl.ds(8 * u, 8), :] = _gather(v, pat)

    def b_stat(b):
        s2 = [jnp.zeros((8, 128), F32) for _ in range(4)]
        for u in range(NU):
            o = _butterfly([xg[b][j, zrow(u), :] for j in range(4)])
            for l2 in range(4):
                xp[4 * l2 + b, pl.ds(8 * u, 8), :] = o[l2]
                e_, o_ = _unpack2(o[l2])
                s2[l2] = s2[l2] + (e_ * e_ + o_ * o_)
        for l2 in range(4):
            stat[b][l2, pl.ds(16, 8), :] = s2[l2]

    def b_dot(b):
        lhs = _bf(wr16b[...])
        for j in range(4):
            rows = pl.ds(pl.multiple_of(zero * zero * 8, 8), D // 2)
            stat[b][j, pl.ds(0, 16), :] = jnp.dot(lhs, _bf(xg[b][j, rows, :]), preferred_element_type=F32)

    def b_norm(b0):
        wx = sx = q = None
        for b in (b0, b0 + 1):
            wxs = _butterfly([stat[b][j, zrow(0), :] for j in range(4)])
            sxs = _butterfly([stat[b][j, zrow(1), :] for j in range(4)])
            for l2 in range(4):
                qq = jnp.sum(stat[b][l2, zrow(2), :], axis=0, keepdims=True)
                here = sub8 == 4 * (b - b0) + l2
                wx = wxs[l2] if wx is None else jnp.where(here, wxs[l2], wx)
                sx = sxs[l2] if sx is None else jnp.where(here, sxs[l2], sx)
                q = jnp.broadcast_to(qq, (8, 128)) if q is None else jnp.where(here, qq, q)
        m = sx * jnp.float32(1.0 / D)
        var = _rbf(jnp.maximum(q * jnp.float32(1.0 / D) - m * m, 0.0))
        rs = 1.0 / _rbf(jnp.sqrt(_rbf(var + jnp.float32(EPS))))
        mb = _rbf(m)
        r = _rbf((wx - mb * wsum[...]) * rs)
        r = jnp.where(r == 0.0, 0.0, r)
        bits = pltpu.bitcast(r, I32)
        mono = ((bits ^ ((bits >> 31) & jnp.int32(0x7FFFFFFF))) >> 16) + 32768
        l2v = sub8 & 3
        tok = 512 * (b0 + (sub8 >> 2)) + 4 * (32 * ((lane8 >> 5) ^ l2v) + (lane8 & 31)) + l2v
        topk[b0 // 2] = pltpu.bitcast((mono << 11) + (2047 - tok) + jnp.int32(0x00800000), F32)
        for b in (b0, b0 + 1):
            st = [[jnp.broadcast_to(v[4 * (b - b0) + l2:4 * (b - b0) + l2 + 1], (8, 128)) for v in (mb, rs)]
                  for l2 in range(4)]
            for us in (range(CB // 16), range(CB // 16, NU)):
                for l2 in range(4):
                    for u in us:
                        e_, o_ = _unpack2(xp[4 * l2 + b, zrow(u), :])
                        xnp[4 * l2 + b, pl.ds(8 * u, 8), :] = _pack2((e_ - st[l2][0]) * st[l2][1],
                                                                     (o_ - st[l2][0]) * st[l2][1])

    def b_init():
        wrow = wr[...].reshape(1, D)
        wr16b[...] = pltpu.bitcast(
            jnp.concatenate([jnp.broadcast_to(wrow, (8, D)), jnp.ones((8, D), BF16)], axis=0), I32)
        wsum[...] = jnp.broadcast_to(jnp.sum(wrow.astype(F32), axis=1, keepdims=True), (8, 128))
        topk[2] = jnp.zeros((8, 128), F32)
        cols[...] = jnp.zeros(cols.shape, I32)

    elt_dep = []

    def c_fwd(i):
        h0 = i.off(CB // 2, 0, 8)
        r0 = i.off(CB, 0, 8)
        for l2 in range(4):
            lhs = _bf(xnp[pl.ds(4 * l2, 4), pl.ds(h0, CB // 2), :].reshape(2 * CB, 128))
            res = jnp.dot(lhs, _bf(fpk[l2, pl.ds(step_zero(i), 64), :]), preferred_element_type=F32)
            for ri in range(2):
                y = res[:, 128 * ri:128 * ri + 128]
                if l2 == 3 and ri == 1 and isinstance(i.i, int) and i.i < 2:
                    y = pad_tail(y, i)
                uhat[2 * l2 + ri, :, pl.ds(r0, CB), :] = y.reshape(4, CB, 128)
            yield

    def c_mid(i):
        for k in range(CB // 8):
            rows = pl.ds(i.off(CB, 8 * k, 8), 8)
            krows = pl.ds(i.off(CB, 16 * (k // 2) + k % 2), 8, stride=2)
            uu = [_fft4([(uhat[2 * l2, b, rows, :], uhat[2 * l2 + 1, b, rows, :]) for l2 in range(4)], -1)
                  for b in range(4)]
            yy = [[None] * 4 for _ in range(4)]
            for k2s in ((0, 2), (1, 3)):
                pps = {k2: [None] * 4 for k2 in k2s}
                for k2, pp in pps.items():
                    for dl in range(3, -1, -1):
                        kk = (khat[2 * k2, dl, krows, :], khat[2 * k2 + 1, dl, krows, :])
                        for m in range(3, dl - 1, -1):
                            t = _cmul(*uu[m - dl][k2], *kk)
                            pp[m] = t if pp[m] is None else (pp[m][0] + t[0], pp[m][1] + t[1])
                for k2, pp in pps.items():
                    for m in range(3, -1, -1):
                        yy[m][k2] = pp[0] if m == 0 else (pp[m][0] - pp[m - 1][1], pp[m][1] + pp[m - 1][0])
            un = i.off(CB // 8, k)
            for bp in range(2):
                ww = [_fft4(yy[m], 1) for m in (2 * bp, 2 * bp + 1)]
                for l2 in range(4):
                    for ri in range(2):
                        yhat[2 * l2 + ri, bp, un] = _pack2(ww[0][l2][ri], ww[1][l2][ri])
            yield

    def c_inv(i):
        u0 = i.off(CB // 8)
        r0 = i.off(2 * CB, 0, 8)
        for l2 in range(4):
            for ri in range(2):
                lhs = _bf(yhat[2 * l2 + ri, :, pl.ds(u0, CB // 8)].reshape(2 * CB, 128))
                y = lax.dot_general(lhs, _bf(fpk[l2, pl.ds(step_zero(i), 64), pl.ds(128 * ri, 128)]), _NT,
                                    preferred_element_type=F32)
                if l2 == 3 and ri == 1 and isinstance(i.i, int):
                    y = pad_tail(y, i)
                ybuf[2 * l2 + ri, :, pl.ds(r0, 2 * CB), :] = y.reshape(2, 2 * CB, 128)
            yield

    def c_elt(i):
        for k in range(CB // 16):
            hr = pl.ds(i.off(CB // 2, 8 * k, 8), 8)
            sk = [skip[pl.ds(i.off(CB, 16 * k + e), 8, stride=2), :] for e in range(2)]
            for b in range(4):
                o = []
                for l2 in range(4):
                    w = xnp[4 * l2 + b, hr, :]
                    if elt_dep:
                        w = after(w, elt_dep)
                    xn = _unpack2(w)
                    xx = _unpack2(xp[4 * l2 + b, hr, :])
                    ss, v = [], []
                    for e in range(2):
                        yr = pl.ds(i.off(2 * CB, 32 * k + 2 * e + b % 2), 8, stride=4)
                        ss.append(ybuf[2 * l2, b // 2, yr, :] + ybuf[2 * l2 + 1, b // 2, yr, :] + xn[e] * sk[e])
                        v.append(xx[e] + ss[e] * _silu(xn[e]))
                    spk[4 * l2 + b, hr, :] = _pack2(*ss)
                    o.append(_pack2(*v))
                p = _butterfly(o)
                for j in range(4):
                    opk[4 * b + j, hr, :] = p[j]
                yield

    def c_top(i):
        k0, k1 = topk[i.off(0, 0)], topk[i.off(0, 1)]
        mx = jnp.max(jnp.max(jnp.maximum(k0, k1), axis=0, keepdims=True), axis=1, keepdims=True)
        topk[i.off(0, 0)] = jnp.where(k0 == mx, 0.0, k0)
        topk[i.off(0, 1)] = jnp.where(k1 == mx, 0.0, k1)
        topk[i.off(0, 2)] = jnp.where(sub8 == i.idx(), mx, topk[i.off(0, 2)])
        yield

    def c_first(i):
        yield from c_fwd(i)
        yield from c_top(i)

    c_pro, c_loop, _ = _pipeline([c_first, c_mid, c_inv, c_elt], NB, newz,
                                 weave=[1] * (CB // 8) + [3] * (CB // 4) + [0, 0, 2, 2, 0, 0, 2, 2])

    def first_fwd():
        for _ in c_first(_Idx(0, 0)):
            pass

    def each(fn, *bs):
        return [lambda b=b: fn(b) for b in bs]

    def add_dskip():
        skip[...] = skip[...] + column(dsk[...].astype(F32).reshape(1, D))

    b_init()
    a_tail[0]()
    b_gather(0)
    b_gather(1)
    block(add_dskip, a_tail[1], *each(b_gather, 2, 3), *each(b_dot, 0, 1), *each(b_stat, 0, 1))
    block(*each(b_stat, 2, 3), *each(b_norm, 0), *each(b_dot, 2, 3))
    block(*each(b_norm, 2), first_fwd)
    block(c_pro[1])
    block(c_pro[2])
    c_loop()

    sel = pltpu.bitcast(topk[2], I32) - jnp.int32(0x00800000)
    mono = (sel >> 11) - 32768
    r_sel = pltpu.bitcast((mono ^ ((mono >> 31) & jnp.int32(0x7FFF))) << 16, F32)
    gate_r = _rbf(jax.nn.sigmoid(r_sel))
    posv[...] = 2047 - (sel & 2047)
    tok = [posv[c, 0] for c in range(C)]
    nat = [(t >> 7, t & 127) for t in tok]
    prm = []
    for t in tok:
        l2, l1 = t & 3, (t >> 2) & 127
        prm.append((4 * l2 + (t >> 9), 32 * ((l1 >> 5) ^ l2) + (l1 & 31)))

    def extract(src, k):
        for c, (tp, pp) in enumerate(prm):
            sh = (c - pp) & 127
            for u in range(NU):
                pltpu.store(cols.at[k, pl.ds(8 * u, 8), :], pltpu.roll(src[tp, pl.ds(8 * u, 8), :], sh, 1),
                            mask=lane8 == c)

    for c, (tp, pp) in enumerate(prm):
        ohb[c] = jnp.where(jnp.logical_and(sub8 == c // 2, lane8 == pp), jnp.int32(0x3F80 << (16 * (c % 2))), 0)

    def take_rows():
        for c, (tp, pp) in enumerate(prm):
            xsel_ref[c] = lax.dot_general(_bf(ohb[c]), _bf(xnp[tp]), _NT, preferred_element_type=F32)[:8]

    def stages(*items):
        def run():
            z = newz()
            for fn, k in items:
                for _ in fn(_Idx(k, 0, z)):
                    pass
        return run

    stages((c_mid, NB - 1), (c_inv, NB - 2))()
    block(stages((c_elt, NB - 3), (c_inv, NB - 1)), take_rows, lambda: extract(xp, 0))

    def o_gather(us):
        for j in range(4):
            pat = pats[4 + j]
            for b in range(4):
                for u in us:
                    v = _gather(opk[4 * b + j, pl.ds(8 * u, 8), :], pat)
                    og[4 * b + j, pl.ds(8 * u, 8), :] = v
                    o_store(u, v, pl.ds(512 * b + 128 * j, 128))

    def o_store(u, v, col):
        obuf[pl.ds(16 * u, 8), col] = _bf(v[0:4])
        obuf[pl.ds(16 * u + 8, 8), col] = _bf(pltpu.roll(v, 4, 0)[0:4])

    bits = jnp.int32(0)
    for c in range(C):
        bits = bits | (jnp.int32(1) << nat[c][0])

    cp_bar.start()

    def send(routed, a, n):
        for t in range(16):
            @pl.when(((bits >> t) & 1) == routed)
            def _():
                col = pl.ds(128 * t, 128)
                pltpu.make_async_copy(obuf.at[pl.ds(a, n), col], out_hbm.at[pl.ds(a, n), col], sem_out).start()

    late = {1: (0, 256), 3: (256, 256), 4: (512, 64)}

    def project(w, post, ks):
        fill = [g for k in ks for g in [c_elt(_Idx(k, 0))] * (CB // 4)]
        nt, done = F // 128, 0
        for t in range(nt):
            ps = [jnp.dot(xsel_b[:, a:a + n], w[pl.ds(a, n), pl.ds(128 * t, 128)],
                          preferred_element_type=F32)[:8] for a, n in chunks]
            v = _rbf((ps[0] + ps[1]) + (ps[2] + ps[3]) + ps[4])
            elt_dep[:] = [v]
            post(t, v)
            while done * nt < (t + 1) * len(fill):
                next(fill[done], None)
                done += 1
        elt_dep.clear()

    def post_gate(t, ga):
        hbuf[:, pl.ds(128 * t, 128)] = _rbf(ga * _rbf(_sigmoid(ga)))

    def post_up(t, up):
        h = hbuf[:, pl.ds(128 * t, 128)] * up
        hpk[:, pl.ds(128 * t, 128)] = pltpu.bitcast(
            jnp.concatenate([h, jnp.zeros((8, 128), F32)], axis=0).astype(BF16), I32)

    cp_g.wait()
    xsel = xsel_ref[0]
    for c in range(1, C):
        xsel = xsel + xsel_ref[c]
    xsel_b = jnp.concatenate([xsel, jnp.zeros((8, D), F32)], axis=0).astype(BF16)
    project(wg, post_gate, (NB - 2, NB - 1))
    o_gather(range(28))
    cp_u.wait()
    project(wu, post_up, ())
    o_gather(range(28, 32))
    o_gather(range(32, NU))
    extract(spk, 1)
    pr = (r128 & (-16)) + 2 * (r128 & 7) + ((r128 >> 3) & 1)
    perm = jnp.where(pr == c128, 1.0, 0.0).astype(BF16)

    def patch(q, y):
        a, n = chunks[q]
        z = _rbf(xsel[:8, a:a + n] + _rbf(_rbf(y[:8]) * gate_r[:, :1]))
        g = z * _rbf(_sigmoid(z))
        g = jnp.concatenate([g, jnp.zeros((120, n), F32)], axis=0).astype(BF16)
        gt = lax.dot_general(perm[:n, :n], g, _NT, preferred_element_type=F32)
        us = range(a // 16, (a + n) // 16)
        zz = newz()
        for u in us:
            hr = pl.ds(pl.multiple_of(zz + 8 * u, 8), 8)
            xx, ss = _unpack2(cols[0, hr, :]), _unpack2(cols[1, hr, :])
            r0 = 16 * u - a
            w = _pack2(*[xx[e] + _rbf(ss[e] * gt[r0 + 8 * e:r0 + 8 * e + 8]) for e in range(2)])
            for c, (tn, pn) in enumerate(nat):
                tt = 4 * (tn >> 2) + (tn & 3)
                pltpu.store(og.at[tt, pl.ds(8 * u, 8), :], pltpu.roll(w, (pn - c) & 127, 1), mask=lane8 == pn)
        for c, (tn, pn) in enumerate(nat):
            for u in us:
                v = og[tn, pl.ds(8 * u, 8), :]
                o_store(u, v, pl.ds(pl.multiple_of(tn * 128, 128), 128))
        if q in late:
            send(1, *late[q])

    send(0, 0, D)
    def down(q, f0, f1):
        a, n = chunks[q]
        return lax.dot_general(_bf(hpk[:, pl.ds(f0, f1 - f0)]), wd[pl.ds(a, n), pl.ds(f0, f1 - f0)], _NT,
                               preferred_element_type=F32)[:8]

    prev = None
    for q, fs in enumerate((0, 1280, 1280, 0, 2560)):
        if q % 3 == 0:
            for cp in cp_d[q:q + 3]:
                cp.wait()
        y0 = down(q, 0, fs) if fs else None
        if prev is not None:
            patch(*prev)
        y = down(q, fs, F)
        prev = (q, y if y0 is None else y0 + y)
    cp_bar.wait()
    patch(*prev)
    pltpu.make_async_copy(obuf, out_hbm, sem_out).wait()


def _scratch():
    return [
        pltpu.VMEM((D, L), BF16),
        pltpu.VMEM((6, D, N), BF16),
        pltpu.VMEM((D,), BF16),
        pltpu.VMEM((D,), BF16),
        pltpu.VMEM((D,), BF16),
        pltpu.VMEM((D, F), BF16),
        pltpu.VMEM((D, F), BF16),
        pltpu.VMEM((D, F), BF16),
        pltpu.VMEM((4, 64, 256), I32),
        pltpu.VMEM(_PROWS.shape, I32),
        pltpu.VMEM((_NPAT, 8, 128), I32),
        pltpu.VMEM((D, 128), F32),
        pltpu.VMEM((D, 128), F32),
        pltpu.VMEM((5, 2 * D, 128), I32),
        pltpu.VMEM((5, 2 * D, 128), I32),
        pltpu.VMEM((8, 2 * D, 128), I32),
        pltpu.VMEM((8, 2 * D, 128), I32),
        pltpu.VMEM((2, 4 * D, 128), F32),
        pltpu.VMEM((8, 4, D, 128), F32),
        pltpu.VMEM((16, D // 2, 128), I32),
        pltpu.VMEM((16, D // 2, 128), I32),
        pltpu.VMEM((8, 4, D, 128), F32),
        pltpu.VMEM((8, 2, D // 8, 8, 128), I32),
        pltpu.VMEM((8, 2, 2 * D, 128), F32),
        pltpu.VMEM((16, D // 2, 128), I32),
        pltpu.VMEM((3, 8, 128), F32),
        pltpu.VMEM((8, 128), I32),
        pltpu.VMEM((8, D), I32),
        pltpu.VMEM((8, 128), F32),
        pltpu.VMEM((C, 8, 128), I32),
        pltpu.VMEM((C, 8, D), F32),
        pltpu.VMEM((8, F), F32),
        pltpu.VMEM((8, F), I32),
        pltpu.VMEM((2, D // 2, 128), I32),
        pltpu.VMEM((16, D // 2, 128), I32),
        pltpu.VMEM((16, D // 2, 128), I32),
        pltpu.VMEM((D, L), BF16),
        pltpu.SemaphoreType.DMA((9,)),
        pltpu.SemaphoreType.DMA,
        pltpu.SemaphoreType.DMA,
    ] + [pltpu.VMEM((4, D // 2, 128), I32)] * 4 + [pltpu.VMEM((4, 24, 128), F32)] * 4


@jax.jit
def pallas_recurrent_scan__ssm_conv_s4__moe_arch_mod__prompt_kernel(
    A_u: jax.Array,
    A_A_re: jax.Array,
    A_A_im: jax.Array,
    A_B_re: jax.Array,
    A_B_im: jax.Array,
    A_C_re: jax.Array,
    A_C_im: jax.Array,
    A_log_dt: jax.Array,
    A_Dskip: jax.Array,
    B_x: jax.Array,
    B_w_r: jax.Array,
    B_w_gate: jax.Array,
    B_w_up: jax.Array,
    B_w_down: jax.Array,
):
    hbm = pl.BlockSpec(memory_space=pltpu.HBM)
    out = pl.pallas_call(
        _kernel,
        out_shape=jax.ShapeDtypeStruct((D, L), BF16),
        in_specs=[hbm] * 14,
        out_specs=hbm,
        scratch_shapes=_scratch(),
        compiler_params=pltpu.CompilerParams(vmem_limit_bytes=110 * 1024 * 1024),
        name="s4_mod",
    )(A_u[0].T, A_A_re, A_A_im, A_B_re, A_B_im, A_C_re, A_C_im, A_log_dt, A_Dskip, B_w_r,
      B_w_gate, B_w_up, B_w_down.T, jnp.asarray(_PROWS))
    return out.T[None]
```

```python
import numpy as np
import jax
import jax.numpy as jnp
from jax import lax
import jax.experimental.pallas as pl
import jax.experimental.pallas.tpu as pltpu

L, D, N, F, C = 2048, 576, 128, 4608, 8
NU = D // 16
CB = 64
NB = D // CB
FG0 = 3
UA = 4
F32, BF16, I32 = jnp.float32, jnp.bfloat16, jnp.int32
EPS = 1e-5


def _bf16_round_np(x):
    u = np.asarray(x, np.float32).view(np.uint32).astype(np.uint64)
    r = ((u + 0x7FFF + ((u >> 16) & 1)) >> 16) << 16
    return r.astype(np.uint32)


_LROUND = _bf16_round_np(np.arange(L)).view(np.float32).astype(np.int64)
_HI = [(1, 3, 516, 1032), (5, 7, 520, 1288), (4, 260, 772, 1544), (8, 264, 776, 1800), (2, 6, 258, 262)]


def _comp_q():
    t = np.arange(8)[:, None]
    lane = np.arange(128)[None, :]
    return ((lane - 8 - 7 * (t % 4)) % 16) // 4


def _make_tables():
    lane = np.arange(128)
    lo = 8 * (4 * (lane // 16) + lane % 4)
    tab = [dict(), dict()]
    amask = np.zeros(128, bool)
    for q in range(5):
        for e in range(4):
            for par in range(2):
                t = 4 * par + e
                for h in range(2):
                    src = lane[(lane // 4) % 4 == 2 * h + par]
                    dst = (src + (4 * (q % 4) - 8 * h + 8) + 7 * t) % 128
                    assert np.all(_comp_q()[t, dst] == q % 4)
                    sid = e if q < 4 else 4 + e // 2
                    for sl, dl_ in zip(src, dst):
                        ent = (sid, int(dl_))
                        assert tab[par].setdefault(_HI[q][e] + int(lo[sl]), ent) == ent
                    if q == 4 and e % 2 == 1:
                        amask[dst % 16 + 16 * np.arange(8)[:, None]] = True
    pats = []
    for j in range(4):
        pats.append(np.tile(4 * (lane % 32) + ((lane // 32) ^ j), (8, 1)))
    for j in range(4):
        pats.append(np.tile(32 * ((lane % 4) ^ j) + lane // 4, (8, 1)))
    npat0 = len(pats)
    tiles, tile_of = [], {}
    for dl in range(4):
        for l2 in range(4):
            v = _LROUND[512 * dl + 4 * lane + l2]
            key = tuple(v.tolist())
            if key in tile_of:
                tile_of[dl, l2] = tile_of[key]
                continue
            sid = np.array([tab[0][x][0] if x else -1 for x in v])
            ln = np.array([[tab[s8 % 2][x][1] if x else 0 for x in v] for s8 in range(8)])
            steps = []
            for s in sorted(set(sid.tolist()), key=lambda s: -(sid == s).sum()):
                lanes = np.nonzero(sid == s)[0]
                if s < 0:
                    steps.append((-1, None, lanes))
                    continue
                care = sid == s
                kk = None
                for k in range(npat0, len(pats)):
                    oldp, oldc, olds = pats[k]
                    both = care & oldc
                    if olds == s and np.array_equal(oldp[:, both], ln[:, both]):
                        pats[k] = (np.where(care, ln, oldp), care | oldc, s)
                        kk = k
                        break
                if kk is None:
                    pats.append((np.where(care, ln, 0), care, s))
                    kk = len(pats) - 1
                steps.append((s, kk, lanes))
            tiles.append(steps)
            tile_of[key] = tile_of[dl, l2] = len(tiles) - 1
    pats = np.stack([p if k < npat0 else p[0] for k, p in enumerate(pats)]).astype(np.int32)
    tile_of = {k: v for k, v in tile_of.items() if len(k) == 2}
    rows = np.concatenate([pats[:, :2].reshape(-1, 128), amask[None].astype(np.int32)])
    rows = np.concatenate([rows, np.zeros((-len(rows) % 8, 128), np.int32)])
    return tiles, tile_of, len(pats), rows


_TILES, _TILE_OF, _NGAT, _PROWS = _make_tables()
_NPAT = _NGAT + 3


def _cmul(ar, ai, br, bi):
    return ar * br - ai * bi, ar * bi + ai * br


def _sincos(b):
    magic = jnp.float32(12582912.0)
    t = b * jnp.float32(2.0 / np.pi) + magic
    k = t - magic
    ki = pltpu.bitcast(t, I32)
    r = b - k * jnp.float32(1.5703125)
    r = r - k * jnp.float32(0.0004837512969970703)
    r = r - k * jnp.float32(7.549790126404332e-08)
    u = r * r
    ps = (jnp.float32(-0.0001958295761141926) * u + jnp.float32(0.008332725614309311)) * u \
        + jnp.float32(-0.166666641831398)
    sn = r + (r * u) * ps
    pc = ((jnp.float32(2.437065268168226e-05) * u + jnp.float32(-0.0013886778615415096)) * u
          + jnp.float32(0.04166663438081741)) * u + jnp.float32(-0.5)
    cs = pc * u + jnp.float32(1.0)
    odd = (ki & 1) == 1
    s1 = jnp.where(odd, cs, sn)
    c1 = jnp.where(odd, sn, cs)
    sign = jnp.int32(-2147483648)
    s1 = pltpu.bitcast(pltpu.bitcast(s1, I32) ^ ((ki << 30) & sign), F32)
    c1 = pltpu.bitcast(pltpu.bitcast(c1, I32) ^ (((ki + 1) << 30) & sign), F32)
    return s1, c1


def _gather(x, idx):
    return jnp.take_along_axis(x, idx, axis=1, mode="promise_in_bounds")


def _lanes_mask(lanes):
    lane = lax.broadcasted_iota(I32, (8, 128), 1)
    lanes = sorted(int(x) for x in lanes)
    runs, start, prev = [], lanes[0], lanes[0]
    for x in lanes[1:]:
        if x != prev + 1:
            runs.append((start, prev))
            start = x
        prev = x
    runs.append((start, prev))
    m = None
    for a, b in runs:
        t = (lane == a) if a == b else jnp.logical_and(lane >= a, lane <= b)
        m = t if m is None else jnp.logical_or(m, t)
    return m


def _butterfly(p):
    lane = lax.broadcasted_iota(I32, p[0].shape, 1)
    b0 = (lane & 32) != 0
    b1 = (lane & 64) != 0
    t = [jnp.where(b0, p[k ^ 1], p[k]) for k in range(4)]
    return [jnp.where(b1, t[k ^ 2], t[k]) for k in range(4)]


def _fft4(x, sgn):
    (ar, ai), (br, bi), (cr, ci), (dr, di) = x
    s0r, s0i, d0r, d0i = ar + cr, ai + ci, ar - cr, ai - ci
    s1r, s1i, d1r, d1i = br + dr, bi + di, br - dr, bi - di
    y0 = (s0r + s1r, s0i + s1i)
    y2 = (s0r - s1r, s0i - s1i)
    p = (d0r - d1i, d0i + d1r)
    m = (d0r + d1i, d0i - d1r)
    return [y0, p, y2, m] if sgn > 0 else [y0, m, y2, p]


def _silu(z):
    h = z * jnp.float32(0.5)
    return h + h * jnp.tanh(h)


def _sigmoid(z):
    return jnp.tanh(z * jnp.float32(0.5)) * jnp.float32(0.5) + jnp.float32(0.5)


def _rbf(x):
    return x.astype(BF16).astype(F32)


def _pack2(a, b):
    p = pltpu.pack_elementwise([a, b], packed_dtype=BF16)
    return p if p.dtype == I32 else pltpu.bitcast(p, I32)


def _unpack2(x):
    return [pltpu.unpack_elementwise(x, index=i, packed_dtype=BF16, unpacked_dtype=F32) for i in range(2)]


def _bf(x):
    return pltpu.bitcast(x, BF16)


_NT = (((1,), (1,)), ((), ()))


class _Idx:
    def __init__(self, i, lag, z=None):
        self.i, self.lag, self.z = i, lag, z

    def off(self, stride, const=0, align=None):
        c = const - self.lag * stride
        if isinstance(self.i, int):
            if self.z is None:
                return self.i * stride + c
            v = self.z + (self.i * stride + c)
        else:
            v = self.i * stride + c
        return pl.multiple_of(v, align) if align else v

    def idx(self):
        return self.i - self.lag


def _pipeline(stages, n, newz, weave=None, reset=None):
    ns = len(stages)

    def step(i, lo, hi):
        z = newz() if isinstance(i, int) else None
        gens = {k: stages[k](_Idx(i, k, z)) for k in range(lo, hi)}
        if reset is not None:
            reset()
        if callable(weave):
            weave(gens)
        else:
            for k in weave or ():
                if k in gens:
                    next(gens[k], None)
        for k in range(hi - 1, lo - 1, -1):
            for _ in gens[k]:
                pass

    def body(i, carry):
        step(i, 0, ns)
        return carry

    return ([lambda i=i: step(i, 0, i + 1) for i in range(ns - 1)],
            lambda: lax.fori_loop(ns - 1, n, body, 0),
            [lambda i=i: step(n + i, i + 1, ns) for i in range(ns - 1)])


def _kernel(x_hbm, are_hbm, aim_hbm, bre_hbm, bim_hbm, cre_hbm, cim_hbm, ldt_hbm, dsk_hbm, wr_hbm,
            wg_hbm, wu_hbm, wd_hbm, pat_hbm,
            out_hbm,
            xbuf, par, ldt, dsk, wr, wg, wu, wd, fpk, prow, pats,
            dtcol, skip, hi_re, hi_im, lo_re, lo_im, comp, khat,
            xp, xnp, uhat, yhat, ybuf, spk, topk, posv, wr16b, wsum, ohb, xsel_ref, hbuf, hpk, cols, opk, og, obuf,
            sem_in, sem_out, sem_bar, *perb):
    xg, stat = perb[0:4], perb[4:8]
    p_hbm = (are_hbm, aim_hbm, bre_hbm, bim_hbm, cre_hbm, cim_hbm)
    r1 = 16 * UA
    small = [(ldt_hbm, ldt), (pat_hbm, prow)]
    for a, n in ((0, r1), (r1, r1), (2 * r1, D - 2 * r1)):
        small += [(h.at[pl.ds(a, n)], par.at[i, pl.ds(a, n)]) for i, h in enumerate(p_hbm)]
    small += [(wr_hbm, wr), (dsk_hbm, dsk)]
    cps = [pltpu.make_async_copy(s, d, sem_in.at[min((i + 4) // 6, 3)]) for i, (s, d) in enumerate(small)]
    ns = 4
    cp_x = pltpu.make_async_copy(x_hbm, xbuf, sem_in.at[ns])
    cp_g = pltpu.make_async_copy(wg_hbm, wg, sem_in.at[ns + 1])
    cp_u = pltpu.make_async_copy(wu_hbm, wu, sem_in.at[ns + 2])
    chunks = [(0, 128), (128, 128), (256, 128), (384, 128), (512, 64)]
    cp_d = [pltpu.make_async_copy(wd_hbm.at[pl.ds(a, n)], wd.at[pl.ds(a, n)], sem_in.at[ns + 3 + (0, 1, 1, 2, 2)[q]])
            for q, (a, n) in enumerate(chunks)]
    cp_bar = pltpu.make_async_copy(pat_hbm.at[pl.ds(0, 8)], posv, sem_bar)
    for cp in cps + [cp_x, cp_g, cp_u] + cp_d:
        cp.start()

    sub8 = lax.broadcasted_iota(I32, (8, 128), 0)
    lane8 = lax.broadcasted_iota(I32, (8, 128), 1)

    def dft_rows(l2):
        for g in range(8):
            cs = []
            for e in range(2):
                p = 16 * g + 2 * sub8 + e
                t = 4 * (32 * ((p >> 5) ^ l2) + (p & 31)) + l2
                n = ((4 * lane8 + 1) * t) & 2047
                cs.append(_sincos(n.astype(F32) * jnp.float32(-2.0 * np.pi / 2048)))
            fpk[l2, pl.ds(8 * g, 8), pl.ds(0, 128)] = _pack2(cs[0][1], cs[1][1])
            fpk[l2, pl.ds(8 * g, 8), pl.ds(128, 128)] = _pack2(cs[0][0], cs[1][0])

    for l2 in range(FG0):
        dft_rows(l2)

    for cp in cps[:2]:
        cp.wait()
    for l2 in range(FG0, 4):
        dft_rows(l2)
    for k in range(_NGAT):
        pats[k] = jnp.where((sub8 & 1) == 1, jnp.broadcast_to(prow[pl.ds(2 * k + 1, 1), :], (8, 128)),
                            jnp.broadcast_to(prow[pl.ds(2 * k, 1), :], (8, 128)))
    cq = ((lane8 - 8 - 7 * (sub8 & 3)) & 15) >> 2
    pats[_NGAT] = cq & 1
    pats[_NGAT + 1] = cq >> 1
    pats[_NGAT + 2] = jnp.broadcast_to(prow[pl.ds(2 * _NGAT, 1), :], (8, 128))
    r128 = lax.broadcasted_iota(I32, (128, 128), 0)
    c128 = lax.broadcasted_iota(I32, (128, 128), 1)

    def column(row):
        pk = pltpu.bitcast(jnp.broadcast_to(row, (8, D)), I32)
        lhs = []
        for u in range(NU):
            t = u // 8
            v = pk[:, 128 * t:128 * t + 128] if t < 4 else jnp.concatenate([pk[:, 512:], pk[:, 512:]], axis=1)
            c0 = 16 * (u % 8) + 2 * sub8
            lhs.append(jnp.where(lane8 == c0, lax.shift_right_logical(v, 16), jnp.where(lane8 == c0 + 1, v, 0)))
        ones = jnp.ones((128, 128), BF16)
        return jnp.concatenate([jnp.dot(_bf(jnp.concatenate(lhs[k:k + NU // 4], axis=0)), ones,
                                        preferred_element_type=F32) for k in range(0, NU, NU // 4)], axis=0)

    dtcol[...] = column(_rbf(jnp.exp(ldt[...].astype(F32).reshape(1, D))))

    zero = prow[0, 0]
    zcount = [0]

    def newz():
        zcount[0] += 1
        return zero * (64 * zcount[0])

    def block(*fns):
        def body(k, carry):
            for fn in fns:
                fn()
            return carry

        lax.fori_loop(0, zero + 1, body, 0)

    def step_zero(i):
        t = i.off(1) * zero if not isinstance(i.i, int) or i.z is None else i.z
        return pl.multiple_of(t * 8, 8)

    def after(x, deps):
        never = pats[0] < 0
        d = None
        for v in deps:
            v = v if v.dtype == I32 else pltpu.bitcast(v, I32)
            d = v if d is None else d ^ v
        return jnp.where(never, d if x.dtype == I32 else pltpu.bitcast(d, x.dtype), x)

    def pad_tail(y, i):
        n, k = 16, y.shape[0] - 64
        base = i.off(1)
        mid = after(y[k:k + 8], [pats[j % _NPAT] * (base + j) for j in range(n)])
        return jnp.concatenate([y[:k], mid, y[k + 8:]], axis=0)

    class Sched:
        tok, g, pre = {}, 0, []

        @classmethod
        def reset(cls):
            cls.tok, cls.g, cls.pre = {}, 0, []

        @classmethod
        def gate(cls, x):
            deps = cls.tok.pop(cls.g, [])
            cls.g += 1
            if not deps:
                return x
            return jnp.concatenate([after(x[:8], deps), after(x[8:], deps[-1:])], axis=0)

    slot = {h: (q, e) for q, ent in enumerate(_HI) for e, h in enumerate(ent)}

    def a_prep(i):
        gate = Sched.gate
        for u in range(UA):
            rows = pl.ds(i.off(16 * UA, 16 * u, 16), 16)
            ev = pl.ds(i.off(32 * UA, 32 * u), 16, stride=2)
            od = pl.ds(i.off(32 * UA, 32 * u + 1), 16, stride=2)
            dt = gate(dtcol[rows, :])
            al = dt * par[0, rows, :].astype(F32)
            be = dt * par[1, rows, :].astype(F32)
            cr, ci = _cmul(par[4, rows, :].astype(F32), par[5, rows, :].astype(F32),
                           par[2, rows, :].astype(F32), par[3, rows, :].astype(F32))
            dts = dt * jnp.float32(1.0 / 512)
            cr, ci = cr * dts, ci * dts
            k0 = jnp.sum(cr, axis=1, keepdims=True) * jnp.float32(512.0)
            skip[rows, :] = jnp.broadcast_to(k0, (16, 128))
            yield cr
            s, c = _sincos(gate(be))
            yield c
            pw = {1: (c, s)}
            e = 1
            while e < 256:
                if e in (1, 16):
                    c = gate(c)
                c, s = (c - s) * (c + s), (c + c) * s
                e *= 2
                pw[e] = (c, s)
                if e in (16, 256):
                    yield c
            z = {}
            for e in (1, 8, 256):
                mag = jnp.exp(al * jnp.float32(e))
                c, s = pw[e]
                z[e] = (mag * c, mag * s)
            pend = {}

            def put(tab, q, ee, v):
                key = (tab[0] is hi_re, q, ee // 2)
                if key not in pend:
                    pend[key] = (ee % 2, v)
                    return
                w, o = pend.pop(key)
                lo_, hi_ = (o, v) if w == 0 else (v, o)
                dst = od if ee // 2 else ev
                tab[0][q, dst, :] = _pack2(lo_[0], hi_[0])
                tab[1][q, dst, :] = _pack2(lo_[1], hi_[1])

            h = (cr, ci)
            cnt = 0
            for e in range(1, 9):
                g, ee, m = h, e, z[1]
                while ee in slot:
                    if cnt % 4 == 0:
                        g = (gate(g[0]), g[1])
                    g = _cmul(*g, *m)
                    put((hi_re, hi_im), *slot[ee], g)
                    if ee == e:
                        h = g
                    ee, m = ee + 256, z[256]
                    cnt += 1
                    if cnt % 4 == 0:
                        yield g[0]
            w1 = (gate(z[8][0]), -z[8][1])
            v = [(jnp.ones((16, 128), F32), jnp.zeros((16, 128), F32)), w1]
            v.append(_cmul(*w1, *w1))
            v.append(_cmul(*v[2], *w1))
            w4 = _cmul(*v[2], *v[2])
            for j in range(8):
                for f in range(4):
                    put((lo_re, lo_im), j, f, v[f])
                yield v[3][0]
                if j < 7:
                    w4 = (gate(w4[0]), w4[1])
                    v = [w4 if (j == 0 and f == 0) else _cmul(*v[f], *w4) for f in range(4)]

    def a_gen(i):
        b0 = pats[_NPAT - 3] != 0
        b1 = pats[_NPAT - 2] != 0
        for k in range(4 * UA):
            rows = pl.ds(i.off(32 * UA, 8 * k, 8), 8)
            lo = jnp.concatenate([lo_re[:, rows, :].reshape(64, 128), lo_im[:, rows, :].reshape(64, 128)], axis=1)
            h0 = hi_re[0, rows, :]
            if k % 2 == 0 and Sched.pre:
                h0 = after(h0, Sched.pre)
                Sched.pre = []
            hi = jnp.concatenate([jnp.concatenate([h0, hi_re[1:5, rows, :].reshape(32, 128)], axis=0),
                                  hi_im[:, rows, :].reshape(40, 128)], axis=1)
            o = lax.dot_general(_bf(hi), _bf(lo), _NT, preferred_element_type=F32)
            for q in range(5):
                Sched.tok.setdefault(13 + int(0.9 * (5 * (k // 2) + q)), []).append(o[16 * q + 8:16 * q + 16])
            for h in range(2):
                g = [pltpu.roll(o[16 * q + 8 * h:16 * q + 8 * h + 8], 4 * (q % 4) - 8 * h + 8, 1,
                                stride=7, stride_axis=0) for q in range(5)]
                dst = pl.ds(i.off(64 * UA, 16 * k + 8 * h, 8), 8)
                comp[0, dst, :] = jnp.where(b1, jnp.where(b0, g[3], g[2]), jnp.where(b0, g[1], g[0]))
                comp[1, dst, :] = g[4]
            if k % 2 == 1:
                yield

    def a_exp(i):
        bm = pats[_NPAT - 1] != 0
        srcs = []
        for u in range(UA):
            def ld(a, e):
                return _pack2(comp[a, pl.ds(i.off(64 * UA, 64 * u + e), 8, stride=4), :],
                              comp[a, pl.ds(i.off(64 * UA, 64 * u + 32 + e), 8, stride=4), :])

            srcs.append([ld(0, e) for e in range(4)]
                        + [jnp.where(bm, ld(1, 2 * k + 1), ld(1, 2 * k)) for k in range(2)])
        cache = {}

        def gat(s, key):
            if key not in cache:
                pat = pats[key]
                cache[key] = [_gather(srcs[u][s], pat) for u in range(UA)]
            return cache[key]

        tiles = []
        for steps in _TILES:
            t = None
            for s, key, lanes in steps:
                v = [jnp.zeros((8, 128), I32)] * UA if s < 0 else gat(s, key)
                t = v if t is None else [jnp.where(_lanes_mask(lanes), v[u], t[u]) for u in range(UA)]
            tiles.append(t)
        yield
        for u0 in range(0, UA, 2):
            lhs = [_bf(jnp.concatenate([tiles[_TILE_OF[dl, l2]][u] for dl in range(4) for u in (u0, u0 + 1)], axis=0))
                   for l2 in range(4)]
            z0 = 0 if u0 == 0 else zero * 8

            def dots(ri):
                return [jnp.dot(lhs[l2], _bf(jnp.concatenate(
                    [fpk[l2, pl.ds(z0 + 16 * (j ^ l2), 16) if u0 == 0 else
                         pl.ds(pl.multiple_of(z0 + 16 * (j ^ l2), 8), 16), pl.ds(128 * ri, 128)]
                     for j in range(4)], axis=0)), preferred_element_type=F32) for l2 in range(4)]

            def store(k2, ri, v):
                khat[2 * k2 + ri, :, pl.ds(i.off(16 * UA, 16 * u0, 16), 32), :] = v.reshape(4, 32, 128)

            def toks(v, step0):
                for j in range(8):
                    g = 13 + 9 * UA + int(0.7 * (step0 + j))
                    Sched.tok.setdefault(g, []).append(v[16 * j + 8:16 * j + 16])

            re = dots(0)
            s0, d0r, s1, d1r = re[0] + re[2], re[0] - re[2], re[1] + re[3], re[1] - re[3]
            store(0, 0, s0 + s1)
            v = s0 - s1
            store(2, 0, v)
            toks(v, 8 * u0)
            im = dots(1)
            s0, d0i, s1, d1i = im[0] + im[2], im[0] - im[2], im[1] + im[3], im[1] - im[3]
            store(0, 1, s0 + s1)
            store(2, 1, s0 - s1)
            store(1, 0, d0r + d1i)
            store(1, 1, d0i - d1r)
            store(3, 0, d0r - d1i)
            v = d0i + d1r
            store(3, 1, v)
            toks(v, 8 * u0 + 8)
            yield

    def a_weave(gens):
        if 2 in gens:
            next(gens[2])
        if 0 in gens and 1 in gens:
            for n in (3, 5, 4):
                for _ in range(n):
                    v = next(gens[0])
                Sched.pre = [v[:8], v[8:]]
                next(gens[1])
        for k in (1, 2, 0):
            if k in gens:
                for _ in gens[k]:
                    pass

    a_pro, a_loop, a_tail = _pipeline([a_prep, a_gen, a_exp], NU // UA, newz, reset=Sched.reset, weave=a_weave)
    for cp in cps[2:8]:
        cp.wait()
    a_pro[0]()
    for cp in cps[8:14]:
        cp.wait()
    a_pro[1]()
    for cp in cps[14:]:
        cp.wait()
    a_loop()

    cp_x.wait()

    def zrow(u):
        return pl.ds(pl.multiple_of(zero * 8 + 8 * u, 8), 8)

    def b_gather(b):
        for j in range(4):
            pat = pats[j]
            for u in range(NU):
                v = pltpu.bitcast(xbuf[pl.ds(16 * u, 16), pl.ds(512 * b + 128 * j, 128)], I32)
                v = _gather(v, pat)
                xg[b][j, pl.ds(8 * u, 8), :] = v
                gtok.setdefault(b, []).append(v)

    gtok = {}

    def b_stat(b, ride=None):
        s2 = [jnp.zeros((8, 128), F32) for _ in range(4)]
        for u in range(NU):
            x = [xg[b][j, zrow(u), :] for j in range(4)]
            if ride is not None:
                x = [after(x[0], [gtok[ride][4 * u]]), x[1], after(x[2], [gtok[ride][4 * u]]), x[3]]
            o = _butterfly(x)
            for l2 in range(4):
                xp[4 * l2 + b, pl.ds(8 * u, 8), :] = o[l2]
                e_, o_ = _unpack2(o[l2])
                s2[l2] = s2[l2] + (e_ * e_ + o_ * o_)
        for l2 in range(4):
            stat[b][l2, pl.ds(16, 8), :] = s2[l2]

    def b_dot(b):
        lhs = _bf(wr16b[...])
        for j in range(4):
            rows = pl.ds(pl.multiple_of(zero * zero * 8, 8), D // 2)
            stat[b][j, pl.ds(0, 16), :] = jnp.dot(lhs, _bf(xg[b][j, rows, :]), preferred_element_type=F32)

    def b_fin(b0):
        wx = sx = q = None
        for b in (b0, b0 + 1):
            wxs = _butterfly([stat[b][j, zrow(0), :] for j in range(4)])
            sxs = _butterfly([stat[b][j, zrow(1), :] for j in range(4)])
            for l2 in range(4):
                qq = jnp.sum(stat[b][l2, zrow(2), :], axis=0, keepdims=True)
                here = sub8 == 4 * (b - b0) + l2
                wx = wxs[l2] if wx is None else jnp.where(here, wxs[l2], wx)
                sx = sxs[l2] if sx is None else jnp.where(here, sxs[l2], sx)
                q = jnp.broadcast_to(qq, (8, 128)) if q is None else jnp.where(here, qq, q)
        m = sx * jnp.float32(1.0 / D)
        var = _rbf(jnp.maximum(q * jnp.float32(1.0 / D) - m * m, 0.0))
        rs = 1.0 / _rbf(jnp.sqrt(_rbf(var + jnp.float32(EPS))))
        mb = _rbf(m)
        r = _rbf((wx - mb * wsum[...]) * rs)
        r = jnp.where(r == 0.0, 0.0, r)
        bits = pltpu.bitcast(r, I32)
        mono = ((bits ^ ((bits >> 31) & jnp.int32(0x7FFFFFFF))) >> 16) + 32768
        l2v = sub8 & 3
        tok = 512 * (b0 + (sub8 >> 2)) + 4 * (32 * ((lane8 >> 5) ^ l2v) + (lane8 & 31)) + l2v
        topk[b0 // 2] = pltpu.bitcast((mono << 11) + (2047 - tok) + jnp.int32(0x00800000), F32)
        return mb, rs

    def b_scale(b0, st, us):
        for k in range(8):
            t = 4 * (k % 4) + b0 + k // 4
            mk, rk = [jnp.broadcast_to(v[k:k + 1], (8, 128)) for v in st]
            for u in us:
                e_, o_ = _unpack2(xp[t, zrow(u), :])
                xnp[t, pl.ds(8 * u, 8), :] = _pack2((e_ - mk) * rk, (o_ - mk) * rk)

    def b_norm(b0):
        st = b_fin(b0)
        for us in (range(CB // 16), range(CB // 16, NU)):
            b_scale(b0, st, us)

    def b_init():
        wrow = wr[...].reshape(1, D)
        wr16b[...] = pltpu.bitcast(
            jnp.concatenate([jnp.broadcast_to(wrow, (8, D)), jnp.ones((8, D), BF16)], axis=0), I32)
        wsum[...] = jnp.broadcast_to(jnp.sum(wrow.astype(F32), axis=1, keepdims=True), (8, 128))
        topk[2] = jnp.zeros((8, 128), F32)
        cols[...] = jnp.zeros(cols.shape, I32)

    elt_dep = []

    def c_fwd(i):
        h0 = i.off(CB // 2, 0, 8)
        r0 = i.off(CB, 0, 8)
        for l2 in range(4):
            lhs = _bf(xnp[pl.ds(4 * l2, 4), pl.ds(h0, CB // 2), :].reshape(2 * CB, 128))
            res = jnp.dot(lhs, _bf(fpk[l2, pl.ds(step_zero(i), 64), :]), preferred_element_type=F32)
            for ri in range(2):
                y = res[:, 128 * ri:128 * ri + 128]
                if l2 == 3 and ri == 1 and isinstance(i.i, int) and i.i < 2:
                    y = pad_tail(y, i)
                uhat[2 * l2 + ri, :, pl.ds(r0, CB), :] = y.reshape(4, CB, 128)
            yield

    def c_mid(i):
        for k in range(CB // 8):
            rows = pl.ds(i.off(CB, 8 * k, 8), 8)
            krows = pl.ds(i.off(CB, 16 * (k // 2) + k % 2), 8, stride=2)
            uu = [_fft4([(uhat[2 * l2, b, rows, :], uhat[2 * l2 + 1, b, rows, :]) for l2 in range(4)], -1)
                  for b in range(4)]
            yy = [[None] * 4 for _ in range(4)]
            for k2s in ((0, 2), (1, 3)):
                pps = {k2: [None] * 4 for k2 in k2s}
                for k2, pp in pps.items():
                    for dl in range(3, -1, -1):
                        kk = (khat[2 * k2, dl, krows, :], khat[2 * k2 + 1, dl, krows, :])
                        for m in range(3, dl - 1, -1):
                            t = _cmul(*uu[m - dl][k2], *kk)
                            pp[m] = t if pp[m] is None else (pp[m][0] + t[0], pp[m][1] + t[1])
                for k2, pp in pps.items():
                    for m in range(3, -1, -1):
                        yy[m][k2] = pp[0] if m == 0 else (pp[m][0] - pp[m - 1][1], pp[m][1] + pp[m - 1][0])
            un = i.off(CB // 8, k)
            for bp in range(2):
                ww = [_fft4(yy[m], 1) for m in (2 * bp, 2 * bp + 1)]
                for l2 in range(4):
                    for ri in range(2):
                        yhat[2 * l2 + ri, bp, un] = _pack2(ww[0][l2][ri], ww[1][l2][ri])
            yield

    def c_inv(i):
        u0 = i.off(CB // 8)
        r0 = i.off(2 * CB, 0, 8)
        for l2 in range(4):
            for ri in range(2):
                lhs = _bf(yhat[2 * l2 + ri, :, pl.ds(u0, CB // 8)].reshape(2 * CB, 128))
                y = lax.dot_general(lhs, _bf(fpk[l2, pl.ds(step_zero(i), 64), pl.ds(128 * ri, 128)]), _NT,
                                    preferred_element_type=F32)
                if l2 == 3 and ri == 1 and isinstance(i.i, int):
                    y = pad_tail(y, i)
                ybuf[2 * l2 + ri, :, pl.ds(r0, 2 * CB), :] = y.reshape(2, 2 * CB, 128)
            yield

    def c_elt(i):
        for k in range(CB // 16):
            hr = pl.ds(i.off(CB // 2, 8 * k, 8), 8)
            sk = [skip[pl.ds(i.off(CB, 16 * k + e), 8, stride=2), :] for e in range(2)]
            for b in range(4):
                o = []
                for l2 in range(4):
                    w = xnp[4 * l2 + b, hr, :]
                    if elt_dep:
                        w = after(w, elt_dep)
                    xn = _unpack2(w)
                    xx = _unpack2(xp[4 * l2 + b, hr, :])
                    ss, v = [], []
                    for e in range(2):
                        yr = pl.ds(i.off(2 * CB, 32 * k + 2 * e + b % 2), 8, stride=4)
                        ss.append(ybuf[2 * l2, b // 2, yr, :] + ybuf[2 * l2 + 1, b // 2, yr, :] + xn[e] * sk[e])
                        v.append(xx[e] + ss[e] * _silu(xn[e]))
                    spk[4 * l2 + b, hr, :] = _pack2(*ss)
                    o.append(_pack2(*v))
                p = _butterfly(o)
                for j in range(4):
                    opk[4 * b + j, hr, :] = p[j]
                yield

    def c_top(i):
        k0, k1 = topk[i.off(0, 0)], topk[i.off(0, 1)]
        mx = jnp.max(jnp.max(jnp.maximum(k0, k1), axis=0, keepdims=True), axis=1, keepdims=True)
        topk[i.off(0, 0)] = jnp.where(k0 == mx, 0.0, k0)
        topk[i.off(0, 1)] = jnp.where(k1 == mx, 0.0, k1)
        topk[i.off(0, 2)] = jnp.where(sub8 == i.idx(), mx, topk[i.off(0, 2)])
        yield

    def c_first(i):
        yield from c_fwd(i)
        yield from c_top(i)

    c_pro, c_loop, _ = _pipeline([c_first, c_mid, c_inv, c_elt], NB, newz,
                                 weave=[1] * (CB // 8) + [3] * (CB // 4) + [0, 0, 2, 2, 0, 0, 2, 2])

    def first_fwd():
        for _ in c_first(_Idx(0, 0)):
            pass

    def each(fn, *bs):
        return [lambda b=b: fn(b) for b in bs]

    def add_dskip():
        skip[...] = skip[...] + column(dsk[...].astype(F32).reshape(1, D))

    b_init()
    a_tail[0]()
    b_gather(0)
    b_gather(1)
    b_stat(0, 1)
    block(add_dskip, a_tail[1], *each(b_gather, 2, 3), *each(b_dot, 0, 1),
          lambda: b_stat(1, 2), lambda: b_stat(2, 3))
    block(*each(b_stat, 3), *each(b_norm, 0), *each(b_dot, 2, 3))
    block(*each(b_norm, 2), first_fwd)
    block(c_pro[1])
    block(c_pro[2])
    c_loop()

    sel = pltpu.bitcast(topk[2], I32) - jnp.int32(0x00800000)
    mono = (sel >> 11) - 32768
    r_sel = pltpu.bitcast((mono ^ ((mono >> 31) & jnp.int32(0x7FFF))) << 16, F32)
    gate_r = _rbf(jax.nn.sigmoid(r_sel))
    posv[...] = 2047 - (sel & 2047)
    tok = [posv[c, 0] for c in range(C)]
    nat = [(t >> 7, t & 127) for t in tok]
    prm = []
    for t in tok:
        l2, l1 = t & 3, (t >> 2) & 127
        prm.append((4 * l2 + (t >> 9), 32 * ((l1 >> 5) ^ l2) + (l1 & 31)))

    xtok = []

    def extract(src, k):
        for c, (tp, pp) in enumerate(prm):
            sh = (c - pp) & 127
            for u in range(NU):
                v = pltpu.roll(src[tp, pl.ds(8 * u, 8), :], sh, 1)
                pltpu.store(cols.at[k, pl.ds(8 * u, 8), :], v, mask=lane8 == c)
                xtok.append(v)

    for c, (tp, pp) in enumerate(prm):
        ohb[c] = jnp.where(jnp.logical_and(sub8 == c // 2, lane8 == pp), jnp.int32(0x3F80 << (16 * (c % 2))), 0)

    def take_rows():
        for c, (tp, pp) in enumerate(prm):
            xsel_ref[c] = lax.dot_general(_bf(ohb[c]), _bf(xnp[tp]), _NT, preferred_element_type=F32)[:8]

    def drain(*gens):
        for g in gens:
            for _ in g:
                pass

    z = newz()
    drain(c_mid(_Idx(NB - 1, 0, z)), c_inv(_Idx(NB - 2, 0, z)))

    def last_inverse():
        z = newz()
        drain(c_inv(_Idx(NB - 1, 0, z)))
        take_rows()
        extract(xp, 0)
        fill = [g for k in (NB - 3, NB - 2) for g in [c_elt(_Idx(k, 0, z))] * (CB // 4)]
        for n, g in enumerate(fill):
            elt_dep[:] = [xtok[n * len(xtok) // len(fill)]]
            next(g, None)
        elt_dep.clear()

    block(last_inverse)

    def o_gather(us):
        for j in range(4):
            pat = pats[4 + j]
            for b in range(4):
                for u in us:
                    v = _gather(opk[4 * b + j, pl.ds(8 * u, 8), :], pat)
                    og[4 * b + j, pl.ds(8 * u, 8), :] = v
                    o_store(u, v, pl.ds(512 * b + 128 * j, 128))

    def o_store(u, v, col):
        obuf[pl.ds(16 * u, 8), col] = _bf(v[0:4])
        obuf[pl.ds(16 * u + 8, 8), col] = _bf(pltpu.roll(v, 4, 0)[0:4])

    bits = jnp.int32(0)
    for c in range(C):
        bits = bits | (jnp.int32(1) << nat[c][0])

    cp_bar.start()

    def send(routed, a, n):
        for t in range(16):
            @pl.when(((bits >> t) & 1) == routed)
            def _():
                col = pl.ds(128 * t, 128)
                pltpu.make_async_copy(obuf.at[pl.ds(a, n), col], out_hbm.at[pl.ds(a, n), col], sem_out).start()

    late = {1: (0, 256), 3: (256, 256), 4: (512, 64)}

    def project(w, post, ks):
        fill = [g for k in ks for g in [c_elt(_Idx(k, 0))] * (CB // 4)]
        nt, done = F // 128, 0
        for t in range(nt):
            ps = [jnp.dot(xsel_b[:, a:a + n], w[pl.ds(a, n), pl.ds(128 * t, 128)],
                          preferred_element_type=F32)[:8] for a, n in chunks]
            v = _rbf((ps[0] + ps[1]) + (ps[2] + ps[3]) + ps[4])
            elt_dep[:] = [v]
            post(t, v)
            while done * nt < (t + 1) * len(fill):
                next(fill[done], None)
                done += 1
        elt_dep.clear()

    def post_gate(t, ga):
        hbuf[:, pl.ds(128 * t, 128)] = _rbf(ga * _rbf(_sigmoid(ga)))

    def post_up(t, up):
        h = hbuf[:, pl.ds(128 * t, 128)] * up
        hpk[:, pl.ds(128 * t, 128)] = pltpu.bitcast(
            jnp.concatenate([h, jnp.zeros((8, 128), F32)], axis=0).astype(BF16), I32)

    cp_g.wait()
    xsel = xsel_ref[0]
    for c in range(1, C):
        xsel = xsel + xsel_ref[c]
    xsel_b = jnp.concatenate([xsel, jnp.zeros((8, D), F32)], axis=0).astype(BF16)
    project(wg, post_gate, (NB - 1,))
    o_gather(range(28))
    cp_u.wait()
    project(wu, post_up, ())
    o_gather(range(28, 32))
    o_gather(range(32, NU))
    extract(spk, 1)
    pr = (r128 & (-16)) + 2 * (r128 & 7) + ((r128 >> 3) & 1)
    perm = jnp.where(pr == c128, 1.0, 0.0).astype(BF16)

    def patch(q, y):
        a, n = chunks[q]
        z = _rbf(xsel[:8, a:a + n] + _rbf(_rbf(y[:8]) * gate_r[:, :1]))
        g = z * _rbf(_sigmoid(z))
        g = jnp.concatenate([g, jnp.zeros((120, n), F32)], axis=0).astype(BF16)
        gt = lax.dot_general(perm[:n, :n], g, _NT, preferred_element_type=F32)
        us = range(a // 16, (a + n) // 16)
        zz = newz()
        for u in us:
            hr = pl.ds(pl.multiple_of(zz + 8 * u, 8), 8)
            xx, ss = _unpack2(cols[0, hr, :]), _unpack2(cols[1, hr, :])
            r0 = 16 * u - a
            w = _pack2(*[xx[e] + _rbf(ss[e] * gt[r0 + 8 * e:r0 + 8 * e + 8]) for e in range(2)])
            for c, (tn, pn) in enumerate(nat):
                tt = 4 * (tn >> 2) + (tn & 3)
                pltpu.store(og.at[tt, pl.ds(8 * u, 8), :], pltpu.roll(w, (pn - c) & 127, 1), mask=lane8 == pn)
        for c, (tn, pn) in enumerate(nat):
            for u in us:
                v = og[tn, pl.ds(8 * u, 8), :]
                o_store(u, v, pl.ds(pl.multiple_of(tn * 128, 128), 128))
        if q in late:
            send(1, *late[q])

    def down(q, f0, f1):
        a, n = chunks[q]
        return lax.dot_general(_bf(hpk[:, pl.ds(f0, f1 - f0)]), wd[pl.ds(a, n), pl.ds(f0, f1 - f0)], _NT,
                               preferred_element_type=F32)[:8]

    cp_d[0].wait()
    y0 = down(0, 0, 1024)
    send(0, 0, D)
    cp_d[1].wait()
    cp_d[2].wait()
    prev = (0, y0 + down(0, 1024, F))
    for q, fs in ((1, 1280), (2, 1280), (3, 0), (4, 2560)):
        if q == 3:
            cp_d[3].wait()
            cp_d[4].wait()
        y0 = down(q, 0, fs) if fs else None
        patch(*prev)
        y = down(q, fs, F)
        prev = (q, y if y0 is None else y0 + y)
    cp_bar.wait()
    patch(*prev)
    pltpu.make_async_copy(obuf, out_hbm, sem_out).wait()


def _scratch():
    return [
        pltpu.VMEM((D, L), BF16),
        pltpu.VMEM((6, D, N), BF16),
        pltpu.VMEM((D,), BF16),
        pltpu.VMEM((D,), BF16),
        pltpu.VMEM((D,), BF16),
        pltpu.VMEM((D, F), BF16),
        pltpu.VMEM((D, F), BF16),
        pltpu.VMEM((D, F), BF16),
        pltpu.VMEM((4, 64, 256), I32),
        pltpu.VMEM(_PROWS.shape, I32),
        pltpu.VMEM((_NPAT, 8, 128), I32),
        pltpu.VMEM((D, 128), F32),
        pltpu.VMEM((D, 128), F32),
        pltpu.VMEM((5, 2 * D, 128), I32),
        pltpu.VMEM((5, 2 * D, 128), I32),
        pltpu.VMEM((8, 2 * D, 128), I32),
        pltpu.VMEM((8, 2 * D, 128), I32),
        pltpu.VMEM((2, 4 * D, 128), F32),
        pltpu.VMEM((8, 4, D, 128), F32),
        pltpu.VMEM((16, D // 2, 128), I32),
        pltpu.VMEM((16, D // 2, 128), I32),
        pltpu.VMEM((8, 4, D, 128), F32),
        pltpu.VMEM((8, 2, D // 8, 8, 128), I32),
        pltpu.VMEM((8, 2, 2 * D, 128), F32),
        pltpu.VMEM((16, D // 2, 128), I32),
        pltpu.VMEM((3, 8, 128), F32),
        pltpu.VMEM((8, 128), I32),
        pltpu.VMEM((8, D), I32),
        pltpu.VMEM((8, 128), F32),
        pltpu.VMEM((C, 8, 128), I32),
        pltpu.VMEM((C, 8, D), F32),
        pltpu.VMEM((8, F), F32),
        pltpu.VMEM((8, F), I32),
        pltpu.VMEM((2, D // 2, 128), I32),
        pltpu.VMEM((16, D // 2, 128), I32),
        pltpu.VMEM((16, D // 2, 128), I32),
        pltpu.VMEM((D, L), BF16),
        pltpu.SemaphoreType.DMA((10,)),
        pltpu.SemaphoreType.DMA,
        pltpu.SemaphoreType.DMA,
    ] + [pltpu.VMEM((4, D // 2, 128), I32)] * 4 + [pltpu.VMEM((4, 24, 128), F32)] * 4


@jax.jit
def pallas_recurrent_scan__ssm_conv_s4__moe_arch_mod__prompt_kernel(
    A_u: jax.Array,
    A_A_re: jax.Array,
    A_A_im: jax.Array,
    A_B_re: jax.Array,
    A_B_im: jax.Array,
    A_C_re: jax.Array,
    A_C_im: jax.Array,
    A_log_dt: jax.Array,
    A_Dskip: jax.Array,
    B_x: jax.Array,
    B_w_r: jax.Array,
    B_w_gate: jax.Array,
    B_w_up: jax.Array,
    B_w_down: jax.Array,
):
    hbm = pl.BlockSpec(memory_space=pltpu.HBM)
    out = pl.pallas_call(
        _kernel,
        out_shape=jax.ShapeDtypeStruct((D, L), BF16),
        in_specs=[hbm] * 14,
        out_specs=hbm,
        scratch_shapes=_scratch(),
        compiler_params=pltpu.CompilerParams(vmem_limit_bytes=110 * 1024 * 1024),
        name="s4_mod",
    )(A_u[0].T, A_A_re, A_A_im, A_B_re, A_B_im, A_C_re, A_C_im, A_log_dt, A_Dskip, B_w_r,
      B_w_gate, B_w_up, B_w_down.T, jnp.asarray(_PROWS))
    return out.T[None]
```

```python
import numpy as np
import jax
import jax.numpy as jnp
from jax import lax
import jax.experimental.pallas as pl
import jax.experimental.pallas.tpu as pltpu

L, D, N, F, C = 2048, 576, 128, 4608, 8
NU = D // 16
CB = 64
NB = D // CB
LAST = 24
FG0 = 3
UA = 4
F32, BF16, I32 = jnp.float32, jnp.bfloat16, jnp.int32
EPS = 1e-5


def _bf16_round_np(x):
    u = np.asarray(x, np.float32).view(np.uint32).astype(np.uint64)
    r = ((u + 0x7FFF + ((u >> 16) & 1)) >> 16) << 16
    return r.astype(np.uint32)


_LROUND = _bf16_round_np(np.arange(L)).view(np.float32).astype(np.int64)
_HI = [(1, 3, 516, 1032), (5, 7, 520, 1288), (4, 260, 772, 1544), (8, 264, 776, 1800), (2, 6, 258, 262)]


def _comp_q():
    t = np.arange(8)[:, None]
    lane = np.arange(128)[None, :]
    return ((lane - 8 - 7 * (t % 4)) % 16) // 4


def _make_tables():
    lane = np.arange(128)
    lo = 8 * (4 * (lane // 16) + lane % 4)
    tab = [dict(), dict()]
    amask = np.zeros(128, bool)
    for q in range(5):
        for e in range(4):
            for par in range(2):
                t = 4 * par + e
                for h in range(2):
                    src = lane[(lane // 4) % 4 == 2 * h + par]
                    dst = (src + (4 * (q % 4) - 8 * h + 8) + 7 * t) % 128
                    assert np.all(_comp_q()[t, dst] == q % 4)
                    sid = e if q < 4 else 4 + e // 2
                    for sl, dl_ in zip(src, dst):
                        ent = (sid, int(dl_))
                        assert tab[par].setdefault(_HI[q][e] + int(lo[sl]), ent) == ent
                    if q == 4 and e % 2 == 1:
                        amask[dst % 16 + 16 * np.arange(8)[:, None]] = True
    pats = []
    for j in range(4):
        pats.append(np.tile(4 * (lane % 32) + ((lane // 32) ^ j), (8, 1)))
    for j in range(4):
        pats.append(np.tile(32 * ((lane % 4) ^ j) + lane // 4, (8, 1)))
    npat0 = len(pats)
    tiles, tile_of = [], {}
    for dl in range(4):
        for l2 in range(4):
            v = _LROUND[512 * dl + 4 * lane + l2]
            key = tuple(v.tolist())
            if key in tile_of:
                tile_of[dl, l2] = tile_of[key]
                continue
            sid = np.array([tab[0][x][0] if x else -1 for x in v])
            ln = np.array([[tab[s8 % 2][x][1] if x else 0 for x in v] for s8 in range(8)])
            steps = []
            for s in sorted(set(sid.tolist()), key=lambda s: -(sid == s).sum()):
                lanes = np.nonzero(sid == s)[0]
                if s < 0:
                    steps.append((-1, None, lanes))
                    continue
                care = sid == s
                kk = None
                for k in range(npat0, len(pats)):
                    oldp, oldc, olds = pats[k]
                    both = care & oldc
                    if olds == s and np.array_equal(oldp[:, both], ln[:, both]):
                        pats[k] = (np.where(care, ln, oldp), care | oldc, s)
                        kk = k
                        break
                if kk is None:
                    pats.append((np.where(care, ln, 0), care, s))
                    kk = len(pats) - 1
                steps.append((s, kk, lanes))
            tiles.append(steps)
            tile_of[key] = tile_of[dl, l2] = len(tiles) - 1
    pats = np.stack([p if k < npat0 else p[0] for k, p in enumerate(pats)]).astype(np.int32)
    tile_of = {k: v for k, v in tile_of.items() if len(k) == 2}
    rows = np.concatenate([pats[:, :2].reshape(-1, 128), amask[None].astype(np.int32)])
    rows = np.concatenate([rows, np.zeros((64 - len(rows), 128), np.int32)]).reshape(16, 4, 128)
    rows = sum(rows[:, k] << (8 * k) for k in range(4)).astype(np.int32)
    return tiles, tile_of, len(pats), rows


_TILES, _TILE_OF, _NGAT, _PROWS = _make_tables()
_NPAT = _NGAT + 3


def _cmul(ar, ai, br, bi):
    return ar * br - ai * bi, ar * bi + ai * br


def _sincos(b):
    magic = jnp.float32(12582912.0)
    t = b * jnp.float32(2.0 / np.pi) + magic
    k = t - magic
    ki = pltpu.bitcast(t, I32)
    r = b - k * jnp.float32(1.5703125)
    r = r - k * jnp.float32(0.0004837512969970703)
    r = r - k * jnp.float32(7.549790126404332e-08)
    u = r * r
    ps = (jnp.float32(-0.0001958295761141926) * u + jnp.float32(0.008332725614309311)) * u \
        + jnp.float32(-0.166666641831398)
    sn = r + (r * u) * ps
    pc = ((jnp.float32(2.437065268168226e-05) * u + jnp.float32(-0.0013886778615415096)) * u
          + jnp.float32(0.04166663438081741)) * u + jnp.float32(-0.5)
    cs = pc * u + jnp.float32(1.0)
    odd = (ki & 1) == 1
    s1 = jnp.where(odd, cs, sn)
    c1 = jnp.where(odd, sn, cs)
    sign = jnp.int32(-2147483648)
    s1 = pltpu.bitcast(pltpu.bitcast(s1, I32) ^ ((ki << 30) & sign), F32)
    c1 = pltpu.bitcast(pltpu.bitcast(c1, I32) ^ (((ki + 1) << 30) & sign), F32)
    return s1, c1


def _gather(x, idx):
    return jnp.take_along_axis(x, idx, axis=1, mode="promise_in_bounds")


def _lanes_mask(lanes):
    lane = lax.broadcasted_iota(I32, (8, 128), 1)
    lanes = sorted(int(x) for x in lanes)
    runs, start, prev = [], lanes[0], lanes[0]
    for x in lanes[1:]:
        if x != prev + 1:
            runs.append((start, prev))
            start = x
        prev = x
    runs.append((start, prev))
    m = None
    for a, b in runs:
        t = (lane == a) if a == b else jnp.logical_and(lane >= a, lane <= b)
        m = t if m is None else jnp.logical_or(m, t)
    return m


def _butterfly(p):
    lane = lax.broadcasted_iota(I32, p[0].shape, 1)
    b0 = (lane & 32) != 0
    b1 = (lane & 64) != 0
    t = [jnp.where(b0, p[k ^ 1], p[k]) for k in range(4)]
    return [jnp.where(b1, t[k ^ 2], t[k]) for k in range(4)]


def _fft4(x, sgn):
    (ar, ai), (br, bi), (cr, ci), (dr, di) = x
    s0r, s0i, d0r, d0i = ar + cr, ai + ci, ar - cr, ai - ci
    s1r, s1i, d1r, d1i = br + dr, bi + di, br - dr, bi - di
    y0 = (s0r + s1r, s0i + s1i)
    y2 = (s0r - s1r, s0i - s1i)
    p = (d0r - d1i, d0i + d1r)
    m = (d0r + d1i, d0i - d1r)
    return [y0, p, y2, m] if sgn > 0 else [y0, m, y2, p]


def _silu(z):
    h = z * jnp.float32(0.5)
    return h + h * jnp.tanh(h)


def _sigmoid(z):
    return jnp.tanh(z * jnp.float32(0.5)) * jnp.float32(0.5) + jnp.float32(0.5)


def _rbf(x):
    return x.astype(BF16).astype(F32)


def _pack2(a, b):
    p = pltpu.pack_elementwise([a, b], packed_dtype=BF16)
    return p if p.dtype == I32 else pltpu.bitcast(p, I32)


def _unpack2(x):
    return [pltpu.bitcast(x << 16, F32), pltpu.bitcast(x & jnp.int32(-65536), F32)]


def _bf(x):
    return pltpu.bitcast(x, BF16)


_NT = (((1,), (1,)), ((), ()))


class _Idx:
    def __init__(self, i, lag, z=None):
        self.i, self.lag, self.z = i, lag, z

    def off(self, stride, const=0, align=None):
        c = const - self.lag * stride
        if isinstance(self.i, int):
            if self.z is None:
                return self.i * stride + c
            v = self.z + (self.i * stride + c)
        else:
            v = self.i * stride + c
        return pl.multiple_of(v, align) if align else v

    def idx(self):
        return self.i - self.lag


def _pipeline(stages, n, newz, weave=None, reset=None):
    ns = len(stages)

    def step(i, lo, hi):
        z = newz() if isinstance(i, int) else None
        gens = {k: stages[k](_Idx(i, k, z)) for k in range(lo, hi)}
        if reset is not None:
            reset()
        if callable(weave):
            weave(gens)
        else:
            for k in weave or ():
                if k in gens:
                    next(gens[k], None)
        for k in range(hi - 1, lo - 1, -1):
            for _ in gens[k]:
                pass

    def body(i, carry):
        step(i, 0, ns)
        return carry

    return ([lambda i=i: step(i, 0, i + 1) for i in range(ns - 1)],
            lambda: lax.fori_loop(ns - 1, n, body, 0),
            [lambda i=i: step(n + i, i + 1, ns) for i in range(ns - 1)])


def _kernel(x_hbm, are_hbm, aim_hbm, bre_hbm, bim_hbm, cre_hbm, cim_hbm, ldt_hbm, dsk_hbm, wr_hbm,
            wg_hbm, wu_hbm, wd_hbm, pat_hbm,
            out_hbm,
            xbuf, par, ldt, dsk, wr, wg, wu, wd, fpk, prow, pats,
            dtcol, skip, hi_re, hi_im, lo_re, lo_im, comp, khat,
            xp, xnp, uhat, yhat, ybuf, spk, topk, posv, dummy, wr16b, wsum, ohb, xsel_ref, hbuf, hpk, cols, opk, og, obuf,
            sem_in, *perb):
    xg, stat = perb[0:4], perb[4:8]
    sem_out = sem_in.at[1]
    p_hbm = (are_hbm, aim_hbm, bre_hbm, bim_hbm, cre_hbm, cim_hbm)
    r1 = 16 * UA
    small = [(ldt_hbm, ldt), (pat_hbm, prow)]
    for a, n in ((0, r1), (r1, r1), (2 * r1, D - 2 * r1)):
        small += [(h.at[pl.ds(a, n)], par.at[i, pl.ds(a, n)]) for i, h in enumerate(p_hbm)]
    small += [(wr_hbm, wr), (dsk_hbm, dsk)]
    cps = [pltpu.make_async_copy(s, d, sem_in.at[min((i + 4) // 6, 3)]) for i, (s, d) in enumerate(small)]
    ns = 4
    cp_x = pltpu.make_async_copy(x_hbm, xbuf, sem_in.at[ns])
    cp_g = pltpu.make_async_copy(wg_hbm, wg, sem_in.at[ns + 1])
    cp_u = pltpu.make_async_copy(wu_hbm, wu, sem_in.at[ns + 2])
    chunks = [(0, 128), (128, 128), (256, 128), (384, 128), (512, 64)]
    cp_d = [pltpu.make_async_copy(wd_hbm.at[pl.ds(a, n)], wd.at[pl.ds(a, n)], sem_in.at[ns + 3 + q - (q > 1)])
            for q, (a, n) in enumerate(chunks[:4] + [(512, 64 - LAST), (D - LAST, LAST)])]
    cp_bar = [pltpu.make_async_copy(pat_hbm.at[pl.ds(0, 8)], dummy.at[k], sem_in.at[(0, 2, 3)[k]]) for k in range(3)]
    for cp in cps + [cp_x, cp_g, cp_u] + cp_d:
        cp.start()

    sub8 = lax.broadcasted_iota(I32, (8, 128), 0)
    lane8 = lax.broadcasted_iota(I32, (8, 128), 1)

    def dft_rows(l2):
        for g in range(8):
            cs = []
            for e in range(2):
                p = 16 * g + 2 * sub8 + e
                t = 4 * (32 * ((p >> 5) ^ l2) + (p & 31)) + l2
                n = ((4 * lane8 + 1) * t) & 2047
                cs.append(_sincos(n.astype(F32) * jnp.float32(-2.0 * np.pi / 2048)))
            fpk[l2, pl.ds(8 * g, 8), pl.ds(0, 128)] = _pack2(cs[0][1], cs[1][1])
            fpk[l2, pl.ds(8 * g, 8), pl.ds(128, 128)] = _pack2(cs[0][0], cs[1][0])

    for l2 in range(FG0):
        dft_rows(l2)

    for cp in cps[:2]:
        cp.wait()
    for l2 in range(FG0, 4):
        dft_rows(l2)
    for k in range(_NGAT):
        w = jnp.broadcast_to(prow[pl.ds(k // 2, 1), :], (8, 128))
        pats[k] = (w >> (16 * (k % 2) + 8 * (sub8 & 1))) & 127
    cq = ((lane8 - 8 - 7 * (sub8 & 3)) & 15) >> 2
    pats[_NGAT] = cq & 1
    pats[_NGAT + 1] = cq >> 1
    pats[_NGAT + 2] = (jnp.broadcast_to(prow[pl.ds(_NGAT // 2, 1), :], (8, 128)) >> (16 * (_NGAT % 2))) & 127
    r128 = lax.broadcasted_iota(I32, (128, 128), 0)
    c128 = lax.broadcasted_iota(I32, (128, 128), 1)

    def column(row):
        pk = pltpu.bitcast(jnp.broadcast_to(row, (8, D)), I32)
        lhs = []
        for u in range(NU):
            t = u // 8
            v = pk[:, 128 * t:128 * t + 128] if t < 4 else jnp.concatenate([pk[:, 512:], pk[:, 512:]], axis=1)
            c0 = 16 * (u % 8) + 2 * sub8
            lhs.append(jnp.where(lane8 == c0, lax.shift_right_logical(v, 16), jnp.where(lane8 == c0 + 1, v, 0)))
        ones = jnp.ones((128, 128), BF16)
        return jnp.concatenate([jnp.dot(_bf(jnp.concatenate(lhs[k:k + NU // 4], axis=0)), ones,
                                        preferred_element_type=F32) for k in range(0, NU, NU // 4)], axis=0)

    dtcol[...] = column(_rbf(jnp.exp(ldt[...].astype(F32).reshape(1, D))))

    zero = pl.program_id(0)
    zcount = [0]

    def newz():
        zcount[0] += 1
        return zero * (64 * zcount[0])

    def block(*fns):
        def body(k, carry):
            for fn in fns:
                fn()
            return carry

        lax.fori_loop(0, zero + 1, body, 0)

    def step_zero(i):
        t = i.off(1) * zero if not isinstance(i.i, int) or i.z is None else i.z
        return pl.multiple_of(t * 8, 8)

    def after(x, deps):
        never = pats[0] < 0
        d = None
        for v in deps:
            v = v if v.dtype == I32 else pltpu.bitcast(v, I32)
            d = v if d is None else d ^ v
        return jnp.where(never, d if x.dtype == I32 else pltpu.bitcast(d, x.dtype), x)

    def pad_tail(y, i):
        n, k = 16, y.shape[0] - 64
        base = i.off(1)
        mid = after(y[k:k + 8], [pats[j % _NPAT] * (base + j) for j in range(n)])
        return jnp.concatenate([y[:k], mid, y[k + 8:]], axis=0)

    class Sched:
        tok, g, pre = {}, 0, []

        @classmethod
        def reset(cls):
            cls.tok, cls.g, cls.pre = {}, 0, []

        @classmethod
        def gate(cls, x):
            deps = cls.tok.pop(cls.g, [])
            cls.g += 1
            if not deps:
                return x
            return jnp.concatenate([after(x[:8], deps), after(x[8:], deps[-1:])], axis=0)

    slot = {h: (q, e) for q, ent in enumerate(_HI) for e, h in enumerate(ent)}

    def a_prep(i):
        gate = Sched.gate
        for u in range(UA):
            rows = pl.ds(i.off(16 * UA, 16 * u, 16), 16)
            ev = pl.ds(i.off(32 * UA, 32 * u), 16, stride=2)
            od = pl.ds(i.off(32 * UA, 32 * u + 1), 16, stride=2)
            dt = gate(dtcol[rows, :])
            al = dt * par[0, rows, :].astype(F32)
            be = dt * par[1, rows, :].astype(F32)
            cr, ci = _cmul(par[4, rows, :].astype(F32), par[5, rows, :].astype(F32),
                           par[2, rows, :].astype(F32), par[3, rows, :].astype(F32))
            dts = dt * jnp.float32(1.0 / 512)
            cr, ci = cr * dts, ci * dts
            k0 = jnp.sum(cr, axis=1, keepdims=True) * jnp.float32(512.0)
            skip[rows, :] = jnp.broadcast_to(k0, (16, 128))
            yield cr
            s, c = _sincos(gate(be))
            yield c
            pw = {1: (c, s)}
            e = 1
            while e < 256:
                if e in (1, 16):
                    c = gate(c)
                c, s = (c - s) * (c + s), (c + c) * s
                e *= 2
                pw[e] = (c, s)
                if e in (16, 256):
                    yield c
            z = {}
            for e in (1, 8, 256):
                mag = jnp.exp(al * jnp.float32(e))
                c, s = pw[e]
                z[e] = (mag * c, mag * s)
            pend = {}

            def put(tab, q, ee, v):
                key = (tab[0] is hi_re, q, ee // 2)
                if key not in pend:
                    pend[key] = (ee % 2, v)
                    return
                w, o = pend.pop(key)
                lo_, hi_ = (o, v) if w == 0 else (v, o)
                dst = od if ee // 2 else ev
                tab[0][q, dst, :] = _pack2(lo_[0], hi_[0])
                tab[1][q, dst, :] = _pack2(lo_[1], hi_[1])

            h = (cr, ci)
            cnt = 0
            for e in range(1, 9):
                g, ee, m = h, e, z[1]
                while ee in slot:
                    if cnt % 4 == 0:
                        g = (gate(g[0]), g[1])
                    g = _cmul(*g, *m)
                    put((hi_re, hi_im), *slot[ee], g)
                    if ee == e:
                        h = g
                    ee, m = ee + 256, z[256]
                    cnt += 1
                    if cnt % 4 == 0:
                        yield g[0]
            w1 = (gate(z[8][0]), -z[8][1])
            v = [(jnp.ones((16, 128), F32), jnp.zeros((16, 128), F32)), w1]
            v.append(_cmul(*w1, *w1))
            v.append(_cmul(*v[2], *w1))
            w4 = _cmul(*v[2], *v[2])
            for j in range(8):
                for f in range(4):
                    put((lo_re, lo_im), j, f, v[f])
                yield v[3][0]
                if j < 7:
                    w4 = (gate(w4[0]), w4[1])
                    v = [w4 if (j == 0 and f == 0) else _cmul(*v[f], *w4) for f in range(4)]

    def a_gen(i):
        b0 = pats[_NPAT - 3] != 0
        b1 = pats[_NPAT - 2] != 0
        for k in range(4 * UA):
            rows = pl.ds(i.off(32 * UA, 8 * k, 8), 8)
            lo = jnp.concatenate([lo_re[:, rows, :].reshape(64, 128), lo_im[:, rows, :].reshape(64, 128)], axis=1)
            h0 = hi_re[0, rows, :]
            if k % 2 == 0 and Sched.pre:
                h0 = after(h0, Sched.pre)
                Sched.pre = []
            hi = jnp.concatenate([jnp.concatenate([h0, hi_re[1:5, rows, :].reshape(32, 128)], axis=0),
                                  hi_im[:, rows, :].reshape(40, 128)], axis=1)
            o = lax.dot_general(_bf(hi), _bf(lo), _NT, preferred_element_type=F32)
            for q in range(5):
                Sched.tok.setdefault(13 + int(0.9 * (5 * (k // 2) + q)), []).append(o[16 * q + 8:16 * q + 16])
            for h in range(2):
                g = [pltpu.roll(o[16 * q + 8 * h:16 * q + 8 * h + 8], 4 * (q % 4) - 8 * h + 8, 1,
                                stride=7, stride_axis=0) for q in range(5)]
                dst = pl.ds(i.off(64 * UA, 16 * k + 8 * h, 8), 8)
                comp[0, dst, :] = jnp.where(b1, jnp.where(b0, g[3], g[2]), jnp.where(b0, g[1], g[0]))
                comp[1, dst, :] = g[4]
            if k % 2 == 1:
                yield

    def a_exp(i):
        bm = pats[_NPAT - 1] != 0
        srcs = []
        for u in range(UA):
            def ld(a, e):
                return _pack2(comp[a, pl.ds(i.off(64 * UA, 64 * u + e), 8, stride=4), :],
                              comp[a, pl.ds(i.off(64 * UA, 64 * u + 32 + e), 8, stride=4), :])

            srcs.append([ld(0, e) for e in range(4)]
                        + [jnp.where(bm, ld(1, 2 * k + 1), ld(1, 2 * k)) for k in range(2)])
        cache = {}

        def gat(s, key):
            if key not in cache:
                pat = pats[key]
                cache[key] = [_gather(srcs[u][s], pat) for u in range(UA)]
            return cache[key]

        tiles = []
        for steps in _TILES:
            t = None
            for s, key, lanes in steps:
                v = [jnp.zeros((8, 128), I32)] * UA if s < 0 else gat(s, key)
                t = v if t is None else [jnp.where(_lanes_mask(lanes), v[u], t[u]) for u in range(UA)]
            tiles.append(t)
        yield
        for u0 in range(0, UA, 2):
            lhs = [_bf(jnp.concatenate([tiles[_TILE_OF[dl, l2]][u] for dl in range(4) for u in (u0, u0 + 1)], axis=0))
                   for l2 in range(4)]
            z0 = 0 if u0 == 0 else zero * 8

            def dots(ri):
                return [jnp.dot(lhs[l2], _bf(jnp.concatenate(
                    [fpk[l2, pl.ds(z0 + 16 * (j ^ l2), 16) if u0 == 0 else
                         pl.ds(pl.multiple_of(z0 + 16 * (j ^ l2), 8), 16), pl.ds(128 * ri, 128)]
                     for j in range(4)], axis=0)), preferred_element_type=F32) for l2 in range(4)]

            def store(k2, ri, v):
                khat[2 * k2 + ri, :, pl.ds(i.off(16 * UA, 16 * u0, 16), 32), :] = v.reshape(4, 32, 128)

            def toks(v, step0):
                for j in range(8):
                    g = 13 + 9 * UA + int(0.7 * (step0 + j))
                    Sched.tok.setdefault(g, []).append(v[16 * j + 8:16 * j + 16])

            re = dots(0)
            s0, d0r, s1, d1r = re[0] + re[2], re[0] - re[2], re[1] + re[3], re[1] - re[3]
            store(0, 0, s0 + s1)
            v = s0 - s1
            store(2, 0, v)
            toks(v, 8 * u0)
            im = dots(1)
            s0, d0i, s1, d1i = im[0] + im[2], im[0] - im[2], im[1] + im[3], im[1] - im[3]
            store(0, 1, s0 + s1)
            store(2, 1, s0 - s1)
            store(1, 0, d0r + d1i)
            store(1, 1, d0i - d1r)
            store(3, 0, d0r - d1i)
            v = d0i + d1r
            store(3, 1, v)
            toks(v, 8 * u0 + 8)
            yield

    def a_weave(gens):
        if 2 in gens:
            next(gens[2])
        if 0 in gens and 1 in gens:
            for n in (3, 5, 4):
                for _ in range(n):
                    v = next(gens[0])
                Sched.pre = [v[:8], v[8:]]
                next(gens[1])
        for k in (1, 2, 0):
            if k in gens:
                for _ in gens[k]:
                    pass

    a_pro, a_loop, a_tail = _pipeline([a_prep, a_gen, a_exp], NU // UA, newz, reset=Sched.reset, weave=a_weave)
    for cp in cps[2:8]:
        cp.wait()
    a_pro[0]()
    for cp in cps[8:14]:
        cp.wait()
    a_pro[1]()
    for cp in cps[14:]:
        cp.wait()
    a_loop()

    cp_x.wait()

    def zrow(u):
        return pl.ds(pl.multiple_of(zero * 8 + 8 * u, 8), 8)

    def b_gather(b):
        for j in range(4):
            pat = pats[j]
            for u in range(NU):
                v = pltpu.bitcast(xbuf[pl.ds(16 * u, 16), pl.ds(512 * b + 128 * j, 128)], I32)
                v = _gather(v, pat)
                xg[b][j, pl.ds(8 * u, 8), :] = v
                gtok.setdefault(b, []).append(v)

    gtok = {}

    def b_stat(b, ride=None):
        s2 = [jnp.zeros((8, 128), F32) for _ in range(4)]
        for u in range(NU):
            x = [xg[b][j, zrow(u), :] for j in range(4)]
            if ride is not None:
                x = [after(x[0], [gtok[ride][4 * u]]), x[1], after(x[2], [gtok[ride][4 * u]]), x[3]]
            o = _butterfly(x)
            for l2 in range(4):
                xp[4 * l2 + b, pl.ds(8 * u, 8), :] = o[l2]
                e_, o_ = _unpack2(o[l2])
                s2[l2] = s2[l2] + (e_ * e_ + o_ * o_)
        for l2 in range(4):
            stat[b][l2, pl.ds(16, 8), :] = s2[l2]

    def b_dot(b):
        lhs = _bf(wr16b[...])
        for j in range(4):
            rows = pl.ds(pl.multiple_of(zero * zero * 8, 8), D // 2)
            stat[b][j, pl.ds(0, 16), :] = jnp.dot(lhs, _bf(xg[b][j, rows, :]), preferred_element_type=F32)

    def b_fin(b0):
        wx = sx = q = None
        for b in (b0, b0 + 1):
            wxs = _butterfly([stat[b][j, zrow(0), :] for j in range(4)])
            sxs = _butterfly([stat[b][j, zrow(1), :] for j in range(4)])
            for l2 in range(4):
                qq = jnp.sum(stat[b][l2, zrow(2), :], axis=0, keepdims=True)
                here = sub8 == 4 * (b - b0) + l2
                wx = wxs[l2] if wx is None else jnp.where(here, wxs[l2], wx)
                sx = sxs[l2] if sx is None else jnp.where(here, sxs[l2], sx)
                q = jnp.broadcast_to(qq, (8, 128)) if q is None else jnp.where(here, qq, q)
        m = sx * jnp.float32(1.0 / D)
        var = _rbf(jnp.maximum(q * jnp.float32(1.0 / D) - m * m, 0.0))
        rs = 1.0 / _rbf(jnp.sqrt(_rbf(var + jnp.float32(EPS))))
        mb = _rbf(m)
        r = _rbf((wx - mb * wsum[...]) * rs)
        r = jnp.where(r == 0.0, 0.0, r)
        bits = pltpu.bitcast(r, I32)
        mono = ((bits ^ ((bits >> 31) & jnp.int32(0x7FFFFFFF))) >> 16) + 32768
        l2v = sub8 & 3
        tok = 512 * (b0 + (sub8 >> 2)) + 4 * (32 * ((lane8 >> 5) ^ l2v) + (lane8 & 31)) + l2v
        topk[b0 // 2] = pltpu.bitcast((mono << 11) + (2047 - tok) + jnp.int32(0x00800000), F32)
        return mb, rs

    def b_scale(b0, st, us):
        for k in range(8):
            t = 4 * (k % 4) + b0 + k // 4
            mk, rk = [jnp.broadcast_to(v[k:k + 1], (8, 128)) for v in st]
            for u in us:
                e_, o_ = _unpack2(xp[t, zrow(u), :])
                xnp[t, pl.ds(8 * u, 8), :] = _pack2((e_ - mk) * rk, (o_ - mk) * rk)

    def b_norm(b0):
        st = b_fin(b0)
        for us in (range(CB // 16), range(CB // 16, NU)):
            b_scale(b0, st, us)

    def b_init():
        wrow = wr[...].reshape(1, D)
        wr16b[...] = pltpu.bitcast(
            jnp.concatenate([jnp.broadcast_to(wrow, (8, D)), jnp.ones((8, D), BF16)], axis=0), I32)
        wsum[...] = jnp.broadcast_to(jnp.sum(wrow.astype(F32), axis=1, keepdims=True), (8, 128))
        topk[2] = jnp.zeros((8, 128), F32)
        cols[...] = jnp.zeros(cols.shape, I32)

    elt_dep, toks = [], []

    def c_fwd(i):
        h0 = i.off(CB // 2, 0, 8)
        r0 = i.off(CB, 0, 8)
        for l2 in range(4):
            lhs = _bf(xnp[pl.ds(4 * l2, 4), pl.ds(h0, CB // 2), :].reshape(2 * CB, 128))
            res = jnp.dot(lhs, _bf(fpk[l2, pl.ds(step_zero(i), 64), :]), preferred_element_type=F32)
            for ri in range(2):
                y = res[:, 128 * ri:128 * ri + 128]
                if l2 == 3 and ri == 1 and isinstance(i.i, int) and i.i < 2:
                    y = pad_tail(y, i)
                uhat[2 * l2 + ri, :, pl.ds(r0, CB), :] = y.reshape(4, CB, 128)
            yield

    def c_mid(i, units=range(CB // 8)):
        for k in units:
            rows = pl.ds(i.off(CB, 8 * k, 8), 8)
            krows = pl.ds(i.off(CB, 16 * (k // 2) + k % 2), 8, stride=2)
            x = [[(uhat[2 * l2, b, rows, :], uhat[2 * l2 + 1, b, rows, :]) for l2 in range(4)] for b in range(4)]
            if elt_dep:
                for b in range(4):
                    x[b][0] = (after(x[b][0][0], elt_dep), x[b][0][1])
            uu = [_fft4(x[b], -1) for b in range(4)]
            yy = [[None] * 4 for _ in range(4)]
            for k2s in ((0, 2), (1, 3)):
                pps = {k2: [None] * 4 for k2 in k2s}
                for k2, pp in pps.items():
                    for dl in range(3, -1, -1):
                        kk = (khat[2 * k2, dl, krows, :], khat[2 * k2 + 1, dl, krows, :])
                        for m in range(3, dl - 1, -1):
                            t = _cmul(*uu[m - dl][k2], *kk)
                            pp[m] = t if pp[m] is None else (pp[m][0] + t[0], pp[m][1] + t[1])
                for k2, pp in pps.items():
                    for m in range(3, -1, -1):
                        yy[m][k2] = pp[0] if m == 0 else (pp[m][0] - pp[m - 1][1], pp[m][1] + pp[m - 1][0])
            un = i.off(CB // 8, k)
            for bp in range(2):
                ww = [_fft4(yy[m], 1) for m in (2 * bp, 2 * bp + 1)]
                for l2 in range(4):
                    for ri in range(2):
                        yhat[2 * l2 + ri, bp, un] = _pack2(ww[0][l2][ri], ww[1][l2][ri])
            yield

    def c_inv(i, l2s=range(4)):
        u0 = i.off(CB // 8)
        r0 = i.off(2 * CB, 0, 8)
        for l2 in l2s:
            for ri in range(2):
                lhs = _bf(yhat[2 * l2 + ri, :, pl.ds(u0, CB // 8)].reshape(2 * CB, 128))
                y = lax.dot_general(lhs, _bf(fpk[l2, pl.ds(step_zero(i), 64), pl.ds(128 * ri, 128)]), _NT,
                                    preferred_element_type=F32)
                if l2 == 3 and ri == 1 and isinstance(i.i, int):
                    y = pad_tail(y, i)
                ybuf[2 * l2 + ri, :, pl.ds(r0, 2 * CB), :] = y.reshape(2, 2 * CB, 128)
                toks.extend(y[32 * j:32 * j + 8] for j in range(CB // 8))
            yield

    def c_elt(i):
        for k in range(CB // 16):
            hr = pl.ds(i.off(CB // 2, 8 * k, 8), 8)
            sk = [skip[pl.ds(i.off(CB, 16 * k + e), 8, stride=2), :] for e in range(2)]
            for b in range(4):
                o = []
                for l2 in range(4):
                    w = xnp[4 * l2 + b, hr, :]
                    if elt_dep:
                        w = after(w, elt_dep)
                    xn = _unpack2(w)
                    xx = _unpack2(xp[4 * l2 + b, hr, :])
                    ss, v = [], []
                    for e in range(2):
                        yr = pl.ds(i.off(2 * CB, 32 * k + 2 * e + b % 2), 8, stride=4)
                        ss.append(ybuf[2 * l2, b // 2, yr, :] + ybuf[2 * l2 + 1, b // 2, yr, :] + xn[e] * sk[e])
                        v.append(xx[e] + ss[e] * _silu(xn[e]))
                    spk[4 * l2 + b, hr, :] = _pack2(*ss)
                    o.append(_pack2(*v))
                p = _butterfly(o)
                for j in range(4):
                    opk[4 * b + j, hr, :] = p[j]
                yield

    def c_top(i):
        k0, k1 = topk[i.off(0, 0)], topk[i.off(0, 1)]
        mx = jnp.max(jnp.max(jnp.maximum(k0, k1), axis=0, keepdims=True), axis=1, keepdims=True)
        topk[i.off(0, 0)] = jnp.where(k0 == mx, 0.0, k0)
        topk[i.off(0, 1)] = jnp.where(k1 == mx, 0.0, k1)
        topk[i.off(0, 2)] = jnp.where(sub8 == i.idx(), mx, topk[i.off(0, 2)])
        yield

    def c_first(i):
        yield from c_fwd(i)
        yield from c_top(i)

    c_pro, c_loop, _ = _pipeline([c_first, c_mid, c_inv, c_elt], NB, newz,
                                 weave=[1] * (CB // 8) + [3] * (CB // 4) + [0, 0, 2, 2, 0, 0, 2, 2])

    def first_fwd():
        for _ in c_first(_Idx(0, 0)):
            pass

    def each(fn, *bs):
        return [lambda b=b: fn(b) for b in bs]

    def add_dskip():
        skip[...] = skip[...] + column(dsk[...].astype(F32).reshape(1, D))

    b_init()
    a_tail[0]()
    b_gather(0)
    b_gather(1)
    b_stat(0, 1)
    block(add_dskip, a_tail[1], *each(b_gather, 2, 3), *each(b_dot, 0, 1),
          lambda: b_stat(1, 2), lambda: b_stat(2, 3))
    block(*each(b_stat, 3), *each(b_norm, 0), *each(b_dot, 2, 3))
    block(*each(b_norm, 2), first_fwd)
    block(c_pro[1])
    block(c_pro[2])
    c_loop()

    sel = pltpu.bitcast(topk[2], I32) - jnp.int32(0x00800000)
    mono = (sel >> 11) - 32768
    r_sel = pltpu.bitcast((mono ^ ((mono >> 31) & jnp.int32(0x7FFF))) << 16, F32)
    gate_r = _rbf(jax.nn.sigmoid(r_sel))
    posv[...] = 2047 - (sel & 2047)
    tok = [posv[c, 0] for c in range(C)]
    nat = [(jnp.clip(t >> 7, 0, 15), t & 127) for t in tok]
    prm = []
    for t in tok:
        l2, l1 = t & 3, (t >> 2) & 127
        prm.append((jnp.clip(4 * l2 + (t >> 9), 0, 15), 32 * ((l1 >> 5) ^ l2) + (l1 & 31)))

    def extract(src, k, us):
        for c, (tp, pp) in enumerate(prm):
            sh = (c - pp) & 127
            for u in us:
                v = pltpu.roll(src[tp, pl.ds(8 * u, 8), :], sh, 1)
                pltpu.store(cols.at[k, pl.ds(8 * u, 8), :], v, mask=lane8 == c)
                toks.append(v)

    for c, (tp, pp) in enumerate(prm):
        ohb[c] = jnp.where(jnp.logical_and(sub8 == c // 2, lane8 == pp), jnp.int32(0x3F80 << (16 * (c % 2))), 0)

    def take_rows():
        for c, (tp, pp) in enumerate(prm):
            xsel_ref[c] = lax.dot_general(_bf(ohb[c]), _bf(xnp[tp]), _NT, preferred_element_type=F32)[:8]

    def o_gather(us):
        for j in range(4):
            pat = pats[4 + j]
            for b in range(4):
                for u in us:
                    v = _gather(opk[4 * b + j, pl.ds(8 * u, 8), :], pat)
                    og[4 * b + j, pl.ds(8 * u, 8), :] = v
                    toks.append(v)
                    o_store(u, v, pl.ds(512 * b + 128 * j, 128))

    def o_store(u, v, col):
        obuf[pl.ds(16 * u, 8), col] = _bf(v[0:4])
        obuf[pl.ds(16 * u + 8, 8), col] = _bf(pltpu.roll(v, 4, 0)[0:4])

    def project(w, post):
        xs = xsel_ref[0]
        for c in range(1, C):
            xs = xs + xsel_ref[c]
        xs = jnp.concatenate([xs, jnp.zeros((8, D), F32)], axis=0).astype(BF16)
        for t in range(F // 128):
            ps = [jnp.dot(xs[:, a:a + n], w[pl.ds(a, n), pl.ds(128 * t, 128)],
                          preferred_element_type=F32)[:8] for a, n in chunks]
            v = _rbf((ps[0] + ps[1]) + (ps[2] + ps[3]) + ps[4])
            toks.append(v)
            post(t, v)

    def post_gate(t, ga):
        hbuf[:, pl.ds(128 * t, 128)] = _rbf(ga * _rbf(_sigmoid(ga)))

    def post_up(t, up):
        h = hbuf[:, pl.ds(128 * t, 128)] * up
        hpk[:, pl.ds(128 * t, 128)] = pltpu.bitcast(
            jnp.concatenate([h, jnp.zeros((8, 128), F32)], axis=0).astype(BF16), I32)

    pr = (r128 & (-16)) + 2 * (r128 & 7) + ((r128 >> 3) & 1)
    perm = jnp.where(pr == c128, 1.0, 0.0).astype(BF16)

    acc = {}
    out_cp = [pltpu.make_async_copy(obuf.at[pl.ds(a, n)], out_hbm.at[pl.ds(a, n)], sem_out) for a, n in chunks]

    def patch(q):
        a, n = chunks[q]
        xs = xsel_ref[0, :, pl.ds(a, n)]
        for c in range(1, C):
            xs = xs + xsel_ref[c, :, pl.ds(a, n)]
        z = _rbf(xs + _rbf(_rbf(acc[q]) * gate_r[:, :1]))
        g = z * _rbf(_sigmoid(z))
        g = jnp.concatenate([g, jnp.zeros((120, n), F32)], axis=0).astype(BF16)
        gt = lax.dot_general(perm[:n, :n], g, _NT, preferred_element_type=F32)
        us = range(a // 16, (a + n) // 16)
        zz = newz()
        for u in us:
            hr = pl.ds(pl.multiple_of(zz + 8 * u, 8), 8)
            xx, ss = _unpack2(cols[0, hr, :]), _unpack2(cols[1, hr, :])
            r0 = 16 * u - a
            w = _pack2(*[xx[e] + _rbf(ss[e] * gt[r0 + 8 * e:r0 + 8 * e + 8]) for e in range(2)])
            for c, (tn, pn) in enumerate(nat):
                pltpu.store(og.at[tn, pl.ds(8 * u, 8), :], pltpu.roll(w, (pn - c) & 127, 1), mask=lane8 == pn)
        for c, (tn, pn) in enumerate(nat):
            for u in us:
                v = og[tn, pl.ds(8 * u, 8), :]
                o_store(u, v, pl.ds(pl.multiple_of(tn * 128, 128), 128))

    def down(q, f0, f1):
        a, n = chunks[q]
        for f in range(f0, f1, 2):
            col = pl.ds(128 * f, 256)
            y = lax.dot_general(_bf(hpk[:, col]), wd[pl.ds(a, n), col], _NT, preferred_element_type=F32)[:8]
            acc[q] = y if q not in acc else acc[q] + y
            if n == 128:
                toks.append(y)

    def inverse(k, l2s):
        for _ in c_inv(_Idx(k, 0), l2s):
            pass

    def ride(gen, n, frac=1.0):
        for j in range(n):
            elt_dep[:] = [toks[int(frac * len(toks)) * j // n]]
            next(gen, None)
        elt_dep.clear()

    def elementwise(k, frac=1.0):
        ride(c_elt(_Idx(k, 0)), CB // 4, frac)

    def products(u0, u1):
        ride(c_mid(_Idx(NB - 1, 0), range(u0, u1)), u1 - u0)

    for cp in cp_bar:
        cp.start()
    take_rows()
    toks.clear()
    extract(xp, 0, range(NU))
    elementwise(NB - 3)
    cp_g.wait()
    project(wg, post_gate)
    o_gather(range(24))
    cp_u.wait()
    project(wu, post_up)
    extract(spk, 1, range(24))
    cp_d[0].wait()
    toks.clear()
    down(0, 0, 36)
    products(0, 4)
    inverse(NB - 2, range(0, 2))
    cp_d[1].wait()
    cp_d[2].wait()
    toks.clear()
    down(1, 0, 10)
    patch(0)
    down(1, 10, 36)
    down(2, 0, 10)
    products(4, 8)
    cp_d[4].wait()
    out_cp[0].start()
    cp_d[3].wait()
    patch(1)
    down(2, 10, 36)
    inverse(NB - 2, range(2, 4))
    cp_d[5].wait()
    out_cp[1].start()
    cp_bar[0].wait()
    toks.clear()
    patch(2)
    out_cp[2].start()
    inverse(NB - 1, range(4))
    down(3, 0, 12)
    elementwise(NB - 2)
    cp_bar[1].wait()
    toks.clear()
    down(3, 12, 36)
    o_gather(range(24, 32))
    extract(spk, 1, range(24, 32))
    down(4, 0, 10)
    patch(3)
    out_cp[3].start()
    down(4, 10, 36)
    elementwise(NB - 1, 0.8)
    cp_bar[2].wait()
    o_gather(range(32, NU))
    extract(spk, 1, range(32, NU))
    patch(4)
    out_cp[4].start()
    for cp in out_cp:
        cp.wait()


def _scratch():
    return [
        pltpu.VMEM((D, L), BF16),
        pltpu.VMEM((6, D, N), BF16),
        pltpu.VMEM((D,), BF16),
        pltpu.VMEM((D,), BF16),
        pltpu.VMEM((D,), BF16),
        pltpu.VMEM((D, F), BF16),
        pltpu.VMEM((D, F), BF16),
        pltpu.VMEM((D, F), BF16),
        pltpu.VMEM((4, 64, 256), I32),
        pltpu.VMEM(_PROWS.shape, I32),
        pltpu.VMEM((_NPAT, 8, 128), I32),
        pltpu.VMEM((D, 128), F32),
        pltpu.VMEM((D, 128), F32),
        pltpu.VMEM((5, 2 * D, 128), I32),
        pltpu.VMEM((5, 2 * D, 128), I32),
        pltpu.VMEM((8, 2 * D, 128), I32),
        pltpu.VMEM((8, 2 * D, 128), I32),
        pltpu.VMEM((2, 4 * D, 128), F32),
        pltpu.VMEM((8, 4, D, 128), F32),
        pltpu.VMEM((16, D // 2, 128), I32),
        pltpu.VMEM((16, D // 2, 128), I32),
        pltpu.VMEM((8, 4, D, 128), F32),
        pltpu.VMEM((8, 2, D // 8, 8, 128), I32),
        pltpu.VMEM((8, 2, 2 * D, 128), F32),
        pltpu.VMEM((16, D // 2, 128), I32),
        pltpu.VMEM((3, 8, 128), F32),
        pltpu.VMEM((8, 128), I32),
        pltpu.VMEM((3, 8, 128), I32),
        pltpu.VMEM((8, D), I32),
        pltpu.VMEM((8, 128), F32),
        pltpu.VMEM((C, 8, 128), I32),
        pltpu.VMEM((C, 8, D), F32),
        pltpu.VMEM((8, F), F32),
        pltpu.VMEM((8, F), I32),
        pltpu.VMEM((2, D // 2, 128), I32),
        pltpu.VMEM((16, D // 2, 128), I32),
        pltpu.VMEM((16, D // 2, 128), I32),
        pltpu.VMEM((D, L), BF16),
        pltpu.SemaphoreType.DMA((12,)),
    ] + [pltpu.VMEM((4, D // 2, 128), I32)] * 4 + [pltpu.VMEM((4, 24, 128), F32)] * 4


@jax.jit
def pallas_recurrent_scan__ssm_conv_s4__moe_arch_mod__prompt_kernel(
    A_u: jax.Array,
    A_A_re: jax.Array,
    A_A_im: jax.Array,
    A_B_re: jax.Array,
    A_B_im: jax.Array,
    A_C_re: jax.Array,
    A_C_im: jax.Array,
    A_log_dt: jax.Array,
    A_Dskip: jax.Array,
    B_x: jax.Array,
    B_w_r: jax.Array,
    B_w_gate: jax.Array,
    B_w_up: jax.Array,
    B_w_down: jax.Array,
):
    hbm = pl.BlockSpec(memory_space=pltpu.HBM)
    out = pl.pallas_call(
        _kernel,
        out_shape=jax.ShapeDtypeStruct((D, L), BF16),
        grid=(1,),
        in_specs=[hbm] * 14,
        out_specs=hbm,
        scratch_shapes=_scratch(),
        compiler_params=pltpu.CompilerParams(vmem_limit_bytes=110 * 1024 * 1024),
        name="s4_mod",
    )(A_u[0].T, A_A_re, A_A_im, A_B_re, A_B_im, A_C_re, A_C_im, A_log_dt, A_Dskip, B_w_r,
      B_w_gate, B_w_up, B_w_down.T, jnp.asarray(_PROWS))
    return out.T[None]
```

```python
import numpy as np
import jax
import jax.numpy as jnp
from jax import lax
import jax.experimental.pallas as pl
import jax.experimental.pallas.tpu as pltpu

L, D, N, F, C = 2048, 576, 128, 4608, 8
NU = D // 16
CB = 64
NB = D // CB
LAST = 32
FG0 = 3
UA = 4
F32, BF16, I32 = jnp.float32, jnp.bfloat16, jnp.int32
EPS = 1e-5


def _bf16_round_np(x):
    u = np.asarray(x, np.float32).view(np.uint32).astype(np.uint64)
    r = ((u + 0x7FFF + ((u >> 16) & 1)) >> 16) << 16
    return r.astype(np.uint32)


_LROUND = _bf16_round_np(np.arange(L)).view(np.float32).astype(np.int64)
_HI = [(1, 3, 516, 1032), (5, 7, 520, 1288), (4, 260, 772, 1544), (8, 264, 776, 1800), (2, 6, 258, 262)]


def _comp_q():
    t = np.arange(8)[:, None]
    lane = np.arange(128)[None, :]
    return ((lane - 8 - 7 * (t % 4)) % 16) // 4


def _make_tables():
    lane = np.arange(128)
    lo = 8 * (4 * (lane // 16) + lane % 4)
    tab = [dict(), dict()]
    amask = np.zeros(128, bool)
    for q in range(5):
        for e in range(4):
            for par in range(2):
                t = 4 * par + e
                for h in range(2):
                    src = lane[(lane // 4) % 4 == 2 * h + par]
                    dst = (src + (4 * (q % 4) - 8 * h + 8) + 7 * t) % 128
                    assert np.all(_comp_q()[t, dst] == q % 4)
                    sid = e if q < 4 else 4 + e // 2
                    for sl, dl_ in zip(src, dst):
                        ent = (sid, int(dl_))
                        assert tab[par].setdefault(_HI[q][e] + int(lo[sl]), ent) == ent
                    if q == 4 and e % 2 == 1:
                        amask[dst % 16 + 16 * np.arange(8)[:, None]] = True
    pats = []
    for j in range(4):
        pats.append(np.tile(4 * (lane % 32) + ((lane // 32) ^ j), (8, 1)))
    for j in range(4):
        pats.append(np.tile(32 * ((lane % 4) ^ j) + lane // 4, (8, 1)))
    npat0 = len(pats)
    tiles, tile_of = [], {}
    for dl in range(4):
        for l2 in range(4):
            v = _LROUND[512 * dl + 4 * lane + l2]
            key = tuple(v.tolist())
            if key in tile_of:
                tile_of[dl, l2] = tile_of[key]
                continue
            sid = np.array([tab[0][x][0] if x else -1 for x in v])
            ln = np.array([[tab[s8 % 2][x][1] if x else 0 for x in v] for s8 in range(8)])
            steps = []
            for s in sorted(set(sid.tolist()), key=lambda s: -(sid == s).sum()):
                lanes = np.nonzero(sid == s)[0]
                if s < 0:
                    steps.append((-1, None, lanes))
                    continue
                care = sid == s
                kk = None
                for k in range(npat0, len(pats)):
                    oldp, oldc, olds = pats[k]
                    both = care & oldc
                    if olds == s and np.array_equal(oldp[:, both], ln[:, both]):
                        pats[k] = (np.where(care, ln, oldp), care | oldc, s)
                        kk = k
                        break
                if kk is None:
                    pats.append((np.where(care, ln, 0), care, s))
                    kk = len(pats) - 1
                steps.append((s, kk, lanes))
            tiles.append(steps)
            tile_of[key] = tile_of[dl, l2] = len(tiles) - 1
    pats = np.stack([p if k < npat0 else p[0] for k, p in enumerate(pats)]).astype(np.int32)
    tile_of = {k: v for k, v in tile_of.items() if len(k) == 2}
    rows = np.concatenate([pats[:, :2].reshape(-1, 128), amask[None].astype(np.int32)])
    rows = np.concatenate([rows, np.zeros((64 - len(rows), 128), np.int32)]).reshape(16, 4, 128)
    rows = sum(rows[:, k] << (8 * k) for k in range(4)).astype(np.int32)
    return tiles, tile_of, len(pats), rows


_TILES, _TILE_OF, _NGAT, _PROWS = _make_tables()
_NPAT = _NGAT + 3


def _cmul(ar, ai, br, bi):
    return ar * br - ai * bi, ar * bi + ai * br


def _sincos(b):
    magic = jnp.float32(12582912.0)
    t = b * jnp.float32(2.0 / np.pi) + magic
    k = t - magic
    ki = pltpu.bitcast(t, I32)
    r = b - k * jnp.float32(1.5703125)
    r = r - k * jnp.float32(0.0004837512969970703)
    r = r - k * jnp.float32(7.549790126404332e-08)
    u = r * r
    ps = (jnp.float32(-0.0001958295761141926) * u + jnp.float32(0.008332725614309311)) * u \
        + jnp.float32(-0.166666641831398)
    sn = r + (r * u) * ps
    pc = ((jnp.float32(2.437065268168226e-05) * u + jnp.float32(-0.0013886778615415096)) * u
          + jnp.float32(0.04166663438081741)) * u + jnp.float32(-0.5)
    cs = pc * u + jnp.float32(1.0)
    odd = (ki & 1) == 1
    s1 = jnp.where(odd, cs, sn)
    c1 = jnp.where(odd, sn, cs)
    sign = jnp.int32(-2147483648)
    s1 = pltpu.bitcast(pltpu.bitcast(s1, I32) ^ ((ki << 30) & sign), F32)
    c1 = pltpu.bitcast(pltpu.bitcast(c1, I32) ^ (((ki + 1) << 30) & sign), F32)
    return s1, c1


def _gather(x, idx):
    return jnp.take_along_axis(x, idx, axis=1, mode="promise_in_bounds")


def _lanes_mask(lanes):
    lane = lax.broadcasted_iota(I32, (8, 128), 1)
    lanes = sorted(int(x) for x in lanes)
    runs, start, prev = [], lanes[0], lanes[0]
    for x in lanes[1:]:
        if x != prev + 1:
            runs.append((start, prev))
            start = x
        prev = x
    runs.append((start, prev))
    m = None
    for a, b in runs:
        t = (lane == a) if a == b else jnp.logical_and(lane >= a, lane <= b)
        m = t if m is None else jnp.logical_or(m, t)
    return m


def _butterfly(p):
    lane = lax.broadcasted_iota(I32, p[0].shape, 1)
    b0 = (lane & 32) != 0
    b1 = (lane & 64) != 0
    t = [jnp.where(b0, p[k ^ 1], p[k]) for k in range(4)]
    return [jnp.where(b1, t[k ^ 2], t[k]) for k in range(4)]


def _fft4(x, sgn):
    (ar, ai), (br, bi), (cr, ci), (dr, di) = x
    s0r, s0i, d0r, d0i = ar + cr, ai + ci, ar - cr, ai - ci
    s1r, s1i, d1r, d1i = br + dr, bi + di, br - dr, bi - di
    y0 = (s0r + s1r, s0i + s1i)
    y2 = (s0r - s1r, s0i - s1i)
    p = (d0r - d1i, d0i + d1r)
    m = (d0r + d1i, d0i - d1r)
    return [y0, p, y2, m] if sgn > 0 else [y0, m, y2, p]


def _silu(z):
    h = z * jnp.float32(0.5)
    return h + h * jnp.tanh(h)


def _sigmoid(z):
    return jnp.tanh(z * jnp.float32(0.5)) * jnp.float32(0.5) + jnp.float32(0.5)


def _rbf(x):
    return x.astype(BF16).astype(F32)


def _pack2(a, b):
    p = pltpu.pack_elementwise([a, b], packed_dtype=BF16)
    return p if p.dtype == I32 else pltpu.bitcast(p, I32)


def _unpack2(x):
    return [pltpu.bitcast(x << 16, F32), pltpu.bitcast(x & jnp.int32(-65536), F32)]


def _bf(x):
    return pltpu.bitcast(x, BF16)


_NT = (((1,), (1,)), ((), ()))


class _Idx:
    def __init__(self, i, lag=0):
        self.i, self.lag = i, lag

    def off(self, stride, const=0, align=None):
        v = self.i * stride + (const - self.lag * stride)
        return pl.multiple_of(v, align) if align and not isinstance(v, int) else v

    def idx(self):
        return self.i - self.lag


def _pipeline(stages, n, weave=None, reset=None):
    ns = len(stages)

    def step(i, lo, hi):
        gens = {k: stages[k](_Idx(i, k)) for k in range(lo, hi)}
        if reset is not None:
            reset()
        if callable(weave):
            weave(gens)
        else:
            for k in weave or ():
                if k in gens:
                    next(gens[k], None)
        for k in range(hi - 1, lo - 1, -1):
            for _ in gens[k]:
                pass

    def body(i, carry):
        step(i, 0, ns)
        return carry

    return ([lambda i=i: step(i, 0, i + 1) for i in range(ns - 1)],
            lambda: lax.fori_loop(ns - 1, n, body, 0),
            [lambda i=i: step(n + i, i + 1, ns) for i in range(ns - 1)])


def _kernel(x_hbm, are_hbm, aim_hbm, bre_hbm, bim_hbm, cre_hbm, cim_hbm, ldt_hbm, dsk_hbm, wr_hbm,
            wg_hbm, wu_hbm, wd_hbm, pat_hbm,
            out_hbm,
            xbuf, par, ldt, dsk, wr, wg, wu, wd, fpk, prow, pats,
            dtcol, skip, hi_re, hi_im, lo_re, lo_im, comp, khat,
            xp, xnp, uhat, yhat, ybuf, spk, topk, posv, dummy, wr16b, wsum, ohb, xsel_ref, hbuf, hpk, cols, opk, og, obuf,
            sem_in, *perb):
    xg, stat = perb[0:4], perb[4:8]
    sem_out = sem_in.at[1]
    p_hbm = (are_hbm, aim_hbm, bre_hbm, bim_hbm, cre_hbm, cim_hbm)
    r1 = 16 * UA
    small = [(ldt_hbm, ldt), (pat_hbm, prow)]
    for a, n in ((0, r1), (r1, r1), (2 * r1, D - 2 * r1)):
        small += [(h.at[pl.ds(a, n)], par.at[i, pl.ds(a, n)]) for i, h in enumerate(p_hbm)]
    small += [(wr_hbm, wr), (dsk_hbm, dsk)]
    cps = [pltpu.make_async_copy(s, d, sem_in.at[min((i + 4) // 6, 3)]) for i, (s, d) in enumerate(small)]
    ns = 4
    cp_x = pltpu.make_async_copy(x_hbm, xbuf, sem_in.at[ns])
    cp_g = pltpu.make_async_copy(wg_hbm, wg, sem_in.at[ns + 1])
    cp_u = pltpu.make_async_copy(wu_hbm, wu, sem_in.at[ns + 2])
    chunks = [(0, 128), (128, 128), (256, 128), (384, 128), (512, 64)]
    cp_d = [pltpu.make_async_copy(wd_hbm.at[pl.ds(a, n)], wd.at[pl.ds(a, n)], sem_in.at[ns + 3 + q - (q > 1)])
            for q, (a, n) in enumerate(chunks[:4] + [(512, 64 - LAST), (D - LAST, LAST)])]
    cp_bar = [pltpu.make_async_copy(prow.at[pl.ds(0, 8)], dummy.at[k], sem_in.at[(0, 2, 3)[k]]) for k in range(3)]
    for cp in cps + [cp_x, cp_g, cp_u] + cp_d:
        cp.start()

    sub8 = lax.broadcasted_iota(I32, (8, 128), 0)
    lane8 = lax.broadcasted_iota(I32, (8, 128), 1)

    def dft_rows(l2):
        for g in range(8):
            cs = []
            for e in range(2):
                p = 16 * g + 2 * sub8 + e
                t = 4 * (32 * ((p >> 5) ^ l2) + (p & 31)) + l2
                n = ((4 * lane8 + 1) * t) & 2047
                cs.append(_sincos(n.astype(F32) * jnp.float32(-2.0 * np.pi / 2048)))
            fpk[l2, pl.ds(8 * g, 8), pl.ds(0, 128)] = _pack2(cs[0][1], cs[1][1])
            fpk[l2, pl.ds(8 * g, 8), pl.ds(128, 128)] = _pack2(cs[0][0], cs[1][0])

    for l2 in range(FG0):
        dft_rows(l2)

    for cp in cps[:2]:
        cp.wait()
    for l2 in range(FG0, 4):
        dft_rows(l2)
    for k in range(_NGAT):
        w = jnp.broadcast_to(prow[pl.ds(k // 2, 1), :], (8, 128))
        pats[k] = (w >> (16 * (k % 2) + 8 * (sub8 & 1))) & 127
    cq = ((lane8 - 8 - 7 * (sub8 & 3)) & 15) >> 2
    pats[_NGAT] = cq & 1
    pats[_NGAT + 1] = cq >> 1
    pats[_NGAT + 2] = (jnp.broadcast_to(prow[pl.ds(_NGAT // 2, 1), :], (8, 128)) >> (16 * (_NGAT % 2))) & 127
    r128 = lax.broadcasted_iota(I32, (128, 128), 0)
    c128 = lax.broadcasted_iota(I32, (128, 128), 1)

    def column(row):
        pk = pltpu.bitcast(jnp.broadcast_to(row, (8, D)), I32)
        lhs = []
        for u in range(NU):
            t = u // 8
            v = pk[:, 128 * t:128 * t + 128] if t < 4 else jnp.concatenate([pk[:, 512:], pk[:, 512:]], axis=1)
            c0 = 16 * (u % 8) + 2 * sub8
            lhs.append(jnp.where(lane8 == c0, lax.shift_right_logical(v, 16), jnp.where(lane8 == c0 + 1, v, 0)))
        ones = jnp.ones((128, 128), BF16)
        return jnp.concatenate([jnp.dot(_bf(jnp.concatenate(lhs[k:k + NU // 4], axis=0)), ones,
                                        preferred_element_type=F32) for k in range(0, NU, NU // 4)], axis=0)

    dtcol[...] = column(_rbf(jnp.exp(ldt[...].astype(F32).reshape(1, D))))

    def block(*fns):
        def body(k, carry):
            for fn in fns:
                fn()
            return carry

        lax.fori_loop(0, pl.program_id(0) + 1, body, 0)

    def after(x, deps):
        never = pats[0] < 0
        d = None
        for v in deps:
            v = v if v.dtype == I32 else pltpu.bitcast(v, I32)
            d = v if d is None else d ^ v
        return jnp.where(never, d if x.dtype == I32 else pltpu.bitcast(d, x.dtype), x)

    def pad_tail(y, i):
        n, k = 16, y.shape[0] - 64
        base = i.off(1)
        mid = after(y[k:k + 8], [pats[j % _NPAT] * (base + j) for j in range(n)])
        return jnp.concatenate([y[:k], mid, y[k + 8:]], axis=0)

    class Sched:
        tok, g, pre = {}, 0, []

        @classmethod
        def reset(cls):
            cls.tok, cls.g, cls.pre = {}, 0, []

        @classmethod
        def gate(cls, x):
            deps = cls.tok.pop(cls.g, [])
            cls.g += 1
            if not deps:
                return x
            return jnp.concatenate([after(x[:8], deps), after(x[8:], deps[-1:])], axis=0)

    slot = {h: (q, e) for q, ent in enumerate(_HI) for e, h in enumerate(ent)}

    def a_prep(i):
        gate = Sched.gate
        for u in range(UA):
            rows = pl.ds(i.off(16 * UA, 16 * u, 16), 16)
            ev = pl.ds(i.off(32 * UA, 32 * u), 16, stride=2)
            od = pl.ds(i.off(32 * UA, 32 * u + 1), 16, stride=2)
            dt = gate(dtcol[rows, :])
            al = dt * par[0, rows, :].astype(F32)
            be = dt * par[1, rows, :].astype(F32)
            cr, ci = _cmul(par[4, rows, :].astype(F32), par[5, rows, :].astype(F32),
                           par[2, rows, :].astype(F32), par[3, rows, :].astype(F32))
            dts = dt * jnp.float32(1.0 / 512)
            cr, ci = cr * dts, ci * dts
            k0 = jnp.sum(cr, axis=1, keepdims=True) * jnp.float32(512.0)
            skip[rows, :] = jnp.broadcast_to(k0, (16, 128))
            yield cr
            s, c = _sincos(gate(be))
            yield c
            pw = {1: (c, s)}
            e = 1
            while e < 256:
                if e in (1, 16):
                    c = gate(c)
                c, s = (c - s) * (c + s), (c + c) * s
                e *= 2
                pw[e] = (c, s)
                if e in (16, 256):
                    yield c
            z = {}
            for e in (1, 8, 256):
                mag = jnp.exp(al * jnp.float32(e))
                c, s = pw[e]
                z[e] = (mag * c, mag * s)
            pend = {}

            def put(tab, q, ee, v):
                key = (tab[0] is hi_re, q, ee // 2)
                if key not in pend:
                    pend[key] = (ee % 2, v)
                    return
                w, o = pend.pop(key)
                lo_, hi_ = (o, v) if w == 0 else (v, o)
                dst = od if ee // 2 else ev
                tab[0][q, dst, :] = _pack2(lo_[0], hi_[0])
                tab[1][q, dst, :] = _pack2(lo_[1], hi_[1])

            h = (cr, ci)
            cnt = 0
            for e in range(1, 9):
                g, ee, m = h, e, z[1]
                while ee in slot:
                    if cnt % 4 == 0:
                        g = (gate(g[0]), g[1])
                    g = _cmul(*g, *m)
                    put((hi_re, hi_im), *slot[ee], g)
                    if ee == e:
                        h = g
                    ee, m = ee + 256, z[256]
                    cnt += 1
                    if cnt % 4 == 0:
                        yield g[0]
            w1 = (gate(z[8][0]), -z[8][1])
            v = [(jnp.ones((16, 128), F32), jnp.zeros((16, 128), F32)), w1]
            v.append(_cmul(*w1, *w1))
            v.append(_cmul(*v[2], *w1))
            w4 = _cmul(*v[2], *v[2])
            for j in range(8):
                for f in range(4):
                    put((lo_re, lo_im), j, f, v[f])
                yield v[3][0]
                if j < 7:
                    w4 = (gate(w4[0]), w4[1])
                    v = [w4 if (j == 0 and f == 0) else _cmul(*v[f], *w4) for f in range(4)]

    def a_gen(i):
        b0 = pats[_NPAT - 3] != 0
        b1 = pats[_NPAT - 2] != 0
        for k in range(4 * UA):
            rows = pl.ds(i.off(32 * UA, 8 * k, 8), 8)
            lo = jnp.concatenate([lo_re[:, rows, :].reshape(64, 128), lo_im[:, rows, :].reshape(64, 128)], axis=1)
            h0 = hi_re[0, rows, :]
            if k % 2 == 0 and Sched.pre:
                h0 = after(h0, Sched.pre)
                Sched.pre = []
            hi = jnp.concatenate([jnp.concatenate([h0, hi_re[1:5, rows, :].reshape(32, 128)], axis=0),
                                  hi_im[:, rows, :].reshape(40, 128)], axis=1)
            o = lax.dot_general(_bf(hi), _bf(lo), _NT, preferred_element_type=F32)
            for q in range(5):
                Sched.tok.setdefault(13 + int(0.9 * (5 * (k // 2) + q)), []).append(o[16 * q + 8:16 * q + 16])
            for h in range(2):
                g = [pltpu.roll(o[16 * q + 8 * h:16 * q + 8 * h + 8], 4 * (q % 4) - 8 * h + 8, 1,
                                stride=7, stride_axis=0) for q in range(5)]
                dst = pl.ds(i.off(64 * UA, 16 * k + 8 * h, 8), 8)
                comp[0, dst, :] = jnp.where(b1, jnp.where(b0, g[3], g[2]), jnp.where(b0, g[1], g[0]))
                comp[1, dst, :] = g[4]
            if k % 2 == 1:
                yield

    def a_exp(i):
        bm = pats[_NPAT - 1] != 0
        srcs = []
        for u in range(UA):
            def ld(a, e):
                return _pack2(comp[a, pl.ds(i.off(64 * UA, 64 * u + e), 8, stride=4), :],
                              comp[a, pl.ds(i.off(64 * UA, 64 * u + 32 + e), 8, stride=4), :])

            srcs.append([ld(0, e) for e in range(4)]
                        + [jnp.where(bm, ld(1, 2 * k + 1), ld(1, 2 * k)) for k in range(2)])
        cache = {}

        def gat(s, key):
            if key not in cache:
                pat = pats[key]
                cache[key] = [_gather(srcs[u][s], pat) for u in range(UA)]
            return cache[key]

        tiles = []
        for steps in _TILES:
            t = None
            for s, key, lanes in steps:
                v = [jnp.zeros((8, 128), I32)] * UA if s < 0 else gat(s, key)
                t = v if t is None else [jnp.where(_lanes_mask(lanes), v[u], t[u]) for u in range(UA)]
            tiles.append(t)
        yield
        for u0 in range(0, UA, 2):
            lhs = [_bf(jnp.concatenate([tiles[_TILE_OF[dl, l2]][u] for dl in range(4) for u in (u0, u0 + 1)], axis=0))
                   for l2 in range(4)]

            def dots(ri):
                return [jnp.dot(lhs[l2], _bf(jnp.concatenate(
                    [fpk[l2, pl.ds(16 * (j ^ l2), 16), pl.ds(128 * ri, 128)] for j in range(4)], axis=0)),
                    preferred_element_type=F32) for l2 in range(4)]

            def store(k2, ri, v):
                khat[2 * k2 + ri, :, pl.ds(i.off(16 * UA, 16 * u0, 16), 32), :] = v.reshape(4, 32, 128)

            def toks(v, step0):
                for j in range(8):
                    g = 13 + 9 * UA + int(0.7 * (step0 + j))
                    Sched.tok.setdefault(g, []).append(v[16 * j + 8:16 * j + 16])

            re = dots(0)
            s0, d0r, s1, d1r = re[0] + re[2], re[0] - re[2], re[1] + re[3], re[1] - re[3]
            store(0, 0, s0 + s1)
            v = s0 - s1
            store(2, 0, v)
            toks(v, 8 * u0)
            im = dots(1)
            s0, d0i, s1, d1i = im[0] + im[2], im[0] - im[2], im[1] + im[3], im[1] - im[3]
            store(0, 1, s0 + s1)
            store(2, 1, s0 - s1)
            store(1, 0, d0r + d1i)
            store(1, 1, d0i - d1r)
            store(3, 0, d0r - d1i)
            v = d0i + d1r
            store(3, 1, v)
            toks(v, 8 * u0 + 8)
            yield

    def a_weave(gens):
        if 2 in gens:
            next(gens[2])
        if 0 in gens and 1 in gens:
            for n in (3, 5, 4):
                for _ in range(n):
                    v = next(gens[0])
                Sched.pre = [v[:8], v[8:]]
                next(gens[1])
        for k in (1, 2, 0):
            if k in gens:
                for _ in gens[k]:
                    pass

    a_pro, a_loop, a_tail = _pipeline([a_prep, a_gen, a_exp], NU // UA, reset=Sched.reset, weave=a_weave)
    for cp in cps[2:8]:
        cp.wait()
    a_pro[0]()
    for cp in cps[8:14]:
        cp.wait()
    a_pro[1]()
    for cp in cps[14:]:
        cp.wait()
    a_loop()

    cp_x.wait()

    def b_gather(b):
        for j in range(4):
            pat = pats[j]
            for u in range(NU):
                v = pltpu.bitcast(xbuf[pl.ds(16 * u, 16), pl.ds(512 * b + 128 * j, 128)], I32)
                v = _gather(v, pat)
                xg[b][j, pl.ds(8 * u, 8), :] = v
                gtok.setdefault(b, []).append(v)

    gtok = {}

    def b_stat(b, ride=None):
        s2 = [jnp.zeros((8, 128), F32) for _ in range(4)]
        for u in range(NU):
            x = [xg[b][j, pl.ds(8 * u, 8), :] for j in range(4)]
            if ride is not None:
                x = [after(x[0], [gtok[ride][4 * u]]), x[1], after(x[2], [gtok[ride][4 * u]]), x[3]]
            o = _butterfly(x)
            for l2 in range(4):
                xp[4 * l2 + b, pl.ds(8 * u, 8), :] = o[l2]
                e_, o_ = _unpack2(o[l2])
                s2[l2] = s2[l2] + (e_ * e_ + o_ * o_)
        for l2 in range(4):
            stat[b][l2, pl.ds(16, 8), :] = s2[l2]

    def b_dot(b):
        lhs = _bf(wr16b[...])
        for j in range(4):
            stat[b][j, pl.ds(0, 16), :] = jnp.dot(lhs, _bf(xg[b][j]), preferred_element_type=F32)

    def b_fin(b0):
        wx = sx = q = None
        for b in (b0, b0 + 1):
            wxs = _butterfly([stat[b][j, pl.ds(0, 8), :] for j in range(4)])
            sxs = _butterfly([stat[b][j, pl.ds(8, 8), :] for j in range(4)])
            for l2 in range(4):
                qq = jnp.sum(stat[b][l2, pl.ds(16, 8), :], axis=0, keepdims=True)
                here = sub8 == 4 * (b - b0) + l2
                wx = wxs[l2] if wx is None else jnp.where(here, wxs[l2], wx)
                sx = sxs[l2] if sx is None else jnp.where(here, sxs[l2], sx)
                q = jnp.broadcast_to(qq, (8, 128)) if q is None else jnp.where(here, qq, q)
        m = sx * jnp.float32(1.0 / D)
        var = _rbf(jnp.maximum(q * jnp.float32(1.0 / D) - m * m, 0.0))
        rs = 1.0 / _rbf(jnp.sqrt(_rbf(var + jnp.float32(EPS))))
        mb = _rbf(m)
        r = _rbf((wx - mb * wsum[...]) * rs)
        r = jnp.where(r == 0.0, 0.0, r)
        bits = pltpu.bitcast(r, I32)
        mono = ((bits ^ ((bits >> 31) & jnp.int32(0x7FFFFFFF))) >> 16) + 32768
        l2v = sub8 & 3
        tok = 512 * (b0 + (sub8 >> 2)) + 4 * (32 * ((lane8 >> 5) ^ l2v) + (lane8 & 31)) + l2v
        topk[b0 // 2] = pltpu.bitcast((mono << 11) + (2047 - tok) + jnp.int32(0x00800000), F32)
        return mb, rs

    def b_scale(b0, st, us):
        for k in range(8):
            t = 4 * (k % 4) + b0 + k // 4
            mk, rk = [jnp.broadcast_to(v[k:k + 1], (8, 128)) for v in st]
            for u in us:
                e_, o_ = _unpack2(xp[t, pl.ds(8 * u, 8), :])
                xnp[t, pl.ds(8 * u, 8), :] = _pack2((e_ - mk) * rk, (o_ - mk) * rk)

    def b_norm(b0):
        st = b_fin(b0)
        for us in (range(CB // 16), range(CB // 16, NU)):
            b_scale(b0, st, us)

    def b_init():
        wrow = wr[...].reshape(1, D)
        wr16b[...] = pltpu.bitcast(
            jnp.concatenate([jnp.broadcast_to(wrow, (8, D)), jnp.ones((8, D), BF16)], axis=0), I32)
        wsum[...] = jnp.broadcast_to(jnp.sum(wrow.astype(F32), axis=1, keepdims=True), (8, 128))
        topk[2] = jnp.zeros((8, 128), F32)
        cols[...] = jnp.zeros(cols.shape, I32)

    elt_dep, toks = [], []

    def c_fwd(i):
        h0 = i.off(CB // 2, 0, 8)
        r0 = i.off(CB, 0, 8)
        for l2 in range(4):
            lhs = _bf(xnp[pl.ds(4 * l2, 4), pl.ds(h0, CB // 2), :].reshape(2 * CB, 128))
            res = jnp.dot(lhs, _bf(fpk[l2]), preferred_element_type=F32)
            for ri in range(2):
                y = res[:, 128 * ri:128 * ri + 128]
                if l2 == 3 and ri == 1 and isinstance(i.i, int) and i.i < 2:
                    y = pad_tail(y, i)
                uhat[2 * l2 + ri, :, pl.ds(r0, CB), :] = y.reshape(4, CB, 128)
            yield

    def c_mid(i, units=range(CB // 8)):
        for k in units:
            rows = pl.ds(i.off(CB, 8 * k, 8), 8)
            krows = pl.ds(i.off(CB, 16 * (k // 2) + k % 2), 8, stride=2)
            x = [[(uhat[2 * l2, b, rows, :], uhat[2 * l2 + 1, b, rows, :]) for l2 in range(4)] for b in range(4)]
            if elt_dep:
                for b in range(4):
                    x[b][0] = (after(x[b][0][0], elt_dep), x[b][0][1])
            uu = [_fft4(x[b], -1) for b in range(4)]
            yy = [[None] * 4 for _ in range(4)]
            for k2s in ((0, 2), (1, 3)):
                pps = {k2: [None] * 4 for k2 in k2s}
                for k2, pp in pps.items():
                    for dl in range(3, -1, -1):
                        kk = (khat[2 * k2, dl, krows, :], khat[2 * k2 + 1, dl, krows, :])
                        for m in range(3, dl - 1, -1):
                            t = _cmul(*uu[m - dl][k2], *kk)
                            pp[m] = t if pp[m] is None else (pp[m][0] + t[0], pp[m][1] + t[1])
                for k2, pp in pps.items():
                    for m in range(3, -1, -1):
                        yy[m][k2] = pp[0] if m == 0 else (pp[m][0] - pp[m - 1][1], pp[m][1] + pp[m - 1][0])
            un = i.off(CB // 8, k)
            for bp in range(2):
                ww = [_fft4(yy[m], 1) for m in (2 * bp, 2 * bp + 1)]
                for l2 in range(4):
                    for ri in range(2):
                        yhat[2 * l2 + ri, bp, un] = _pack2(ww[0][l2][ri], ww[1][l2][ri])
            yield

    def c_inv(i, l2s=range(4)):
        u0 = i.off(CB // 8)
        r0 = i.off(2 * CB, 0, 8)
        for l2 in l2s:
            for ri in range(2):
                lhs = _bf(yhat[2 * l2 + ri, :, pl.ds(u0, CB // 8)].reshape(2 * CB, 128))
                y = lax.dot_general(lhs, _bf(fpk[l2, :, pl.ds(128 * ri, 128)]), _NT,
                                    preferred_element_type=F32)
                if l2 == 3 and ri == 1 and isinstance(i.i, int):
                    y = pad_tail(y, i)
                ybuf[2 * l2 + ri, :, pl.ds(r0, 2 * CB), :] = y.reshape(2, 2 * CB, 128)
                toks.extend(y[32 * j:32 * j + 8] for j in range(CB // 8))
            yield

    def c_elt(i):
        for k in range(CB // 16):
            hr = pl.ds(i.off(CB // 2, 8 * k, 8), 8)
            sk = [skip[pl.ds(i.off(CB, 16 * k + e), 8, stride=2), :] for e in range(2)]
            for b in range(4):
                o = []
                for l2 in range(4):
                    w = xnp[4 * l2 + b, hr, :]
                    if elt_dep:
                        w = after(w, elt_dep)
                    xn = _unpack2(w)
                    xx = _unpack2(xp[4 * l2 + b, hr, :])
                    ss, v = [], []
                    for e in range(2):
                        yr = pl.ds(i.off(2 * CB, 32 * k + 2 * e + b % 2), 8, stride=4)
                        ss.append(ybuf[2 * l2, b // 2, yr, :] + ybuf[2 * l2 + 1, b // 2, yr, :] + xn[e] * sk[e])
                        v.append(xx[e] + ss[e] * _silu(xn[e]))
                    spk[4 * l2 + b, hr, :] = _pack2(*ss)
                    o.append(_pack2(*v))
                p = _butterfly(o)
                for j in range(4):
                    opk[4 * b + j, hr, :] = p[j]
                yield

    def c_top(i):
        k0, k1 = topk[0], topk[1]
        mx = jnp.max(jnp.max(jnp.maximum(k0, k1), axis=0, keepdims=True), axis=1, keepdims=True)
        topk[0] = jnp.where(k0 == mx, 0.0, k0)
        topk[1] = jnp.where(k1 == mx, 0.0, k1)
        topk[2] = jnp.where(sub8 == i.idx(), mx, topk[2])
        yield

    def c_first(i):
        yield from c_fwd(i)
        yield from c_top(i)

    c_pro, c_loop, _ = _pipeline([c_first, c_mid, c_inv, c_elt], NB,
                                 weave=[1] * (CB // 8) + [3] * (CB // 4) + [0, 0, 2, 2, 0, 0, 2, 2])

    def first_fwd():
        for _ in c_first(_Idx(0)):
            pass

    def each(fn, *bs):
        return [lambda b=b: fn(b) for b in bs]

    def add_dskip():
        skip[...] = skip[...] + column(dsk[...].astype(F32).reshape(1, D))

    b_init()
    a_tail[0]()
    b_gather(0)
    b_gather(1)
    b_stat(0, 1)
    block(add_dskip, a_tail[1], *each(b_gather, 2, 3), *each(b_dot, 0, 1),
          lambda: b_stat(1, 2), lambda: b_stat(2, 3))
    block(*each(b_stat, 3), *each(b_norm, 0), *each(b_dot, 2, 3))
    block(*each(b_norm, 2), first_fwd)
    block(c_pro[1])
    block(c_pro[2])
    c_loop()

    sel = pltpu.bitcast(topk[2], I32) - jnp.int32(0x00800000)
    mono = (sel >> 11) - 32768
    r_sel = pltpu.bitcast((mono ^ ((mono >> 31) & jnp.int32(0x7FFF))) << 16, F32)
    gate_r = _rbf(jax.nn.sigmoid(r_sel))
    posv[...] = 2047 - (sel & 2047)
    tok = [posv[c, 0] for c in range(C)]
    nat = [(jnp.clip(t >> 7, 0, 15), t & 127) for t in tok]
    prm = []
    for t in tok:
        l2, l1 = t & 3, (t >> 2) & 127
        prm.append((jnp.clip(4 * l2 + (t >> 9), 0, 15), 32 * ((l1 >> 5) ^ l2) + (l1 & 31)))

    def extract(src, k, us):
        for c, (tp, pp) in enumerate(prm):
            sh = (c - pp) & 127
            for u in us:
                v = pltpu.roll(src[tp, pl.ds(8 * u, 8), :], sh, 1)
                pltpu.store(cols.at[k, pl.ds(8 * u, 8), :], v, mask=lane8 == c)
                toks.append(v)

    for c, (tp, pp) in enumerate(prm):
        ohb[c] = jnp.where(jnp.logical_and(sub8 == c // 2, lane8 == pp), jnp.int32(0x3F80 << (16 * (c % 2))), 0)

    def take_rows():
        for c, (tp, pp) in enumerate(prm):
            xsel_ref[c] = lax.dot_general(_bf(ohb[c]), _bf(xnp[tp]), _NT, preferred_element_type=F32)[:8]

    def o_gather(us):
        for j in range(4):
            pat = pats[4 + j]
            for b in range(4):
                for u in us:
                    v = _gather(opk[4 * b + j, pl.ds(8 * u, 8), :], pat)
                    og[4 * b + j, pl.ds(8 * u, 8), :] = v
                    toks.append(v)
                    o_store(u, v, pl.ds(512 * b + 128 * j, 128))

    def o_store(u, v, col):
        obuf[pl.ds(16 * u, 8), col] = _bf(v[0:4])
        obuf[pl.ds(16 * u + 8, 8), col] = _bf(pltpu.roll(v, 4, 0)[0:4])

    def project(w, post):
        xs = xsel_ref[0]
        for c in range(1, C):
            xs = xs + xsel_ref[c]
        xs = jnp.concatenate([xs, jnp.zeros((8, D), F32)], axis=0).astype(BF16)
        for t in range(F // 128):
            ps = [jnp.dot(xs[:, a:a + n], w[pl.ds(a, n), pl.ds(128 * t, 128)],
                          preferred_element_type=F32)[:8] for a, n in chunks]
            v = _rbf((ps[0] + ps[1]) + (ps[2] + ps[3]) + ps[4])
            toks.append(v)
            post(t, v)

    def post_gate(t, ga):
        hbuf[:, pl.ds(128 * t, 128)] = _rbf(ga * _rbf(_sigmoid(ga)))

    def post_up(t, up):
        h = hbuf[:, pl.ds(128 * t, 128)] * up
        hpk[:, pl.ds(128 * t, 128)] = pltpu.bitcast(
            jnp.concatenate([h, jnp.zeros((8, 128), F32)], axis=0).astype(BF16), I32)

    pr = (r128 & (-16)) + 2 * (r128 & 7) + ((r128 >> 3) & 1)
    perm = jnp.where(pr == c128, 1.0, 0.0).astype(BF16)

    acc = {}
    out_cp = [pltpu.make_async_copy(obuf.at[pl.ds(a, n)], out_hbm.at[pl.ds(a, n)], sem_out) for a, n in chunks]

    def patch(q):
        a, n = chunks[q]
        xs = xsel_ref[0, :, pl.ds(a, n)]
        for c in range(1, C):
            xs = xs + xsel_ref[c, :, pl.ds(a, n)]
        z = _rbf(xs + _rbf(_rbf(acc[q]) * gate_r[:, :1]))
        g = z * _rbf(_sigmoid(z))
        g = jnp.concatenate([g, jnp.zeros((120, n), F32)], axis=0).astype(BF16)
        gt = lax.dot_general(perm[:n, :n], g, _NT, preferred_element_type=F32)
        us = range(a // 16, (a + n) // 16)
        for u in us:
            hr = pl.ds(8 * u, 8)
            xx, ss = _unpack2(cols[0, hr, :]), _unpack2(cols[1, hr, :])
            r0 = 16 * u - a
            w = _pack2(*[xx[e] + _rbf(ss[e] * gt[r0 + 8 * e:r0 + 8 * e + 8]) for e in range(2)])
            for c, (tn, pn) in enumerate(nat):
                pltpu.store(og.at[tn, pl.ds(8 * u, 8), :], pltpu.roll(w, (pn - c) & 127, 1), mask=lane8 == pn)
        for c, (tn, pn) in enumerate(nat):
            for u in us:
                v = og[tn, pl.ds(8 * u, 8), :]
                o_store(u, v, pl.ds(pl.multiple_of(tn * 128, 128), 128))

    def down(q, f0, f1):
        a, n = chunks[q]
        for f in range(f0, f1, 2):
            col = pl.ds(128 * f, 256)
            y = lax.dot_general(_bf(hpk[:, col]), wd[pl.ds(a, n), col], _NT, preferred_element_type=F32)[:8]
            acc[q] = y if q not in acc else acc[q] + y
            if n == 128:
                toks.append(y)

    def inverse(k, l2s):
        for _ in c_inv(_Idx(k), l2s):
            pass

    def ride(gen, n, frac=1.0):
        for j in range(n):
            elt_dep[:] = [toks[int(frac * len(toks)) * j // n]]
            next(gen, None)
        elt_dep.clear()

    def elementwise(k, frac=1.0):
        ride(c_elt(_Idx(k)), CB // 4, frac)

    def products(u0, u1):
        ride(c_mid(_Idx(NB - 1), range(u0, u1)), u1 - u0)

    for cp in cp_bar:
        cp.start()
    take_rows()
    toks.clear()
    extract(xp, 0, range(NU))
    elementwise(NB - 3)
    cp_g.wait()
    project(wg, post_gate)
    o_gather(range(24))
    cp_u.wait()
    project(wu, post_up)
    extract(spk, 1, range(24))
    cp_d[0].wait()
    toks.clear()
    down(0, 0, 36)
    products(0, 4)
    inverse(NB - 2, range(0, 2))
    cp_d[1].wait()
    cp_d[2].wait()
    toks.clear()
    down(1, 0, 10)
    patch(0)
    down(1, 10, 36)
    down(2, 0, 10)
    products(4, 8)
    cp_d[4].wait()
    out_cp[0].start()
    cp_d[3].wait()
    patch(1)
    down(2, 10, 36)
    inverse(NB - 2, range(2, 4))
    cp_d[5].wait()
    out_cp[1].start()
    cp_bar[0].wait()
    toks.clear()
    patch(2)
    out_cp[2].start()
    inverse(NB - 1, range(4))
    down(3, 0, 12)
    elementwise(NB - 2)
    cp_bar[1].wait()
    toks.clear()
    down(3, 12, 36)
    o_gather(range(24, 32))
    extract(spk, 1, range(24, 32))
    down(4, 0, 10)
    patch(3)
    out_cp[3].start()
    down(4, 10, 36)
    elementwise(NB - 1, 0.8)
    cp_bar[2].wait()
    o_gather(range(32, NU))
    extract(spk, 1, range(32, NU))
    patch(4)
    out_cp[4].start()
    for cp in out_cp:
        cp.wait()


def _scratch():
    return [
        pltpu.VMEM((D, L), BF16),
        pltpu.VMEM((6, D, N), BF16),
        pltpu.VMEM((D,), BF16),
        pltpu.VMEM((D,), BF16),
        pltpu.VMEM((D,), BF16),
        pltpu.VMEM((D, F), BF16),
        pltpu.VMEM((D, F), BF16),
        pltpu.VMEM((D, F), BF16),
        pltpu.VMEM((4, 64, 256), I32),
        pltpu.VMEM(_PROWS.shape, I32),
        pltpu.VMEM((_NPAT, 8, 128), I32),
        pltpu.VMEM((D, 128), F32),
        pltpu.VMEM((D, 128), F32),
        pltpu.VMEM((5, 2 * D, 128), I32),
        pltpu.VMEM((5, 2 * D, 128), I32),
        pltpu.VMEM((8, 2 * D, 128), I32),
        pltpu.VMEM((8, 2 * D, 128), I32),
        pltpu.VMEM((2, 4 * D, 128), F32),
        pltpu.VMEM((8, 4, D, 128), F32),
        pltpu.VMEM((16, D // 2, 128), I32),
        pltpu.VMEM((16, D // 2, 128), I32),
        pltpu.VMEM((8, 4, D, 128), F32),
        pltpu.VMEM((8, 2, D // 8, 8, 128), I32),
        pltpu.VMEM((8, 2, 2 * D, 128), F32),
        pltpu.VMEM((16, D // 2, 128), I32),
        pltpu.VMEM((3, 8, 128), F32),
        pltpu.VMEM((8, 128), I32),
        pltpu.VMEM((3, 8, 128), I32),
        pltpu.VMEM((8, D), I32),
        pltpu.VMEM((8, 128), F32),
        pltpu.VMEM((C, 8, 128), I32),
        pltpu.VMEM((C, 8, D), F32),
        pltpu.VMEM((8, F), F32),
        pltpu.VMEM((8, F), I32),
        pltpu.VMEM((2, D // 2, 128), I32),
        pltpu.VMEM((16, D // 2, 128), I32),
        pltpu.VMEM((16, D // 2, 128), I32),
        pltpu.VMEM((D, L), BF16),
        pltpu.SemaphoreType.DMA((12,)),
    ] + [pltpu.VMEM((4, D // 2, 128), I32)] * 4 + [pltpu.VMEM((4, 24, 128), F32)] * 4


@jax.jit
def pallas_recurrent_scan__ssm_conv_s4__moe_arch_mod__prompt_kernel(
    A_u: jax.Array,
    A_A_re: jax.Array,
    A_A_im: jax.Array,
    A_B_re: jax.Array,
    A_B_im: jax.Array,
    A_C_re: jax.Array,
    A_C_im: jax.Array,
    A_log_dt: jax.Array,
    A_Dskip: jax.Array,
    B_x: jax.Array,
    B_w_r: jax.Array,
    B_w_gate: jax.Array,
    B_w_up: jax.Array,
    B_w_down: jax.Array,
):
    hbm = pl.BlockSpec(memory_space=pltpu.HBM)
    out = pl.pallas_call(
        _kernel,
        out_shape=jax.ShapeDtypeStruct((D, L), BF16),
        grid=(1,),
        in_specs=[hbm] * 14,
        out_specs=hbm,
        scratch_shapes=_scratch(),
        compiler_params=pltpu.CompilerParams(vmem_limit_bytes=110 * 1024 * 1024),
        name="s4_mod",
    )(A_u.reshape(L, D).T, A_A_re, A_A_im, A_B_re, A_B_im, A_C_re, A_C_im, A_log_dt, A_Dskip, B_w_r,
      B_w_gate, B_w_up, B_w_down.T, jnp.asarray(_PROWS))
    return out.T.reshape(1, L, D)
```
